```python
import jax
import jax.numpy as jnp

def _softmax(x, axis=-1):
    return jax.nn.softmax(x, axis=axis)

def _gelu(x):
    return jax.nn.gelu(x, approximate=True)

def _silu(x):
    return jax.nn.silu(x)

def _sigmoid(x):
    return jax.nn.sigmoid(x)

def _layernorm(x, axis=-1, eps=1e-05):
    m = jnp.mean(x, axis=axis, keepdims=True)
    v = jnp.var(x, axis=axis, keepdims=True)
    return (x - m) / jnp.sqrt(v + eps)

def _scatter_add(tgt, idx, src, axis=0):
    return tgt.at[idx].add(src)

def _segment_sum(src, seg, n):
    return jax.ops.segment_sum(src, seg, n)

class _Rng:

    def __init__(self, key):
        self._k = key

    def _next(self):
        self._k, sub = jax.random.split(self._k)
        return sub

    def normal(self, shape):
        return jax.random.normal(self._next(), shape, dtype=jnp.bfloat16)

    def randint(self, lo, hi, shape):
        return jax.random.randint(self._next(), shape, lo, hi, dtype=jnp.int32)

    def uniform(self, shape, lo=0.0, hi=1.0):
        return jax.random.uniform(self._next(), shape, jnp.bfloat16, lo, hi)

    def permutation(self, n):
        return jax.random.permutation(self._next(), n)
kernel_name = 'interleave_layers__memory_aug_recurrent_mem_tr__linear_kernel_hedgehog__prompt'

def setup_inputs():
    _rng = _Rng(jax.random.key(int.from_bytes(__import__("os").urandom(4), "little")))
    _w = lambda a: (lambda t: t.astype(jnp.bfloat16) if jnp.issubdtype(t.dtype, jnp.floating) else t)(jnp.asarray(a))

    def _A_setup():
        B, S, Dm = (1, 2048, 640)
        H, Dh = (32, 192)
        M, seg = (8, 32)
        seg = min(seg, S)
        S = S // seg * seg
        return {'x': _w((lambda *s: _rng.normal(s) * 0.05)(B, S, Dm)), 'mem0': _w((lambda *s: _rng.normal(s) * 0.05)(B, M, Dm)), 'Wq': _w((lambda *s: _rng.normal(s) * 0.05)(Dm, H, Dh) * Dm ** (-0.5)), 'Wk': _w((lambda *s: _rng.normal(s) * 0.05)(Dm, H, Dh) * Dm ** (-0.5)), 'Wv': _w((lambda *s: _rng.normal(s) * 0.05)(Dm, H, Dh) * Dm ** (-0.5)), 'Wo': _w((lambda *s: _rng.normal(s) * 0.05)(H, Dh, Dm) * (H * Dh) ** (-0.5)), 'seg_len': seg}
    _A_in = _A_setup()

    def _B_setup():
        B, S, D, H = (1, 2048, 640, 32)
        Dh = D // H
        return {'x': _w((lambda *s: _rng.normal(s) * 0.05)(B, S, D)), 'wqkv': _w((lambda *s: _rng.normal(s) * 0.05)(D, 3 * D)), 'w_phi': _w((lambda *s: _rng.normal(s) * 0.05)(H, Dh, Dh) * Dh ** (-0.5)), 'wo': _w((lambda *s: _rng.normal(s) * 0.05)(D, D))}
    _B_in = _B_setup()
    return {'A_x': _A_in['x'], 'A_mem0': _A_in['mem0'], 'A_Wq': _A_in['Wq'], 'A_Wk': _A_in['Wk'], 'A_Wv': _A_in['Wv'], 'A_Wo': _A_in['Wo'], 'A_seg_len': _A_in['seg_len'], 'B_x': _B_in['x'], 'B_wqkv': _B_in['wqkv'], 'B_w_phi': _B_in['w_phi'], 'B_wo': _B_in['wo']}

def reference(A_x, A_mem0, A_Wq, A_Wk, A_Wv, A_Wo, A_seg_len, B_x, B_wqkv, B_w_phi, B_wo):

    def _A_ref(x, mem0, Wq, Wk, Wv, Wo, seg_len):
        B, S, Dm = x.shape
        H, Dh = (Wq.shape[1], Wq.shape[2])
        M = mem0.shape[1]
        scale = Dh ** (-0.5)
        n_seg = S // seg_len
        L = M + seg_len
        idx = jnp.arange(L)
        mask = (idx[:, None] < M) | (idx[:, None] >= idx[None, :])
        mem = mem0
        outs = []
        for s in range(n_seg):
            xs = x[:, s * seg_len:(s + 1) * seg_len, :].copy()
            h = jnp.concatenate([mem, xs], axis=1)
            q = jnp.einsum('btd,dhe->bhte', h, Wq)
            k = jnp.einsum('btd,dhe->bhte', h, Wk)
            v = jnp.einsum('btd,dhe->bhte', h, Wv)
            scores = jnp.einsum('bhqe,bhke->bhqk', q, k) * scale
            scores = jnp.where(mask[None, None], scores, -1000000000.0)
            p = _softmax(scores, axis=-1)
            o = jnp.einsum('bhqk,bhke->bhqe', p, v)
            o = jnp.einsum('bhte,hed->btd', o, Wo)
            mem = o[:, :M, :].copy()
            outs.append(o[:, M:, :])
        return jnp.concatenate(outs, axis=1)

    def _B_ref(x, wqkv, w_phi, wo):
        B, S, D = x.shape
        H = 32
        Dh = D // H
        qkv = (lambda x, *d: x.transpose(*d))((x @ wqkv).reshape(B, S, 3, H, Dh), 2, 0, 3, 1, 4)
        q, k, v = (qkv[0], qkv[1], qkv[2])
        pq = jnp.einsum('bhsd,hdf->bhsf', q, w_phi)
        pk = jnp.einsum('bhsd,hdf->bhsf', k, w_phi)
        phi_q = jnp.concatenate([_softmax(pq, axis=-1), _softmax(-pq, axis=-1)], axis=-1)
        phi_k = jnp.concatenate([_softmax(pk, axis=-1), _softmax(-pk, axis=-1)], axis=-1)
        kv = jnp.einsum('bhsf,bhsd->bhfd', phi_k, v)
        z = jnp.einsum('bhsf->bhf', phi_k)
        num = jnp.einsum('bhqf,bhfd->bhqd', phi_q, kv)
        den = jnp.einsum('bhqf,bhf->bhq', phi_q, z)[..., None] + 1e-06
        o = num / den
        return (lambda x, *d: x.transpose(*d))(o, 0, 2, 1, 3).reshape(B, S, D) @ wo
    x = A_x
    x = x + _A_ref(_layernorm(x, axis=-1), A_mem0, A_Wq, A_Wk, A_Wv, A_Wo, A_seg_len)
    x = x + _B_ref(_layernorm(x, axis=-1), B_wqkv, B_w_phi, B_wo)
    x = x + _A_ref(_layernorm(x, axis=-1), A_mem0, A_Wq, A_Wk, A_Wv, A_Wo, A_seg_len)
    x = x + _B_ref(_layernorm(x, axis=-1), B_wqkv, B_w_phi, B_wo)
    return x
```

```python
import functools

import jax
import jax.numpy as jnp
from jax import lax
import jax.experimental.pallas as pl
import jax.experimental.pallas.tpu as pltpu

F32 = jnp.float32
BF16 = jnp.bfloat16

B_HEADS = 32
LN_EPS = 1e-05
DEN_EPS = 1e-06
MASK_FILL = -1000000000.0

_NN = (((1,), (0,)), ((), ()))
_NT = (((1,), (1,)), ((), ()))


def _mm(a, b):
    return lax.dot_general(a, b, _NN, preferred_element_type=F32)


def _mm_nt(a, b):
    return lax.dot_general(a, b, _NT, preferred_element_type=F32)


def _iota(shape, dim):
    return lax.broadcasted_iota(jnp.int32, shape, dim)


def _div_const(r, d):
    mul = (1 << 18) // d + 1
    assert all((v * mul) >> 18 == v // d for v in range(4096))
    return (r * mul) >> 18


def _layernorm(x):
    m = jnp.mean(x, axis=-1, keepdims=True)
    xc = x - m
    v = jnp.mean(xc * xc, axis=-1, keepdims=True)
    return xc * lax.rsqrt(v + LN_EPS)


def _pair_reduce(v, op):
    v = op(v, pltpu.roll(v, 4, 0))
    return op(v, pltpu.roll(v, 2, 0))


def _hedgehog(p):
    rows = [p[i:i + 8] for i in range(0, p.shape[0], 8)]
    hi = _pair_reduce(functools.reduce(jnp.maximum, rows), jnp.maximum)
    lo = _pair_reduce(functools.reduce(jnp.minimum, rows), jnp.minimum)
    ep = [jnp.exp(r - hi) for r in rows]
    en = [jnp.exp(lo - r) for r in rows]
    rp = 1.0 / _pair_reduce(functools.reduce(jnp.add, ep), jnp.add)
    rn = 1.0 / _pair_reduce(functools.reduce(jnp.add, en), jnp.add)
    return jnp.concatenate([e * rp for e in ep] + [e * rn for e in en], axis=0)


def _kernel(
    x_hbm, mem0_ref, wq_hbm, wk_hbm, wv_hbm, wo_hbm, bqkv_hbm, wphi_ref, bwo_hbm,
    out_hbm,
    xin_ref, xres_ref, hn_ref, wqkv_ref, wo_ref, stage_ref, bqkv_ref, bwo_ref,
    bq_ref, bkv_ref, bo_ref, o_ref, pt_ref, ot_ref, kv_ref,
    sem_x, sem_b, sem_w, sem_wo, sem_out,
    *, seg, heads, dh, chunk,
):
    seq, dm = xres_ref.shape
    n_mem = mem0_ref.shape[0]
    n_seg = seq // seg
    rows = n_mem + seg
    pairs = heads // 2
    pw = 2 * dh
    off = -(-rows // 16) * 16
    scale = dh ** (-0.5)
    bdh = dm // B_HEADS
    grp = 2 * bdh
    n_grp = B_HEADS // 2

    cp_x = pltpu.make_async_copy(x_hbm, xin_ref, sem_x)
    cp_bqkv = pltpu.make_async_copy(bqkv_hbm, bqkv_ref, sem_b.at[0])
    cp_bwo = pltpu.make_async_copy(bwo_hbm, bwo_ref, sem_b.at[1])
    cp_wo = pltpu.make_async_copy(wo_hbm, wo_ref, sem_wo)

    def cp_w(m, j):
        src = (wq_hbm, wk_hbm, wv_hbm)[m]
        return pltpu.make_async_copy(
            src.at[pl.ds(pl.multiple_of(j * pw, pw), pw)], stage_ref.at[j, m], sem_w.at[j, m])

    cp_bqkv.start()
    cp_bwo.start()
    cp_x.start()
    for j in range(pairs):
        for m in range(3):
            cp_w(m, j).start()
    cp_wo.start()

    r = _iota((dm, dm), 0)
    c = _iota((dm, dm), 1)
    r_grp = _div_const(r, grp)
    r_feat = (r - r_grp * grp) >> 1
    r_head = 2 * r_grp + (r & 1)
    c_head = _div_const(c, bdh)
    c_feat = c - c_head * bdh
    same_head = r_head == c_head
    perm = jnp.where(same_head & (r_feat == c_feat), 1.0, 0.0).astype(BF16)

    eh_r = _iota((B_HEADS, dm), 0)
    eh_c = _iota((B_HEADS, dm), 1)
    phi_f = None
    for d in range(bdh):
        eh = jnp.where(eh_c == eh_r * bdh + d, 1.0, 0.0).astype(BF16)
        t = _mm(wphi_ref[d], eh)
        phi_f = t if phi_f is None else phi_f + t
    ef_r = _iota((dm, bdh), 0)
    ef_feat = (ef_r - _div_const(ef_r, grp) * grp) >> 1
    ef = jnp.where(ef_feat == _iota((dm, bdh), 1), 1.0, 0.0).astype(BF16)
    phi_t = jnp.where(same_head, _mm(ef, phi_f.astype(BF16)), 0.0).astype(BF16)

    cp_bqkv.wait()
    bq_ref[...] = _mm_nt(phi_t, bqkv_ref[:, 0:dm]).astype(BF16)
    bkv_ref[0:dm, :] = _mm_nt(phi_t, bqkv_ref[:, dm:2 * dm]).astype(BF16)
    bkv_ref[dm:2 * dm, :] = _mm_nt(perm, bqkv_ref[:, 2 * dm:3 * dm]).astype(BF16)
    cp_bwo.wait()
    bo_ref[...] = _mm(perm, bwo_ref[...]).astype(BF16)

    cp_x.wait()

    def init_body(i, carry):
        sl = pl.ds(pl.multiple_of(i * chunk, chunk), chunk)
        x = xin_ref[sl, :].astype(F32)
        xres_ref[sl, :] = x
        hn_ref[sl, :] = _layernorm(x)
        return carry

    lax.fori_loop(0, seq // chunk, init_body, 0)

    def tr_body(j, carry):
        for m in range(3):
            cp_w(m, j).wait()
            wqkv_ref[j, :, m * pw:(m + 1) * pw] = stage_ref[j, m].T
        return carry

    lax.fori_loop(0, pairs, tr_body, 0)
    cp_wo.wait()

    def block_diag(t):
        lane = _iota((rows, pw), 1)
        gap = jnp.zeros((off - rows, pw), F32)
        tail = jnp.zeros((128 - off - rows, pw), F32)
        first = jnp.where(lane < dh, t, 0.0)
        second = jnp.where(lane >= dh, t, 0.0)
        return jnp.concatenate([first, gap, second, tail], axis=0).astype(BF16)

    def a_step(s, mem):
        sl = pl.ds(pl.multiple_of(s * seg, seg), seg)
        h = jnp.concatenate([mem, hn_ref[sl, :]], axis=0)
        qi = _iota((rows, 128), 0)
        ki = _iota((rows, 128), 1)
        in_a = ki < rows
        in_b = (ki >= off) & (ki < off + rows)
        see_a = in_a & ((qi < n_mem) | (qi >= ki))
        see_b = in_b & ((qi < n_mem) | (qi >= ki - off))
        fill_a = jnp.where(in_a, MASK_FILL, -jnp.inf)
        fill_b = jnp.where(in_b, MASK_FILL, -jnp.inf)

        qkv, prob = {}, {}
        for j in range(pairs + 2):
            if j < pairs:
                qkv[j] = _mm(h, wqkv_ref[j])
            if 0 <= j - 1 < pairs:
                t = qkv[j - 1]
                sc = _mm_nt(t[:, 0:pw], block_diag(t[:, pw:2 * pw])) * scale
                sa = jnp.where(see_a, sc, fill_a)
                sb = jnp.where(see_b, sc, fill_b)
                ea = jnp.exp(sa - jnp.max(sa, axis=-1, keepdims=True))
                eb = jnp.exp(sb - jnp.max(sb, axis=-1, keepdims=True))
                ra = 1.0 / jnp.sum(ea, axis=-1, keepdims=True)
                rb = 1.0 / jnp.sum(eb, axis=-1, keepdims=True)
                prob[j - 1] = ea * ra + eb * rb
            if 0 <= j - 2 < pairs:
                t = qkv[j - 2]
                o_ref[:, (j - 2) * pw:(j - 1) * pw] = _mm(prob[j - 2], block_diag(t[:, 2 * pw:3 * pw]))
        y = _mm(o_ref[...], wo_ref[...])
        xn = xres_ref[sl, :] + y[n_mem:]
        xres_ref[sl, :] = xn
        hn_ref[sl, :] = _layernorm(xn)
        return y[:n_mem]

    def b_kv(i, carry):
        sl = pl.ds(pl.multiple_of(i * chunk, chunk), chunk)
        pt_ref[...] = _mm_nt(bkv_ref[...], hn_ref[sl, :].astype(BF16))
        ones = jnp.ones((8, chunk), F32)
        for g in range(n_grp):
            phi = _hedgehog(pt_ref[g * grp:(g + 1) * grp, :]).astype(BF16)
            v1 = jnp.concatenate([pt_ref[dm + g * grp:dm + (g + 1) * grp, :], ones], axis=0)
            kv_ref[g] += _mm_nt(v1, phi)
        return carry

    def b_out(i, carry):
        sl = pl.ds(pl.multiple_of(i * chunk, chunk), chunk)
        pt_ref[0:dm, :] = _mm_nt(bq_ref[...], hn_ref[sl, :].astype(BF16))
        for g in range(n_grp):
            phi = _hedgehog(pt_ref[g * grp:(g + 1) * grp, :]).astype(BF16)
            nd = _mm(kv_ref[g], phi)
            inv = 1.0 / (nd[grp:grp + 8] + DEN_EPS)
            ot_ref[g * grp:(g + 1) * grp, :] = jnp.concatenate(
                [nd[k:k + 8] * inv for k in range(0, grp, 8)], axis=0)
        o = ot_ref[...].astype(BF16).T
        xn = xres_ref[sl, :] + _mm(o, bo_ref[...])
        xres_ref[sl, :] = xn
        hn_ref[sl, :] = _layernorm(xn)
        return carry

    def layer_pair(_, carry):
        lax.fori_loop(0, n_seg, a_step, mem0_ref[...].astype(F32))
        kv_ref[...] = jnp.zeros(kv_ref.shape, F32)
        lax.fori_loop(0, seq // chunk, b_kv, 0)
        same = ((_iota(kv_ref.shape, 1) ^ _iota(kv_ref.shape, 2)) & 1) == 0
        kv_ref[...] = jnp.where(same, kv_ref[...], 0.0)
        lax.fori_loop(0, seq // chunk, b_out, 0)
        return carry

    lax.fori_loop(0, 2, layer_pair, 0)

    def fin_body(i, carry):
        sl = pl.ds(pl.multiple_of(i * chunk, chunk), chunk)
        xin_ref[sl, :] = xres_ref[sl, :].astype(BF16)
        return carry

    lax.fori_loop(0, seq // chunk, fin_body, 0)
    cp_out = pltpu.make_async_copy(xin_ref, out_hbm, sem_out)
    cp_out.start()
    cp_out.wait()


@functools.partial(jax.jit, static_argnames=("A_seg_len",))
def pallas_interleave_layers__memory_aug_recurrent_mem_tr__linear_kernel_hedgehog__prompt_kernel(
    A_x: jax.Array,
    A_mem0: jax.Array,
    A_Wq: jax.Array,
    A_Wk: jax.Array,
    A_Wv: jax.Array,
    A_Wo: jax.Array,
    A_seg_len: int,
    B_x: jax.Array,
    B_wqkv: jax.Array,
    B_w_phi: jax.Array,
    B_wo: jax.Array,
):
    del B_x
    batch, seq, dm = A_x.shape
    _, heads, dh = A_Wq.shape
    n_mem = A_mem0.shape[1]
    seg = int(A_seg_len)
    chunk = 256
    rows = n_mem + seg
    pw = 2 * dh
    pairs = heads // 2
    bdh = dm // B_HEADS
    assert batch == 1 and seq % seg == 0 and seq % chunk == 0
    assert n_mem % 8 == 0 and seg % 8 == 0 and -(-rows // 16) * 16 + rows <= 128
    assert heads % 2 == 0 and pw % 128 == 0 and dm % 128 == 0 and (2 * bdh) % 8 == 0

    w_t = lambda w: jnp.transpose(w, (1, 2, 0)).reshape(heads * dh, dm)
    hbm = pl.BlockSpec(memory_space=pl.ANY)
    vmem = pl.BlockSpec(memory_space=pltpu.VMEM)

    out = pl.pallas_call(
        functools.partial(_kernel, seg=seg, heads=heads, dh=dh, chunk=chunk),
        out_shape=jax.ShapeDtypeStruct((seq, dm), A_x.dtype),
        in_specs=[hbm, vmem, hbm, hbm, hbm, hbm, hbm, vmem, hbm],
        out_specs=hbm,
        scratch_shapes=[
            pltpu.VMEM((seq, dm), BF16),
            pltpu.VMEM((seq, dm), F32),
            pltpu.VMEM((seq, dm), F32),
            pltpu.VMEM((pairs, dm, 3 * pw), BF16),
            pltpu.VMEM((heads * dh, dm), BF16),
            pltpu.VMEM((pairs, 3, pw, dm), BF16),
            pltpu.VMEM((dm, 3 * dm), BF16),
            pltpu.VMEM((dm, dm), BF16),
            pltpu.VMEM((dm, dm), BF16),
            pltpu.VMEM((2 * dm, dm), BF16),
            pltpu.VMEM((dm, dm), BF16),
            pltpu.VMEM((rows, heads * dh), F32),
            pltpu.VMEM((2 * dm, chunk), F32),
            pltpu.VMEM((dm, chunk), F32),
            pltpu.VMEM((B_HEADS // 2, 2 * bdh + 8, 4 * bdh), F32),
            pltpu.SemaphoreType.DMA,
            pltpu.SemaphoreType.DMA((2,)),
            pltpu.SemaphoreType.DMA((pairs, 3)),
            pltpu.SemaphoreType.DMA,
            pltpu.SemaphoreType.DMA,
        ],
        compiler_params=pltpu.CompilerParams(vmem_limit_bytes=110 * 1024 * 1024),
    )(
        A_x.reshape(seq, dm),
        A_mem0.reshape(n_mem, dm),
        w_t(A_Wq), w_t(A_Wk), w_t(A_Wv),
        A_Wo.reshape(heads * dh, dm),
        B_wqkv,
        jnp.transpose(B_w_phi, (1, 2, 0)),
        B_wo,
    )
    return out.reshape(batch, seq, dm)
```

```python
import functools

import jax
import jax.numpy as jnp
from jax import lax
import jax.experimental.pallas as pl
import jax.experimental.pallas.tpu as pltpu

F32 = jnp.float32
BF16 = jnp.bfloat16

B_HEADS = 32
LN_EPS = 1e-05
DEN_EPS = 1e-06
MASK_FILL = -1000000000.0

LAG = 4
EARLY = 8
RING = 3
CHUNK = 256

_NN = (((1,), (0,)), ((), ()))
_NT = (((1,), (1,)), ((), ()))


def _mm(a, b):
    return lax.dot_general(a, b, _NN, preferred_element_type=F32)


def _mm_nt(a, b):
    return lax.dot_general(a, b, _NT, preferred_element_type=F32)


def _pack(w):
    return pltpu.bitcast(w, jnp.uint32)


def _unpack(w):
    return pltpu.bitcast(w, BF16)


def _iota(shape, dim):
    return lax.broadcasted_iota(jnp.int32, shape, dim)


def _div_const(r, d):
    mul = (1 << 18) // d + 1
    assert all((v * mul) >> 18 == v // d for v in range(4096))
    return (r * mul) >> 18


def _layernorm(x):
    m = jnp.mean(x, axis=-1, keepdims=True)
    xc = x - m
    v = jnp.mean(xc * xc, axis=-1, keepdims=True)
    return xc * lax.rsqrt(v + LN_EPS)


def _pair_reduce(v, op):
    v = op(v, pltpu.roll(v, 4, 0))
    return op(v, pltpu.roll(v, 2, 0))


def _hedgehog(p):
    rows = [p[i:i + 8] for i in range(0, p.shape[0], 8)]
    hi = _pair_reduce(functools.reduce(jnp.maximum, rows), jnp.maximum)
    lo = _pair_reduce(functools.reduce(jnp.minimum, rows), jnp.minimum)
    ep = [jnp.exp(r - hi) for r in rows]
    en = [jnp.exp(lo - r) for r in rows]
    rp = 1.0 / _pair_reduce(functools.reduce(jnp.add, ep), jnp.add)
    rn = 1.0 / _pair_reduce(functools.reduce(jnp.add, en), jnp.add)
    return jnp.concatenate([e * rp for e in ep] + [e * rn for e in en], axis=0)


def _kernel(
    x_hbm, mem0_ref, wq_hbm, wk_hbm, wv_hbm, wo_hbm, bqkv_hbm, wphi_ref, bwo_hbm,
    out_hbm,
    xin_ref, xe_ref, he_ref, xres_ref, hn_ref, wqkv_ref, wo_ref, stage_ref, early_ref,
    bqkv_ref, bwo_ref, bq_ref, bkv_ref, bo_ref,
    o_ref, y_ref, kt_ref, vb_ref, p_ref, pt_ref, ot_ref, kv_ref,
    sem_x, sem_b, sem_w, sem_out,
    *, seg, heads, dh,
):
    seq, dm = out_hbm.shape
    n_mem = mem0_ref.shape[0]
    n_seg = seq // seg
    rows = n_mem + seg
    pairs = heads // 2
    pw = 2 * dh
    off = -(-rows // 16) * 16
    scale = dh ** (-0.5)
    bdh = dm // B_HEADS
    grp = 2 * bdh
    n_grp = B_HEADS // 2

    cp_xe = pltpu.make_async_copy(x_hbm.at[:, seg // EARLY - 1], xe_ref, sem_x.at[0])
    cp_x = pltpu.make_async_copy(x_hbm, xin_ref, sem_x.at[1])
    cp_bqkv = pltpu.make_async_copy(bqkv_hbm, bqkv_ref, sem_b.at[0])
    cp_bwo = pltpu.make_async_copy(bwo_hbm, bwo_ref, sem_b.at[1])

    def cp_w(m, j):
        src = (wq_hbm, wk_hbm, wv_hbm, wo_hbm)[m]
        start = j * pw if isinstance(j, int) else pl.multiple_of(j * pw, pw)
        slot = j % RING
        return pltpu.make_async_copy(
            src.at[pl.ds(start, pw)], stage_ref.at[slot, m], sem_w.at[slot, m])

    cp_xe.start()
    for j in range(RING - 1):
        for m in (1, 2, 0, 3):
            cp_w(m, j).start()

    cp_xe.wait()
    he_ref[...] = _layernorm(xe_ref[...].astype(F32).reshape(n_seg * EARLY, dm))

    def load_body(j, carry):
        @pl.when(j + RING - 1 < pairs)
        def _():
            for m in (1, 2, 0, 3):
                cp_w(m, j + RING - 1).start()

        @pl.when(j + RING - 1 == pairs)
        def _():
            cp_x.start()

        for m in (1, 2, 0, 3):
            cp_w(m, j).wait()
        slot = j % RING
        for m in (1, 2):
            early_ref[j, :, (m - 1) * pw:m * pw] = _mm_nt(he_ref[...], stage_ref[slot, m])
        for m in range(3):
            wqkv_ref[j, :, m * pw:(m + 1) * pw] = _pack(stage_ref[slot, m].T)
        wo_ref[pl.ds(pl.multiple_of(j * dh, dh), dh), :] = _pack(stage_ref[slot, 3])
        return carry

    lax.fori_loop(0, pairs, load_body, 0)
    cp_x.wait()
    cp_bqkv.start()
    cp_bwo.start()

    def init_body(i, carry):
        sl = pl.ds(pl.multiple_of(i * CHUNK, CHUNK), CHUNK)
        n = CHUNK // seg
        x = xin_ref[pl.ds(i * n, n)].astype(F32).reshape(CHUNK, dm)
        xres_ref[sl, :] = x
        hn_ref[sl, :] = _layernorm(x)
        return carry

    lax.fori_loop(0, seq // CHUNK, init_body, 0)
    xres_ref[seq:seq + seg, :] = jnp.zeros((seg, dm), F32)

    def block_diag(t):
        lane = _iota((rows, pw), 1)
        gap = jnp.zeros((off - rows, pw), F32)
        tail = jnp.zeros((128 - off - rows, pw), F32)
        first = jnp.where(lane < dh, t, 0.0)
        second = jnp.where(lane >= dh, t, 0.0)
        return jnp.concatenate([first, gap, second, tail], axis=0).astype(BF16)

    def a_residual(s):
        sl = pl.ds(pl.multiple_of(s * seg, seg), seg)
        xn = xres_ref[sl, :] + y_ref[n_mem:rows, :]
        xres_ref[sl, :] = xn
        hn_ref[sl, :] = _layernorm(xn)

    def a_step(s, carry, *, first_layer):
        sl = pl.ds(pl.multiple_of(s * seg, seg), seg)
        h = jnp.concatenate([y_ref[0:n_mem, :], hn_ref[sl, :]], axis=0)
        a_residual(jnp.where(s == 0, n_seg, s - 1))
        qi = _iota((rows, 128), 0)
        ki = _iota((rows, 128), 1)
        in_a = ki < rows
        in_b = (ki >= off) & (ki < off + rows)
        see_a = in_a & ((qi < n_mem) | (qi >= ki))
        see_b = in_b & ((qi < n_mem) | (qi >= ki - off))
        fill_a = jnp.where(in_a, MASK_FILL, -jnp.inf)
        fill_b = jnp.where(in_b, MASK_FILL, -jnp.inf)

        def proj(m, j):
            w = _unpack(wqkv_ref[j, :, m * pw:(m + 1) * pw])
            if first_layer and m > 0:
                done = early_ref[j, pl.ds(pl.multiple_of(s * EARLY, EARLY), EARLY), (m - 1) * pw:m * pw]
                return jnp.concatenate([_mm(h[:rows - EARLY], w), done], axis=0)
            return _mm(h, w)

        def scores(j):
            sc = _mm(o_ref[:, j * pw:(j + 1) * pw], _unpack(kt_ref[j])) * scale
            sa = jnp.where(see_a, sc, fill_a)
            sb = jnp.where(see_b, sc, fill_b)
            ea = jnp.exp(sa - jnp.max(sa, axis=-1, keepdims=True))
            eb = jnp.exp(sb - jnp.max(sb, axis=-1, keepdims=True))
            ra = 1.0 / jnp.sum(ea, axis=-1, keepdims=True)
            rb = 1.0 / jnp.sum(eb, axis=-1, keepdims=True)
            p_ref[j] = ea * ra + eb * rb

        def attend(j):
            o_ref[:, j * pw:(j + 1) * pw] = _mm(p_ref[j], _unpack(vb_ref[j]))

        def out_proj(j0, j1):
            return _mm(o_ref[:, j0 * pw:j1 * pw], _unpack(wo_ref[j0 * dh:j1 * dh, :]))

        for j in range(pairs):
            kt_ref[j] = _pack(block_diag(proj(1, j)).T)
        for j in range(pairs):
            o_ref[:, j * pw:(j + 1) * pw] = proj(0, j)
            if j >= LAG:
                scores(j - LAG)
        for j in range(pairs):
            v = proj(2, j)
            if j < LAG:
                scores(pairs - LAG + j)
            vb_ref[j] = _pack(block_diag(v))
            if j >= LAG:
                attend(j - LAG)
        y = out_proj(0, pairs // 2)
        for j in range(pairs - LAG, pairs):
            attend(j)
        y_ref[...] = y + out_proj(pairs // 2, pairs)
        return carry

    def b_fold_weights():
        r = _iota((dm, dm), 0)
        c = _iota((dm, dm), 1)
        r_grp = _div_const(r, grp)
        r_feat = (r - r_grp * grp) >> 1
        r_head = 2 * r_grp + (r & 1)
        c_head = _div_const(c, bdh)
        c_feat = c - c_head * bdh
        same_head = r_head == c_head
        perm = jnp.where(same_head & (r_feat == c_feat), 1.0, 0.0).astype(BF16)

        eh_r = _iota((B_HEADS, dm), 0)
        eh_c = _iota((B_HEADS, dm), 1)
        phi_f = None
        for d in range(bdh):
            eh = jnp.where(eh_c == eh_r * bdh + d, 1.0, 0.0).astype(BF16)
            t = _mm(wphi_ref[d], eh)
            phi_f = t if phi_f is None else phi_f + t
        ef_r = _iota((dm, bdh), 0)
        ef_feat = (ef_r - _div_const(ef_r, grp) * grp) >> 1
        ef = jnp.where(ef_feat == _iota((dm, bdh), 1), 1.0, 0.0).astype(BF16)
        phi_t = jnp.where(same_head, _mm(ef, phi_f.astype(BF16)), 0.0).astype(BF16)

        cp_bqkv.wait()
        bq_ref[...] = _pack(_mm_nt(phi_t, bqkv_ref[:, 0:dm]).astype(BF16))
        bkv_ref[0:dm // 2, :] = _pack(_mm_nt(phi_t, bqkv_ref[:, dm:2 * dm]).astype(BF16))
        bkv_ref[dm // 2:dm, :] = _pack(_mm_nt(perm, bqkv_ref[:, 2 * dm:3 * dm]).astype(BF16))
        cp_bwo.wait()
        bo_ref[...] = _pack(_mm(perm, bwo_ref[...]).astype(BF16))

    def b_kv(i, carry):
        sl = pl.ds(pl.multiple_of(i * CHUNK, CHUNK), CHUNK)
        pt_ref[...] = _mm_nt(_unpack(bkv_ref[...]), hn_ref[sl, :].astype(BF16))
        ones = jnp.ones((8, CHUNK), F32)
        for g in range(n_grp):
            phi = _hedgehog(pt_ref[g * grp:(g + 1) * grp, :]).astype(BF16)
            v1 = jnp.concatenate([pt_ref[dm + g * grp:dm + (g + 1) * grp, :], ones], axis=0)
            kv_ref[g] += _mm_nt(v1, phi)
        return carry

    def b_out(i, carry):
        sl = pl.ds(pl.multiple_of(i * CHUNK, CHUNK), CHUNK)
        pt_ref[0:dm, :] = _mm_nt(_unpack(bq_ref[...]), hn_ref[sl, :].astype(BF16))
        for g in range(n_grp):
            phi = _hedgehog(pt_ref[g * grp:(g + 1) * grp, :]).astype(BF16)
            nd = _mm(kv_ref[g], phi)
            inv = 1.0 / (nd[grp:grp + 8] + DEN_EPS)
            ot_ref[g * grp:(g + 1) * grp, :] = jnp.concatenate(
                [nd[k:k + 8] * inv for k in range(0, grp, 8)], axis=0)
        o = ot_ref[...].astype(BF16).T
        xn = xres_ref[sl, :] + _mm(o, _unpack(bo_ref[...]))
        xres_ref[sl, :] = xn
        hn_ref[sl, :] = _layernorm(xn)
        return carry

    def layer_pair(it, carry):
        y_ref[0:n_mem, :] = mem0_ref[...].astype(F32)
        y_ref[n_mem:rows, :] = jnp.zeros((seg, dm), F32)

        @pl.when(it == 0)
        def _():
            lax.fori_loop(0, n_seg, functools.partial(a_step, first_layer=True), 0)
            b_fold_weights()

        @pl.when(it == 1)
        def _():
            lax.fori_loop(0, n_seg, functools.partial(a_step, first_layer=False), 0)

        a_residual(n_seg - 1)
        kv_ref[...] = jnp.zeros(kv_ref.shape, F32)
        lax.fori_loop(0, seq // CHUNK, b_kv, 0)
        same = ((_iota(kv_ref.shape, 1) ^ _iota(kv_ref.shape, 2)) & 1) == 0
        kv_ref[...] = jnp.where(same, kv_ref[...], 0.0)
        lax.fori_loop(0, seq // CHUNK, b_out, 0)
        return carry

    lax.fori_loop(0, 2, layer_pair, 0)

    def fin_body(i, carry):
        sl = pl.ds(pl.multiple_of(i * CHUNK, CHUNK), CHUNK)
        pt_out_ref[sl, :] = xres_ref[sl, :].astype(BF16)
        return carry

    pt_out_ref = xin_ref.reshape(seq, dm)
    lax.fori_loop(0, seq // CHUNK, fin_body, 0)
    cp_out = pltpu.make_async_copy(pt_out_ref, out_hbm, sem_out)
    cp_out.start()
    cp_out.wait()


@functools.partial(jax.jit, static_argnames=("A_seg_len",))
def pallas_interleave_layers__memory_aug_recurrent_mem_tr__linear_kernel_hedgehog__prompt_kernel(
    A_x: jax.Array,
    A_mem0: jax.Array,
    A_Wq: jax.Array,
    A_Wk: jax.Array,
    A_Wv: jax.Array,
    A_Wo: jax.Array,
    A_seg_len: int,
    B_x: jax.Array,
    B_wqkv: jax.Array,
    B_w_phi: jax.Array,
    B_wo: jax.Array,
):
    del B_x
    batch, seq, dm = A_x.shape
    _, heads, dh = A_Wq.shape
    n_mem = A_mem0.shape[1]
    seg = int(A_seg_len)
    n_seg = seq // seg
    rows = n_mem + seg
    pw = 2 * dh
    pairs = heads // 2
    bdh = dm // B_HEADS
    assert batch == 1 and seq % CHUNK == 0 and CHUNK % seg == 0 and seg % EARLY == 0
    assert n_mem % 8 == 0 and -(-rows // 16) * 16 + rows <= 128
    assert heads % 2 == 0 and pw % 128 == 0 and dm % 128 == 0 and (2 * bdh) % 8 == 0

    w_t = lambda w: jnp.transpose(w, (1, 2, 0)).reshape(heads * dh, dm)
    hbm = pl.BlockSpec(memory_space=pl.ANY)
    vmem = pl.BlockSpec(memory_space=pltpu.VMEM)

    out = pl.pallas_call(
        functools.partial(_kernel, seg=seg, heads=heads, dh=dh),
        out_shape=jax.ShapeDtypeStruct((seq, dm), A_x.dtype),
        in_specs=[hbm, vmem, hbm, hbm, hbm, hbm, hbm, vmem, hbm],
        out_specs=hbm,
        scratch_shapes=[
            pltpu.VMEM((n_seg, seg // EARLY, EARLY, dm), BF16),
            pltpu.VMEM((n_seg, EARLY, dm), BF16),
            pltpu.VMEM((n_seg * EARLY, dm), F32),
            pltpu.VMEM((seq + seg, dm), F32),
            pltpu.VMEM((seq + seg, dm), F32),
            pltpu.VMEM((pairs, dm // 2, 3 * pw), jnp.uint32),
            pltpu.VMEM((pairs * dh, dm), jnp.uint32),
            pltpu.VMEM((RING, 4, pw, dm), BF16),
            pltpu.VMEM((pairs, n_seg * EARLY, 2 * pw), F32),
            pltpu.VMEM((dm, 3 * dm), BF16),
            pltpu.VMEM((dm, dm), BF16),
            pltpu.VMEM((dm // 2, dm), jnp.uint32),
            pltpu.VMEM((dm, dm), jnp.uint32),
            pltpu.VMEM((dm // 2, dm), jnp.uint32),
            pltpu.VMEM((rows, heads * dh), F32),
            pltpu.VMEM((rows, dm), F32),
            pltpu.VMEM((pairs, dh, 128), jnp.uint32),
            pltpu.VMEM((pairs, 64, pw), jnp.uint32),
            pltpu.VMEM((pairs, rows, 128), F32),
            pltpu.VMEM((2 * dm, CHUNK), F32),
            pltpu.VMEM((dm, CHUNK), F32),
            pltpu.VMEM((B_HEADS // 2, 2 * bdh + 8, 4 * bdh), F32),
            pltpu.SemaphoreType.DMA((2,)),
            pltpu.SemaphoreType.DMA((2,)),
            pltpu.SemaphoreType.DMA((RING, 4)),
            pltpu.SemaphoreType.DMA,
        ],
        compiler_params=pltpu.CompilerParams(vmem_limit_bytes=120 * 1024 * 1024),
    )(
        A_x.reshape(n_seg, seg // EARLY, EARLY, dm),
        A_mem0.reshape(n_mem, dm),
        w_t(A_Wq), w_t(A_Wk), w_t(A_Wv),
        A_Wo.reshape(heads * dh, dm),
        B_wqkv,
        jnp.transpose(B_w_phi, (1, 2, 0)),
        B_wo,
    )
    return out.reshape(batch, seq, dm)
```

```python
import functools

import jax
import jax.numpy as jnp
from jax import lax
import jax.experimental.pallas as pl
import jax.experimental.pallas.tpu as pltpu

F32 = jnp.float32
BF16 = jnp.bfloat16

B_HEADS = 32
LN_EPS = 1e-05
DEN_EPS = 1e-06
MASK_FILL = -1000000000.0

LAG = 4
EARLY = 8
RING = 3
CHUNK = 256
B_LAG = 2

_NN = (((1,), (0,)), ((), ()))
_NT = (((1,), (1,)), ((), ()))


def _mm(a, b):
    return lax.dot_general(a, b, _NN, preferred_element_type=F32)


def _mm_nt(a, b):
    return lax.dot_general(a, b, _NT, preferred_element_type=F32)


def _pack(w):
    return pltpu.bitcast(w, jnp.uint32)


def _unpack(w):
    return pltpu.bitcast(w, BF16)


def _iota(shape, dim):
    return lax.broadcasted_iota(jnp.int32, shape, dim)


def _div_const(r, d):
    mul = (1 << 18) // d + 1
    assert all((v * mul) >> 18 == v // d for v in range(4096))
    return (r * mul) >> 18


def _layernorm(x):
    m = jnp.mean(x, axis=-1, keepdims=True)
    xc = x - m
    v = jnp.mean(xc * xc, axis=-1, keepdims=True)
    return xc * lax.rsqrt(v + LN_EPS)


def _pair_reduce(v, op):
    v = op(v, pltpu.roll(v, 4, 0))
    return op(v, pltpu.roll(v, 2, 0))


def _hedgehog(p):
    rows = [p[i:i + 8] for i in range(0, p.shape[0], 8)]
    hi = _pair_reduce(functools.reduce(jnp.maximum, rows), jnp.maximum)
    lo = _pair_reduce(functools.reduce(jnp.minimum, rows), jnp.minimum)
    ep = [jnp.exp(r - hi) for r in rows]
    en = [jnp.exp(lo - r) for r in rows]
    rp = 1.0 / _pair_reduce(functools.reduce(jnp.add, ep), jnp.add)
    rn = 1.0 / _pair_reduce(functools.reduce(jnp.add, en), jnp.add)
    return jnp.concatenate([e * rp for e in ep] + [e * rn for e in en], axis=0)


def _kernel(
    x_hbm, mem0_ref, wq_hbm, wk_hbm, wv_hbm, wo_hbm, bqkv_hbm, wphi_ref, bwo_hbm,
    out_hbm,
    xin_ref, xe_ref, he_ref, xres_ref, hn_ref, wqkv_ref, wo_ref, stage_ref, early_ref,
    bqkv_ref, bwo_ref, sel_ref, bq_ref, bkv_ref, bo_ref,
    o_ref, y_ref, kt_ref, vb_ref, p_ref, ht_ref, ot_ref, kv_ref, res_ref,
    sem_x, sem_b, sem_w, sem_out,
    *, seg, heads, dh,
):
    seq, dm = out_hbm.shape
    n_mem = mem0_ref.shape[0]
    n_seg = seq // seg
    rows = n_mem + seg
    pairs = heads // 2
    pw = 2 * dh
    off = -(-rows // 16) * 16
    scale = dh ** (-0.5)
    bdh = dm // B_HEADS
    grp = 2 * bdh
    n_grp = B_HEADS // 2

    cp_xe = pltpu.make_async_copy(x_hbm.at[:, seg // EARLY - 1], xe_ref, sem_x.at[0])
    cp_x = pltpu.make_async_copy(x_hbm, xin_ref, sem_x.at[1])
    cp_bqkv = pltpu.make_async_copy(bqkv_hbm, bqkv_ref, sem_b.at[0])
    cp_bwo = pltpu.make_async_copy(bwo_hbm, bwo_ref, sem_b.at[1])

    def cp_w(m, j):
        src = (wq_hbm, wk_hbm, wv_hbm, wo_hbm)[m]
        start = j * pw if isinstance(j, int) else pl.multiple_of(j * pw, pw)
        slot = j % RING
        return pltpu.make_async_copy(
            src.at[pl.ds(start, pw)], stage_ref.at[slot, m], sem_w.at[slot, m])

    def groups_of(kt):
        return range(128 * kt // grp, (128 * kt + 127) // grp + 1)

    def build_selectors():
        eh_r = _iota((B_HEADS, dm), 0)
        eh_c = _iota((B_HEADS, dm), 1)
        phi_f = None
        for d in range(bdh):
            eh = jnp.where(eh_c == eh_r * bdh + d, 1.0, 0.0).astype(BF16)
            t = _mm(wphi_ref[d], eh)
            phi_f = t if phi_f is None else phi_f + t
        pick = jnp.where((_iota((grp, bdh), 0) >> 1) == _iota((grp, bdh), 1), 1.0, 0.0)
        phi_rows = _mm(pick, phi_f.astype(BF16))
        r = _iota((grp, 128), 0)
        for kt in range(dm // 128):
            c = _iota((grp, 128), 1) + 128 * kt
            c_head = _div_const(c, bdh)
            for i, g in enumerate(groups_of(kt)):
                head = 2 * g + (r & 1)
                sel_ref[0, kt, i] = jnp.where(c_head == head, phi_rows[:, 128 * kt:128 * kt + 128], 0.0)
                sel_ref[1, kt, i] = jnp.where(c == head * bdh + (r >> 1), 1.0, 0.0)

    cp_xe.start()
    for j in range(RING - 1):
        for m in (1, 2, 0, 3):
            cp_w(m, j).start()

    build_selectors()
    cp_xe.wait()
    he_ref[...] = _layernorm(xe_ref[...].astype(F32).reshape(n_seg * EARLY, dm))

    def load_body(j, carry):
        @pl.when(j + RING - 1 < pairs)
        def _():
            for m in (1, 2, 0, 3):
                cp_w(m, j + RING - 1).start()

        @pl.when(j + RING - 1 == pairs)
        def _():
            cp_x.start()

        for m in (1, 2, 0, 3):
            cp_w(m, j).wait()
        slot = j % RING
        for m in (1, 2):
            early_ref[j, :, (m - 1) * pw:m * pw] = _mm_nt(he_ref[...], stage_ref[slot, m])
        for m in range(3):
            wqkv_ref[j, :, m * pw:(m + 1) * pw] = _pack(stage_ref[slot, m].T)
        wo_ref[pl.ds(pl.multiple_of(j * dh, dh), dh), :] = _pack(stage_ref[slot, 3])
        return carry

    lax.fori_loop(0, pairs, load_body, 0)
    cp_x.wait()
    cp_bqkv.start()
    cp_bwo.start()

    def init_body(i, carry):
        sl = pl.ds(pl.multiple_of(i * CHUNK, CHUNK), CHUNK)
        n = CHUNK // seg
        x = xin_ref[pl.ds(i * n, n)].astype(F32).reshape(CHUNK, dm)
        xres_ref[sl, :] = x
        hn_ref[sl, :] = _layernorm(x)
        return carry

    lax.fori_loop(0, seq // CHUNK, init_body, 0)
    xres_ref[seq:seq + seg, :] = jnp.zeros((seg, dm), F32)

    def block_diag(t):
        lane = _iota((rows, pw), 1)
        gap = jnp.zeros((off - rows, pw), F32)
        tail = jnp.zeros((128 - off - rows, pw), F32)
        first = jnp.where(lane < dh, t, 0.0)
        second = jnp.where(lane >= dh, t, 0.0)
        return jnp.concatenate([first, gap, second, tail], axis=0).astype(BF16)

    def a_residual(s):
        sl = pl.ds(s * seg if isinstance(s, int) else pl.multiple_of(s * seg, seg), seg)
        xn = xres_ref[sl, :] + y_ref[n_mem:rows, :]
        xres_ref[sl, :] = xn
        hn_ref[sl, :] = _layernorm(xn)

    def a_step(s, carry, *, first_layer):
        sl = pl.ds(pl.multiple_of(s * seg, seg), seg)
        h = jnp.concatenate([y_ref[0:n_mem, :], hn_ref[sl, :]], axis=0)
        a_residual(jnp.where(s == 0, n_seg, s - 1))
        qi = _iota((rows, 128), 0)
        ki = _iota((rows, 128), 1)
        in_a = ki < rows
        in_b = (ki >= off) & (ki < off + rows)
        see_a = in_a & ((qi < n_mem) | (qi >= ki))
        see_b = in_b & ((qi < n_mem) | (qi >= ki - off))
        fill_a = jnp.where(in_a, MASK_FILL, -jnp.inf)
        fill_b = jnp.where(in_b, MASK_FILL, -jnp.inf)

        def proj(m, j):
            w = _unpack(wqkv_ref[j, :, m * pw:(m + 1) * pw])
            if first_layer and m > 0:
                done = early_ref[j, pl.ds(pl.multiple_of(s * EARLY, EARLY), EARLY), (m - 1) * pw:m * pw]
                return jnp.concatenate([_mm(h[:rows - EARLY], w), done], axis=0)
            return _mm(h, w)

        def scores(j):
            sc = _mm(o_ref[:, j * pw:(j + 1) * pw], _unpack(kt_ref[j])) * scale
            sa = jnp.where(see_a, sc, fill_a)
            sb = jnp.where(see_b, sc, fill_b)
            ea = jnp.exp(sa - jnp.max(sa, axis=-1, keepdims=True))
            eb = jnp.exp(sb - jnp.max(sb, axis=-1, keepdims=True))
            ra = 1.0 / jnp.sum(ea, axis=-1, keepdims=True)
            rb = 1.0 / jnp.sum(eb, axis=-1, keepdims=True)
            p_ref[j] = ea * ra + eb * rb

        def attend(j):
            o_ref[:, j * pw:(j + 1) * pw] = _mm(p_ref[j], _unpack(vb_ref[j]))

        def out_proj(j0, j1):
            return _mm(o_ref[:, j0 * pw:j1 * pw], _unpack(wo_ref[j0 * dh:j1 * dh, :]))

        for j in range(pairs):
            kt_ref[j] = _pack(block_diag(proj(1, j)).T)
        for j in range(pairs):
            o_ref[:, j * pw:(j + 1) * pw] = proj(0, j)
            if j >= LAG:
                scores(j - LAG)
        for j in range(pairs):
            v = proj(2, j)
            if j < LAG:
                scores(pairs - LAG + j)
            vb_ref[j] = _pack(block_diag(v))
            if j >= LAG:
                attend(j - LAG)
        y = out_proj(0, pairs // 2)
        for j in range(pairs - LAG, pairs):
            attend(j)
        y_ref[...] = y + out_proj(pairs // 2, pairs)
        return carry

    def b_fold_weights():
        def fold(which, product):
            out = {}
            for kt in range(dm // 128):
                gs = groups_of(kt)
                block = jnp.concatenate([sel_ref[which, kt, i] for i in range(len(gs))], axis=0)
                part = product(block, 128 * kt)
                for i, g in enumerate(gs):
                    t = part[i * grp:(i + 1) * grp]
                    out[g] = out[g] + t if g in out else t
            return out

        def store(ref, blocks):
            for i in range(0, len(blocks), 2):
                two = jnp.concatenate(blocks[i:i + 2], axis=0).astype(BF16)
                ref[i * bdh:(i + 2) * bdh, :] = _pack(two)

        def from_qkv(m):
            return lambda b, c: _mm_nt(b, bqkv_ref[:, m * dm + c:m * dm + c + 128])

        cp_bqkv.wait()
        cp_bwo.wait()
        wk, wv = fold(0, from_qkv(1)), fold(1, from_qkv(2))
        store(bkv_ref, [w[g] for g in range(n_grp) for w in (wk, wv)])
        wq = fold(0, from_qkv(0))
        store(bq_ref, [wq[g] for g in range(n_grp)])
        wo = fold(1, lambda b, c: _mm(b, bwo_ref[c:c + 128, :]))
        store(bo_ref, [wo[g] for g in range(n_grp)])

    n_chunk = seq // CHUNK
    tokens = lambda i: slice(i * CHUNK, (i + 1) * CHUNK)

    def b_kv():
        ones = jnp.ones((8, CHUNK), F32)

        def transpose(i):
            ht_ref[:, tokens(i)] = _pack(hn_ref[tokens(i), :].astype(BF16).T)

        work = [(i, g) for i in range(n_chunk) for g in range(n_grp)]
        ready = {}
        transpose(0)
        for n in range(len(work) + B_LAG):
            if n < len(work):
                i, g = work[n]
                if g == 0 and i + 1 < n_chunk:
                    transpose(i + 1)
                t = _mm(_unpack(bkv_ref[g * grp:(g + 1) * grp, :]), _unpack(ht_ref[:, tokens(i)]))
                ready[n] = (jnp.concatenate([t[grp:], ones], axis=0), _hedgehog(t[:grp]).astype(BF16))
            if n >= B_LAG:
                i, g = work[n - B_LAG]
                t = _mm_nt(*ready.pop(n - B_LAG))
                kv_ref[g] = t if i == 0 else kv_ref[g] + t
        same = ((_iota(kv_ref.shape, 1) ^ _iota(kv_ref.shape, 2)) & 1) == 0
        kv_ref[...] = jnp.where(same, kv_ref[...], 0.0)

    def cp_out(i):
        return pltpu.make_async_copy(res_ref.at[tokens(i)], out_hbm.at[tokens(i)], sem_out.at[i])

    def b_out():
        half = n_grp // 2
        work = [(i, gg) for i in range(n_chunk) for gg in range(half)]
        ready = {}

        def finish(i):
            o = ot_ref[i % 2].astype(BF16).T
            xn = xres_ref[tokens(i), :] + _mm(o, _unpack(bo_ref[...]))
            xres_ref[tokens(i), :] = xn
            hn_ref[tokens(i), :] = _layernorm(xn)
            res_ref[tokens(i), :] = xn.astype(BF16)
            cp_out(i).start()

        for n in range(len(work) + B_LAG):
            if n < len(work):
                i, gg = work[n]
                t = _mm(_unpack(bq_ref[gg * grp:(gg + 1) * grp, :]), _unpack(ht_ref[:, tokens(i)]))
                ready[n] = [_hedgehog(t[k * grp:(k + 1) * grp]).astype(BF16) for k in range(2)]
                if i > 0 and gg == half - 1:
                    finish(i - 1)
            if n >= B_LAG:
                i, gg = work[n - B_LAG]
                for k, phi in enumerate(ready.pop(n - B_LAG)):
                    g = 2 * gg + k
                    nd = _mm(kv_ref[g], phi)
                    inv = 1.0 / (nd[grp:grp + 8] + DEN_EPS)
                    ot_ref[i % 2, g * grp:(g + 1) * grp, :] = jnp.concatenate(
                        [nd[r:r + 8] * inv for r in range(0, grp, 8)], axis=0)
        finish(n_chunk - 1)

    def layer_pair(it, carry):
        y_ref[0:n_mem, :] = mem0_ref[...].astype(F32)
        y_ref[n_mem:rows, :] = jnp.zeros((seg, dm), F32)

        @pl.when(it == 0)
        def _():
            lax.fori_loop(0, n_seg, functools.partial(a_step, first_layer=True), 0)
            b_fold_weights()

        @pl.when(it == 1)
        def _():
            lax.fori_loop(0, n_seg, functools.partial(a_step, first_layer=False), 0)
            for i in range(n_chunk):
                cp_out(i).wait()

        a_residual(n_seg - 1)
        with jax.named_scope("L_b_kv"):
            b_kv()
        with jax.named_scope("L_b_out"):
            b_out()
        return carry

    lax.fori_loop(0, 2, layer_pair, 0)
    for i in range(n_chunk):
        cp_out(i).wait()


@functools.partial(jax.jit, static_argnames=("A_seg_len",))
def pallas_interleave_layers__memory_aug_recurrent_mem_tr__linear_kernel_hedgehog__prompt_kernel(
    A_x: jax.Array,
    A_mem0: jax.Array,
    A_Wq: jax.Array,
    A_Wk: jax.Array,
    A_Wv: jax.Array,
    A_Wo: jax.Array,
    A_seg_len: int,
    B_x: jax.Array,
    B_wqkv: jax.Array,
    B_w_phi: jax.Array,
    B_wo: jax.Array,
):
    del B_x
    batch, seq, dm = A_x.shape
    _, heads, dh = A_Wq.shape
    n_mem = A_mem0.shape[1]
    seg = int(A_seg_len)
    n_seg = seq // seg
    rows = n_mem + seg
    pw = 2 * dh
    pairs = heads // 2
    bdh = dm // B_HEADS
    assert batch == 1 and seq % CHUNK == 0 and CHUNK % seg == 0 and seg % EARLY == 0
    assert n_mem % 8 == 0 and -(-rows // 16) * 16 + rows <= 128
    assert heads % 2 == 0 and pw % 128 == 0 and dm % 128 == 0 and (2 * bdh) % 8 == 0

    w_t = lambda w: jnp.transpose(w, (1, 2, 0)).reshape(heads * dh, dm)
    hbm = pl.BlockSpec(memory_space=pl.ANY)
    vmem = pl.BlockSpec(memory_space=pltpu.VMEM)

    out = pl.pallas_call(
        functools.partial(_kernel, seg=seg, heads=heads, dh=dh),
        out_shape=jax.ShapeDtypeStruct((seq, dm), A_x.dtype),
        in_specs=[hbm, vmem, hbm, hbm, hbm, hbm, hbm, vmem, hbm],
        out_specs=hbm,
        scratch_shapes=[
            pltpu.VMEM((n_seg, seg // EARLY, EARLY, dm), BF16),
            pltpu.VMEM((n_seg, EARLY, dm), BF16),
            pltpu.VMEM((n_seg * EARLY, dm), F32),
            pltpu.VMEM((seq + seg, dm), F32),
            pltpu.VMEM((seq + seg, dm), F32),
            pltpu.VMEM((pairs, dm // 2, 3 * pw), jnp.uint32),
            pltpu.VMEM((pairs * dh, dm), jnp.uint32),
            pltpu.VMEM((RING, 4, pw, dm), BF16),
            pltpu.VMEM((pairs, n_seg * EARLY, 2 * pw), F32),
            pltpu.VMEM((dm, 3 * dm), BF16),
            pltpu.VMEM((dm, dm), BF16),
            pltpu.VMEM((2, dm // 128, 127 // (2 * bdh) + 2, 2 * bdh, 128), F32),
            pltpu.VMEM((dm // 2, dm), jnp.uint32),
            pltpu.VMEM((dm, dm), jnp.uint32),
            pltpu.VMEM((dm // 2, dm), jnp.uint32),
            pltpu.VMEM((rows, heads * dh), F32),
            pltpu.VMEM((rows, dm), F32),
            pltpu.VMEM((pairs, dh, 128), jnp.uint32),
            pltpu.VMEM((pairs, 64, pw), jnp.uint32),
            pltpu.VMEM((pairs, rows, 128), F32),
            pltpu.VMEM((dm // 2, seq), jnp.uint32),
            pltpu.VMEM((2, dm, CHUNK), F32),
            pltpu.VMEM((B_HEADS // 2, 2 * bdh + 8, 4 * bdh), F32),
            pltpu.VMEM((seq, dm), BF16),
            pltpu.SemaphoreType.DMA((2,)),
            pltpu.SemaphoreType.DMA((2,)),
            pltpu.SemaphoreType.DMA((RING, 4)),
            pltpu.SemaphoreType.DMA((seq // CHUNK,)),
        ],
        compiler_params=pltpu.CompilerParams(vmem_limit_bytes=120 * 1024 * 1024),
    )(
        A_x.reshape(n_seg, seg // EARLY, EARLY, dm),
        A_mem0.reshape(n_mem, dm),
        w_t(A_Wq), w_t(A_Wk), w_t(A_Wv),
        A_Wo.reshape(heads * dh, dm),
        B_wqkv,
        jnp.transpose(B_w_phi, (1, 2, 0)),
        B_wo,
    )
    return out.reshape(batch, seq, dm)
```

```python
import functools

import jax
import jax.numpy as jnp
from jax import lax
import jax.experimental.pallas as pl
import jax.experimental.pallas.tpu as pltpu

F32 = jnp.float32
BF16 = jnp.bfloat16

B_HEADS = 32
LN_EPS = 1e-05
DEN_EPS = 1e-06
MASK_FILL = -1000000000.0

LAG = 4
EARLY = 8
UNROLL = 2
RING = 4
CHUNK = 256
B_LAG = 2

_NN = (((1,), (0,)), ((), ()))
_NT = (((1,), (1,)), ((), ()))


def _mm(a, b):
    return lax.dot_general(a, b, _NN, preferred_element_type=F32)


def _mm_nt(a, b):
    return lax.dot_general(a, b, _NT, preferred_element_type=F32)


def _pack(w):
    return pltpu.bitcast(w, jnp.uint32)


def _unpack(w):
    return pltpu.bitcast(w, BF16)


def _iota(shape, dim):
    return lax.broadcasted_iota(jnp.int32, shape, dim)


def _div_const(r, d):
    mul = (1 << 18) // d + 1
    assert all((v * mul) >> 18 == v // d for v in range(4096))
    return (r * mul) >> 18


def _layernorm(x):
    m = jnp.mean(x, axis=-1, keepdims=True)
    xc = x - m
    v = jnp.mean(xc * xc, axis=-1, keepdims=True)
    return xc * lax.rsqrt(v + LN_EPS)


def _pair_reduce(v, op):
    v = op(v, pltpu.roll(v, 4, 0))
    return op(v, pltpu.roll(v, 2, 0))


def _hedgehog(p):
    rows = [p[i:i + 8] for i in range(0, p.shape[0], 8)]
    hi = _pair_reduce(functools.reduce(jnp.maximum, rows), jnp.maximum)
    lo = _pair_reduce(functools.reduce(jnp.minimum, rows), jnp.minimum)
    ep = [jnp.exp(r - hi) for r in rows]
    en = [jnp.exp(lo - r) for r in rows]
    rp = 1.0 / _pair_reduce(functools.reduce(jnp.add, ep), jnp.add)
    rn = 1.0 / _pair_reduce(functools.reduce(jnp.add, en), jnp.add)
    return jnp.concatenate([e * rp for e in ep] + [e * rn for e in en], axis=0)


def _kernel(
    x_hbm, mem0_ref, wq_hbm, wk_hbm, wv_hbm, wo_hbm, bqkv_hbm, wphi_ref, bwo_hbm,
    out_hbm,
    xin_ref, xe_ref, he_ref, xres_ref, hn_ref, hb_ref, wqkv_ref, wo_ref, stage_ref, early_ref,
    bqkv_ref, bwo_ref, sel_ref, bq_ref, bkv_ref, bo_ref,
    o_ref, y_ref, kt_ref, vb_ref, p_ref, ht_ref, ot_ref, kv_ref, res_ref,
    sem_x, sem_b, sem_w, sem_out,
    *, seg, heads, dh,
):
    seq, dm = out_hbm.shape
    n_mem = mem0_ref.shape[0]
    n_seg = seq // seg
    rows = n_mem + seg
    pairs = heads // 2
    pw = 2 * dh
    off = -(-rows // 16) * 16
    scale = dh ** (-0.5)
    bdh = dm // B_HEADS
    grp = 2 * bdh
    n_grp = B_HEADS // 2

    cp_xe = pltpu.make_async_copy(x_hbm.at[:, seg // EARLY - 1], xe_ref, sem_x)
    cp_bqkv = pltpu.make_async_copy(bqkv_hbm, bqkv_ref, sem_b.at[0])
    cp_bwo = pltpu.make_async_copy(bwo_hbm, bwo_ref, sem_b.at[1])

    def rows_of(j, n):
        return pl.ds(j * n if isinstance(j, int) else pl.multiple_of(j * n, n), n)

    def cp_w(m, j):
        slot = j & (RING - 1)
        if m == 4:
            n = n_seg // pairs
            return pltpu.make_async_copy(x_hbm.at[pl.ds(j * n, n)], xin_ref.at[slot], sem_w.at[slot, m])
        src = (wq_hbm, wk_hbm, wv_hbm, wo_hbm)[m]
        return pltpu.make_async_copy(src.at[rows_of(j, pw)], stage_ref.at[slot, m], sem_w.at[slot, m])

    def groups_of(kt):
        return range(128 * kt // grp, (128 * kt + 127) // grp + 1)

    def build_selectors():
        eh_r = _iota((B_HEADS, dm), 0)
        eh_c = _iota((B_HEADS, dm), 1)
        phi_f = None
        for d in range(bdh):
            eh = jnp.where(eh_c == eh_r * bdh + d, 1.0, 0.0).astype(BF16)
            t = _mm(wphi_ref[d], eh)
            phi_f = t if phi_f is None else phi_f + t
        pick = jnp.where((_iota((grp, bdh), 0) >> 1) == _iota((grp, bdh), 1), 1.0, 0.0)
        phi_rows = _mm(pick, phi_f.astype(BF16))
        r = _iota((grp, 128), 0)
        for kt in range(dm // 128):
            c = _iota((grp, 128), 1) + 128 * kt
            c_head = _div_const(c, bdh)
            for i, g in enumerate(groups_of(kt)):
                head = 2 * g + (r & 1)
                sel_ref[0, kt, i] = jnp.where(c_head == head, phi_rows[:, 128 * kt:128 * kt + 128], 0.0)
                sel_ref[1, kt, i] = jnp.where(c == head * bdh + (r >> 1), 1.0, 0.0)

    skew, ahead = 2, 2

    def copies(j, has_kv, has_rest):
        return [cp_w(m, j) for m in (1, 2) if has_kv] + [cp_w(m, j - skew) for m in (0, 3, 4) if has_rest]

    def parts(j):
        return j < pairs, skew <= j < pairs + skew

    def load_round(j, now, later):
        for cp in copies(j, *now):
            cp.wait()
        prefetch = copies(j + ahead, *later)
        if now[0]:
            slot = j & (RING - 1)
            for m in (1, 2):
                early_ref[j, :, (m - 1) * pw:m * pw] = _mm_nt(he_ref[...], stage_ref[slot, m])
                if m == 1:
                    for cp in prefetch:
                        cp.start()
                wqkv_ref[j, :, m * pw:(m + 1) * pw] = _pack(stage_ref[slot, m].T)
        else:
            for cp in prefetch:
                cp.start()
        if now[1]:
            i = j - skew
            slot = i & (RING - 1)
            n = seq // pairs
            x = xin_ref[slot].astype(F32).reshape(n, dm)
            xres_ref[rows_of(i, n), :] = x
            hn_ref[rows_of(i, n), :] = _layernorm(x)
            wqkv_ref[i, :, 0:pw] = _pack(stage_ref[slot, 0].T)
            wo_ref[rows_of(i, dh), :] = _pack(stage_ref[slot, 3])

    cp_xe.start()
    for cp in copies(0, *parts(0)):
        cp.start()
    build_selectors()
    cp_xe.wait()
    for j in range(1, ahead):
        for cp in copies(j, *parts(j)):
            cp.start()
    he_ref[...] = _layernorm(xe_ref[...].astype(F32).reshape(n_seg * EARLY, dm))

    def load_body(j, carry):
        load_round(j, (True, True), (True, True))
        return carry

    for j in range(skew):
        load_round(j, parts(j), parts(j + ahead))
    lax.fori_loop(skew, pairs - ahead, load_body, 0)
    for j in range(pairs - ahead, pairs + skew):
        load_round(j, parts(j), parts(j + ahead))
    cp_bqkv.start()
    cp_bwo.start()
    xres_ref[seq:seq + seg, :] = jnp.zeros((seg, dm), F32)

    def block_diag(t):
        lane = _iota((rows, pw), 1)
        gap = jnp.zeros((off - rows, pw), F32)
        tail = jnp.zeros((128 - off - rows, pw), F32)
        first = jnp.where(lane < dh, t, 0.0)
        second = jnp.where(lane >= dh, t, 0.0)
        return jnp.concatenate([first, gap, second, tail], axis=0).astype(BF16)

    def a_residual(s):
        sl = rows_of(s, seg)
        xn = xres_ref[sl, :] + y_ref[n_mem:rows, :]
        xres_ref[sl, :] = xn
        hb_ref[sl, :] = _layernorm(xn).astype(BF16)

    def a_step(s, first_layer):
        h = jnp.concatenate([y_ref[0:n_mem, :], hn_ref[rows_of(s, seg), :]], axis=0)
        a_residual(jnp.where(s == 0, n_seg, s - 1))
        qi = _iota((rows, 128), 0)
        ki = _iota((rows, 128), 1)
        in_a = ki < rows
        in_b = (ki >= off) & (ki < off + rows)
        see_a = in_a & ((qi < n_mem) | (qi >= ki))
        see_b = in_b & ((qi < n_mem) | (qi >= ki - off))
        fill_a = jnp.where(in_a, MASK_FILL, -jnp.inf)
        fill_b = jnp.where(in_b, MASK_FILL, -jnp.inf)

        def proj(m, j):
            w = _unpack(wqkv_ref[j, :, m * pw:(m + 1) * pw])
            if first_layer and m > 0:
                done = early_ref[j, rows_of(s, EARLY), (m - 1) * pw:m * pw]
                return jnp.concatenate([_mm(h[:rows - EARLY], w), done], axis=0)
            return _mm(h, w)

        def scores(j):
            sc = _mm(o_ref[:, j * pw:(j + 1) * pw], _unpack(kt_ref[j])) * scale
            sa = jnp.where(see_a, sc, fill_a)
            sb = jnp.where(see_b, sc, fill_b)
            ea = jnp.exp(sa - jnp.max(sa, axis=-1, keepdims=True))
            eb = jnp.exp(sb - jnp.max(sb, axis=-1, keepdims=True))
            ra = 1.0 / jnp.sum(ea, axis=-1, keepdims=True)
            rb = 1.0 / jnp.sum(eb, axis=-1, keepdims=True)
            p_ref[j] = ea * ra + eb * rb

        def attend(j):
            o_ref[:, j * pw:(j + 1) * pw] = _mm(p_ref[j], _unpack(vb_ref[j]))

        def out_proj(j0, j1, cols):
            return _mm(o_ref[:, j0 * pw:j1 * pw], _unpack(wo_ref[j0 * dh:j1 * dh, cols]))

        for j in range(pairs):
            kt_ref[j] = _pack(block_diag(proj(1, j)).T)
        for j in range(pairs):
            o_ref[:, j * pw:(j + 1) * pw] = proj(0, j)
            if j >= LAG:
                scores(j - LAG)
        for j in range(pairs):
            v = proj(2, j)
            if j < LAG:
                scores(pairs - LAG + j)
            vb_ref[j] = _pack(block_diag(v))
            if j >= LAG:
                attend(j - LAG)
        y = out_proj(0, pairs // 2, slice(0, dm))
        for j in range(pairs - LAG, pairs):
            attend(j)
        for cols in (slice(0, dm - 256), slice(dm - 256, dm)):
            y_ref[:, cols] = y[:, cols] + out_proj(pairs // 2, pairs, cols)

    def a_layer(first_layer):
        def a_body(i, carry):
            for u in range(UNROLL):
                a_step(i * UNROLL + u, first_layer)
            return carry

        lax.fori_loop(0, n_seg // UNROLL, a_body, 0)

    def b_fold_weights():
        def fold(which, product):
            out = {}
            for kt in range(dm // 128):
                gs = groups_of(kt)
                block = jnp.concatenate([sel_ref[which, kt, i] for i in range(len(gs))], axis=0)
                part = product(block, 128 * kt)
                for i, g in enumerate(gs):
                    t = part[i * grp:(i + 1) * grp]
                    out[g] = out[g] + t if g in out else t
            return out

        def store(ref, blocks):
            for i in range(0, len(blocks), 2):
                two = jnp.concatenate(blocks[i:i + 2], axis=0).astype(BF16)
                ref[i * bdh:(i + 2) * bdh, :] = _pack(two)

        def from_qkv(m):
            return lambda b, c: _mm_nt(b, bqkv_ref[:, m * dm + c:m * dm + c + 128])

        cp_bqkv.wait()
        cp_bwo.wait()
        wk, wv = fold(0, from_qkv(1)), fold(1, from_qkv(2))
        store(bkv_ref, [w[g] for g in range(n_grp) for w in (wk, wv)])
        wq = fold(0, from_qkv(0))
        store(bq_ref, [wq[g] for g in range(n_grp)])
        wo = fold(1, lambda b, c: _mm(b, bwo_ref[c:c + 128, :]))
        store(bo_ref, [wo[g] for g in range(n_grp)])

    n_chunk = seq // CHUNK
    tokens = lambda i: slice(i * CHUNK, (i + 1) * CHUNK)

    def b_kv():
        ones = jnp.ones((8, CHUNK), F32)

        def transpose(i):
            ht_ref[:, tokens(i)] = _pack(hb_ref[tokens(i), :].T)

        work = [(i, g) for i in range(n_chunk) for g in range(n_grp)]
        ready = {}
        transpose(0)
        for n in range(len(work) + B_LAG):
            if n < len(work):
                i, g = work[n]
                if g == 0 and i + 1 < n_chunk:
                    transpose(i + 1)
                t = _mm(_unpack(bkv_ref[g * grp:(g + 1) * grp, :]), _unpack(ht_ref[:, tokens(i)]))
                ready[n] = (jnp.concatenate([t[grp:], ones], axis=0), _hedgehog(t[:grp]).astype(BF16))
            if n >= B_LAG:
                i, g = work[n - B_LAG]
                t = _mm_nt(*ready.pop(n - B_LAG))
                kv_ref[g] = t if i == 0 else kv_ref[g] + t
        same = ((_iota(kv_ref.shape, 1) ^ _iota(kv_ref.shape, 2)) & 1) == 0
        kv_ref[...] = jnp.where(same, kv_ref[...], 0.0)

    def cp_out(i):
        return pltpu.make_async_copy(res_ref.at[tokens(i)], out_hbm.at[tokens(i)], sem_out.at[i])

    def b_out():
        half = n_grp // 2
        work = [(i, gg) for i in range(n_chunk) for gg in range(half)]
        ready = {}

        def finish(i):
            o = ot_ref[i % 2].astype(BF16).T
            xn = xres_ref[tokens(i), :] + _mm(o, _unpack(bo_ref[...]))
            xres_ref[tokens(i), :] = xn
            hn_ref[tokens(i), :] = _layernorm(xn)
            res_ref[tokens(i), :] = xn.astype(BF16)
            cp_out(i).start()

        for n in range(len(work) + B_LAG):
            if n < len(work):
                i, gg = work[n]
                t = _mm(_unpack(bq_ref[gg * grp:(gg + 1) * grp, :]), _unpack(ht_ref[:, tokens(i)]))
                ready[n] = [_hedgehog(t[k * grp:(k + 1) * grp]).astype(BF16) for k in range(2)]
                if i > 0 and gg == half - 1:
                    finish(i - 1)
            if n >= B_LAG:
                i, gg = work[n - B_LAG]
                for k, phi in enumerate(ready.pop(n - B_LAG)):
                    g = 2 * gg + k
                    nd = _mm(kv_ref[g], phi)
                    inv = 1.0 / (nd[grp:grp + 8] + DEN_EPS)
                    ot_ref[i % 2, g * grp:(g + 1) * grp, :] = jnp.concatenate(
                        [nd[r:r + 8] * inv for r in range(0, grp, 8)], axis=0)
        finish(n_chunk - 1)

    def layer_pair(it, carry):
        y_ref[0:n_mem, :] = mem0_ref[...].astype(F32)
        y_ref[n_mem:rows, :] = jnp.zeros((seg, dm), F32)

        @pl.when(it == 0)
        def _():
            a_layer(True)
            b_fold_weights()

        @pl.when(it == 1)
        def _():
            a_layer(False)
            for i in range(n_chunk):
                cp_out(i).wait()

        a_residual(n_seg - 1)
        with jax.named_scope("L_b_kv"):
            b_kv()
        with jax.named_scope("L_b_out"):
            b_out()
        return carry

    lax.fori_loop(0, 2, layer_pair, 0)
    for i in range(n_chunk):
        cp_out(i).wait()


@functools.partial(jax.jit, static_argnames=("A_seg_len",))
def pallas_interleave_layers__memory_aug_recurrent_mem_tr__linear_kernel_hedgehog__prompt_kernel(
    A_x: jax.Array,
    A_mem0: jax.Array,
    A_Wq: jax.Array,
    A_Wk: jax.Array,
    A_Wv: jax.Array,
    A_Wo: jax.Array,
    A_seg_len: int,
    B_x: jax.Array,
    B_wqkv: jax.Array,
    B_w_phi: jax.Array,
    B_wo: jax.Array,
):
    del B_x
    batch, seq, dm = A_x.shape
    _, heads, dh = A_Wq.shape
    n_mem = A_mem0.shape[1]
    seg = int(A_seg_len)
    n_seg = seq // seg
    rows = n_mem + seg
    pw = 2 * dh
    pairs = heads // 2
    bdh = dm // B_HEADS
    assert batch == 1 and seq % CHUNK == 0 and CHUNK % seg == 0 and seg % EARLY == 0
    assert n_mem % 8 == 0 and -(-rows // 16) * 16 + rows <= 128
    assert heads % 2 == 0 and pw % 128 == 0 and dm % 128 == 0 and (2 * bdh) % 8 == 0

    w_t = lambda w: jnp.transpose(w, (1, 2, 0)).reshape(heads * dh, dm)
    hbm = pl.BlockSpec(memory_space=pl.ANY)
    vmem = pl.BlockSpec(memory_space=pltpu.VMEM)

    out = pl.pallas_call(
        functools.partial(_kernel, seg=seg, heads=heads, dh=dh),
        out_shape=jax.ShapeDtypeStruct((seq, dm), A_x.dtype),
        in_specs=[hbm, vmem, hbm, hbm, hbm, hbm, hbm, vmem, hbm],
        out_specs=hbm,
        scratch_shapes=[
            pltpu.VMEM((RING, n_seg // pairs, seg // EARLY, EARLY, dm), BF16),
            pltpu.VMEM((n_seg, EARLY, dm), BF16),
            pltpu.VMEM((n_seg * EARLY, dm), F32),
            pltpu.VMEM((seq + seg, dm), F32),
            pltpu.VMEM((seq, dm), F32),
            pltpu.VMEM((seq + seg, dm), BF16),
            pltpu.VMEM((pairs, dm // 2, 3 * pw), jnp.uint32),
            pltpu.VMEM((pairs * dh, dm), jnp.uint32),
            pltpu.VMEM((RING, 4, pw, dm), BF16),
            pltpu.VMEM((pairs, n_seg * EARLY, 2 * pw), F32),
            pltpu.VMEM((dm, 3 * dm), BF16),
            pltpu.VMEM((dm, dm), BF16),
            pltpu.VMEM((2, dm // 128, 127 // (2 * bdh) + 2, 2 * bdh, 128), F32),
            pltpu.VMEM((dm // 2, dm), jnp.uint32),
            pltpu.VMEM((dm, dm), jnp.uint32),
            pltpu.VMEM((dm // 2, dm), jnp.uint32),
            pltpu.VMEM((rows, heads * dh), F32),
            pltpu.VMEM((rows, dm), F32),
            pltpu.VMEM((pairs, dh, 128), jnp.uint32),
            pltpu.VMEM((pairs, 64, pw), jnp.uint32),
            pltpu.VMEM((pairs, rows, 128), F32),
            pltpu.VMEM((dm // 2, seq), jnp.uint32),
            pltpu.VMEM((2, dm, CHUNK), F32),
            pltpu.VMEM((B_HEADS // 2, 2 * bdh + 8, 4 * bdh), F32),
            pltpu.VMEM((seq, dm), BF16),
            pltpu.SemaphoreType.DMA,
            pltpu.SemaphoreType.DMA((2,)),
            pltpu.SemaphoreType.DMA((RING, 5)),
            pltpu.SemaphoreType.DMA((seq // CHUNK,)),
        ],
        compiler_params=pltpu.CompilerParams(
            vmem_limit_bytes=120 * 1024 * 1024, disable_bounds_checks=True),
    )(
        A_x.reshape(n_seg, seg // EARLY, EARLY, dm),
        A_mem0.reshape(n_mem, dm),
        w_t(A_Wq), w_t(A_Wk), w_t(A_Wv),
        A_Wo.reshape(heads * dh, dm),
        B_wqkv,
        jnp.transpose(B_w_phi, (1, 2, 0)),
        B_wo,
    )
    return out.reshape(batch, seq, dm)
```

```python
import functools

import jax
import jax.numpy as jnp
from jax import lax
import jax.experimental.pallas as pl
import jax.experimental.pallas.tpu as pltpu

F32 = jnp.float32
BF16 = jnp.bfloat16

B_HEADS = 32
LN_EPS = 1e-05
DEN_EPS = 1e-06
MASK_FILL = -1000000000.0

LAG = 4
EARLY = 8
UNROLL = 2
LEAD = 2
RING = 4
CHUNK = 256
B_LAG = 2

_NN = (((1,), (0,)), ((), ()))
_NT = (((1,), (1,)), ((), ()))


def _mm(a, b):
    return lax.dot_general(a, b, _NN, preferred_element_type=F32)


def _mm_nt(a, b):
    return lax.dot_general(a, b, _NT, preferred_element_type=F32)


def _pack(w):
    return pltpu.bitcast(w, jnp.uint32)


def _unpack(w):
    return pltpu.bitcast(w, BF16)


def _iota(shape, dim):
    return lax.broadcasted_iota(jnp.int32, shape, dim)


def _div_const(r, d):
    mul = (1 << 18) // d + 1
    assert all((v * mul) >> 18 == v // d for v in range(4096))
    return (r * mul) >> 18


def _layernorm(x):
    m = jnp.mean(x, axis=-1, keepdims=True)
    xc = x - m
    v = jnp.mean(xc * xc, axis=-1, keepdims=True)
    return xc * lax.rsqrt(v + LN_EPS)


def _pair_reduce(v, op):
    v = op(v, pltpu.roll(v, 4, 0))
    return op(v, pltpu.roll(v, 2, 0))


def _hedgehog(p):
    rows = [p[i:i + 8] for i in range(0, p.shape[0], 8)]
    hi = _pair_reduce(functools.reduce(jnp.maximum, rows), jnp.maximum)
    lo = _pair_reduce(functools.reduce(jnp.minimum, rows), jnp.minimum)
    ep = [jnp.exp(r - hi) for r in rows]
    en = [jnp.exp(lo - r) for r in rows]
    rp = 1.0 / _pair_reduce(functools.reduce(jnp.add, ep), jnp.add)
    rn = 1.0 / _pair_reduce(functools.reduce(jnp.add, en), jnp.add)
    return jnp.concatenate([e * rp for e in ep] + [e * rn for e in en], axis=0)


def _kernel(
    x_hbm, mem0_ref, wq_hbm, wk_hbm, wv_hbm, wo_hbm, bqkv_hbm, wphi_ref, bwo_hbm,
    out_hbm,
    xin_ref, xe_ref, he_ref, xres_ref, hn_ref, hb_ref, wqkv_ref, wo_ref, stage_ref, early_ref,
    bqkv_ref, bwo_ref, sel_ref, bq_ref, bkv_ref, bo_ref,
    o_ref, y_ref, kt_ref, v_ref, p_ref, ht_ref, ot_ref, kv_ref, res_ref,
    sem_x, sem_b, sem_w, sem_out,
    *, seg, heads, dh,
):
    seq, dm = out_hbm.shape
    n_mem = mem0_ref.shape[0]
    n_seg = seq // seg
    rows = n_mem + seg
    pairs = heads // 2
    pw = 2 * dh
    off = -(-rows // 16) * 16
    scale = dh ** (-0.5)
    bdh = dm // B_HEADS
    grp = 2 * bdh
    n_grp = B_HEADS // 2

    cp_xe = pltpu.make_async_copy(x_hbm.at[:, seg // EARLY - 1], xe_ref, sem_x)
    cp_bqkv = pltpu.make_async_copy(bqkv_hbm, bqkv_ref, sem_b.at[0])
    cp_bwo = pltpu.make_async_copy(bwo_hbm, bwo_ref, sem_b.at[1])

    def rows_of(j, n):
        return pl.ds(j * n if isinstance(j, int) else pl.multiple_of(j * n, n), n)

    def cp_w(m, j):
        slot = j & (RING - 1)
        if m == 4:
            n = n_seg // pairs
            return pltpu.make_async_copy(x_hbm.at[pl.ds(j * n, n)], xin_ref.at[slot], sem_w.at[slot, m])
        src = (wq_hbm, wk_hbm, wv_hbm, wo_hbm)[m]
        return pltpu.make_async_copy(src.at[rows_of(j, pw)], stage_ref.at[slot, m], sem_w.at[slot, m])

    def groups_of(kt):
        return range(128 * kt // grp, (128 * kt + 127) // grp + 1)

    def build_selectors():
        eh_r = _iota((B_HEADS, dm), 0)
        eh_c = _iota((B_HEADS, dm), 1)
        phi_f = None
        for d in range(bdh):
            eh = jnp.where(eh_c == eh_r * bdh + d, 1.0, 0.0).astype(BF16)
            t = _mm(wphi_ref[d], eh)
            phi_f = t if phi_f is None else phi_f + t
        pick = jnp.where((_iota((grp, bdh), 0) >> 1) == _iota((grp, bdh), 1), 1.0, 0.0)
        phi_rows = _mm(pick, phi_f.astype(BF16))
        r = _iota((grp, 128), 0)
        for kt in range(dm // 128):
            c = _iota((grp, 128), 1) + 128 * kt
            c_head = _div_const(c, bdh)
            for i, g in enumerate(groups_of(kt)):
                head = 2 * g + (r & 1)
                sel_ref[0, kt, i] = jnp.where(c_head == head, phi_rows[:, 128 * kt:128 * kt + 128], 0.0)
                sel_ref[1, kt, i] = jnp.where(c == head * bdh + (r >> 1), 1.0, 0.0)

    skew, ahead = 2, 2

    def copies(j, has_kv, has_rest):
        return [cp_w(m, j) for m in (1, 2) if has_kv] + [cp_w(m, j - skew) for m in (0, 3, 4) if has_rest]

    def parts(j):
        return j < pairs, skew <= j < pairs + skew

    def load_round(j, now, later):
        for cp in copies(j, *now):
            cp.wait()
        prefetch = copies(j + ahead, *later)
        if now[0]:
            slot = j & (RING - 1)
            for m in (1, 2):
                early_ref[j, :, (m - 1) * pw:m * pw] = _mm_nt(he_ref[...], stage_ref[slot, m])
                if m == 1:
                    for cp in prefetch:
                        cp.start()
                wqkv_ref[j, :, m * pw:(m + 1) * pw] = _pack(stage_ref[slot, m].T)
        else:
            for cp in prefetch:
                cp.start()
        if now[1]:
            i = j - skew
            slot = i & (RING - 1)
            n = seq // pairs
            x = xin_ref[slot].astype(F32).reshape(n, dm)
            xres_ref[rows_of(i, n), :] = x
            hn_ref[rows_of(i, n), :] = _layernorm(x)
            wqkv_ref[i, :, 0:pw] = _pack(stage_ref[slot, 0].T)
            wo_ref[rows_of(i, dh), :] = _pack(stage_ref[slot, 3])

    cp_xe.start()
    for cp in copies(0, *parts(0)):
        cp.start()
    build_selectors()
    cp_xe.wait()
    for j in range(1, ahead):
        for cp in copies(j, *parts(j)):
            cp.start()
    he_ref[...] = _layernorm(xe_ref[...].astype(F32).reshape(n_seg * EARLY, dm))

    def load_body(j, carry):
        load_round(j, (True, True), (True, True))
        return carry

    for j in range(skew):
        load_round(j, parts(j), parts(j + ahead))
    lax.fori_loop(skew, pairs - ahead, load_body, 0)
    for j in range(pairs - ahead, pairs + skew):
        load_round(j, parts(j), parts(j + ahead))
    cp_bqkv.start()
    cp_bwo.start()
    xres_ref[seq:seq + seg, :] = jnp.zeros((seg, dm), F32)

    cut = dh % 128

    def stack(a, b):
        gap = jnp.zeros((off - rows, a.shape[1]), F32)
        tail = jnp.zeros((128 - off - rows, a.shape[1]), F32)
        return jnp.concatenate([a, gap, b, tail], axis=0).astype(BF16)

    def store_keys(j, t):
        outer = _pack(stack(t[:, 0:128], t[:, 256:384]).T)
        inner = _pack(stack(t[:, 128:256], t[:, 128:256]).T)
        low = _iota((64, 128), 1) < off
        kt_ref[j, 0:64] = jnp.where(low, outer, 0)
        kt_ref[j, 64:64 + cut // 2] = jnp.where(low[:cut // 2], inner[:cut // 2], 0)
        kt_ref[j, 64 + cut // 2:128] = jnp.where(low[cut // 2:], 0, inner[cut // 2:])
        kt_ref[j, 128:192] = jnp.where(low, 0, outer)

    def load_values(j):
        t = v_ref[j]
        low = _iota((rows, 128), 1) < cut
        none = jnp.zeros((rows, 128), F32)
        first = jnp.concatenate([t[:, 0:128], jnp.where(low, t[:, 128:256], 0.0), none], axis=1)
        second = jnp.concatenate([none, jnp.where(low, 0.0, t[:, 128:256]), t[:, 256:384]], axis=1)
        return stack(first, second)

    def a_residual(s):
        sl = rows_of(s, seg)
        xn = xres_ref[sl, :] + y_ref[n_mem:rows, :]
        xres_ref[sl, :] = xn
        hb_ref[sl, :] = _layernorm(xn).astype(BF16)

    def a_step(s, first_layer):
        h = jnp.concatenate([y_ref[0:n_mem, :], hn_ref[rows_of(s, seg), :]], axis=0)
        a_residual(jnp.where(s == 0, n_seg, s - 1))
        qi = _iota((rows, 128), 0)
        ki = _iota((rows, 128), 1)
        in_a = ki < rows
        in_b = (ki >= off) & (ki < off + rows)
        see_a = in_a & ((qi < n_mem) | (qi >= ki))
        see_b = in_b & ((qi < n_mem) | (qi >= ki - off))
        fill_a = jnp.where(in_a, MASK_FILL, -jnp.inf)
        fill_b = jnp.where(in_b, MASK_FILL, -jnp.inf)

        def partial_proj(m, j, d0, d1):
            n = rows - EARLY if first_layer and m > 0 else rows
            return _mm(h[:n, d0:d1], _unpack(wqkv_ref[j, d0 // 2:d1 // 2, m * pw:(m + 1) * pw]))

        def with_early(m, j, t):
            if first_layer and m > 0:
                done = early_ref[j, rows_of(s, EARLY), (m - 1) * pw:m * pw]
                return jnp.concatenate([t, done], axis=0)
            return t

        def proj(m, j):
            return with_early(m, j, partial_proj(m, j, 0, dm))

        def scores(j):
            sc = _mm(o_ref[:, j * pw:(j + 1) * pw], _unpack(kt_ref[j])) * scale
            sa = jnp.where(see_a, sc, fill_a)
            sb = jnp.where(see_b, sc, fill_b)
            ea = jnp.exp(sa - jnp.max(sa, axis=-1, keepdims=True))
            eb = jnp.exp(sb - jnp.max(sb, axis=-1, keepdims=True))
            ra = 1.0 / jnp.sum(ea, axis=-1, keepdims=True)
            rb = 1.0 / jnp.sum(eb, axis=-1, keepdims=True)
            p_ref[j] = ea * ra + eb * rb

        def attend(j):
            o_ref[:, j * pw:(j + 1) * pw] = _mm(p_ref[j], load_values(j))

        def out_proj(j0, j1, cols):
            return _mm(o_ref[:, j0 * pw:j1 * pw], _unpack(wo_ref[j0 * dh:j1 * dh, cols]))

        split = dm - 256
        nk = rows - EARLY if first_layer else rows
        for j in range(LEAD):
            v_ref[j, 0:nk] = partial_proj(1, j, 0, split)
        for j in range(LEAD):
            v_ref[LEAD + j, 0:nk] = partial_proj(1, j, split, dm)
        for j in range(LEAD):
            store_keys(j, with_early(1, j, v_ref[j, 0:nk] + v_ref[LEAD + j, 0:nk]))
        for j in range(LEAD, pairs):
            store_keys(j, proj(1, j))
        for j in range(pairs):
            o_ref[:, j * pw:(j + 1) * pw] = proj(0, j)
            if j >= LAG:
                scores(j - LAG)
        for j in range(pairs):
            v = proj(2, j)
            if j < LAG:
                scores(pairs - LAG + j)
            v_ref[j] = v
            if j >= LAG:
                attend(j - LAG)
        y = out_proj(0, pairs // 2, slice(0, dm))
        for j in range(pairs - LAG, pairs):
            attend(j)
        for cols in (slice(0, split), slice(split, dm)):
            y_ref[:, cols] = y[:, cols] + out_proj(pairs // 2, pairs, cols)

    def a_layer(first_layer):
        def a_body(i, carry):
            for u in range(UNROLL):
                a_step(i * UNROLL + u, first_layer)
            return carry

        lax.fori_loop(0, n_seg // UNROLL, a_body, 0)

    def b_fold_weights():
        def fold(which, product):
            out = {}
            for kt in range(dm // 128):
                gs = groups_of(kt)
                block = jnp.concatenate([sel_ref[which, kt, i] for i in range(len(gs))], axis=0)
                part = product(block, 128 * kt)
                for i, g in enumerate(gs):
                    t = part[i * grp:(i + 1) * grp]
                    out[g] = out[g] + t if g in out else t
            return out

        def store(ref, blocks):
            for i in range(0, len(blocks), 2):
                two = jnp.concatenate(blocks[i:i + 2], axis=0).astype(BF16)
                ref[i * bdh:(i + 2) * bdh, :] = _pack(two)

        def from_qkv(m):
            return lambda b, c: _mm_nt(b, bqkv_ref[:, m * dm + c:m * dm + c + 128])

        cp_bqkv.wait()
        cp_bwo.wait()
        wk, wv = fold(0, from_qkv(1)), fold(1, from_qkv(2))
        store(bkv_ref, [w[g] for g in range(n_grp) for w in (wk, wv)])
        wq = fold(0, from_qkv(0))
        store(bq_ref, [wq[g] for g in range(n_grp)])
        wo = fold(1, lambda b, c: _mm(b, bwo_ref[c:c + 128, :]))
        store(bo_ref, [wo[g] for g in range(n_grp)])

    n_chunk = seq // CHUNK
    tokens = lambda i: slice(i * CHUNK, (i + 1) * CHUNK)

    def b_kv():
        ones = jnp.ones((8, CHUNK), F32)

        def transpose(i):
            ht_ref[:, tokens(i)] = _pack(hb_ref[tokens(i), :].T)

        work = [(i, g) for i in range(n_chunk) for g in range(n_grp)]
        ready = {}
        transpose(0)
        for n in range(len(work) + B_LAG):
            if n < len(work):
                i, g = work[n]
                if g == 0 and i + 1 < n_chunk:
                    transpose(i + 1)
                t = _mm(_unpack(bkv_ref[g * grp:(g + 1) * grp, :]), _unpack(ht_ref[:, tokens(i)]))
                ready[n] = (jnp.concatenate([t[grp:], ones], axis=0), _hedgehog(t[:grp]).astype(BF16))
            if n >= B_LAG:
                i, g = work[n - B_LAG]
                t = _mm_nt(*ready.pop(n - B_LAG))
                kv_ref[g] = t if i == 0 else kv_ref[g] + t
        same = ((_iota(kv_ref.shape, 1) ^ _iota(kv_ref.shape, 2)) & 1) == 0
        kv_ref[...] = jnp.where(same, kv_ref[...], 0.0)

    def cp_out(i):
        return pltpu.make_async_copy(res_ref.at[tokens(i)], out_hbm.at[tokens(i)], sem_out.at[i])

    def b_out():
        half = n_grp // 2
        work = [(i, gg) for i in range(n_chunk) for gg in range(half)]
        ready = {}

        def finish(i):
            o = ot_ref[i % 2].astype(BF16).T
            xn = xres_ref[tokens(i), :] + _mm(o, _unpack(bo_ref[...]))
            xres_ref[tokens(i), :] = xn
            hn_ref[tokens(i), :] = _layernorm(xn)
            res_ref[tokens(i), :] = xn.astype(BF16)
            cp_out(i).start()

        for n in range(len(work) + B_LAG):
            if n < len(work):
                i, gg = work[n]
                t = _mm(_unpack(bq_ref[gg * grp:(gg + 1) * grp, :]), _unpack(ht_ref[:, tokens(i)]))
                ready[n] = [_hedgehog(t[k * grp:(k + 1) * grp]).astype(BF16) for k in range(2)]
                if i > 0 and gg == half - 1:
                    finish(i - 1)
            if n >= B_LAG:
                i, gg = work[n - B_LAG]
                for k, phi in enumerate(ready.pop(n - B_LAG)):
                    g = 2 * gg + k
                    nd = _mm(kv_ref[g], phi)
                    inv = 1.0 / (nd[grp:grp + 8] + DEN_EPS)
                    ot_ref[i % 2, g * grp:(g + 1) * grp, :] = jnp.concatenate(
                        [nd[r:r + 8] * inv for r in range(0, grp, 8)], axis=0)
        finish(n_chunk - 1)

    def layer_pair(it, carry):
        y_ref[0:n_mem, :] = mem0_ref[...].astype(F32)
        y_ref[n_mem:rows, :] = jnp.zeros((seg, dm), F32)

        @pl.when(it == 0)
        def _():
            a_layer(True)
            b_fold_weights()

        @pl.when(it == 1)
        def _():
            a_layer(False)
            for i in range(n_chunk):
                cp_out(i).wait()

        a_residual(n_seg - 1)
        with jax.named_scope("L_b_kv"):
            b_kv()
        with jax.named_scope("L_b_out"):
            b_out()
        return carry

    lax.fori_loop(0, 2, layer_pair, 0)
    for i in range(n_chunk):
        cp_out(i).wait()


@functools.partial(jax.jit, static_argnames=("A_seg_len",))
def pallas_interleave_layers__memory_aug_recurrent_mem_tr__linear_kernel_hedgehog__prompt_kernel(
    A_x: jax.Array,
    A_mem0: jax.Array,
    A_Wq: jax.Array,
    A_Wk: jax.Array,
    A_Wv: jax.Array,
    A_Wo: jax.Array,
    A_seg_len: int,
    B_x: jax.Array,
    B_wqkv: jax.Array,
    B_w_phi: jax.Array,
    B_wo: jax.Array,
):
    del B_x
    batch, seq, dm = A_x.shape
    _, heads, dh = A_Wq.shape
    n_mem = A_mem0.shape[1]
    seg = int(A_seg_len)
    n_seg = seq // seg
    rows = n_mem + seg
    pw = 2 * dh
    pairs = heads // 2
    bdh = dm // B_HEADS
    assert batch == 1 and seq % CHUNK == 0 and CHUNK % seg == 0 and seg % EARLY == 0
    assert n_mem % 8 == 0 and rows <= 48
    assert heads % 2 == 0 and pw == 3 * 128 and dm % 128 == 0 and (2 * bdh) % 8 == 0

    w_t = lambda w: jnp.transpose(w, (1, 2, 0)).reshape(heads * dh, dm)
    hbm = pl.BlockSpec(memory_space=pl.ANY)
    vmem = pl.BlockSpec(memory_space=pltpu.VMEM)

    out = pl.pallas_call(
        functools.partial(_kernel, seg=seg, heads=heads, dh=dh),
        out_shape=jax.ShapeDtypeStruct((seq, dm), A_x.dtype),
        in_specs=[hbm, vmem, hbm, hbm, hbm, hbm, hbm, vmem, hbm],
        out_specs=hbm,
        scratch_shapes=[
            pltpu.VMEM((RING, n_seg // pairs, seg // EARLY, EARLY, dm), BF16),
            pltpu.VMEM((n_seg, EARLY, dm), BF16),
            pltpu.VMEM((n_seg * EARLY, dm), F32),
            pltpu.VMEM((seq + seg, dm), F32),
            pltpu.VMEM((seq, dm), F32),
            pltpu.VMEM((seq + seg, dm), BF16),
            pltpu.VMEM((pairs, dm // 2, 3 * pw), jnp.uint32),
            pltpu.VMEM((pairs * dh, dm), jnp.uint32),
            pltpu.VMEM((RING, 4, pw, dm), BF16),
            pltpu.VMEM((pairs, n_seg * EARLY, 2 * pw), F32),
            pltpu.VMEM((dm, 3 * dm), BF16),
            pltpu.VMEM((dm, dm), BF16),
            pltpu.VMEM((2, dm // 128, 127 // (2 * bdh) + 2, 2 * bdh, 128), F32),
            pltpu.VMEM((dm // 2, dm), jnp.uint32),
            pltpu.VMEM((dm, dm), jnp.uint32),
            pltpu.VMEM((dm // 2, dm), jnp.uint32),
            pltpu.VMEM((rows, heads * dh), F32),
            pltpu.VMEM((rows, dm), F32),
            pltpu.VMEM((pairs, dh, 128), jnp.uint32),
            pltpu.VMEM((pairs, rows, pw), F32),
            pltpu.VMEM((pairs, rows, 128), F32),
            pltpu.VMEM((dm // 2, seq), jnp.uint32),
            pltpu.VMEM((2, dm, CHUNK), F32),
            pltpu.VMEM((B_HEADS // 2, 2 * bdh + 8, 4 * bdh), F32),
            pltpu.VMEM((seq, dm), BF16),
            pltpu.SemaphoreType.DMA,
            pltpu.SemaphoreType.DMA((2,)),
            pltpu.SemaphoreType.DMA((RING, 5)),
            pltpu.SemaphoreType.DMA((seq // CHUNK,)),
        ],
        compiler_params=pltpu.CompilerParams(vmem_limit_bytes=120 * 1024 * 1024),
    )(
        A_x.reshape(n_seg, seg // EARLY, EARLY, dm),
        A_mem0.reshape(n_mem, dm),
        w_t(A_Wq), w_t(A_Wk), w_t(A_Wv),
        A_Wo.reshape(heads * dh, dm),
        B_wqkv,
        jnp.transpose(B_w_phi, (1, 2, 0)),
        B_wo,
    )
    return out.reshape(batch, seq, dm)
```

```python
import functools

import jax
import jax.numpy as jnp
from jax import lax
import jax.experimental.pallas as pl
import jax.experimental.pallas.tpu as pltpu

F32 = jnp.float32
BF16 = jnp.bfloat16

B_HEADS = 32
LN_EPS = 1e-05
DEN_EPS = 1e-06
MASK_FILL = -1000000000.0

LAG = 4
EARLY = 8
UNROLL = 2
LEAD = 2
RING = 4
CHUNK = 256
B_LAG = 2

_NN = (((1,), (0,)), ((), ()))
_NT = (((1,), (1,)), ((), ()))


def _mm(a, b):
    return lax.dot_general(a, b, _NN, preferred_element_type=F32)


def _mm_nt(a, b):
    return lax.dot_general(a, b, _NT, preferred_element_type=F32)


def _pack(w):
    return pltpu.bitcast(w, jnp.uint32)


def _unpack(w):
    return pltpu.bitcast(w, BF16)


def _iota(shape, dim):
    return lax.broadcasted_iota(jnp.int32, shape, dim)


def _div_const(r, d):
    mul = (1 << 18) // d + 1
    assert all((v * mul) >> 18 == v // d for v in range(4096))
    return (r * mul) >> 18


def _layernorm(x):
    m = jnp.mean(x, axis=-1, keepdims=True)
    xc = x - m
    v = jnp.mean(xc * xc, axis=-1, keepdims=True)
    return xc * lax.rsqrt(v + LN_EPS)


def _pair_reduce(v, op):
    v = op(v, pltpu.roll(v, 4, 0))
    return op(v, pltpu.roll(v, 2, 0))


def _hedgehog(p):
    rows = [p[i:i + 8] for i in range(0, p.shape[0], 8)]
    hi = _pair_reduce(functools.reduce(jnp.maximum, rows), jnp.maximum)
    lo = _pair_reduce(functools.reduce(jnp.minimum, rows), jnp.minimum)
    ep = [jnp.exp(r - hi) for r in rows]
    en = [jnp.exp(lo - r) for r in rows]
    rp = 1.0 / _pair_reduce(functools.reduce(jnp.add, ep), jnp.add)
    rn = 1.0 / _pair_reduce(functools.reduce(jnp.add, en), jnp.add)
    return jnp.concatenate([e * rp for e in ep] + [e * rn for e in en], axis=0)


def _kernel(
    x_hbm, mem0_ref, wq_hbm, wk_hbm, wv_hbm, wo_hbm, bqkv_hbm, wphi_ref, bwo_hbm,
    out_hbm,
    xin_ref, xe_ref, he_ref, xres_ref, hn_ref, ya_ref, wqkv_ref, wo_ref, stage_ref, early_ref,
    bqkv_ref, bwo_ref, sel_ref, bq_ref, bkv_ref, bo_ref,
    o_ref, mem_ref, kt_ref, v_ref, p_ref, ht_ref, ot_ref, kv_ref, res_ref,
    sem_x, sem_b, sem_w, sem_out,
    *, seg, heads, dh,
):
    seq, dm = out_hbm.shape
    n_mem = mem0_ref.shape[0]
    n_seg = seq // seg
    rows = n_mem + seg
    pairs = heads // 2
    pw = 2 * dh
    off = -(-rows // 16) * 16
    scale = dh ** (-0.5)
    bdh = dm // B_HEADS
    grp = 2 * bdh
    n_grp = B_HEADS // 2

    cp_xe = pltpu.make_async_copy(x_hbm.at[:, seg // EARLY - 1], xe_ref, sem_x)
    cp_bqkv = pltpu.make_async_copy(bqkv_hbm, bqkv_ref, sem_b.at[0])
    cp_bwo = pltpu.make_async_copy(bwo_hbm, bwo_ref, sem_b.at[1])

    def rows_of(j, n):
        return pl.ds(j * n if isinstance(j, int) else pl.multiple_of(j * n, n), n)

    def cp_w(m, j):
        slot = j & (RING - 1)
        if m == 4:
            n = n_seg // pairs
            return pltpu.make_async_copy(x_hbm.at[pl.ds(j * n, n)], xin_ref.at[slot], sem_w.at[slot, m])
        src = (wq_hbm, wk_hbm, wv_hbm, wo_hbm)[m]
        return pltpu.make_async_copy(src.at[rows_of(j, pw)], stage_ref.at[slot, m], sem_w.at[slot, m])

    def groups_of(kt):
        return range(128 * kt // grp, (128 * kt + 127) // grp + 1)

    def build_selectors():
        eh_r = _iota((B_HEADS, dm), 0)
        eh_c = _iota((B_HEADS, dm), 1)
        phi_f = None
        for d in range(bdh):
            eh = jnp.where(eh_c == eh_r * bdh + d, 1.0, 0.0).astype(BF16)
            t = _mm(wphi_ref[d], eh)
            phi_f = t if phi_f is None else phi_f + t
        pick = jnp.where((_iota((grp, bdh), 0) >> 1) == _iota((grp, bdh), 1), 1.0, 0.0)
        phi_rows = _mm(pick, phi_f.astype(BF16))
        r = _iota((grp, 128), 0)
        for kt in range(dm // 128):
            c = _iota((grp, 128), 1) + 128 * kt
            c_head = _div_const(c, bdh)
            for i, g in enumerate(groups_of(kt)):
                head = 2 * g + (r & 1)
                sel_ref[0, kt, i] = jnp.where(c_head == head, phi_rows[:, 128 * kt:128 * kt + 128], 0.0)
                sel_ref[1, kt, i] = jnp.where(c == head * bdh + (r >> 1), 1.0, 0.0)

    skew, ahead = 2, 2

    def copies(j, has_kv, has_rest):
        return [cp_w(m, j) for m in (1, 2) if has_kv] + [cp_w(m, j - skew) for m in (0, 3, 4) if has_rest]

    def parts(j):
        return j < pairs, skew <= j < pairs + skew

    def load_round(j, now, later):
        for cp in copies(j, *now):
            cp.wait()
        prefetch = copies(j + ahead, *later)
        if now[0]:
            slot = j & (RING - 1)
            for m in (1, 2):
                early_ref[j, :, (m - 1) * pw:m * pw] = _mm_nt(he_ref[...], stage_ref[slot, m])
                if m == 1:
                    for cp in prefetch:
                        cp.start()
                wqkv_ref[j, :, m * pw:(m + 1) * pw] = _pack(stage_ref[slot, m].T)
        else:
            for cp in prefetch:
                cp.start()
        if now[1]:
            i = j - skew
            slot = i & (RING - 1)
            n = seq // pairs
            x = xin_ref[slot].astype(F32).reshape(n, dm)
            xres_ref[rows_of(i, n), :] = x
            hn_ref[rows_of(i, n), :] = _layernorm(x)
            wqkv_ref[i, :, 0:pw] = _pack(stage_ref[slot, 0].T)
            wo_ref[rows_of(i, dh), :] = _pack(stage_ref[slot, 3])

    cp_xe.start()
    for cp in copies(0, *parts(0)):
        cp.start()
    build_selectors()
    cp_xe.wait()
    for j in range(1, ahead):
        for cp in copies(j, *parts(j)):
            cp.start()
    he_ref[...] = _layernorm(xe_ref[...].astype(F32).reshape(n_seg * EARLY, dm))

    def load_body(j, carry):
        load_round(j, (True, True), (True, True))
        return carry

    for j in range(skew):
        load_round(j, parts(j), parts(j + ahead))
    lax.fori_loop(skew, pairs - ahead, load_body, 0)
    for j in range(pairs - ahead, pairs + skew):
        load_round(j, parts(j), parts(j + ahead))
    cp_bqkv.start()
    cp_bwo.start()

    cut = dh % 128

    def stack(a, b):
        gap = jnp.zeros((off - rows, a.shape[1]), F32)
        tail = jnp.zeros((128 - off - rows, a.shape[1]), F32)
        return jnp.concatenate([a, gap, b, tail], axis=0).astype(BF16)

    def store_keys(j, t):
        outer = _pack(stack(t[:, 0:128], t[:, 256:384]).T)
        inner = _pack(stack(t[:, 128:256], t[:, 128:256]).T)
        low = _iota((64, 128), 1) < off
        kt_ref[j, 0:64] = jnp.where(low, outer, 0)
        kt_ref[j, 64:64 + cut // 2] = jnp.where(low[:cut // 2], inner[:cut // 2], 0)
        kt_ref[j, 64 + cut // 2:128] = jnp.where(low[cut // 2:], 0, inner[cut // 2:])
        kt_ref[j, 128:192] = jnp.where(low, 0, outer)

    def load_values(j):
        t = v_ref[j]
        low = _iota((rows, 128), 1) < cut
        none = jnp.zeros((rows, 128), F32)
        first = jnp.concatenate([t[:, 0:128], jnp.where(low, t[:, 128:256], 0.0), none], axis=1)
        second = jnp.concatenate([none, jnp.where(low, 0.0, t[:, 128:256]), t[:, 256:384]], axis=1)
        return stack(first, second)

    def a_step(s, first_layer):
        h = jnp.concatenate([mem_ref[...], hn_ref[rows_of(s, seg), :]], axis=0)
        qi = _iota((rows, 128), 0)
        ki = _iota((rows, 128), 1)
        in_a = ki < rows
        in_b = (ki >= off) & (ki < off + rows)
        see_a = in_a & ((qi < n_mem) | (qi >= ki))
        see_b = in_b & ((qi < n_mem) | (qi >= ki - off))
        fill_a = jnp.where(in_a, MASK_FILL, -jnp.inf)
        fill_b = jnp.where(in_b, MASK_FILL, -jnp.inf)

        def partial_proj(m, j, d0, d1):
            n = rows - EARLY if first_layer and m > 0 else rows
            return _mm(h[:n, d0:d1], _unpack(wqkv_ref[j, d0 // 2:d1 // 2, m * pw:(m + 1) * pw]))

        def with_early(m, j, t):
            if first_layer and m > 0:
                done = early_ref[j, rows_of(s, EARLY), (m - 1) * pw:m * pw]
                return jnp.concatenate([t, done], axis=0)
            return t

        def proj(m, j):
            return with_early(m, j, partial_proj(m, j, 0, dm))

        def scores(j):
            sc = _mm(o_ref[:, j * pw:(j + 1) * pw], _unpack(kt_ref[j])) * scale
            sa = jnp.where(see_a, sc, fill_a)
            sb = jnp.where(see_b, sc, fill_b)
            ea = jnp.exp(sa - jnp.max(sa, axis=-1, keepdims=True))
            eb = jnp.exp(sb - jnp.max(sb, axis=-1, keepdims=True))
            ra = 1.0 / jnp.sum(ea, axis=-1, keepdims=True)
            rb = 1.0 / jnp.sum(eb, axis=-1, keepdims=True)
            p_ref[j] = ea * ra + eb * rb

        def attend(j):
            o_ref[:, j * pw:(j + 1) * pw] = _mm(p_ref[j], load_values(j))

        def out_proj(j0, j1, cols):
            return _mm(o_ref[:, j0 * pw:j1 * pw], _unpack(wo_ref[j0 * dh:j1 * dh, cols]))

        split = dm - 256
        nk = rows - EARLY if first_layer else rows
        for j in range(LEAD):
            v_ref[j, 0:nk] = partial_proj(1, j, 0, split)
        for j in range(LEAD):
            v_ref[LEAD + j, 0:nk] = partial_proj(1, j, split, dm)
        for j in range(LEAD):
            store_keys(j, with_early(1, j, v_ref[j, 0:nk] + v_ref[LEAD + j, 0:nk]))
        for j in range(LEAD, pairs):
            store_keys(j, proj(1, j))
        for j in range(pairs):
            o_ref[:, j * pw:(j + 1) * pw] = proj(0, j)
            if j >= LAG:
                scores(j - LAG)
        for j in range(pairs):
            v = proj(2, j)
            if j < LAG:
                scores(pairs - LAG + j)
            v_ref[j] = v
            if j >= LAG:
                attend(j - LAG)
        y = out_proj(0, pairs // 2, slice(0, dm))
        for j in range(pairs - LAG, pairs):
            attend(j)
        for cols in (slice(0, split), slice(split, dm)):
            t = y[:, cols] + out_proj(pairs // 2, pairs, cols)
            mem_ref[:, cols] = t[:n_mem]
            ya_ref[rows_of(s, seg), cols] = t[n_mem:]

    def a_layer(first_layer):
        def a_body(i, carry):
            for u in range(UNROLL):
                a_step(i * UNROLL + u, first_layer)
            return carry

        lax.fori_loop(0, n_seg // UNROLL, a_body, 0)

    def b_fold_weights():
        def fold(which, product):
            out = {}
            for kt in range(dm // 128):
                gs = groups_of(kt)
                block = jnp.concatenate([sel_ref[which, kt, i] for i in range(len(gs))], axis=0)
                part = product(block, 128 * kt)
                for i, g in enumerate(gs):
                    t = part[i * grp:(i + 1) * grp]
                    out[g] = out[g] + t if g in out else t
            return out

        def store(ref, blocks):
            for i in range(0, len(blocks), 2):
                two = jnp.concatenate(blocks[i:i + 2], axis=0).astype(BF16)
                ref[i * bdh:(i + 2) * bdh, :] = _pack(two)

        def from_qkv(m):
            return lambda b, c: _mm_nt(b, bqkv_ref[:, m * dm + c:m * dm + c + 128])

        cp_bqkv.wait()
        cp_bwo.wait()
        wk, wv = fold(0, from_qkv(1)), fold(1, from_qkv(2))
        store(bkv_ref, [w[g] for g in range(n_grp) for w in (wk, wv)])
        wq = fold(0, from_qkv(0))
        store(bq_ref, [wq[g] for g in range(n_grp)])
        wo = fold(1, lambda b, c: _mm(b, bwo_ref[c:c + 128, :]))
        store(bo_ref, [wo[g] for g in range(n_grp)])

    n_chunk = seq // CHUNK
    tokens = lambda i: slice(i * CHUNK, (i + 1) * CHUNK)

    def b_kv():
        ones = jnp.ones((8, CHUNK), F32)

        def normalize(i):
            xn = xres_ref[tokens(i), :] + ya_ref[tokens(i), :]
            xres_ref[tokens(i), :] = xn
            ht_ref[:, tokens(i)] = _pack(_layernorm(xn).astype(BF16).T)

        work = [(i, g) for i in range(n_chunk) for g in range(n_grp)]
        ready = {}
        normalize(0)
        for n in range(len(work) + B_LAG):
            if n < len(work):
                i, g = work[n]
                if g == 0 and i + 1 < n_chunk:
                    normalize(i + 1)
                t = _mm(_unpack(bkv_ref[g * grp:(g + 1) * grp, :]), _unpack(ht_ref[:, tokens(i)]))
                ready[n] = (jnp.concatenate([t[grp:], ones], axis=0), _hedgehog(t[:grp]).astype(BF16))
            if n >= B_LAG:
                i, g = work[n - B_LAG]
                t = _mm_nt(*ready.pop(n - B_LAG))
                kv_ref[g] = t if i == 0 else kv_ref[g] + t
        same = ((_iota(kv_ref.shape, 1) ^ _iota(kv_ref.shape, 2)) & 1) == 0
        kv_ref[...] = jnp.where(same, kv_ref[...], 0.0)

    def cp_out(i):
        return pltpu.make_async_copy(res_ref.at[tokens(i)], out_hbm.at[tokens(i)], sem_out.at[i])

    def b_out():
        half = n_grp // 2
        work = [(i, gg) for i in range(n_chunk) for gg in range(half)]
        ready = {}

        def finish(i):
            o = ot_ref[i % 2].astype(BF16).T
            xn = xres_ref[tokens(i), :] + _mm(o, _unpack(bo_ref[...]))
            xres_ref[tokens(i), :] = xn
            hn_ref[tokens(i), :] = _layernorm(xn)
            res_ref[tokens(i), :] = xn.astype(BF16)
            cp_out(i).start()

        for n in range(len(work) + B_LAG):
            if n < len(work):
                i, gg = work[n]
                t = _mm(_unpack(bq_ref[gg * grp:(gg + 1) * grp, :]), _unpack(ht_ref[:, tokens(i)]))
                ready[n] = [_hedgehog(t[k * grp:(k + 1) * grp]).astype(BF16) for k in range(2)]
                if i > 0 and gg == half - 1:
                    finish(i - 1)
            if n >= B_LAG:
                i, gg = work[n - B_LAG]
                for k, phi in enumerate(ready.pop(n - B_LAG)):
                    g = 2 * gg + k
                    nd = _mm(kv_ref[g], phi)
                    inv = 1.0 / (nd[grp:grp + 8] + DEN_EPS)
                    ot_ref[i % 2, g * grp:(g + 1) * grp, :] = jnp.concatenate(
                        [nd[r:r + 8] * inv for r in range(0, grp, 8)], axis=0)
        finish(n_chunk - 1)

    def layer_pair(it, carry):
        mem_ref[...] = mem0_ref[...].astype(F32)

        @pl.when(it == 0)
        def _():
            a_layer(True)
            b_fold_weights()

        @pl.when(it == 1)
        def _():
            a_layer(False)
            for i in range(n_chunk):
                cp_out(i).wait()

        with jax.named_scope("L_b_kv"):
            b_kv()
        with jax.named_scope("L_b_out"):
            b_out()
        return carry

    lax.fori_loop(0, 2, layer_pair, 0)
    for i in range(n_chunk):
        cp_out(i).wait()


@functools.partial(jax.jit, static_argnames=("A_seg_len",))
def pallas_interleave_layers__memory_aug_recurrent_mem_tr__linear_kernel_hedgehog__prompt_kernel(
    A_x: jax.Array,
    A_mem0: jax.Array,
    A_Wq: jax.Array,
    A_Wk: jax.Array,
    A_Wv: jax.Array,
    A_Wo: jax.Array,
    A_seg_len: int,
    B_x: jax.Array,
    B_wqkv: jax.Array,
    B_w_phi: jax.Array,
    B_wo: jax.Array,
):
    del B_x
    batch, seq, dm = A_x.shape
    _, heads, dh = A_Wq.shape
    n_mem = A_mem0.shape[1]
    seg = int(A_seg_len)
    n_seg = seq // seg
    rows = n_mem + seg
    pw = 2 * dh
    pairs = heads // 2
    bdh = dm // B_HEADS
    assert batch == 1 and seq % CHUNK == 0 and CHUNK % seg == 0 and seg % EARLY == 0
    assert n_mem % 8 == 0 and rows <= 48
    assert heads % 2 == 0 and pw == 3 * 128 and dm % 128 == 0 and (2 * bdh) % 8 == 0

    w_t = lambda w: jnp.transpose(w, (1, 2, 0)).reshape(heads * dh, dm)
    hbm = pl.BlockSpec(memory_space=pl.ANY)
    vmem = pl.BlockSpec(memory_space=pltpu.VMEM)

    out = pl.pallas_call(
        functools.partial(_kernel, seg=seg, heads=heads, dh=dh),
        out_shape=jax.ShapeDtypeStruct((seq, dm), A_x.dtype),
        in_specs=[hbm, vmem, hbm, hbm, hbm, hbm, hbm, vmem, hbm],
        out_specs=hbm,
        scratch_shapes=[
            pltpu.VMEM((RING, n_seg // pairs, seg // EARLY, EARLY, dm), BF16),
            pltpu.VMEM((n_seg, EARLY, dm), BF16),
            pltpu.VMEM((n_seg * EARLY, dm), F32),
            pltpu.VMEM((seq, dm), F32),
            pltpu.VMEM((seq, dm), F32),
            pltpu.VMEM((seq, dm), F32),
            pltpu.VMEM((pairs, dm // 2, 3 * pw), jnp.uint32),
            pltpu.VMEM((pairs * dh, dm), jnp.uint32),
            pltpu.VMEM((RING, 4, pw, dm), BF16),
            pltpu.VMEM((pairs, n_seg * EARLY, 2 * pw), F32),
            pltpu.VMEM((dm, 3 * dm), BF16),
            pltpu.VMEM((dm, dm), BF16),
            pltpu.VMEM((2, dm // 128, 127 // (2 * bdh) + 2, 2 * bdh, 128), F32),
            pltpu.VMEM((dm // 2, dm), jnp.uint32),
            pltpu.VMEM((dm, dm), jnp.uint32),
            pltpu.VMEM((dm // 2, dm), jnp.uint32),
            pltpu.VMEM((rows, heads * dh), F32),
            pltpu.VMEM((n_mem, dm), F32),
            pltpu.VMEM((pairs, dh, 128), jnp.uint32),
            pltpu.VMEM((pairs, rows, pw), F32),
            pltpu.VMEM((pairs, rows, 128), F32),
            pltpu.VMEM((dm // 2, seq), jnp.uint32),
            pltpu.VMEM((2, dm, CHUNK), F32),
            pltpu.VMEM((B_HEADS // 2, 2 * bdh + 8, 4 * bdh), F32),
            pltpu.VMEM((seq, dm), BF16),
            pltpu.SemaphoreType.DMA,
            pltpu.SemaphoreType.DMA((2,)),
            pltpu.SemaphoreType.DMA((RING, 5)),
            pltpu.SemaphoreType.DMA((seq // CHUNK,)),
        ],
        compiler_params=pltpu.CompilerParams(vmem_limit_bytes=120 * 1024 * 1024),
    )(
        A_x.reshape(n_seg, seg // EARLY, EARLY, dm),
        A_mem0.reshape(n_mem, dm),
        w_t(A_Wq), w_t(A_Wk), w_t(A_Wv),
        A_Wo.reshape(heads * dh, dm),
        B_wqkv,
        jnp.transpose(B_w_phi, (1, 2, 0)),
        B_wo,
    )
    return out.reshape(batch, seq, dm)
```

```python
import functools

import jax
import jax.numpy as jnp
from jax import lax
import jax.experimental.pallas as pl
import jax.experimental.pallas.tpu as pltpu

F32 = jnp.float32
BF16 = jnp.bfloat16

B_HEADS = 32
LN_EPS = 1e-05
DEN_EPS = 1e-06
MASK_FILL = -1000000000.0
LOG2E = 1.4426950408889634

LAG = 4
EARLY = 8
UNROLL = 2
LEAD = 2
RING = 4
CHUNK = 256
B_LAG = 3
KV_CHUNK = 128
KV_LAG = 3
SUB = 64
OUT_LAG = 4
LN_LAG = 1

_NN = (((1,), (0,)), ((), ()))
_NT = (((1,), (1,)), ((), ()))


def _mm(a, b):
    return lax.dot_general(a, b, _NN, preferred_element_type=F32)


def _mm_nt(a, b):
    return lax.dot_general(a, b, _NT, preferred_element_type=F32)


def _pack(w):
    return pltpu.bitcast(w, jnp.uint32)


def _unpack(w):
    return pltpu.bitcast(w, BF16)


def _iota(shape, dim):
    return lax.broadcasted_iota(jnp.int32, shape, dim)


def _div_const(r, d):
    mul = (1 << 18) // d + 1
    assert all((v * mul) >> 18 == v // d for v in range(4096))
    return (r * mul) >> 18


def _recip(x):
    r = pl.reciprocal(x, approx=True)
    return r * (2.0 - x * r)


def _layernorm(x):
    m = jnp.mean(x, axis=-1, keepdims=True)
    xc = x - m
    v = jnp.mean(xc * xc, axis=-1, keepdims=True)
    return xc * lax.rsqrt(v + LN_EPS)


def _pair_reduce(v, op):
    v = op(v, pltpu.roll(v, 4, 0))
    return op(v, pltpu.roll(v, 2, 0))


def _hedgehog(p):
    rows = [p[i:i + 8] for i in range(0, p.shape[0], 8)]
    hi = _pair_reduce(functools.reduce(jnp.maximum, rows), jnp.maximum)
    lo = _pair_reduce(functools.reduce(jnp.minimum, rows), jnp.minimum)
    ep = [jnp.exp2(r - hi) for r in rows]
    en = [jnp.exp2(lo - r) for r in rows]
    rp = _recip(_pair_reduce(functools.reduce(jnp.add, ep), jnp.add))
    rn = _recip(_pair_reduce(functools.reduce(jnp.add, en), jnp.add))
    return jnp.concatenate([e * rp for e in ep] + [e * rn for e in en], axis=0)


def _kernel(
    x_hbm, mem0_ref, wq_hbm, wk_hbm, wv_hbm, wo_hbm, bqkv_hbm, wphi_ref, bwo_hbm,
    out_hbm,
    xin_ref, xe_ref, he_ref, xres_ref, hn_ref, ya_ref, wqkv_ref, wo_ref, stage_ref, early_ref,
    bqkv_ref, bwo_ref, sel_ref, bq_ref, bkv_ref, bo_ref,
    o_ref, mem_ref, kt_ref, v_ref, p_ref, ht_ref, ot_ref, kv_ref, z_ref, res_ref,
    sem_x, sem_b, sem_w, sem_out,
    *, seg, heads, dh,
):
    seq, dm = out_hbm.shape
    n_mem = mem0_ref.shape[0]
    n_seg = seq // seg
    rows = n_mem + seg
    pairs = heads // 2
    pw = 2 * dh
    off = -(-rows // 16) * 16
    scale = dh ** (-0.5)
    bdh = dm // B_HEADS
    grp = 2 * bdh
    n_grp = B_HEADS // 2

    cp_xe = pltpu.make_async_copy(x_hbm.at[:, seg // EARLY - 1], xe_ref, sem_x)
    cp_bqkv = pltpu.make_async_copy(bqkv_hbm, bqkv_ref, sem_b.at[0])
    cp_bwo = pltpu.make_async_copy(bwo_hbm, bwo_ref, sem_b.at[1])

    def rows_of(j, n):
        return pl.ds(j * n if isinstance(j, int) else pl.multiple_of(j * n, n), n)

    def cp_w(m, j):
        slot = j & (RING - 1)
        if m == 4:
            n = n_seg // pairs
            return pltpu.make_async_copy(x_hbm.at[pl.ds(j * n, n)], xin_ref.at[slot], sem_w.at[slot, m])
        src = (wq_hbm, wk_hbm, wv_hbm, wo_hbm)[m]
        return pltpu.make_async_copy(src.at[rows_of(j, pw)], stage_ref.at[slot, m], sem_w.at[slot, m])

    def groups_of(kt):
        return range(128 * kt // grp, (128 * kt + 127) // grp + 1)

    def build_selectors():
        eh_r = _iota((B_HEADS, dm), 0)
        eh_c = _iota((B_HEADS, dm), 1)
        phi_f = None
        for d in range(bdh):
            eh = jnp.where(eh_c == eh_r * bdh + d, 1.0, 0.0).astype(BF16)
            t = _mm(wphi_ref[d], eh)
            phi_f = t if phi_f is None else phi_f + t
        pick = jnp.where((_iota((grp, bdh), 0) >> 1) == _iota((grp, bdh), 1), 1.0, 0.0)
        phi_rows = _mm(pick, phi_f.astype(BF16))
        r = _iota((grp, 128), 0)
        for kt in range(dm // 128):
            c = _iota((grp, 128), 1) + 128 * kt
            c_head = _div_const(c, bdh)
            for i, g in enumerate(groups_of(kt)):
                head = 2 * g + (r & 1)
                sel_ref[0, kt, i] = jnp.where(c_head == head, phi_rows[:, 128 * kt:128 * kt + 128], 0.0)
                sel_ref[1, kt, i] = jnp.where(c == head * bdh + (r >> 1), 1.0, 0.0)

    skew, ahead = 2, 2

    def copies(j, has_kv, has_rest):
        return [cp_w(m, j) for m in (1, 2) if has_kv] + [cp_w(m, j - skew) for m in (0, 3, 4) if has_rest]

    def parts(j):
        return j < pairs, skew <= j < pairs + skew

    def load_round(j, now, later):
        for cp in copies(j, *now):
            cp.wait()
        prefetch = copies(j + ahead, *later)
        if now[0]:
            slot = j & (RING - 1)
            for m in (1, 2):
                early_ref[j, :, (m - 1) * pw:m * pw] = _mm_nt(he_ref[...], stage_ref[slot, m])
                if m == 1:
                    for cp in prefetch:
                        cp.start()
                wqkv_ref[j, :, m * pw:(m + 1) * pw] = _pack(stage_ref[slot, m].T)
        else:
            for cp in prefetch:
                cp.start()
        if now[1]:
            i = j - skew
            slot = i & (RING - 1)
            n = seq // pairs
            x = xin_ref[slot].astype(F32).reshape(n, dm)
            xres_ref[rows_of(i, n), :] = x
            hn_ref[rows_of(i, n), :] = _layernorm(x)
            wqkv_ref[i, :, 0:pw] = _pack(stage_ref[slot, 0].T)
            wo_ref[rows_of(i, dh), :] = _pack(stage_ref[slot, 3])

    cp_xe.start()
    for cp in copies(0, *parts(0)):
        cp.start()
    build_selectors()
    cp_xe.wait()
    for j in range(1, ahead):
        for cp in copies(j, *parts(j)):
            cp.start()
    he_ref[...] = _layernorm(xe_ref[...].astype(F32).reshape(n_seg * EARLY, dm))

    def load_body(j, carry):
        load_round(j, (True, True), (True, True))
        return carry

    for j in range(skew):
        load_round(j, parts(j), parts(j + ahead))
    lax.fori_loop(skew, pairs - ahead, load_body, 0)
    for j in range(pairs - ahead, pairs + skew):
        load_round(j, parts(j), parts(j + ahead))
    cp_bqkv.start()
    cp_bwo.start()

    cut = dh % 128

    def stack(a, b):
        gap = jnp.zeros((off - rows, a.shape[1]), F32)
        tail = jnp.zeros((128 - off - rows, a.shape[1]), F32)
        return jnp.concatenate([a, gap, b, tail], axis=0).astype(BF16)

    def store_keys(j, t):
        outer = _pack(stack(t[:, 0:128], t[:, 256:384]).T)
        inner = _pack(stack(t[:, 128:256], t[:, 128:256]).T)
        low = _iota((64, 128), 1) < off
        kt_ref[j, 0:64] = jnp.where(low, outer, 0)
        kt_ref[j, 64:64 + cut // 2] = jnp.where(low[:cut // 2], inner[:cut // 2], 0)
        kt_ref[j, 64 + cut // 2:128] = jnp.where(low[cut // 2:], 0, inner[cut // 2:])
        kt_ref[j, 128:192] = jnp.where(low, 0, outer)

    def load_values(j):
        t = v_ref[j]
        low = _iota((rows, 128), 1) < cut
        none = jnp.zeros((rows, 128), F32)
        first = jnp.concatenate([t[:, 0:128], jnp.where(low, t[:, 128:256], 0.0), none], axis=1)
        second = jnp.concatenate([none, jnp.where(low, 0.0, t[:, 128:256]), t[:, 256:384]], axis=1)
        return stack(first, second)

    def a_step(s, first_layer):
        h = jnp.concatenate([mem_ref[...], hn_ref[rows_of(s, seg), :]], axis=0)
        qi = _iota((rows, 128), 0)
        ki = _iota((rows, 128), 1)
        in_a = ki < rows
        in_b = (ki >= off) & (ki < off + rows)
        see_a = in_a & ((qi < n_mem) | (qi >= ki))
        see_b = in_b & ((qi < n_mem) | (qi >= ki - off))
        fill_a = jnp.where(in_a, MASK_FILL, -jnp.inf)
        fill_b = jnp.where(in_b, MASK_FILL, -jnp.inf)

        def partial_proj(m, j, d0, d1):
            n = rows - EARLY if first_layer and m > 0 else rows
            return _mm(h[:n, d0:d1], _unpack(wqkv_ref[j, d0 // 2:d1 // 2, m * pw:(m + 1) * pw]))

        def with_early(m, j, t):
            if first_layer and m > 0:
                done = early_ref[j, rows_of(s, EARLY), (m - 1) * pw:m * pw]
                return jnp.concatenate([t, done], axis=0)
            return t

        def proj(m, j):
            return with_early(m, j, partial_proj(m, j, 0, dm))

        def scores(j):
            sc = _mm(o_ref[:, j * pw:(j + 1) * pw], _unpack(kt_ref[j])) * scale
            sa = jnp.where(see_a, sc, fill_a)
            sb = jnp.where(see_b, sc, fill_b)
            ea = jnp.exp(sa - jnp.max(sa, axis=-1, keepdims=True))
            eb = jnp.exp(sb - jnp.max(sb, axis=-1, keepdims=True))
            ra = _recip(jnp.sum(ea, axis=-1, keepdims=True))
            rb = _recip(jnp.sum(eb, axis=-1, keepdims=True))
            p_ref[j] = ea * ra + eb * rb

        def attend(j):
            o_ref[:, j * pw:(j + 1) * pw] = _mm(p_ref[j], load_values(j))

        def out_proj(j0, j1, cols):
            return _mm(o_ref[:, j0 * pw:j1 * pw], _unpack(wo_ref[j0 * dh:j1 * dh, cols]))

        split = dm - 256
        nk = rows - EARLY if first_layer else rows
        for j in range(LEAD):
            v_ref[j, 0:nk] = partial_proj(1, j, 0, split)
        for j in range(LEAD):
            v_ref[LEAD + j, 0:nk] = partial_proj(1, j, split, dm)
        for j in range(LEAD):
            store_keys(j, with_early(1, j, v_ref[j, 0:nk] + v_ref[LEAD + j, 0:nk]))
        for j in range(LEAD, pairs):
            store_keys(j, proj(1, j))
        for j in range(pairs):
            o_ref[:, j * pw:(j + 1) * pw] = proj(0, j)
            if j >= LAG:
                scores(j - LAG)
        for j in range(pairs):
            v = proj(2, j)
            if j < LAG:
                scores(pairs - LAG + j)
            v_ref[j] = v
            if j >= LAG:
                attend(j - LAG)
        y = out_proj(0, pairs // 2, slice(0, dm))
        for j in range(pairs - LAG, pairs):
            attend(j)
        for cols in (slice(0, split), slice(split, dm)):
            t = y[:, cols] + out_proj(pairs // 2, pairs, cols)
            mem_ref[:, cols] = t[:n_mem]
            ya_ref[rows_of(s, seg), cols] = t[n_mem:]

    def a_layer(first_layer):
        def a_body(i, carry):
            for u in range(UNROLL):
                a_step(i * UNROLL + u, first_layer)
            return carry

        lax.fori_loop(0, n_seg // UNROLL, a_body, 0)

    def b_fold_weights():
        def fold(which, product):
            out = {}
            for kt in range(dm // 128):
                gs = groups_of(kt)
                block = jnp.concatenate([sel_ref[which, kt, i] for i in range(len(gs))], axis=0)
                part = product(block, 128 * kt)
                for i, g in enumerate(gs):
                    t = part[i * grp:(i + 1) * grp]
                    out[g] = out[g] + t if g in out else t
            return out

        def store(ref, blocks):
            for i in range(0, len(blocks), 2):
                two = jnp.concatenate(blocks[i:i + 2], axis=0).astype(BF16)
                ref[i * bdh:(i + 2) * bdh, :] = _pack(two)

        def from_qkv(m):
            return lambda b, c: _mm_nt(b, bqkv_ref[:, m * dm + c:m * dm + c + 128])

        cp_bqkv.wait()
        cp_bwo.wait()
        wk, wv = fold(0, from_qkv(1)), fold(1, from_qkv(2))
        wk = {g: w * LOG2E for g, w in wk.items()}
        store(bkv_ref, [w[g] for g in range(n_grp) for w in (wk, wv)])
        wq = fold(0, from_qkv(0))
        store(bq_ref, [wq[g] * LOG2E for g in range(n_grp)])
        wo = fold(1, lambda b, c: _mm(b, bwo_ref[c:c + 128, :]))
        store(bo_ref, [wo[g] for g in range(n_grp)])

    def b_kv():
        n_chunk = seq // KV_CHUNK
        tokens = lambda i: slice(i * KV_CHUNK, (i + 1) * KV_CHUNK)

        def normalize(i):
            xn = xres_ref[tokens(i), :] + ya_ref[tokens(i), :]
            xres_ref[tokens(i), :] = xn
            ht_ref[:, tokens(i)] = _pack(_layernorm(xn).astype(BF16).T)

        work = [(i, g) for i in range(n_chunk) for g in range(n_grp)]
        ready = {}
        normalize(0)
        for n in range(len(work) + KV_LAG):
            if n < len(work):
                i, g = work[n]
                if g == 0 and i + 1 < n_chunk:
                    normalize(i + 1)
                t = _mm(_unpack(bkv_ref[g * grp:(g + 1) * grp, :]), _unpack(ht_ref[:, tokens(i)]))
                phi = _hedgehog(t[:grp])
                ready[n] = (t[grp:], phi.astype(BF16))
                z = phi if i == 0 else z_ref[g] + phi
                if i == n_chunk - 1:
                    z = jnp.broadcast_to(jnp.sum(z, axis=-1, keepdims=True), z.shape)
                z_ref[g] = z
            if n >= KV_LAG:
                i, g = work[n - KV_LAG]
                t = _mm_nt(*ready.pop(n - KV_LAG))
                if i > 0:
                    t = kv_ref[g] + t
                if i == n_chunk - 1:
                    t = jnp.where(((_iota(t.shape, 0) ^ _iota(t.shape, 1)) & 1) == 0, t, 0.0)
                kv_ref[g] = t

    n_chunk = seq // CHUNK
    tokens = lambda i: slice(i * CHUNK, (i + 1) * CHUNK)

    def cp_out(i):
        return pltpu.make_async_copy(res_ref.at[tokens(i)], out_hbm.at[tokens(i)], sem_out.at[i])

    def b_out(zero):
        half = n_grp // 2
        n_sub = CHUNK // SUB
        work = [(i, gg) for i in range(n_chunk) for gg in range(half)]
        ready = {}

        def staged(i, r0, n):
            return pl.ds(pl.multiple_of(zero + seq + (i % 2) * (CHUNK // 2) + r0, 8), n)

        def features(g, p):
            phi = _hedgehog(p)
            t = phi * jnp.concatenate([z_ref[g]] * (CHUNK // 128), axis=1)
            den = functools.reduce(jnp.add, [t[r:r + 8] for r in range(0, 2 * grp, 8)])
            return phi.astype(BF16), _recip(_pair_reduce(den, jnp.add) + DEN_EPS)

        finished = []

        def normalize():
            sl = finished.pop(0)
            hn_ref[sl, :] = _layernorm(xres_ref[sl, :])

        def finish(i, k):
            if len(finished) > LN_LAG:
                normalize()
            sl = slice(i * CHUNK + k * SUB, i * CHUNK + (k + 1) * SUB)
            o = _unpack(hn_ref[staged(i, k * SUB // 2, SUB // 2), :])
            xn = xres_ref[sl, :] + _mm(o, _unpack(bo_ref[...]))
            xres_ref[sl, :] = xn
            res_ref[sl, :] = xn.astype(BF16)
            finished.append(sl)
            if k == n_sub - 1:
                cp_out(i).start()

        pending = []
        for n in range(len(work) + B_LAG):
            if n < len(work):
                i, gg = work[n]
                t = _mm(_unpack(bq_ref[gg * grp:(gg + 1) * grp, :]), _unpack(ht_ref[:, tokens(i)]))
                ready[n] = [features(2 * gg + k, t[k * grp:(k + 1) * grp]) for k in range(2)]
            while pending and pending[0][0] <= n:
                finish(*pending.pop(0)[1:])
            if n >= B_LAG:
                i, gg = work[n - B_LAG]
                for k, (phi, inv) in enumerate(ready.pop(n - B_LAG)):
                    g = 2 * gg + k
                    num = _mm(kv_ref[g], phi)
                    ot_ref[g * grp:(g + 1) * grp, :] = jnp.concatenate(
                        [num[r:r + 8] * inv for r in range(0, grp, 8)], axis=0)
                if gg == half - 1:
                    hn_ref[staged(i, 0, CHUNK // 2), :] = pltpu.bitcast(ot_ref[...].astype(BF16).T, F32)
                    pending += [(n + OUT_LAG + k * half // n_sub, i, k) for k in range(n_sub)]
        for _, i, k in pending:
            finish(i, k)
        while finished:
            normalize()

    def layer_pair(it, carry):
        mem_ref[...] = mem0_ref[...].astype(F32)

        @pl.when(it == 0)
        def _():
            a_layer(True)
            b_fold_weights()

        @pl.when(it == 1)
        def _():
            a_layer(False)
            for i in range(n_chunk):
                cp_out(i).wait()

        with jax.named_scope("L_b_kv"):
            b_kv()
        with jax.named_scope("L_b_out"):
            b_out(it * (it - 1))
        return carry

    lax.fori_loop(0, 2, layer_pair, 0)
    for i in range(n_chunk):
        cp_out(i).wait()


@functools.partial(jax.jit, static_argnames=("A_seg_len",))
def pallas_interleave_layers__memory_aug_recurrent_mem_tr__linear_kernel_hedgehog__prompt_kernel(
    A_x: jax.Array,
    A_mem0: jax.Array,
    A_Wq: jax.Array,
    A_Wk: jax.Array,
    A_Wv: jax.Array,
    A_Wo: jax.Array,
    A_seg_len: int,
    B_x: jax.Array,
    B_wqkv: jax.Array,
    B_w_phi: jax.Array,
    B_wo: jax.Array,
):
    del B_x
    batch, seq, dm = A_x.shape
    _, heads, dh = A_Wq.shape
    n_mem = A_mem0.shape[1]
    seg = int(A_seg_len)
    n_seg = seq // seg
    rows = n_mem + seg
    pw = 2 * dh
    pairs = heads // 2
    bdh = dm // B_HEADS
    assert batch == 1 and seq % CHUNK == 0 and CHUNK % seg == 0 and seg % EARLY == 0
    assert n_mem % 8 == 0 and rows <= 48
    assert heads % 2 == 0 and pw == 3 * 128 and dm % 128 == 0 and (2 * bdh) % 8 == 0

    w_t = lambda w: jnp.transpose(w, (1, 2, 0)).reshape(heads * dh, dm)
    hbm = pl.BlockSpec(memory_space=pl.ANY)
    vmem = pl.BlockSpec(memory_space=pltpu.VMEM)

    out = pl.pallas_call(
        functools.partial(_kernel, seg=seg, heads=heads, dh=dh),
        out_shape=jax.ShapeDtypeStruct((seq, dm), A_x.dtype),
        in_specs=[hbm, vmem, hbm, hbm, hbm, hbm, hbm, vmem, hbm],
        out_specs=hbm,
        scratch_shapes=[
            pltpu.VMEM((RING, n_seg // pairs, seg // EARLY, EARLY, dm), BF16),
            pltpu.VMEM((n_seg, EARLY, dm), BF16),
            pltpu.VMEM((n_seg * EARLY, dm), F32),
            pltpu.VMEM((seq, dm), F32),
            pltpu.VMEM((seq + CHUNK, dm), F32),
            pltpu.VMEM((seq, dm), F32),
            pltpu.VMEM((pairs, dm // 2, 3 * pw), jnp.uint32),
            pltpu.VMEM((pairs * dh, dm), jnp.uint32),
            pltpu.VMEM((RING, 4, pw, dm), BF16),
            pltpu.VMEM((pairs, n_seg * EARLY, 2 * pw), F32),
            pltpu.VMEM((dm, 3 * dm), BF16),
            pltpu.VMEM((dm, dm), BF16),
            pltpu.VMEM((2, dm // 128, 127 // (2 * bdh) + 2, 2 * bdh, 128), F32),
            pltpu.VMEM((dm // 2, dm), jnp.uint32),
            pltpu.VMEM((dm, dm), jnp.uint32),
            pltpu.VMEM((dm // 2, dm), jnp.uint32),
            pltpu.VMEM((rows, heads * dh), F32),
            pltpu.VMEM((n_mem, dm), F32),
            pltpu.VMEM((pairs, dh, 128), jnp.uint32),
            pltpu.VMEM((pairs, rows, pw), F32),
            pltpu.VMEM((pairs, rows, 128), F32),
            pltpu.VMEM((dm // 2, seq), jnp.uint32),
            pltpu.VMEM((dm, CHUNK), F32),
            pltpu.VMEM((B_HEADS // 2, 2 * bdh, 4 * bdh), F32),
            pltpu.VMEM((B_HEADS // 2, 4 * bdh, 128), F32),
            pltpu.VMEM((seq, dm), BF16),
            pltpu.SemaphoreType.DMA,
            pltpu.SemaphoreType.DMA((2,)),
            pltpu.SemaphoreType.DMA((RING, 5)),
            pltpu.SemaphoreType.DMA((seq // CHUNK,)),
        ],
        compiler_params=pltpu.CompilerParams(vmem_limit_bytes=120 * 1024 * 1024),
    )(
        A_x.reshape(n_seg, seg // EARLY, EARLY, dm),
        A_mem0.reshape(n_mem, dm),
        w_t(A_Wq), w_t(A_Wk), w_t(A_Wv),
        A_Wo.reshape(heads * dh, dm),
        B_wqkv,
        jnp.transpose(B_w_phi, (1, 2, 0)),
        B_wo,
    )
    return out.reshape(batch, seq, dm)
```

```python
import functools

import jax
import jax.numpy as jnp
from jax import lax
import jax.experimental.pallas as pl
import jax.experimental.pallas.tpu as pltpu

F32 = jnp.float32
BF16 = jnp.bfloat16

B_HEADS = 32
LN_EPS = 1e-05
DEN_EPS = 1e-06
MASK_FILL = -1000000000.0
LOG2E = 1.4426950408889634

LAG = 4
EARLY = 8
EARLY_Q = 2
UNROLL = 2
LEAD = 2
RING = 4
CHUNK = 256
B_LAG = 3
KV_CHUNK = 128
KV_LAG = 3
SUB = 64
OUT_LAG = 4
LN_LAG = 1

_NN = (((1,), (0,)), ((), ()))
_NT = (((1,), (1,)), ((), ()))


def _mm(a, b):
    return lax.dot_general(a, b, _NN, preferred_element_type=F32)


def _mm_nt(a, b):
    return lax.dot_general(a, b, _NT, preferred_element_type=F32)


def _pack(w):
    return pltpu.bitcast(w, jnp.uint32)


def _unpack(w):
    return pltpu.bitcast(w, BF16)


def _iota(shape, dim):
    return lax.broadcasted_iota(jnp.int32, shape, dim)


def _div_const(r, d):
    mul = (1 << 18) // d + 1
    assert all((v * mul) >> 18 == v // d for v in range(4096))
    return (r * mul) >> 18


def _recip(x):
    r = pl.reciprocal(x, approx=True)
    return r * (2.0 - x * r)


def _layernorm(x):
    m = jnp.mean(x, axis=-1, keepdims=True)
    xc = x - m
    v = jnp.mean(xc * xc, axis=-1, keepdims=True)
    return xc * lax.rsqrt(v + LN_EPS)


def _pair_reduce(v, op):
    v = op(v, pltpu.roll(v, 4, 0))
    return op(v, pltpu.roll(v, 2, 0))


def _hedgehog(p):
    rows = [p[i:i + 8] for i in range(0, p.shape[0], 8)]
    hi = _pair_reduce(functools.reduce(jnp.maximum, rows), jnp.maximum)
    lo = _pair_reduce(functools.reduce(jnp.minimum, rows), jnp.minimum)
    ep = [jnp.exp2(r - hi) for r in rows]
    en = [jnp.exp2(lo - r) for r in rows]
    rp = _recip(_pair_reduce(functools.reduce(jnp.add, ep), jnp.add))
    rn = _recip(_pair_reduce(functools.reduce(jnp.add, en), jnp.add))
    return jnp.concatenate([e * rp for e in ep] + [e * rn for e in en], axis=0)


def _kernel(
    x_hbm, mem0_hbm, wq_hbm, wk_hbm, wv_hbm, wo_hbm, bqkv_hbm, wphi_hbm, bwo_hbm,
    out_hbm,
    mem0_ref, wphi_ref,
    xin_ref, xe_ref, he_ref, xres_ref, hn_ref, ya_ref, wqkv_ref, wo_ref, stage_ref, early_ref, early_q_ref,
    bqkv_ref, bwo_ref, sel_ref, bq_ref, bkv_ref, bo_ref,
    o_ref, mem_ref, kt_ref, v_ref, p_ref, ht_ref, ot_ref, kv_ref, z_ref, res_ref,
    sem_x, sem_b, sem_w, sem_out,
    *, seg, heads, dh,
):
    seq, dm = out_hbm.shape
    n_mem = mem0_ref.shape[0]
    n_seg = seq // seg
    rows = n_mem + seg
    pairs = heads // 2
    pw = 2 * dh
    off = -(-rows // 16) * 16
    scale = dh ** (-0.5)
    bdh = dm // B_HEADS
    grp = 2 * bdh
    n_grp = B_HEADS // 2

    cp_xe = pltpu.make_async_copy(x_hbm.at[:, seg // EARLY - 1], xe_ref, sem_x.at[0])
    cp_mem0 = pltpu.make_async_copy(mem0_hbm, mem0_ref, sem_x.at[1])
    cp_wphi = pltpu.make_async_copy(wphi_hbm, wphi_ref, sem_x.at[2])
    cp_bqkv = pltpu.make_async_copy(bqkv_hbm, bqkv_ref, sem_b.at[0])
    cp_bwo = pltpu.make_async_copy(bwo_hbm, bwo_ref, sem_b.at[1])

    def rows_of(j, n):
        return pl.ds(j * n if isinstance(j, int) else pl.multiple_of(j * n, n), n)

    def cp_w(m, j):
        slot = j & (RING - 1)
        if m == 4:
            n = n_seg // pairs
            return pltpu.make_async_copy(x_hbm.at[pl.ds(j * n, n)], xin_ref.at[slot], sem_w.at[slot, m])
        src = (wq_hbm, wk_hbm, wv_hbm, wo_hbm)[m]
        return pltpu.make_async_copy(src.at[rows_of(j, pw)], stage_ref.at[slot, m], sem_w.at[slot, m])

    def groups_of(kt):
        return range(128 * kt // grp, (128 * kt + 127) // grp + 1)

    def build_selectors():
        eh_r = _iota((B_HEADS, dm), 0)
        eh_c = _iota((B_HEADS, dm), 1)
        phi_f = None
        for d in range(bdh):
            eh = jnp.where(eh_c == eh_r * bdh + d, 1.0, 0.0).astype(BF16)
            t = _mm(wphi_ref[d], eh)
            phi_f = t if phi_f is None else phi_f + t
        pick = jnp.where((_iota((grp, bdh), 0) >> 1) == _iota((grp, bdh), 1), 1.0, 0.0)
        phi_rows = _mm(pick, phi_f.astype(BF16))
        r = _iota((grp, 128), 0)
        for kt in range(dm // 128):
            c = _iota((grp, 128), 1) + 128 * kt
            c_head = _div_const(c, bdh)
            for i, g in enumerate(groups_of(kt)):
                head = 2 * g + (r & 1)
                sel_ref[0, kt, i] = jnp.where(c_head == head, phi_rows[:, 128 * kt:128 * kt + 128], 0.0)
                sel_ref[1, kt, i] = jnp.where(c == head * bdh + (r >> 1), 1.0, 0.0)

    skew, ahead = EARLY_Q, RING - 1

    def parts(j):
        early = (1, 2, 0) if j < skew else (1, 2) if j < pairs else ()
        late = () if j < skew else (3, 4) if j < 2 * skew else (0, 3, 4) if j < pairs + skew else ()
        return early, late

    def copies(j, early, late):
        return [cp_w(m, j) for m in early] + [cp_w(m, j - skew) for m in late]

    def project_early(m, j):
        w = stage_ref[j & (RING - 1), m]
        if m == 0:
            early_q_ref[j] = _mm_nt(he_ref[...], w)
        else:
            early_ref[j, :, (m - 1) * pw:m * pw] = _mm_nt(he_ref[...], w)
        wqkv_ref[j, :, m * pw:(m + 1) * pw] = _pack(w.T)

    def unpack_late(i, late):
        slot = i & (RING - 1)
        if 0 in late:
            wqkv_ref[i, :, 0:pw] = _pack(stage_ref[slot, 0].T)
        if late:
            n = seq // pairs
            x = xin_ref[slot].astype(F32).reshape(n, dm)
            xres_ref[rows_of(i, n), :] = x
            hn_ref[rows_of(i, n), :] = _layernorm(x)
            wo_ref[rows_of(i, dh), :] = _pack(stage_ref[slot, 3])

    def load_round(j, now, later):
        for cp in copies(j, *now):
            cp.wait()
        for n, m in enumerate(now[0]):
            project_early(m, j)
            if n == 0:
                for cp in copies(j + ahead, *later):
                    cp.start()
        unpack_late(j - skew, now[1])

    def load_body(j, carry):
        load_round(j, parts(2 * skew), parts(2 * skew))
        return carry

    first, *rest = copies(0, *parts(0))
    for cp in (cp_wphi, cp_mem0, cp_xe, first):
        cp.start()
    cp_wphi.wait()
    build_selectors()
    cp_xe.wait()
    for cp in rest:
        cp.start()
    he_ref[...] = _layernorm(xe_ref[...].astype(F32).reshape(n_seg * EARLY, dm))
    first.wait()
    for j in range(1, ahead):
        for cp in copies(j, *parts(j)):
            cp.start()
    project_early(parts(0)[0][0], 0)
    load_round(0, (parts(0)[0][1:], ()), parts(ahead))
    for j in range(1, 2 * skew):
        load_round(j, parts(j), parts(j + ahead))
    lax.fori_loop(2 * skew, pairs - ahead, load_body, 0)
    for j in range(pairs - ahead, pairs - 1):
        load_round(j, parts(j), parts(j + ahead))
    for cp in copies(pairs, *parts(pairs)):
        cp.wait()
    load_round(pairs - 1, parts(pairs - 1), ((), ()))
    unpack_late(pairs - skew, parts(pairs)[1])
    for j in range(pairs + 1, pairs + skew):
        load_round(j, parts(j), ((), ()))
    cp_mem0.wait()
    cp_bqkv.start()
    cp_bwo.start()

    cut = dh % 128

    def stack(a, b):
        gap = jnp.zeros((off - rows, a.shape[1]), F32)
        tail = jnp.zeros((128 - off - rows, a.shape[1]), F32)
        return jnp.concatenate([a, gap, b, tail], axis=0).astype(BF16)

    def store_keys(j, t):
        outer = _pack(stack(t[:, 0:128], t[:, 256:384]).T)
        inner = _pack(stack(t[:, 128:256], t[:, 128:256]).T)
        low = _iota((64, 128), 1) < off
        kt_ref[j, 0:64] = jnp.where(low, outer, 0)
        kt_ref[j, 64:64 + cut // 2] = jnp.where(low[:cut // 2], inner[:cut // 2], 0)
        kt_ref[j, 64 + cut // 2:128] = jnp.where(low[cut // 2:], 0, inner[cut // 2:])
        kt_ref[j, 128:192] = jnp.where(low, 0, outer)

    def load_values(j):
        t = v_ref[j]
        low = _iota((rows, 128), 1) < cut
        none = jnp.zeros((rows, 128), F32)
        first = jnp.concatenate([t[:, 0:128], jnp.where(low, t[:, 128:256], 0.0), none], axis=1)
        second = jnp.concatenate([none, jnp.where(low, 0.0, t[:, 128:256]), t[:, 256:384]], axis=1)
        return stack(first, second)

    def a_step(s, first_layer):
        h = jnp.concatenate([mem_ref[...], hn_ref[rows_of(s, seg), :]], axis=0)
        qi = _iota((rows, 128), 0)
        ki = _iota((rows, 128), 1)
        in_a = ki < rows
        in_b = (ki >= off) & (ki < off + rows)
        see_a = in_a & ((qi < n_mem) | (qi >= ki))
        see_b = in_b & ((qi < n_mem) | (qi >= ki - off))
        fill_a = jnp.where(in_a, MASK_FILL, -jnp.inf)
        fill_b = jnp.where(in_b, MASK_FILL, -jnp.inf)

        def has_early(m, j):
            return first_layer and (m > 0 or j < EARLY_Q)

        def partial_proj(m, j, d0, d1):
            n = rows - EARLY if has_early(m, j) else rows
            return _mm(h[:n, d0:d1], _unpack(wqkv_ref[j, d0 // 2:d1 // 2, m * pw:(m + 1) * pw]))

        def with_early(m, j, t):
            if not has_early(m, j):
                return t
            sl = rows_of(s, EARLY)
            done = early_ref[j, sl, (m - 1) * pw:m * pw] if m > 0 else early_q_ref[j, sl, :]
            return jnp.concatenate([t, done], axis=0)

        def proj(m, j):
            return with_early(m, j, partial_proj(m, j, 0, dm))

        def scores(j):
            sc = _mm(o_ref[:, j * pw:(j + 1) * pw], _unpack(kt_ref[j])) * scale
            sa = jnp.where(see_a, sc, fill_a)
            sb = jnp.where(see_b, sc, fill_b)
            ea = jnp.exp(sa - jnp.max(sa, axis=-1, keepdims=True))
            eb = jnp.exp(sb - jnp.max(sb, axis=-1, keepdims=True))
            ra = _recip(jnp.sum(ea, axis=-1, keepdims=True))
            rb = _recip(jnp.sum(eb, axis=-1, keepdims=True))
            p_ref[j] = ea * ra + eb * rb

        def attend(j):
            o_ref[:, j * pw:(j + 1) * pw] = _mm(p_ref[j], load_values(j))

        def out_proj(j0, j1, cols):
            return _mm(o_ref[:, j0 * pw:j1 * pw], _unpack(wo_ref[j0 * dh:j1 * dh, cols]))

        split = dm - 256
        nk = rows - EARLY if first_layer else rows
        for j in range(LEAD):
            v_ref[j, 0:nk] = partial_proj(1, j, 0, split)
        for j in range(LEAD):
            v_ref[LEAD + j, 0:nk] = partial_proj(1, j, split, dm)
        for j in range(LEAD):
            store_keys(j, with_early(1, j, v_ref[j, 0:nk] + v_ref[LEAD + j, 0:nk]))
        for j in range(LEAD, pairs):
            store_keys(j, proj(1, j))
        for j in range(pairs):
            o_ref[:, j * pw:(j + 1) * pw] = proj(0, j)
            if j >= LAG:
                scores(j - LAG)
        for j in range(pairs):
            v = proj(2, j)
            if j < LAG:
                scores(pairs - LAG + j)
            v_ref[j] = v
            if j >= LAG:
                attend(j - LAG)
        y = out_proj(0, pairs // 2, slice(0, dm))
        for j in range(pairs - LAG, pairs):
            attend(j)
        for cols in (slice(0, split), slice(split, dm)):
            t = y[:, cols] + out_proj(pairs // 2, pairs, cols)
            mem_ref[:, cols] = t[:n_mem]
            ya_ref[rows_of(s, seg), cols] = t[n_mem:]

    def a_layer(first_layer):
        def a_body(i, carry):
            for u in range(UNROLL):
                a_step(i * UNROLL + u, first_layer)
            return carry

        lax.fori_loop(0, n_seg // UNROLL, a_body, 0)

    def b_fold_weights():
        def fold(which, product):
            out = {}
            for kt in range(dm // 128):
                gs = groups_of(kt)
                block = jnp.concatenate([sel_ref[which, kt, i] for i in range(len(gs))], axis=0)
                part = product(block, 128 * kt)
                for i, g in enumerate(gs):
                    t = part[i * grp:(i + 1) * grp]
                    out[g] = out[g] + t if g in out else t
            return out

        def store(ref, blocks):
            for i in range(0, len(blocks), 2):
                two = jnp.concatenate(blocks[i:i + 2], axis=0).astype(BF16)
                ref[i * bdh:(i + 2) * bdh, :] = _pack(two)

        def from_qkv(m):
            return lambda b, c: _mm_nt(b, bqkv_ref[:, m * dm + c:m * dm + c + 128])

        cp_bqkv.wait()
        cp_bwo.wait()
        wk, wv = fold(0, from_qkv(1)), fold(1, from_qkv(2))
        wk = {g: w * LOG2E for g, w in wk.items()}
        store(bkv_ref, [w[g] for g in range(n_grp) for w in (wk, wv)])
        wq = fold(0, from_qkv(0))
        store(bq_ref, [wq[g] * LOG2E for g in range(n_grp)])
        wo = fold(1, lambda b, c: _mm(b, bwo_ref[c:c + 128, :]))
        store(bo_ref, [wo[g] for g in range(n_grp)])

    def b_kv():
        n_chunk = seq // KV_CHUNK
        tokens = lambda i: slice(i * KV_CHUNK, (i + 1) * KV_CHUNK)

        def normalize(i):
            xn = xres_ref[tokens(i), :] + ya_ref[tokens(i), :]
            xres_ref[tokens(i), :] = xn
            ht_ref[:, tokens(i)] = _pack(_layernorm(xn).astype(BF16).T)

        work = [(i, g) for i in range(n_chunk) for g in range(n_grp)]
        ready = {}
        normalize(0)
        for n in range(len(work) + KV_LAG):
            if n < len(work):
                i, g = work[n]
                if g == 0 and i + 1 < n_chunk:
                    normalize(i + 1)
                t = _mm(_unpack(bkv_ref[g * grp:(g + 1) * grp, :]), _unpack(ht_ref[:, tokens(i)]))
                phi = _hedgehog(t[:grp])
                ready[n] = (t[grp:], phi.astype(BF16))
                z = phi if i == 0 else z_ref[g] + phi
                if i == n_chunk - 1:
                    z = jnp.broadcast_to(jnp.sum(z, axis=-1, keepdims=True), z.shape)
                z_ref[g] = z
            if n >= KV_LAG:
                i, g = work[n - KV_LAG]
                t = _mm_nt(*ready.pop(n - KV_LAG))
                if i > 0:
                    t = kv_ref[g] + t
                if i == n_chunk - 1:
                    t = jnp.where(((_iota(t.shape, 0) ^ _iota(t.shape, 1)) & 1) == 0, t, 0.0)
                kv_ref[g] = t

    n_chunk = seq // CHUNK
    tokens = lambda i: slice(i * CHUNK, (i + 1) * CHUNK)

    def cp_out(i):
        return pltpu.make_async_copy(res_ref.at[tokens(i)], out_hbm.at[tokens(i)], sem_out.at[i])

    def b_out(zero):
        half = n_grp // 2
        n_sub = CHUNK // SUB
        work = [(i, gg) for i in range(n_chunk) for gg in range(half)]
        ready = {}

        def staged(i, r0, n):
            return pl.ds(pl.multiple_of(zero + seq + (i % 2) * (CHUNK // 2) + r0, 8), n)

        def features(g, p):
            phi = _hedgehog(p)
            t = phi * jnp.concatenate([z_ref[g]] * (CHUNK // 128), axis=1)
            den = functools.reduce(jnp.add, [t[r:r + 8] for r in range(0, 2 * grp, 8)])
            return phi.astype(BF16), _recip(_pair_reduce(den, jnp.add) + DEN_EPS)

        finished = []

        def normalize():
            sl = finished.pop(0)
            hn_ref[sl, :] = _layernorm(xres_ref[sl, :])

        def finish(i, k):
            if len(finished) > LN_LAG:
                normalize()
            sl = slice(i * CHUNK + k * SUB, i * CHUNK + (k + 1) * SUB)
            o = _unpack(hn_ref[staged(i, k * SUB // 2, SUB // 2), :])
            xn = xres_ref[sl, :] + _mm(o, _unpack(bo_ref[...]))
            xres_ref[sl, :] = xn
            res_ref[sl, :] = xn.astype(BF16)
            finished.append(sl)
            if k == n_sub - 1:
                cp_out(i).start()

        pending = []
        for n in range(len(work) + B_LAG):
            if n < len(work):
                i, gg = work[n]
                t = _mm(_unpack(bq_ref[gg * grp:(gg + 1) * grp, :]), _unpack(ht_ref[:, tokens(i)]))
                ready[n] = [features(2 * gg + k, t[k * grp:(k + 1) * grp]) for k in range(2)]
            while pending and pending[0][0] <= n:
                finish(*pending.pop(0)[1:])
            if n >= B_LAG:
                i, gg = work[n - B_LAG]
                for k, (phi, inv) in enumerate(ready.pop(n - B_LAG)):
                    g = 2 * gg + k
                    num = _mm(kv_ref[g], phi)
                    ot_ref[g * grp:(g + 1) * grp, :] = jnp.concatenate(
                        [num[r:r + 8] * inv for r in range(0, grp, 8)], axis=0)
                if gg == half - 1:
                    hn_ref[staged(i, 0, CHUNK // 2), :] = pltpu.bitcast(ot_ref[...].astype(BF16).T, F32)
                    pending += [(n + OUT_LAG + k * half // n_sub, i, k) for k in range(n_sub)]
        for _, i, k in pending:
            finish(i, k)
        while finished:
            normalize()

    def layer_pair(it, carry):
        mem_ref[...] = mem0_ref[...].astype(F32)

        @pl.when(it == 0)
        def _():
            a_layer(True)
            b_fold_weights()

        @pl.when(it == 1)
        def _():
            a_layer(False)
            for i in range(n_chunk):
                cp_out(i).wait()

        with jax.named_scope("L_b_kv"):
            b_kv()
        with jax.named_scope("L_b_out"):
            b_out(it * (it - 1))
        return carry

    lax.fori_loop(0, 2, layer_pair, 0)
    for i in range(n_chunk):
        cp_out(i).wait()


@functools.partial(jax.jit, static_argnames=("A_seg_len",))
def pallas_interleave_layers__memory_aug_recurrent_mem_tr__linear_kernel_hedgehog__prompt_kernel(
    A_x: jax.Array,
    A_mem0: jax.Array,
    A_Wq: jax.Array,
    A_Wk: jax.Array,
    A_Wv: jax.Array,
    A_Wo: jax.Array,
    A_seg_len: int,
    B_x: jax.Array,
    B_wqkv: jax.Array,
    B_w_phi: jax.Array,
    B_wo: jax.Array,
):
    del B_x
    batch, seq, dm = A_x.shape
    _, heads, dh = A_Wq.shape
    n_mem = A_mem0.shape[1]
    seg = int(A_seg_len)
    n_seg = seq // seg
    rows = n_mem + seg
    pw = 2 * dh
    pairs = heads // 2
    bdh = dm // B_HEADS
    assert batch == 1 and seq % CHUNK == 0 and CHUNK % seg == 0 and seg % EARLY == 0
    assert n_mem % 8 == 0 and rows <= 48
    assert heads % 2 == 0 and pw == 3 * 128 and dm % 128 == 0 and (2 * bdh) % 8 == 0

    w_t = lambda w: jnp.transpose(w, (1, 2, 0)).reshape(heads * dh, dm)
    hbm = pl.BlockSpec(memory_space=pl.ANY)

    out = pl.pallas_call(
        functools.partial(_kernel, seg=seg, heads=heads, dh=dh),
        out_shape=jax.ShapeDtypeStruct((seq, dm), A_x.dtype),
        in_specs=[hbm] * 9,
        out_specs=hbm,
        scratch_shapes=[
            pltpu.VMEM((n_mem, dm), BF16),
            pltpu.VMEM((bdh, bdh, B_HEADS), BF16),
            pltpu.VMEM((RING, n_seg // pairs, seg // EARLY, EARLY, dm), BF16),
            pltpu.VMEM((n_seg, EARLY, dm), BF16),
            pltpu.VMEM((n_seg * EARLY, dm), F32),
            pltpu.VMEM((seq, dm), F32),
            pltpu.VMEM((seq + CHUNK, dm), F32),
            pltpu.VMEM((seq, dm), F32),
            pltpu.VMEM((pairs, dm // 2, 3 * pw), jnp.uint32),
            pltpu.VMEM((pairs * dh, dm), jnp.uint32),
            pltpu.VMEM((RING, 4, pw, dm), BF16),
            pltpu.VMEM((pairs, n_seg * EARLY, 2 * pw), F32),
            pltpu.VMEM((EARLY_Q, n_seg * EARLY, pw), F32),
            pltpu.VMEM((dm, 3 * dm), BF16),
            pltpu.VMEM((dm, dm), BF16),
            pltpu.VMEM((2, dm // 128, 127 // (2 * bdh) + 2, 2 * bdh, 128), F32),
            pltpu.VMEM((dm // 2, dm), jnp.uint32),
            pltpu.VMEM((dm, dm), jnp.uint32),
            pltpu.VMEM((dm // 2, dm), jnp.uint32),
            pltpu.VMEM((rows, heads * dh), F32),
            pltpu.VMEM((n_mem, dm), F32),
            pltpu.VMEM((pairs, dh, 128), jnp.uint32),
            pltpu.VMEM((pairs, rows, pw), F32),
            pltpu.VMEM((pairs, rows, 128), F32),
            pltpu.VMEM((dm // 2, seq), jnp.uint32),
            pltpu.VMEM((dm, CHUNK), F32),
            pltpu.VMEM((B_HEADS // 2, 2 * bdh, 4 * bdh), F32),
            pltpu.VMEM((B_HEADS // 2, 4 * bdh, 128), F32),
            pltpu.VMEM((seq, dm), BF16),
            pltpu.SemaphoreType.DMA((3,)),
            pltpu.SemaphoreType.DMA((2,)),
            pltpu.SemaphoreType.DMA((RING, 5)),
            pltpu.SemaphoreType.DMA((seq // CHUNK,)),
        ],
        compiler_params=pltpu.CompilerParams(vmem_limit_bytes=120 * 1024 * 1024),
    )(
        A_x.reshape(n_seg, seg // EARLY, EARLY, dm),
        A_mem0.reshape(n_mem, dm),
        w_t(A_Wq), w_t(A_Wk), w_t(A_Wv),
        A_Wo.reshape(heads * dh, dm),
        B_wqkv,
        jnp.transpose(B_w_phi, (1, 2, 0)),
        B_wo,
    )
    return out.reshape(batch, seq, dm)
```

```python
import functools

import jax
import jax.numpy as jnp
from jax import lax
import jax.experimental.pallas as pl
import jax.experimental.pallas.tpu as pltpu

F32 = jnp.float32
BF16 = jnp.bfloat16

B_HEADS = 32
LN_EPS = 1e-05
DEN_EPS = 1e-06
MASK_FILL = -1000000000.0
LOG2E = 1.4426950408889634

LAG = 4
EARLY = 8
EARLY_Q = 2
UNROLL = 2
LEAD = 2
RING = 4
CHUNK = 256
B_LAG = 3
KV_CHUNK = 128
KV_LAG = 3
SUB = 64
OUT_LAG = 4
LN_LAG = 1

_NN = (((1,), (0,)), ((), ()))
_NT = (((1,), (1,)), ((), ()))


def _mm(a, b):
    return lax.dot_general(a, b, _NN, preferred_element_type=F32)


def _mm_nt(a, b):
    return lax.dot_general(a, b, _NT, preferred_element_type=F32)


def _pack(w):
    return pltpu.bitcast(w, jnp.uint32)


def _unpack(w):
    return pltpu.bitcast(w, BF16)


def _iota(shape, dim):
    return lax.broadcasted_iota(jnp.int32, shape, dim)


def _div_const(r, d):
    mul = (1 << 18) // d + 1
    assert all((v * mul) >> 18 == v // d for v in range(4096))
    return (r * mul) >> 18


def _recip(x):
    r = pl.reciprocal(x, approx=True)
    return r * (2.0 - x * r)


def _layernorm(x):
    m = jnp.mean(x, axis=-1, keepdims=True)
    xc = x - m
    v = jnp.mean(xc * xc, axis=-1, keepdims=True)
    return xc * lax.rsqrt(v + LN_EPS)


def _pair_reduce(v, op):
    v = op(v, pltpu.roll(v, 4, 0))
    return op(v, pltpu.roll(v, 2, 0))


def _hedgehog(p):
    rows = [p[i:i + 8] for i in range(0, p.shape[0], 8)]
    hi = _pair_reduce(functools.reduce(jnp.maximum, rows), jnp.maximum)
    lo = _pair_reduce(functools.reduce(jnp.minimum, rows), jnp.minimum)
    ep = [jnp.exp2(r - hi) for r in rows]
    en = [jnp.exp2(lo - r) for r in rows]
    rp = _recip(_pair_reduce(functools.reduce(jnp.add, ep), jnp.add))
    rn = _recip(_pair_reduce(functools.reduce(jnp.add, en), jnp.add))
    return jnp.concatenate([e * rp for e in ep] + [e * rn for e in en], axis=0)


def _kernel(
    x_hbm, mem0_hbm, wq_hbm, wk_hbm, wv_hbm, wo_hbm, bqkv_hbm, wphi_hbm, bwo_hbm,
    out_hbm,
    mem0_ref, wphi_ref,
    xin_ref, xe_ref, he_ref, xres_ref, hn_ref, ya_ref, wqkv_ref, wo_ref, stage_ref, early_ref, early_q_ref,
    bqkv_ref, bwo_ref, sel_ref, bq_ref, bkv_ref, bo_ref,
    o_ref, mem_ref, kt_ref, v_ref, p_ref, ht_ref, ot_ref, kv_ref, z_ref, res_ref, zero_ref,
    sem_x, sem_b, sem_w, sem_out,
    *, seg, heads, dh,
):
    seq, dm = out_hbm.shape
    n_mem = mem0_ref.shape[0]
    n_seg = seq // seg
    rows = n_mem + seg
    pairs = heads // 2
    pw = 2 * dh
    off = -(-rows // 16) * 16
    scale = dh ** (-0.5)
    bdh = dm // B_HEADS
    grp = 2 * bdh
    n_grp = B_HEADS // 2

    cp_xe = pltpu.make_async_copy(x_hbm.at[:, seg // EARLY - 1], xe_ref, sem_x.at[0])
    cp_mem0 = pltpu.make_async_copy(mem0_hbm, mem0_ref, sem_x.at[1])
    cp_wphi = pltpu.make_async_copy(wphi_hbm, wphi_ref, sem_x.at[2])
    cp_bqkv = pltpu.make_async_copy(bqkv_hbm, bqkv_ref, sem_b.at[0])
    cp_bwo = pltpu.make_async_copy(bwo_hbm, bwo_ref, sem_b.at[1])

    def rows_of(j, n):
        return pl.ds(j * n if isinstance(j, int) else pl.multiple_of(j * n, n), n)

    def cp_w(m, j):
        slot = j & (RING - 1)
        if m == 4:
            n = n_seg // pairs
            return pltpu.make_async_copy(x_hbm.at[pl.ds(j * n, n)], xin_ref.at[slot], sem_w.at[slot, m])
        src = (wq_hbm, wk_hbm, wv_hbm, wo_hbm)[m]
        return pltpu.make_async_copy(src.at[rows_of(j, pw)], stage_ref.at[slot, m], sem_w.at[slot, m])

    def groups_of(kt):
        return range(128 * kt // grp, (128 * kt + 127) // grp + 1)

    def build_selectors():
        eh_r = _iota((B_HEADS, dm), 0)
        eh_c = _iota((B_HEADS, dm), 1)
        phi_f = None
        for d in range(bdh):
            eh = jnp.where(eh_c == eh_r * bdh + d, 1.0, 0.0).astype(BF16)
            t = _mm(wphi_ref[d], eh)
            phi_f = t if phi_f is None else phi_f + t
        pick = jnp.where((_iota((grp, bdh), 0) >> 1) == _iota((grp, bdh), 1), 1.0, 0.0)
        phi_rows = _mm(pick, phi_f.astype(BF16))
        r = _iota((grp, 128), 0)
        for kt in range(dm // 128):
            c = _iota((grp, 128), 1) + 128 * kt
            c_head = _div_const(c, bdh)
            for i, g in enumerate(groups_of(kt)):
                head = 2 * g + (r & 1)
                sel_ref[0, kt, i] = jnp.where(c_head == head, phi_rows[:, 128 * kt:128 * kt + 128], 0.0)
                sel_ref[1, kt, i] = jnp.where(c == head * bdh + (r >> 1), 1.0, 0.0)

    skew, ahead = EARLY_Q, RING - 1

    def parts(j):
        early = (1, 2, 0) if j < skew else (1, 2) if j < pairs else ()
        late = () if j < skew else (3, 4) if j < 2 * skew else (0, 3, 4) if j < pairs + skew else ()
        return early, late

    def copies(j, early, late):
        return [cp_w(m, j) for m in early] + [cp_w(m, j - skew) for m in late]

    def project_early(m, j):
        w = stage_ref[j & (RING - 1), m]
        if m == 0:
            early_q_ref[j] = _mm_nt(he_ref[...], w)
        else:
            early_ref[j, :, (m - 1) * pw:m * pw] = _mm_nt(he_ref[...], w)
        wqkv_ref[j, :, m * pw:(m + 1) * pw] = _pack(w.T)

    def unpack_late(i, late):
        slot = i & (RING - 1)
        if 0 in late:
            wqkv_ref[i, :, 0:pw] = _pack(stage_ref[slot, 0].T)
        if late:
            n = seq // pairs
            x = xin_ref[slot].astype(F32).reshape(n, dm)
            xres_ref[rows_of(i, n), :] = x
            hn_ref[rows_of(i, n), :] = _layernorm(x)
            wo_ref[rows_of(i, dh), :] = _pack(stage_ref[slot, 3])

    def load_round(j, now, later):
        for cp in copies(j, *now):
            cp.wait()
        for n, m in enumerate(now[0]):
            project_early(m, j)
            if n == 0:
                for cp in copies(j + ahead, *later):
                    cp.start()
        unpack_late(j - skew, now[1])

    def load_body(j, carry):
        load_round(j, parts(2 * skew), parts(2 * skew))
        return carry

    zero_ref[0] = 0
    first, *rest = copies(0, *parts(0))
    for cp in (cp_wphi, cp_mem0, cp_xe, first):
        cp.start()
    cp_wphi.wait()
    build_selectors()
    cp_xe.wait()
    for cp in rest:
        cp.start()
    he_ref[...] = _layernorm(xe_ref[...].astype(F32).reshape(n_seg * EARLY, dm))
    first.wait()
    for j in range(1, ahead):
        for cp in copies(j, *parts(j)):
            cp.start()
    project_early(parts(0)[0][0], 0)
    load_round(0, (parts(0)[0][1:], ()), parts(ahead))
    for j in range(1, 2 * skew):
        load_round(j, parts(j), parts(j + ahead))
    lax.fori_loop(2 * skew, pairs - ahead, load_body, 0)
    for j in range(pairs - ahead, pairs - 1):
        load_round(j, parts(j), parts(j + ahead))
    for cp in copies(pairs, *parts(pairs)):
        cp.wait()
    load_round(pairs - 1, parts(pairs - 1), ((), ()))
    unpack_late(pairs - skew, parts(pairs)[1])
    for j in range(pairs + 1, pairs + skew):
        load_round(j, parts(j), ((), ()))
    cp_mem0.wait()
    cp_bqkv.start()
    cp_bwo.start()

    cut = dh % 128

    def stack(a, b):
        gap = jnp.zeros((off - rows, a.shape[1]), F32)
        tail = jnp.zeros((128 - off - rows, a.shape[1]), F32)
        return jnp.concatenate([a, gap, b, tail], axis=0).astype(BF16)

    def store_keys(j, t):
        outer = _pack(stack(t[:, 0:128], t[:, 256:384]).T)
        inner = _pack(stack(t[:, 128:256], t[:, 128:256]).T)
        low = _iota((64, 128), 1) < off
        kt_ref[j, 0:64] = jnp.where(low, outer, 0)
        kt_ref[j, 64:64 + cut // 2] = jnp.where(low[:cut // 2], inner[:cut // 2], 0)
        kt_ref[j, 64 + cut // 2:128] = jnp.where(low[cut // 2:], 0, inner[cut // 2:])
        kt_ref[j, 128:192] = jnp.where(low, 0, outer)

    def load_values(j):
        t = v_ref[j]
        low = _iota((rows, 128), 1) < cut
        none = jnp.zeros((rows, 128), F32)
        first = jnp.concatenate([t[:, 0:128], jnp.where(low, t[:, 128:256], 0.0), none], axis=1)
        second = jnp.concatenate([none, jnp.where(low, 0.0, t[:, 128:256]), t[:, 256:384]], axis=1)
        return stack(first, second)

    def a_step(s, first_layer):
        h = jnp.concatenate([mem_ref[...], hn_ref[rows_of(s, seg), :]], axis=0)
        qi = _iota((rows, 128), 0)
        ki = _iota((rows, 128), 1)
        in_a = ki < rows
        in_b = (ki >= off) & (ki < off + rows)
        see_a = in_a & ((qi < n_mem) | (qi >= ki))
        see_b = in_b & ((qi < n_mem) | (qi >= ki - off))
        fill_a = jnp.where(in_a, MASK_FILL, -jnp.inf)
        fill_b = jnp.where(in_b, MASK_FILL, -jnp.inf)

        def has_early(m, j):
            return first_layer and (m > 0 or j < EARLY_Q)

        def partial_proj(m, j, d0, d1):
            n = rows - EARLY if has_early(m, j) else rows
            return _mm(h[:n, d0:d1], _unpack(wqkv_ref[j, d0 // 2:d1 // 2, m * pw:(m + 1) * pw]))

        def with_early(m, j, t):
            if not has_early(m, j):
                return t
            sl = rows_of(s, EARLY)
            done = early_ref[j, sl, (m - 1) * pw:m * pw] if m > 0 else early_q_ref[j, sl, :]
            return jnp.concatenate([t, done], axis=0)

        def proj(m, j):
            return with_early(m, j, partial_proj(m, j, 0, dm))

        def scores(j):
            sc = _mm(o_ref[:, j * pw:(j + 1) * pw], _unpack(kt_ref[j])) * scale
            sa = jnp.where(see_a, sc, fill_a)
            sb = jnp.where(see_b, sc, fill_b)
            ea = jnp.exp(sa - jnp.max(sa, axis=-1, keepdims=True))
            eb = jnp.exp(sb - jnp.max(sb, axis=-1, keepdims=True))
            ra = _recip(jnp.sum(ea, axis=-1, keepdims=True))
            rb = _recip(jnp.sum(eb, axis=-1, keepdims=True))
            p_ref[j] = ea * ra + eb * rb

        def attend(j):
            o_ref[:, j * pw:(j + 1) * pw] = _mm(p_ref[j], load_values(j))

        def out_proj(j0, j1, cols):
            return _mm(o_ref[:, j0 * pw:j1 * pw], _unpack(wo_ref[j0 * dh:j1 * dh, cols]))

        split = dm - 256
        nk = rows - EARLY if first_layer else rows
        for j in range(LEAD):
            v_ref[j, 0:nk] = partial_proj(1, j, 0, split)
        for j in range(LEAD):
            v_ref[LEAD + j, 0:nk] = partial_proj(1, j, split, dm)
        for j in range(LEAD):
            store_keys(j, with_early(1, j, v_ref[j, 0:nk] + v_ref[LEAD + j, 0:nk]))
        for j in range(LEAD, pairs):
            store_keys(j, proj(1, j))
        for j in range(pairs):
            o_ref[:, j * pw:(j + 1) * pw] = proj(0, j)
            if j >= LAG:
                scores(j - LAG)
        for j in range(pairs):
            v = proj(2, j)
            if j < LAG:
                scores(pairs - LAG + j)
            v_ref[j] = v
            if j >= LAG:
                attend(j - LAG)
        y = out_proj(0, pairs // 2, slice(0, dm))
        for j in range(pairs - LAG, pairs):
            attend(j)
        for cols in (slice(0, split), slice(split, dm)):
            t = y[:, cols] + out_proj(pairs // 2, pairs, cols)
            mem_ref[:, cols] = t[:n_mem]
            ya_ref[rows_of(s, seg), cols] = t[n_mem:]

    def a_layer(first_layer):
        def a_body(i, carry):
            for u in range(UNROLL):
                a_step(i * UNROLL + u, first_layer)
            return carry

        mem_ref[...] = mem0_ref[...].astype(F32)
        lax.fori_loop(0, n_seg // UNROLL, a_body, 0)

    def b_fold_weights():
        def fold(which, product):
            out = {}
            for kt in range(dm // 128):
                gs = groups_of(kt)
                block = jnp.concatenate([sel_ref[which, kt, i] for i in range(len(gs))], axis=0)
                part = product(block, 128 * kt)
                for i, g in enumerate(gs):
                    t = part[i * grp:(i + 1) * grp]
                    out[g] = out[g] + t if g in out else t
            return out

        def store(ref, blocks):
            for i in range(0, len(blocks), 2):
                two = jnp.concatenate(blocks[i:i + 2], axis=0).astype(BF16)
                ref[i * bdh:(i + 2) * bdh, :] = _pack(two)

        def from_qkv(m):
            return lambda b, c: _mm_nt(b, bqkv_ref[:, m * dm + c:m * dm + c + 128])

        cp_bqkv.wait()
        cp_bwo.wait()
        wk, wv = fold(0, from_qkv(1)), fold(1, from_qkv(2))
        wk = {g: w * LOG2E for g, w in wk.items()}
        store(bkv_ref, [w[g] for g in range(n_grp) for w in (wk, wv)])
        wq = fold(0, from_qkv(0))
        store(bq_ref, [wq[g] * LOG2E for g in range(n_grp)])
        wo = fold(1, lambda b, c: _mm(b, bwo_ref[c:c + 128, :]))
        store(bo_ref, [wo[g] for g in range(n_grp)])

    def b_kv():
        n_chunk = seq // KV_CHUNK
        tokens = lambda i: slice(i * KV_CHUNK, (i + 1) * KV_CHUNK)

        def normalize(i):
            xn = xres_ref[tokens(i), :] + ya_ref[tokens(i), :]
            xres_ref[tokens(i), :] = xn
            ht_ref[:, tokens(i)] = _pack(_layernorm(xn).astype(BF16).T)

        work = [(i, g) for i in range(n_chunk) for g in range(n_grp)]
        ready = {}
        normalize(0)
        for n in range(len(work) + KV_LAG):
            if n < len(work):
                i, g = work[n]
                if g == 0 and i + 1 < n_chunk:
                    normalize(i + 1)
                t = _mm(_unpack(bkv_ref[g * grp:(g + 1) * grp, :]), _unpack(ht_ref[:, tokens(i)]))
                phi = _hedgehog(t[:grp])
                ready[n] = (t[grp:], phi.astype(BF16))
                z = phi if i == 0 else z_ref[g] + phi
                if i == n_chunk - 1:
                    z = jnp.broadcast_to(jnp.sum(z, axis=-1, keepdims=True), z.shape)
                z_ref[g] = z
            if n >= KV_LAG:
                i, g = work[n - KV_LAG]
                t = _mm_nt(*ready.pop(n - KV_LAG))
                if i > 0:
                    t = kv_ref[g] + t
                if i == n_chunk - 1:
                    t = jnp.where(((_iota(t.shape, 0) ^ _iota(t.shape, 1)) & 1) == 0, t, 0.0)
                kv_ref[g] = t

    n_chunk = seq // CHUNK
    tokens = lambda i: slice(i * CHUNK, (i + 1) * CHUNK)

    def cp_out(i):
        return pltpu.make_async_copy(res_ref.at[tokens(i)], out_hbm.at[tokens(i)], sem_out.at[i])

    def b_out(last_layer):
        zero = zero_ref[0]
        half = n_grp // 2
        n_sub = CHUNK // SUB
        work = [(i, gg) for i in range(n_chunk) for gg in range(half)]
        ready = {}

        def staged(i, r0, n):
            return pl.ds(pl.multiple_of(zero + seq + (i % 2) * (CHUNK // 2) + r0, 8), n)

        def features(g, p):
            phi = _hedgehog(p)
            t = phi * jnp.concatenate([z_ref[g]] * (CHUNK // 128), axis=1)
            den = functools.reduce(jnp.add, [t[r:r + 8] for r in range(0, 2 * grp, 8)])
            return phi.astype(BF16), _recip(_pair_reduce(den, jnp.add) + DEN_EPS)

        finished = []

        def normalize():
            sl = finished.pop(0)
            hn_ref[sl, :] = _layernorm(xres_ref[sl, :])

        def finish(i, k):
            if len(finished) > LN_LAG:
                normalize()
            sl = slice(i * CHUNK + k * SUB, i * CHUNK + (k + 1) * SUB)
            o = _unpack(hn_ref[staged(i, k * SUB // 2, SUB // 2), :])
            xn = xres_ref[sl, :] + _mm(o, _unpack(bo_ref[...]))
            if last_layer:
                res_ref[sl, :] = xn.astype(BF16)
                if k == n_sub - 1:
                    cp_out(i).start()
            else:
                xres_ref[sl, :] = xn
                finished.append(sl)

        pending = []
        for n in range(len(work) + B_LAG):
            if n < len(work):
                i, gg = work[n]
                t = _mm(_unpack(bq_ref[gg * grp:(gg + 1) * grp, :]), _unpack(ht_ref[:, tokens(i)]))
                ready[n] = [features(2 * gg + k, t[k * grp:(k + 1) * grp]) for k in range(2)]
            while pending and pending[0][0] <= n:
                finish(*pending.pop(0)[1:])
            if n >= B_LAG:
                i, gg = work[n - B_LAG]
                for k, (phi, inv) in enumerate(ready.pop(n - B_LAG)):
                    g = 2 * gg + k
                    num = _mm(kv_ref[g], phi)
                    ot_ref[g * grp:(g + 1) * grp, :] = jnp.concatenate(
                        [num[r:r + 8] * inv for r in range(0, grp, 8)], axis=0)
                if gg == half - 1:
                    hn_ref[staged(i, 0, CHUNK // 2), :] = pltpu.bitcast(ot_ref[...].astype(BF16).T, F32)
                    pending += [(n + OUT_LAG + k * half // n_sub, i, k) for k in range(n_sub)]
        for _, i, k in pending:
            finish(i, k)
        while finished:
            normalize()

    a_layer(True)
    b_fold_weights()
    with jax.named_scope("L_b_kv"):
        b_kv()
    with jax.named_scope("L_b_out"):
        b_out(False)
    a_layer(False)
    with jax.named_scope("L_b_kv"):
        b_kv()
    with jax.named_scope("L_b_out"):
        b_out(True)
    for i in range(n_chunk):
        cp_out(i).wait()


@functools.partial(jax.jit, static_argnames=("A_seg_len",))
def pallas_interleave_layers__memory_aug_recurrent_mem_tr__linear_kernel_hedgehog__prompt_kernel(
    A_x: jax.Array,
    A_mem0: jax.Array,
    A_Wq: jax.Array,
    A_Wk: jax.Array,
    A_Wv: jax.Array,
    A_Wo: jax.Array,
    A_seg_len: int,
    B_x: jax.Array,
    B_wqkv: jax.Array,
    B_w_phi: jax.Array,
    B_wo: jax.Array,
):
    del B_x
    batch, seq, dm = A_x.shape
    _, heads, dh = A_Wq.shape
    n_mem = A_mem0.shape[1]
    seg = int(A_seg_len)
    n_seg = seq // seg
    rows = n_mem + seg
    pw = 2 * dh
    pairs = heads // 2
    bdh = dm // B_HEADS
    assert batch == 1 and seq % CHUNK == 0 and CHUNK % seg == 0 and seg % EARLY == 0
    assert n_mem % 8 == 0 and rows <= 48
    assert heads % 2 == 0 and pw == 3 * 128 and dm % 128 == 0 and (2 * bdh) % 8 == 0

    w_t = lambda w: jnp.transpose(w, (1, 2, 0)).reshape(heads * dh, dm)
    hbm = pl.BlockSpec(memory_space=pl.ANY)

    out = pl.pallas_call(
        functools.partial(_kernel, seg=seg, heads=heads, dh=dh),
        out_shape=jax.ShapeDtypeStruct((seq, dm), A_x.dtype),
        in_specs=[hbm] * 9,
        out_specs=hbm,
        scratch_shapes=[
            pltpu.VMEM((n_mem, dm), BF16),
            pltpu.VMEM((bdh, bdh, B_HEADS), BF16),
            pltpu.VMEM((RING, n_seg // pairs, seg // EARLY, EARLY, dm), BF16),
            pltpu.VMEM((n_seg, EARLY, dm), BF16),
            pltpu.VMEM((n_seg * EARLY, dm), F32),
            pltpu.VMEM((seq, dm), F32),
            pltpu.VMEM((seq + CHUNK, dm), F32),
            pltpu.VMEM((seq, dm), F32),
            pltpu.VMEM((pairs, dm // 2, 3 * pw), jnp.uint32),
            pltpu.VMEM((pairs * dh, dm), jnp.uint32),
            pltpu.VMEM((RING, 4, pw, dm), BF16),
            pltpu.VMEM((pairs, n_seg * EARLY, 2 * pw), F32),
            pltpu.VMEM((EARLY_Q, n_seg * EARLY, pw), F32),
            pltpu.VMEM((dm, 3 * dm), BF16),
            pltpu.VMEM((dm, dm), BF16),
            pltpu.VMEM((2, dm // 128, 127 // (2 * bdh) + 2, 2 * bdh, 128), F32),
            pltpu.VMEM((dm // 2, dm), jnp.uint32),
            pltpu.VMEM((dm, dm), jnp.uint32),
            pltpu.VMEM((dm // 2, dm), jnp.uint32),
            pltpu.VMEM((rows, heads * dh), F32),
            pltpu.VMEM((n_mem, dm), F32),
            pltpu.VMEM((pairs, dh, 128), jnp.uint32),
            pltpu.VMEM((pairs, rows, pw), F32),
            pltpu.VMEM((pairs, rows, 128), F32),
            pltpu.VMEM((dm // 2, seq), jnp.uint32),
            pltpu.VMEM((dm, CHUNK), F32),
            pltpu.VMEM((B_HEADS // 2, 2 * bdh, 4 * bdh), F32),
            pltpu.VMEM((B_HEADS // 2, 4 * bdh, 128), F32),
            pltpu.VMEM((seq, dm), BF16),
            pltpu.SMEM((1,), jnp.int32),
            pltpu.SemaphoreType.DMA((3,)),
            pltpu.SemaphoreType.DMA((2,)),
            pltpu.SemaphoreType.DMA((RING, 5)),
            pltpu.SemaphoreType.DMA((seq // CHUNK,)),
        ],
        compiler_params=pltpu.CompilerParams(vmem_limit_bytes=120 * 1024 * 1024),
    )(
        A_x.reshape(n_seg, seg // EARLY, EARLY, dm),
        A_mem0.reshape(n_mem, dm),
        w_t(A_Wq), w_t(A_Wk), w_t(A_Wv),
        A_Wo.reshape(heads * dh, dm),
        B_wqkv,
        jnp.transpose(B_w_phi, (1, 2, 0)),
        B_wo,
    )
    return out.reshape(batch, seq, dm)
```

```python
import functools

import jax
import jax.numpy as jnp
from jax import lax
import jax.experimental.pallas as pl
import jax.experimental.pallas.tpu as pltpu

F32 = jnp.float32
BF16 = jnp.bfloat16

B_HEADS = 32
LN_EPS = 1e-05
DEN_EPS = 1e-06
MASK_FILL = -1000000000.0
LOG2E = 1.4426950408889634

LAG = 4
EARLY = 8
EARLY_Q = 2
UNROLL = 2
LEAD = 2
RING = 4
CHUNK = 256
B_LAG = 3
KV_CHUNK = 128
KV_LAG = 3
SUB = 64
OUT_LAG = 4
LN_LAG = 1

_NN = (((1,), (0,)), ((), ()))
_NT = (((1,), (1,)), ((), ()))


def _mm(a, b):
    return lax.dot_general(a, b, _NN, preferred_element_type=F32)


def _mm_nt(a, b):
    return lax.dot_general(a, b, _NT, preferred_element_type=F32)


def _pack(w):
    return pltpu.bitcast(w, jnp.uint32)


def _unpack(w):
    return pltpu.bitcast(w, BF16)


def _iota(shape, dim):
    return lax.broadcasted_iota(jnp.int32, shape, dim)


def _div_const(r, d):
    mul = (1 << 18) // d + 1
    assert all((v * mul) >> 18 == v // d for v in range(4096))
    return (r * mul) >> 18


def _recip(x):
    r = pl.reciprocal(x, approx=True)
    return r * (2.0 - x * r)


def _layernorm(x):
    m = jnp.mean(x, axis=-1, keepdims=True)
    xc = x - m
    v = jnp.mean(xc * xc, axis=-1, keepdims=True)
    return xc * lax.rsqrt(v + LN_EPS)


def _pair_reduce(v, op):
    v = op(v, pltpu.roll(v, 4, 0))
    return op(v, pltpu.roll(v, 2, 0))


def _hedgehog(p):
    rows = [p[i:i + 8] for i in range(0, p.shape[0], 8)]
    hi = _pair_reduce(functools.reduce(jnp.maximum, rows), jnp.maximum)
    lo = _pair_reduce(functools.reduce(jnp.minimum, rows), jnp.minimum)
    ep = [jnp.exp2(r - hi) for r in rows]
    en = [jnp.exp2(lo - r) for r in rows]
    rp = _recip(_pair_reduce(functools.reduce(jnp.add, ep), jnp.add))
    rn = _recip(_pair_reduce(functools.reduce(jnp.add, en), jnp.add))
    return jnp.concatenate([e * rp for e in ep] + [e * rn for e in en], axis=0)


def _kernel(
    x_hbm, mem0_hbm, wq_hbm, wk_hbm, wv_hbm, wo_hbm, bqkv_hbm, wphi_hbm, bwo_hbm,
    out_hbm,
    mem0_ref, wphi_ref,
    xin_ref, xe_ref, he_ref, xres_ref, hn_ref, ya_ref, wqkv_ref, wo_ref, stage_ref, early_ref, early_q_ref,
    bqkv_ref, bwo_ref, sel_ref, bq_ref, bkv_ref, bo_ref,
    o_ref, mem_ref, qkv0_ref, kt_ref, v_ref, p_ref, ht_ref, ot_ref, kv_ref, z_ref, res_ref, zero_ref,
    sem_x, sem_b, sem_w, sem_out,
    *, seg, heads, dh,
):
    seq, dm = out_hbm.shape
    n_mem = mem0_ref.shape[0]
    n_seg = seq // seg
    rows = n_mem + seg
    pairs = heads // 2
    pw = 2 * dh
    off = -(-rows // 16) * 16
    scale = dh ** (-0.5)
    bdh = dm // B_HEADS
    grp = 2 * bdh
    n_grp = B_HEADS // 2

    cp_xe = pltpu.make_async_copy(x_hbm.at[:, seg // EARLY - 1], xe_ref, sem_x.at[0])
    cp_mem0 = pltpu.make_async_copy(mem0_hbm, mem0_ref, sem_x.at[1])
    cp_wphi = pltpu.make_async_copy(wphi_hbm, wphi_ref, sem_x.at[2])
    cp_bqkv = pltpu.make_async_copy(bqkv_hbm, bqkv_ref, sem_b.at[0])
    cp_bwo = pltpu.make_async_copy(bwo_hbm, bwo_ref, sem_b.at[1])

    def rows_of(j, n):
        return pl.ds(j * n if isinstance(j, int) else pl.multiple_of(j * n, n), n)

    def cp_w(m, j):
        slot = j & (RING - 1)
        if m == 4:
            n = n_seg // pairs
            return pltpu.make_async_copy(x_hbm.at[pl.ds(j * n, n)], xin_ref.at[slot], sem_w.at[slot, m])
        src = (wq_hbm, wk_hbm, wv_hbm, wo_hbm)[m]
        return pltpu.make_async_copy(src.at[rows_of(j, pw)], stage_ref.at[slot, m], sem_w.at[slot, m])

    def groups_of(kt):
        return range(128 * kt // grp, (128 * kt + 127) // grp + 1)

    def build_selectors():
        eh_r = _iota((B_HEADS, dm), 0)
        eh_c = _iota((B_HEADS, dm), 1)
        phi_f = None
        for d in range(bdh):
            eh = jnp.where(eh_c == eh_r * bdh + d, 1.0, 0.0).astype(BF16)
            t = _mm(wphi_ref[d], eh)
            phi_f = t if phi_f is None else phi_f + t
        pick = jnp.where((_iota((grp, bdh), 0) >> 1) == _iota((grp, bdh), 1), 1.0, 0.0)
        phi_rows = _mm(pick, phi_f.astype(BF16))
        r = _iota((grp, 128), 0)
        for kt in range(dm // 128):
            c = _iota((grp, 128), 1) + 128 * kt
            c_head = _div_const(c, bdh)
            for i, g in enumerate(groups_of(kt)):
                head = 2 * g + (r & 1)
                sel_ref[0, kt, i] = jnp.where(c_head == head, phi_rows[:, 128 * kt:128 * kt + 128], 0.0)
                sel_ref[1, kt, i] = jnp.where(c == head * bdh + (r >> 1), 1.0, 0.0)

    skew, ahead = EARLY_Q, RING - 1
    cp_kv = lambda j: [cp_w(m, j) for m in (1, 2)]
    cp_rest = lambda i: [cp_w(m, i) for m in (0, 3, 4)]

    def when(cond, copies, method):
        @pl.when(cond)
        def _():
            for cp in copies():
                getattr(cp, method)()

    def unpack_rest(i):
        slot, i = i & (RING - 1), jnp.maximum(i, 0)
        n = seq // pairs
        x = xin_ref[slot].astype(F32).reshape(n, dm)
        xres_ref[rows_of(i, n), :] = x
        hn_ref[rows_of(i, n), :] = _layernorm(x)
        wqkv_ref[i, :, 0:pw] = _pack(stage_ref[slot, 0].T)
        wo_ref[rows_of(i, dh), :] = _pack(stage_ref[slot, 3])

    def swap_rest(i):
        when(i >= 0, lambda: cp_rest(i), "wait")
        when((i + ahead >= 0) & (i + ahead < pairs), lambda: cp_rest(i + ahead), "start")

    def load_body(j, carry):
        for cp in cp_kv(j):
            cp.wait()
        when(j + ahead < pairs, lambda: cp_kv(j + ahead), "start")
        swap_rest(j - skew)
        for m in (1, 2):
            w = stage_ref[j & (RING - 1), m]
            early_ref[j, :, (m - 1) * pw:m * pw] = _mm_nt(he_ref[...], w)
            wqkv_ref[j, :, m * pw:(m + 1) * pw] = _pack(w.T)
        unpack_rest(j - skew)
        return carry

    def load_tail(t, carry):
        swap_rest(pairs - skew + t)
        early_q_ref[t] = _mm(he_ref[...], _unpack(wqkv_ref[t, :, 0:pw]))
        unpack_rest(pairs - skew + t)
        return carry

    zero_ref[0] = 0
    for cp in [cp_wphi, cp_mem0, cp_xe] + cp_kv(0):
        cp.start()
    cp_wphi.wait()
    build_selectors()
    cp_xe.wait()
    for j in range(1, ahead):
        for cp in cp_kv(j) + (cp_rest(j - skew) if j >= skew else []):
            cp.start()
    he_ref[...] = _layernorm(xe_ref[...].astype(F32).reshape(n_seg * EARLY, dm))
    lax.fori_loop(0, pairs, load_body, 0)
    lax.fori_loop(0, skew, load_tail, 0)
    cp_mem0.wait()
    cp_bqkv.start()
    cp_bwo.start()

    cut = dh % 128

    def stack(a, b):
        gap = jnp.zeros((off - rows, a.shape[1]), F32)
        tail = jnp.zeros((128 - off - rows, a.shape[1]), F32)
        return jnp.concatenate([a, gap, b, tail], axis=0).astype(BF16)

    def store_keys(j, t):
        outer = _pack(stack(t[:, 0:128], t[:, 256:384]).T)
        inner = _pack(stack(t[:, 128:256], t[:, 128:256]).T)
        low = _iota((64, 128), 1) < off
        kt_ref[j, 0:64] = jnp.where(low, outer, 0)
        kt_ref[j, 64:64 + cut // 2] = jnp.where(low[:cut // 2], inner[:cut // 2], 0)
        kt_ref[j, 64 + cut // 2:128] = jnp.where(low[cut // 2:], 0, inner[cut // 2:])
        kt_ref[j, 128:192] = jnp.where(low, 0, outer)

    def load_values(j):
        t = v_ref[j]
        low = _iota((rows, 128), 1) < cut
        none = jnp.zeros((rows, 128), F32)
        first = jnp.concatenate([t[:, 0:128], jnp.where(low, t[:, 128:256], 0.0), none], axis=1)
        second = jnp.concatenate([none, jnp.where(low, 0.0, t[:, 128:256]), t[:, 256:384]], axis=1)
        return stack(first, second)

    def a_step(s, first_layer):
        first_step = isinstance(s, int) and s == 0
        q0 = n_mem if isinstance(s, int) and s == n_seg - 1 else 0
        mem = mem0_ref[...].astype(F32) if first_step else mem_ref[...]
        h = jnp.concatenate([mem, hn_ref[rows_of(s, seg), :]], axis=0)
        qi = _iota((rows - q0, 128), 0) + q0
        ki = _iota((rows - q0, 128), 1)
        in_a = ki < rows
        in_b = (ki >= off) & (ki < off + rows)
        see_a = in_a & ((qi < n_mem) | (qi >= ki))
        see_b = in_b & ((qi < n_mem) | (qi >= ki - off))
        fill_a = jnp.where(in_a, MASK_FILL, -jnp.inf)
        fill_b = jnp.where(in_b, MASK_FILL, -jnp.inf)

        def streamed(m, j):
            if first_layer:
                return (q0 if m == 0 else 0), rows - (EARLY if m > 0 or j < EARLY_Q else 0)
            return (n_mem if first_step else q0 if m == 0 else 0), rows

        def partial_proj(m, j, d0, d1):
            r0, r1 = streamed(m, j)
            return _mm(h[r0:r1, d0:d1], _unpack(wqkv_ref[j, d0 // 2:d1 // 2, m * pw:(m + 1) * pw]))

        def complete(m, j, t):
            cols = slice(m * pw, (m + 1) * pw)
            if first_step and first_layer:
                qkv0_ref[j, :, cols] = t[:n_mem]
            elif first_step:
                t = jnp.concatenate([qkv0_ref[j, :, cols], t], axis=0)
            if streamed(m, j)[1] < rows:
                sl = rows_of(s, EARLY)
                done = early_ref[j, sl, (m - 1) * pw:m * pw] if m > 0 else early_q_ref[j, sl, :]
                t = jnp.concatenate([t, done], axis=0)
            return t

        def proj(m, j):
            return complete(m, j, partial_proj(m, j, 0, dm))

        def scores(j):
            sc = _mm(o_ref[q0:, j * pw:(j + 1) * pw], _unpack(kt_ref[j])) * scale
            sa = jnp.where(see_a, sc, fill_a)
            sb = jnp.where(see_b, sc, fill_b)
            ea = jnp.exp(sa - jnp.max(sa, axis=-1, keepdims=True))
            eb = jnp.exp(sb - jnp.max(sb, axis=-1, keepdims=True))
            ra = _recip(jnp.sum(ea, axis=-1, keepdims=True))
            rb = _recip(jnp.sum(eb, axis=-1, keepdims=True))
            p_ref[j, q0:] = ea * ra + eb * rb

        def attend(j):
            o_ref[q0:, j * pw:(j + 1) * pw] = _mm(p_ref[j, q0:], load_values(j))

        def out_proj(j0, j1, cols):
            return _mm(o_ref[q0:, j0 * pw:j1 * pw], _unpack(wo_ref[j0 * dh:j1 * dh, cols]))

        split = dm - 256
        nk = streamed(1, 0)[1] - streamed(1, 0)[0]
        for j in range(LEAD):
            v_ref[j, 0:nk] = partial_proj(1, j, 0, split)
        for j in range(LEAD):
            v_ref[LEAD + j, 0:nk] = partial_proj(1, j, split, dm)
        for j in range(LEAD):
            store_keys(j, complete(1, j, v_ref[j, 0:nk] + v_ref[LEAD + j, 0:nk]))
        for j in range(LEAD, pairs):
            store_keys(j, proj(1, j))
        for j in range(pairs):
            o_ref[q0:, j * pw:(j + 1) * pw] = proj(0, j)
            if j >= LAG:
                scores(j - LAG)
        for j in range(pairs):
            v = proj(2, j)
            if j < LAG:
                scores(pairs - LAG + j)
            v_ref[j] = v
            if j >= LAG:
                attend(j - LAG)
        y = out_proj(0, pairs // 2, slice(0, dm))
        for j in range(pairs - LAG, pairs):
            attend(j)
        for cols in (slice(0, split), slice(split, dm)):
            t = y[:, cols] + out_proj(pairs // 2, pairs, cols)
            if q0 == 0:
                mem_ref[:, cols] = t[:n_mem]
            ya_ref[rows_of(s, seg), cols] = t[n_mem - q0:]

    def a_layer(first_layer):
        n_loop = (n_seg - 2) // UNROLL

        def a_body(i, carry):
            for u in range(UNROLL):
                a_step(1 + i * UNROLL + u, first_layer)
            return carry

        a_step(0, first_layer)
        lax.fori_loop(0, n_loop, a_body, 0)
        for s in range(1 + n_loop * UNROLL, n_seg):
            a_step(s, first_layer)

    def b_fold_weights():
        def fold(which, product):
            out = {}
            for kt in range(dm // 128):
                gs = groups_of(kt)
                block = jnp.concatenate([sel_ref[which, kt, i] for i in range(len(gs))], axis=0)
                part = product(block, 128 * kt)
                for i, g in enumerate(gs):
                    t = part[i * grp:(i + 1) * grp]
                    out[g] = out[g] + t if g in out else t
            return out

        def store(ref, blocks):
            for i in range(0, len(blocks), 2):
                two = jnp.concatenate(blocks[i:i + 2], axis=0).astype(BF16)
                ref[i * bdh:(i + 2) * bdh, :] = _pack(two)

        def from_qkv(m):
            return lambda b, c: _mm_nt(b, bqkv_ref[:, m * dm + c:m * dm + c + 128])

        cp_bqkv.wait()
        cp_bwo.wait()
        wk, wv = fold(0, from_qkv(1)), fold(1, from_qkv(2))
        wk = {g: w * LOG2E for g, w in wk.items()}
        store(bkv_ref, [w[g] for g in range(n_grp) for w in (wk, wv)])
        wq = fold(0, from_qkv(0))
        store(bq_ref, [wq[g] * LOG2E for g in range(n_grp)])
        wo = fold(1, lambda b, c: _mm(b, bwo_ref[c:c + 128, :]))
        store(bo_ref, [wo[g] for g in range(n_grp)])

    def b_kv():
        n_chunk = seq // KV_CHUNK
        tokens = lambda i: slice(i * KV_CHUNK, (i + 1) * KV_CHUNK)

        def normalize(i):
            xn = xres_ref[tokens(i), :] + ya_ref[tokens(i), :]
            xres_ref[tokens(i), :] = xn
            ht_ref[:, tokens(i)] = _pack(_layernorm(xn).astype(BF16).T)

        work = [(i, g) for i in range(n_chunk) for g in range(n_grp)]
        ready = {}
        normalize(0)
        for n in range(len(work) + KV_LAG):
            if n < len(work):
                i, g = work[n]
                if g == 0 and i + 1 < n_chunk:
                    normalize(i + 1)
                t = _mm(_unpack(bkv_ref[g * grp:(g + 1) * grp, :]), _unpack(ht_ref[:, tokens(i)]))
                phi = _hedgehog(t[:grp])
                ready[n] = (t[grp:], phi.astype(BF16))
                z = phi if i == 0 else z_ref[g] + phi
                if i == n_chunk - 1:
                    z = jnp.broadcast_to(jnp.sum(z, axis=-1, keepdims=True), z.shape)
                z_ref[g] = z
            if n >= KV_LAG:
                i, g = work[n - KV_LAG]
                t = _mm_nt(*ready.pop(n - KV_LAG))
                if i > 0:
                    t = kv_ref[g] + t
                if i == n_chunk - 1:
                    t = jnp.where(((_iota(t.shape, 0) ^ _iota(t.shape, 1)) & 1) == 0, t, 0.0)
                kv_ref[g] = t

    n_chunk = seq // CHUNK
    tokens = lambda i: slice(i * CHUNK, (i + 1) * CHUNK)

    def cp_out(i):
        return pltpu.make_async_copy(res_ref.at[tokens(i)], out_hbm.at[tokens(i)], sem_out.at[i])

    def b_out(last_layer):
        zero = zero_ref[0]
        half = n_grp // 2
        n_sub = CHUNK // SUB
        work = [(i, gg) for i in range(n_chunk) for gg in range(half)]
        ready = {}

        def staged(i, r0, n):
            return pl.ds(pl.multiple_of(zero + seq + (i % 2) * (CHUNK // 2) + r0, 8), n)

        def features(g, p):
            phi = _hedgehog(p)
            t = phi * jnp.concatenate([z_ref[g]] * (CHUNK // 128), axis=1)
            den = functools.reduce(jnp.add, [t[r:r + 8] for r in range(0, 2 * grp, 8)])
            return phi.astype(BF16), _recip(_pair_reduce(den, jnp.add) + DEN_EPS)

        finished = []

        def normalize():
            sl = finished.pop(0)
            hn_ref[sl, :] = _layernorm(xres_ref[sl, :])

        def finish(i, k):
            if len(finished) > LN_LAG:
                normalize()
            sl = slice(i * CHUNK + k * SUB, i * CHUNK + (k + 1) * SUB)
            o = _unpack(hn_ref[staged(i, k * SUB // 2, SUB // 2), :])
            xn = xres_ref[sl, :] + _mm(o, _unpack(bo_ref[...]))
            if last_layer:
                res_ref[sl, :] = xn.astype(BF16)
                if k == n_sub - 1:
                    cp_out(i).start()
            else:
                xres_ref[sl, :] = xn
                finished.append(sl)

        pending = []
        for n in range(len(work) + B_LAG):
            if n < len(work):
                i, gg = work[n]
                t = _mm(_unpack(bq_ref[gg * grp:(gg + 1) * grp, :]), _unpack(ht_ref[:, tokens(i)]))
                ready[n] = [features(2 * gg + k, t[k * grp:(k + 1) * grp]) for k in range(2)]
            while pending and pending[0][0] <= n:
                finish(*pending.pop(0)[1:])
            if n >= B_LAG:
                i, gg = work[n - B_LAG]
                for k, (phi, inv) in enumerate(ready.pop(n - B_LAG)):
                    g = 2 * gg + k
                    num = _mm(kv_ref[g], phi)
                    ot_ref[g * grp:(g + 1) * grp, :] = jnp.concatenate(
                        [num[r:r + 8] * inv for r in range(0, grp, 8)], axis=0)
                if gg == half - 1:
                    hn_ref[staged(i, 0, CHUNK // 2), :] = pltpu.bitcast(ot_ref[...].astype(BF16).T, F32)
                    pending += [(n + OUT_LAG + k * half // n_sub, i, k) for k in range(n_sub)]
        for _, i, k in pending:
            finish(i, k)
        while finished:
            normalize()

    a_layer(True)
    b_fold_weights()
    with jax.named_scope("L_b_kv"):
        b_kv()
    with jax.named_scope("L_b_out"):
        b_out(False)
    a_layer(False)
    with jax.named_scope("L_b_kv"):
        b_kv()
    with jax.named_scope("L_b_out"):
        b_out(True)
    for i in range(n_chunk):
        cp_out(i).wait()


@functools.partial(jax.jit, static_argnames=("A_seg_len",))
def pallas_interleave_layers__memory_aug_recurrent_mem_tr__linear_kernel_hedgehog__prompt_kernel(
    A_x: jax.Array,
    A_mem0: jax.Array,
    A_Wq: jax.Array,
    A_Wk: jax.Array,
    A_Wv: jax.Array,
    A_Wo: jax.Array,
    A_seg_len: int,
    B_x: jax.Array,
    B_wqkv: jax.Array,
    B_w_phi: jax.Array,
    B_wo: jax.Array,
):
    del B_x
    batch, seq, dm = A_x.shape
    _, heads, dh = A_Wq.shape
    n_mem = A_mem0.shape[1]
    seg = int(A_seg_len)
    n_seg = seq // seg
    rows = n_mem + seg
    pw = 2 * dh
    pairs = heads // 2
    bdh = dm // B_HEADS
    assert batch == 1 and seq % CHUNK == 0 and CHUNK % seg == 0 and seg % EARLY == 0
    assert n_mem % 8 == 0 and rows <= 48
    assert heads % 2 == 0 and pw == 3 * 128 and dm % 128 == 0 and (2 * bdh) % 8 == 0

    w_t = lambda w: jnp.transpose(w, (1, 2, 0)).reshape(heads * dh, dm)
    hbm = pl.BlockSpec(memory_space=pl.ANY)

    out = pl.pallas_call(
        functools.partial(_kernel, seg=seg, heads=heads, dh=dh),
        out_shape=jax.ShapeDtypeStruct((seq, dm), A_x.dtype),
        in_specs=[hbm] * 9,
        out_specs=hbm,
        scratch_shapes=[
            pltpu.VMEM((n_mem, dm), BF16),
            pltpu.VMEM((bdh, bdh, B_HEADS), BF16),
            pltpu.VMEM((RING, n_seg // pairs, seg // EARLY, EARLY, dm), BF16),
            pltpu.VMEM((n_seg, EARLY, dm), BF16),
            pltpu.VMEM((n_seg * EARLY, dm), F32),
            pltpu.VMEM((seq, dm), F32),
            pltpu.VMEM((seq + CHUNK, dm), F32),
            pltpu.VMEM((seq, dm), F32),
            pltpu.VMEM((pairs, dm // 2, 3 * pw), jnp.uint32),
            pltpu.VMEM((pairs * dh, dm), jnp.uint32),
            pltpu.VMEM((RING, 4, pw, dm), BF16),
            pltpu.VMEM((pairs, n_seg * EARLY, 2 * pw), F32),
            pltpu.VMEM((EARLY_Q, n_seg * EARLY, pw), F32),
            pltpu.VMEM((dm, 3 * dm), BF16),
            pltpu.VMEM((dm, dm), BF16),
            pltpu.VMEM((2, dm // 128, 127 // (2 * bdh) + 2, 2 * bdh, 128), F32),
            pltpu.VMEM((dm // 2, dm), jnp.uint32),
            pltpu.VMEM((dm, dm), jnp.uint32),
            pltpu.VMEM((dm // 2, dm), jnp.uint32),
            pltpu.VMEM((rows, heads * dh), F32),
            pltpu.VMEM((n_mem, dm), F32),
            pltpu.VMEM((pairs, n_mem, 3 * pw), F32),
            pltpu.VMEM((pairs, dh, 128), jnp.uint32),
            pltpu.VMEM((pairs, rows, pw), F32),
            pltpu.VMEM((pairs, rows, 128), F32),
            pltpu.VMEM((dm // 2, seq), jnp.uint32),
            pltpu.VMEM((dm, CHUNK), F32),
            pltpu.VMEM((B_HEADS // 2, 2 * bdh, 4 * bdh), F32),
            pltpu.VMEM((B_HEADS // 2, 4 * bdh, 128), F32),
            pltpu.VMEM((seq, dm), BF16),
            pltpu.SMEM((1,), jnp.int32),
            pltpu.SemaphoreType.DMA((3,)),
            pltpu.SemaphoreType.DMA((2,)),
            pltpu.SemaphoreType.DMA((RING, 5)),
            pltpu.SemaphoreType.DMA((seq // CHUNK,)),
        ],
        compiler_params=pltpu.CompilerParams(vmem_limit_bytes=120 * 1024 * 1024),
    )(
        A_x.reshape(n_seg, seg // EARLY, EARLY, dm),
        A_mem0.reshape(n_mem, dm),
        w_t(A_Wq), w_t(A_Wk), w_t(A_Wv),
        A_Wo.reshape(heads * dh, dm),
        B_wqkv,
        jnp.transpose(B_w_phi, (1, 2, 0)),
        B_wo,
    )
    return out.reshape(batch, seq, dm)
```

```python
import functools

import jax
import jax.numpy as jnp
from jax import lax
import jax.experimental.pallas as pl
import jax.experimental.pallas.tpu as pltpu

F32 = jnp.float32
BF16 = jnp.bfloat16

B_HEADS = 32
LN_EPS = 1e-05
DEN_EPS = 1e-06
MASK_FILL = -1000000000.0
LOG2E = 1.4426950408889634

LAG = 4
EARLY = 8
EARLY_Q = 2
UNROLL = (2, 3)
LEAD = 2
RING = 4
CHUNK = 256
B_LAG = 3
KV_CHUNK = 128
KV_LAG = 3
SUB = 64
OUT_LAG = 4
LN_LAG = 1

_NN = (((1,), (0,)), ((), ()))
_NT = (((1,), (1,)), ((), ()))


def _mm(a, b):
    return lax.dot_general(a, b, _NN, preferred_element_type=F32)


def _mm_nt(a, b):
    return lax.dot_general(a, b, _NT, preferred_element_type=F32)


def _pack(w):
    return pltpu.bitcast(w, jnp.uint32)


def _unpack(w):
    return pltpu.bitcast(w, BF16)


def _iota(shape, dim):
    return lax.broadcasted_iota(jnp.int32, shape, dim)


def _recip(x):
    r = pl.reciprocal(x, approx=True)
    return r * (2.0 - x * r)


def _layernorm(x):
    m = jnp.mean(x, axis=-1, keepdims=True)
    xc = x - m
    v = jnp.mean(xc * xc, axis=-1, keepdims=True)
    return xc * lax.rsqrt(v + LN_EPS)


def _pair_reduce(v, op):
    v = op(v, pltpu.roll(v, 4, 0))
    return op(v, pltpu.roll(v, 2, 0))


def _hedgehog(p):
    rows = [p[i:i + 8] for i in range(0, p.shape[0], 8)]
    hi = _pair_reduce(functools.reduce(jnp.maximum, rows), jnp.maximum)
    lo = _pair_reduce(functools.reduce(jnp.minimum, rows), jnp.minimum)
    ep = [jnp.exp2(r - hi) for r in rows]
    en = [jnp.exp2(lo - r) for r in rows]
    rp = _recip(_pair_reduce(functools.reduce(jnp.add, ep), jnp.add))
    rn = _recip(_pair_reduce(functools.reduce(jnp.add, en), jnp.add))
    return jnp.concatenate([e * rp for e in ep] + [e * rn for e in en], axis=0)


def _kernel(
    x_hbm, mem0_hbm, wq_hbm, wk_hbm, wv_hbm, wo_hbm, bqkv_hbm, wphi_hbm, bwo_hbm,
    out_hbm,
    mem0_ref, wphi_ref,
    xin_ref, xe_ref, he_ref, xres_ref, hn_ref, ya_ref, wqkv_ref, wo_in_ref, wo_ref, stage_ref, early_ref, early_q_ref,
    bqkv_ref, bwo_ref, sel_ref, bq_ref, bkv_ref, bo_ref,
    o_ref, mem_ref, qkv0_ref, kt_ref, v_ref, p_ref, ht_ref, ot_ref, kv_ref, z_ref, res_ref, zero_ref,
    sem_x, sem_b, sem_w, sem_wo, sem_out,
    *, seg, heads, dh,
):
    seq, dm = out_hbm.shape
    n_mem = mem0_ref.shape[0]
    n_seg = seq // seg
    rows = n_mem + seg
    pairs = heads // 2
    pw = 2 * dh
    off = -(-rows // 16) * 16
    scale = dh ** (-0.5)
    bdh = dm // B_HEADS
    grp = 2 * bdh
    n_grp = B_HEADS // 2

    cp_xe = pltpu.make_async_copy(x_hbm.at[:, seg // EARLY - 1], xe_ref, sem_x.at[0])
    cp_mem0 = pltpu.make_async_copy(mem0_hbm, mem0_ref, sem_x.at[1])
    cp_wphi = pltpu.make_async_copy(wphi_hbm, wphi_ref, sem_x.at[2])
    cp_bqkv = pltpu.make_async_copy(bqkv_hbm, bqkv_ref, sem_b.at[0])
    cp_bwo = pltpu.make_async_copy(bwo_hbm, bwo_ref, sem_b.at[1])

    def rows_of(j, n):
        return pl.ds(j * n if isinstance(j, int) else pl.multiple_of(j * n, n), n)

    def cp_w(m, j):
        slot = j & (RING - 1)
        if m == 3:
            n = n_seg // pairs
            return pltpu.make_async_copy(x_hbm.at[pl.ds(j * n, n)], xin_ref.at[slot], sem_w.at[slot, m])
        src = (wq_hbm, wk_hbm, wv_hbm)[m]
        return pltpu.make_async_copy(src.at[rows_of(j, pw)], stage_ref.at[slot, m], sem_w.at[slot, m])

    def groups_of(kt):
        return range(128 * kt // grp, (128 * kt + 127) // grp + 1)

    def build_selectors():
        eh_r = _iota((B_HEADS, dm), 0)
        eh_c = _iota((B_HEADS, dm), 1)
        phi_f = None
        for d in range(bdh):
            eh = jnp.where(eh_c == eh_r * bdh + d, 1.0, 0.0).astype(BF16)
            t = _mm(wphi_ref[d], eh)
            phi_f = t if phi_f is None else phi_f + t
        pick = jnp.where((_iota((grp, bdh), 0) >> 1) == _iota((grp, bdh), 1), 1.0, 0.0)
        phi_rows = _mm(pick, phi_f.astype(BF16))
        r = _iota((grp, 128), 0)
        for kt in range(dm // 128):
            c = _iota((grp, 128), 1) + 128 * kt
            for i, g in enumerate(groups_of(kt)):
                c0 = (2 * g + (r & 1)) * bdh
                sel_ref[kt, i] = jnp.where(
                    (c >= c0) & (c < c0 + bdh), phi_rows[:, 128 * kt:128 * kt + 128], 0.0)

    skew, ahead = EARLY_Q, RING - 1
    cp_kv = lambda j: [cp_w(m, j) for m in (1, 2)]
    cp_rest = lambda i: [cp_w(m, i) for m in (0, 3)]
    cp_wo = lambda j: pltpu.make_async_copy(
        wo_hbm.at[rows_of(j, pw)], wo_in_ref.at[rows_of(j, pw)], sem_wo)

    def when(cond, copies, method):
        @pl.when(cond)
        def _():
            for cp in copies():
                getattr(cp, method)()

    def unpack_rest(i):
        real = i >= 0
        n = seq // pairs
        x = xin_ref[i & (RING - 1)].astype(F32).reshape(n, dm)
        slot = jnp.where(real, i, i + skew) & (RING - 1)
        i = jnp.maximum(i, 0)
        xres_ref[rows_of(i, n), :] = x
        hn_ref[rows_of(i, n), :] = _pack(_layernorm(x))
        wqkv_ref[i, :, 0:pw] = _pack(stage_ref[slot, jnp.where(real, 0, 1)].T)

    def swap_rest(i):
        when(i >= 0, lambda: cp_rest(i), "wait")
        when((i + ahead >= 0) & (i + ahead < pairs), lambda: cp_rest(i + ahead), "start")

    def load_body(j, carry):
        for cp in cp_kv(j):
            cp.wait()
        when(j + ahead < pairs, lambda: cp_kv(j + ahead), "start")
        swap_rest(j - skew)
        cp_wo(j).start()
        for m in (1, 2):
            w = stage_ref[j & (RING - 1), m]
            early_ref[j, :, (m - 1) * pw:m * pw] = _mm_nt(he_ref[...], w)
            wqkv_ref[j, :, m * pw:(m + 1) * pw] = _pack(w.T)
        unpack_rest(j - skew)
        return carry

    def load_tail(t, carry):
        swap_rest(pairs - skew + t)
        early_q_ref[t] = _mm(he_ref[...], _unpack(wqkv_ref[t, :, 0:pw]))
        unpack_rest(pairs - skew + t)
        return carry

    zero_ref[0] = 0
    for cp in [cp_wphi, cp_mem0, cp_xe] + cp_kv(0):
        cp.start()
    for i in range(-skew, 0):
        xin_ref[i & (RING - 1)] = jnp.zeros(xin_ref.shape[1:], BF16)
    cp_wphi.wait()
    build_selectors()
    cp_xe.wait()
    for j in range(1, ahead):
        for cp in cp_kv(j) + (cp_rest(j - skew) if j >= skew else []):
            cp.start()
    he_ref[...] = _layernorm(xe_ref[...].astype(F32).reshape(n_seg * EARLY, dm))
    lax.fori_loop(0, pairs, load_body, 0)
    lax.fori_loop(0, skew, load_tail, 0)
    cp_mem0.wait()

    cut = dh % 128

    def stack(a, b):
        gap = jnp.zeros((off - rows, a.shape[1]), F32)
        tail = jnp.zeros((128 - off - rows, a.shape[1]), F32)
        return jnp.concatenate([a, gap, b, tail], axis=0).astype(BF16)

    def store_keys(j, t):
        outer = _pack(stack(t[:, 0:128], t[:, 256:384]).T)
        inner = _pack(stack(t[:, 128:256], t[:, 128:256]).T)
        low = _iota((64, 128), 1) < off
        kt_ref[j, 0:64] = jnp.where(low, outer, 0)
        kt_ref[j, 64:64 + cut // 2] = jnp.where(low[:cut // 2], inner[:cut // 2], 0)
        kt_ref[j, 64 + cut // 2:128] = jnp.where(low[cut // 2:], 0, inner[cut // 2:])
        kt_ref[j, 128:192] = jnp.where(low, 0, outer)

    def load_values(j):
        t = v_ref[j]
        low = _iota((rows, 128), 1) < cut
        none = jnp.zeros((rows, 128), F32)
        first = jnp.concatenate([t[:, 0:128], jnp.where(low, t[:, 128:256], 0.0), none], axis=1)
        second = jnp.concatenate([none, jnp.where(low, 0.0, t[:, 128:256]), t[:, 256:384]], axis=1)
        return stack(first, second)

    def a_step(s, first_layer):
        first_step = isinstance(s, int) and s == 0
        q0 = n_mem if isinstance(s, int) and s == n_seg - 1 else 0
        mem = mem0_ref[...].astype(F32) if first_step else mem_ref[...]
        h = jnp.concatenate([mem, pltpu.bitcast(hn_ref[rows_of(s, seg), :], F32)], axis=0)
        qi = _iota((rows - q0, 128), 0) + q0
        ki = _iota((rows - q0, 128), 1)
        in_a = ki < rows
        in_b = (ki >= off) & (ki < off + rows)
        see_a = in_a & ((qi < n_mem) | (qi >= ki))
        see_b = in_b & ((qi < n_mem) | (qi >= ki - off))
        fill_a = jnp.where(in_a, MASK_FILL, -jnp.inf)
        fill_b = jnp.where(in_b, MASK_FILL, -jnp.inf)

        def streamed(m, j):
            if first_layer:
                return (q0 if m == 0 else 0), rows - (EARLY if m > 0 or j < EARLY_Q else 0)
            return (n_mem if first_step else q0 if m == 0 else 0), rows

        def partial_proj(m, j, d0, d1):
            r0, r1 = streamed(m, j)
            return _mm(h[r0:r1, d0:d1], _unpack(wqkv_ref[j, d0 // 2:d1 // 2, m * pw:(m + 1) * pw]))

        def complete(m, j, t):
            cols = slice(m * pw, (m + 1) * pw)
            if first_step and first_layer:
                qkv0_ref[j, :, cols] = t[:n_mem]
            elif first_step:
                t = jnp.concatenate([qkv0_ref[j, :, cols], t], axis=0)
            if streamed(m, j)[1] < rows:
                sl = rows_of(s, EARLY)
                done = early_ref[j, sl, (m - 1) * pw:m * pw] if m > 0 else early_q_ref[j, sl, :]
                t = jnp.concatenate([t, done], axis=0)
            return t

        def proj(m, j):
            return complete(m, j, partial_proj(m, j, 0, dm))

        def scores(j):
            sc = _mm(o_ref[q0:, j * pw:(j + 1) * pw], _unpack(kt_ref[j])) * scale
            sa = jnp.where(see_a, sc, fill_a)
            sb = jnp.where(see_b, sc, fill_b)
            ea = jnp.exp(sa - jnp.max(sa, axis=-1, keepdims=True))
            eb = jnp.exp(sb - jnp.max(sb, axis=-1, keepdims=True))
            ra = _recip(jnp.sum(ea, axis=-1, keepdims=True))
            rb = _recip(jnp.sum(eb, axis=-1, keepdims=True))
            p_ref[j, q0:] = ea * ra + eb * rb

        def attend(j):
            o_ref[q0:, j * pw:(j + 1) * pw] = _mm(p_ref[j, q0:], load_values(j))

        def out_proj(j0, j1, cols):
            return _mm(o_ref[q0:, j0 * pw:j1 * pw], _unpack(wo_ref[j0 * dh:j1 * dh, cols]))

        split = dm - 256
        nk = streamed(1, 0)[1] - streamed(1, 0)[0]
        for j in range(LEAD):
            v_ref[j, 0:nk] = partial_proj(1, j, 0, split)
        for j in range(LEAD):
            v_ref[LEAD + j, 0:nk] = partial_proj(1, j, split, dm)
        for j in range(LEAD):
            store_keys(j, complete(1, j, v_ref[j, 0:nk] + v_ref[LEAD + j, 0:nk]))
        for j in range(LEAD, pairs):
            store_keys(j, proj(1, j))
        for j in range(pairs):
            o_ref[q0:, j * pw:(j + 1) * pw] = proj(0, j)
            if j >= LAG:
                scores(j - LAG)
        for j in range(pairs):
            v = proj(2, j)
            if j < LAG:
                scores(pairs - LAG + j)
            v_ref[j] = v
            if j >= LAG:
                attend(j - LAG)
        y = out_proj(0, pairs // 2, slice(0, dm))
        for j in range(pairs - LAG, pairs):
            attend(j)
        for cols in (slice(0, split), slice(split, dm)):
            t = y[:, cols] + out_proj(pairs // 2, pairs, cols)
            if q0 == 0:
                mem_ref[:, cols] = t[:n_mem]
            ya_ref[rows_of(s, seg), cols] = t[n_mem - q0:]

    def a_layer(first_layer):
        unroll = UNROLL[0 if first_layer else 1]
        n_loop = (n_seg - 2) // unroll

        def a_body(i, carry):
            for u in range(unroll):
                a_step(1 + i * unroll + u, first_layer)
            return carry

        if first_layer:
            pltpu.make_async_copy(wo_hbm, wo_in_ref, sem_wo).wait()
            wo_ref[...] = _pack(wo_in_ref[...])
        a_step(0, first_layer)
        if first_layer:
            cp_bqkv.start()
            cp_bwo.start()
        lax.fori_loop(0, n_loop, a_body, 0)
        if first_layer:
            cp_bqkv.wait()
            cp_bwo.wait()
            b_fold_weights()
        for s in range(1 + n_loop * unroll, n_seg):
            a_step(s, first_layer)

    def b_fold_weights():
        def fold(m):
            out = {}
            for kt in range(dm // 128):
                gs = groups_of(kt)
                block = jnp.concatenate([sel_ref[kt, i] for i in range(len(gs))], axis=0)
                part = _mm_nt(block, bqkv_ref[:, m * dm + 128 * kt:m * dm + 128 * kt + 128])
                for i, g in enumerate(gs):
                    t = part[i * grp:(i + 1) * grp]
                    out[g] = out[g] + t if g in out else t
            return [out[g] * LOG2E for g in range(n_grp)]

        def store(ref, blocks):
            for i in range(0, len(blocks), 2):
                two = jnp.concatenate(blocks[i:i + 2], axis=0).astype(BF16)
                ref[i * bdh:(i + 2) * bdh, :] = _pack(two)

        wk = fold(1)
        wv = bqkv_ref[:, 2 * dm:3 * dm].T.astype(F32)
        store(bkv_ref, [w for g in range(n_grp) for w in (wk[g], wv[g * grp:(g + 1) * grp])])
        store(bq_ref, fold(0))
        bo_ref[...] = _pack(bwo_ref[...])

    def b_kv():
        n_chunk = seq // KV_CHUNK
        tokens = lambda i: slice(i * KV_CHUNK, (i + 1) * KV_CHUNK)

        def normalize(i):
            xn = xres_ref[tokens(i), :] + ya_ref[tokens(i), :]
            xres_ref[tokens(i), :] = xn
            ht_ref[:, tokens(i)] = _pack(_layernorm(xn).astype(BF16).T)

        work = [(i, g) for i in range(n_chunk) for g in range(n_grp)]
        ready = {}
        normalize(0)
        for n in range(len(work) + KV_LAG):
            if n < len(work):
                i, g = work[n]
                if g == 0 and i + 1 < n_chunk:
                    normalize(i + 1)
                t = _mm(_unpack(bkv_ref[g * grp:(g + 1) * grp, :]), _unpack(ht_ref[:, tokens(i)]))
                phi = _hedgehog(t[:grp])
                ready[n] = (t[grp:], phi.astype(BF16))
                z = phi if i == 0 else z_ref[g] + phi
                if i == n_chunk - 1:
                    z = jnp.broadcast_to(jnp.sum(z, axis=-1, keepdims=True), z.shape)
                z_ref[g] = z
            if n >= KV_LAG:
                i, g = work[n - KV_LAG]
                t = _mm_nt(*ready.pop(n - KV_LAG))
                if i > 0:
                    t = kv_ref[g] + t
                if i == n_chunk - 1:
                    second = (_iota(t.shape, 1) & 1) == 1
                    t = jnp.where((_iota(t.shape, 0) >= bdh) == second, t, 0.0)
                kv_ref[g] = t

    n_chunk = seq // CHUNK
    tokens = lambda i: slice(i * CHUNK, (i + 1) * CHUNK)

    def cp_out(i):
        return pltpu.make_async_copy(res_ref.at[tokens(i)], out_hbm.at[tokens(i)], sem_out.at[i])

    def b_out(last_layer):
        zero = zero_ref[0]
        half = n_grp // 2
        n_sub = CHUNK // SUB
        work = [(i, gg) for i in range(n_chunk) for gg in range(half)]
        ready = {}

        def staged(i, r0, n):
            return pl.ds(pl.multiple_of(zero + seq + (i % 2) * (CHUNK // 2) + r0, 8), n)

        def features(g, p):
            phi = _hedgehog(p)
            t = phi * jnp.concatenate([z_ref[g]] * (CHUNK // 128), axis=1)
            den = functools.reduce(jnp.add, [t[r:r + 8] for r in range(0, 2 * grp, 8)])
            inv = _recip(_pair_reduce(den, jnp.add) + DEN_EPS)
            other = pltpu.roll(inv, 1, 0)
            r = _iota(inv.shape, 0)
            return phi.astype(BF16), jnp.concatenate(
                [jnp.where((r + r0 >= bdh) == ((r & 1) == 1), inv, other) for r0 in range(0, grp, 8)],
                axis=0)

        finished = []

        def normalize():
            sl = finished.pop(0)
            hn_ref[sl, :] = _pack(_layernorm(xres_ref[sl, :]))

        def finish(i, k):
            if len(finished) > LN_LAG:
                normalize()
            sl = slice(i * CHUNK + k * SUB, i * CHUNK + (k + 1) * SUB)
            o = _unpack(hn_ref[staged(i, k * SUB // 2, SUB // 2), :])
            xn = xres_ref[sl, :] + _mm(o, _unpack(bo_ref[...]))
            if last_layer:
                res_ref[sl, :] = xn.astype(BF16)
                if k == n_sub - 1:
                    cp_out(i).start()
            else:
                xres_ref[sl, :] = xn
                finished.append(sl)

        pending = []
        for n in range(len(work) + B_LAG):
            if n < len(work):
                i, gg = work[n]
                t = _mm(_unpack(bq_ref[gg * grp:(gg + 1) * grp, :]), _unpack(ht_ref[:, tokens(i)]))
                ready[n] = [features(2 * gg + k, t[k * grp:(k + 1) * grp]) for k in range(2)]
            while pending and pending[0][0] <= n:
                finish(*pending.pop(0)[1:])
            if n >= B_LAG:
                i, gg = work[n - B_LAG]
                for k, (phi, inv) in enumerate(ready.pop(n - B_LAG)):
                    g = 2 * gg + k
                    ot_ref[g * grp:(g + 1) * grp, :] = _mm(kv_ref[g], phi) * inv
                if gg == half - 1:
                    hn_ref[staged(i, 0, CHUNK // 2), :] = _pack(ot_ref[...].astype(BF16).T)
                    pending += [(n + OUT_LAG + k * half // n_sub, i, k) for k in range(n_sub)]
        for _, i, k in pending:
            finish(i, k)
        while finished:
            normalize()

    a_layer(True)
    with jax.named_scope("L_b_kv"):
        b_kv()
    with jax.named_scope("L_b_out"):
        b_out(False)
    a_layer(False)
    with jax.named_scope("L_b_kv"):
        b_kv()
    with jax.named_scope("L_b_out"):
        b_out(True)
    for i in range(n_chunk):
        cp_out(i).wait()


@functools.partial(jax.jit, static_argnames=("A_seg_len",))
def pallas_interleave_layers__memory_aug_recurrent_mem_tr__linear_kernel_hedgehog__prompt_kernel(
    A_x: jax.Array,
    A_mem0: jax.Array,
    A_Wq: jax.Array,
    A_Wk: jax.Array,
    A_Wv: jax.Array,
    A_Wo: jax.Array,
    A_seg_len: int,
    B_x: jax.Array,
    B_wqkv: jax.Array,
    B_w_phi: jax.Array,
    B_wo: jax.Array,
):
    del B_x
    batch, seq, dm = A_x.shape
    _, heads, dh = A_Wq.shape
    n_mem = A_mem0.shape[1]
    seg = int(A_seg_len)
    n_seg = seq // seg
    rows = n_mem + seg
    pw = 2 * dh
    pairs = heads // 2
    bdh = dm // B_HEADS
    assert batch == 1 and seq % CHUNK == 0 and CHUNK % seg == 0 and seg % EARLY == 0
    assert n_mem % 8 == 0 and rows <= 48
    assert heads % 2 == 0 and pw == 3 * 128 and dm % 128 == 0 and (2 * bdh) % 8 == 0

    w_t = lambda w: jnp.transpose(w, (1, 2, 0)).reshape(heads * dh, dm)
    hbm = pl.BlockSpec(memory_space=pl.ANY)

    out = pl.pallas_call(
        functools.partial(_kernel, seg=seg, heads=heads, dh=dh),
        out_shape=jax.ShapeDtypeStruct((seq, dm), A_x.dtype),
        in_specs=[hbm] * 9,
        out_specs=hbm,
        scratch_shapes=[
            pltpu.VMEM((n_mem, dm), BF16),
            pltpu.VMEM((bdh, bdh, B_HEADS), BF16),
            pltpu.VMEM((RING, n_seg // pairs, seg // EARLY, EARLY, dm), BF16),
            pltpu.VMEM((n_seg, EARLY, dm), BF16),
            pltpu.VMEM((n_seg * EARLY, dm), F32),
            pltpu.VMEM((seq, dm), F32),
            pltpu.VMEM((seq + CHUNK, dm), jnp.uint32),
            pltpu.VMEM((seq, dm), F32),
            pltpu.VMEM((pairs, dm // 2, 3 * pw), jnp.uint32),
            pltpu.VMEM((heads * dh, dm), BF16),
            pltpu.VMEM((pairs * dh, dm), jnp.uint32),
            pltpu.VMEM((RING, 3, pw, dm), BF16),
            pltpu.VMEM((pairs, n_seg * EARLY, 2 * pw), F32),
            pltpu.VMEM((EARLY_Q, n_seg * EARLY, pw), F32),
            pltpu.VMEM((dm, 3 * dm), BF16),
            pltpu.VMEM((dm, dm), BF16),
            pltpu.VMEM((dm // 128, 127 // (2 * bdh) + 2, 2 * bdh, 128), F32),
            pltpu.VMEM((dm // 2, dm), jnp.uint32),
            pltpu.VMEM((dm, dm), jnp.uint32),
            pltpu.VMEM((dm // 2, dm), jnp.uint32),
            pltpu.VMEM((rows, heads * dh), F32),
            pltpu.VMEM((n_mem, dm), F32),
            pltpu.VMEM((pairs, n_mem, 3 * pw), F32),
            pltpu.VMEM((pairs, dh, 128), jnp.uint32),
            pltpu.VMEM((pairs, rows, pw), F32),
            pltpu.VMEM((pairs, rows, 128), F32),
            pltpu.VMEM((dm // 2, seq), jnp.uint32),
            pltpu.VMEM((dm, CHUNK), F32),
            pltpu.VMEM((B_HEADS // 2, 2 * bdh, 4 * bdh), F32),
            pltpu.VMEM((B_HEADS // 2, 4 * bdh, 128), F32),
            pltpu.VMEM((seq, dm), BF16),
            pltpu.SMEM((1,), jnp.int32),
            pltpu.SemaphoreType.DMA((3,)),
            pltpu.SemaphoreType.DMA((2,)),
            pltpu.SemaphoreType.DMA((RING, 4)),
            pltpu.SemaphoreType.DMA,
            pltpu.SemaphoreType.DMA((seq // CHUNK,)),
        ],
        compiler_params=pltpu.CompilerParams(vmem_limit_bytes=120 * 1024 * 1024),
    )(
        A_x.reshape(n_seg, seg // EARLY, EARLY, dm),
        A_mem0.reshape(n_mem, dm),
        w_t(A_Wq), w_t(A_Wk), w_t(A_Wv),
        A_Wo.reshape(heads * dh, dm),
        B_wqkv,
        jnp.transpose(B_w_phi, (1, 2, 0)),
        B_wo,
    )
    return out.reshape(batch, seq, dm)
```

```python
import functools
import itertools

import jax
import jax.numpy as jnp
from jax import lax
import jax.experimental.pallas as pl
import jax.experimental.pallas.tpu as pltpu

F32 = jnp.float32
BF16 = jnp.bfloat16
U32 = jnp.uint32

B_HEADS = 32
LN_EPS = 1e-05
DEN_EPS = 1e-06
MASK_FILL = -1000000000.0
LOG2E = 1.4426950408889634

LAMBDA = (-1.75, -0.5625, 0.0, 0.5625, 1.75)
NB = len(LAMBDA)
UNROLL = 3
RING = 3
CHUNK = 256
B_LAG = 3
KV_CHUNK = 128
KV_LAG = 3
SUB = 64
OUT_LAG = 4
LN_LAG = 1

_NN = (((1,), (0,)), ((), ()))
_NT = (((1,), (1,)), ((), ()))


def _mm(a, b):
    return lax.dot_general(a, b, _NN, preferred_element_type=F32)


def _mm_nt(a, b):
    return lax.dot_general(a, b, _NT, preferred_element_type=F32)


def _pack(w):
    return pltpu.bitcast(w, jnp.uint32)


def _unpack(w):
    return pltpu.bitcast(w, BF16)


def _iota(shape, dim):
    return lax.broadcasted_iota(jnp.int32, shape, dim)


def _recip(x):
    r = pl.reciprocal(x, approx=True)
    return r * (2.0 - x * r)


def _layernorm(x):
    m = jnp.mean(x, axis=-1, keepdims=True)
    xc = x - m
    v = jnp.mean(xc * xc, axis=-1, keepdims=True)
    return xc * lax.rsqrt(v + LN_EPS)


def _pair_reduce(v, op):
    v = op(v, pltpu.roll(v, 4, 0))
    return op(v, pltpu.roll(v, 2, 0))


def _hedgehog(p):
    rows = [p[i:i + 8] for i in range(0, p.shape[0], 8)]
    hi = _pair_reduce(functools.reduce(jnp.maximum, rows), jnp.maximum)
    lo = _pair_reduce(functools.reduce(jnp.minimum, rows), jnp.minimum)
    ep = [jnp.exp2(r - hi) for r in rows]
    en = [jnp.exp2(lo - r) for r in rows]
    rp = _recip(_pair_reduce(functools.reduce(jnp.add, ep), jnp.add))
    rn = _recip(_pair_reduce(functools.reduce(jnp.add, en), jnp.add))
    return jnp.concatenate([e * rp for e in ep] + [e * rn for e in en], axis=0)


def _total(terms):
    return functools.reduce(jnp.add, terms)


_BLOCK_PAIRS = tuple(itertools.combinations(range(NB), 2))


def _kappa(i, j):
    return 1.0 / (LAMBDA[j] - LAMBDA[i])


def _others(j):
    return [i for i in range(NB) if i != j]


def _ahead_lhs(a, b):
    c = [b[j] + LAMBDA[j] * a[j] for j in range(NB)]
    return list(a) + [_kappa(i, j) * (c[i] + c[j]) for i, j in _BLOCK_PAIRS]


def _ahead_sums(products):
    y = list(products[:NB])
    for (i, j), t in zip(_BLOCK_PAIRS, products[NB:]):
        y[i], y[j] = y[i] + t, y[j] - t
    return y


def _step_lhs(x, i, j):
    t = x(j) if i == j else x(i) + x(j)
    return jnp.concatenate([t[:-16], t[-8:] + LAMBDA[j] * t[-16:-8]], axis=0)


def _step_rows(prod, ahead):
    y = list(ahead)
    for i, j in _BLOCK_PAIRS:
        g = _kappa(i, j) * (prod[i, j][-8:] + prod[j, i][-8:])
        y[i] = -g if y[i] is None else y[i] - g
        y[j] = g if y[j] is None else y[j] + g
    w = [_total([prod[i, j] for i in range(NB)]) for j in range(NB)]
    return [jnp.concatenate([w[j][:-8], y[j], w[j][-8:] - LAMBDA[j] * y[j]], axis=0)
            for j in range(NB)]


def _kernel(
    x_hbm, x_flat_hbm, mem0_hbm, wq_hbm, wk_hbm, wv_hbm, wo_hbm, bqkv_hbm, wphi_hbm, bwo_hbm,
    out_hbm,
    mem0_ref, al_ref, xres_ref, hn_ref, wqkv_ref, rqkv_ref, wo_ref, ro_ref, ahead_ref, early_ref,
    sel_ref, res_ref, zero_ref,
    sem_x, sem_b, sem_w, sem_last, sem_out,
    *, seg, heads, dh,
):
    seq, dm = out_hbm.shape
    n_mem = mem0_ref.shape[0]
    n_seg = seq // seg
    rows = n_mem + seg
    pairs = heads // 2
    pw = 2 * dh
    off = -(-rows // 16) * 16
    scale = dh ** (-0.5)
    bdh = dm // B_HEADS
    grp = 2 * bdh
    n_grp = B_HEADS // 2
    n_set = pairs // NB
    last = pairs - 1
    tile = lambda k, n=128: slice(k * n, (k + 1) * n)

    def rows_of(j, n):
        return pl.ds(j * n if isinstance(j, int) else pl.multiple_of(j * n, n), n)

    def groups_of(kt):
        return range(128 * kt // grp, (128 * kt + 127) // grp + 1)

    def store_ahead_lhs(a, b):
        split = lambda t: [t[:, tile(k)] for k in range(NB)]
        for r, t in enumerate(_ahead_lhs(split(a), split(b))):
            al_ref[r] = _pack(t.astype(BF16))

    def project_ahead(m, u, rhs, product):
        n = n_seg * 8 // 4
        for r0 in range(0, n_seg * 8, n):
            prods = [product(_unpack(al_ref[r, r0 // 2:(r0 + n) // 2]), w) for r, w in enumerate(rhs)]
            for j, y in enumerate(_ahead_sums(prods)):
                ahead_ref[m * (pairs - 1) + u * NB + j, r0:r0 + n] = y

    def load(wphi_ref, xe_ref, hb_ref, stage_ref, last_ref):
        cp_xe = pltpu.make_async_copy(x_hbm.at[:, pl.ds(seg // 8 - 2, 2)], xe_ref, sem_x.at[0])
        cp_x = pltpu.make_async_copy(x_flat_hbm, res_ref, sem_x.at[3])
        cp_mem0 = pltpu.make_async_copy(mem0_hbm, mem0_ref, sem_x.at[1])
        cp_wphi = pltpu.make_async_copy(wphi_hbm, wphi_ref, sem_x.at[2])

        weights = (wq_hbm, wk_hbm, wv_hbm, wo_hbm)

        def cp_set(m, u):
            return pltpu.make_async_copy(
                weights[m].at[rows_of(u, NB * pw)], stage_ref.at[u], sem_w.at[u])

        def cp_last(m):
            return pltpu.make_async_copy(weights[m].at[rows_of(last, pw)], last_ref.at[m], sem_last.at[m])

        def build_selectors():
            eh_r = _iota((B_HEADS, dm), 0)
            eh_c = _iota((B_HEADS, dm), 1)
            phi_f = None
            for d in range(bdh):
                eh = jnp.where(eh_c == eh_r * bdh + d, 1.0, 0.0).astype(BF16)
                t = _mm(wphi_ref[d], eh)
                phi_f = t if phi_f is None else phi_f + t
            pick = jnp.where((_iota((grp, bdh), 0) >> 1) == _iota((grp, bdh), 1), 1.0, 0.0)
            phi_rows = _mm(pick, phi_f.astype(BF16))
            r = _iota((grp, 128), 0)
            for kt in range(dm // 128):
                c = _iota((grp, 128), 1) + 128 * kt
                for i, g in enumerate(groups_of(kt)):
                    c0 = (2 * g + (r & 1)) * bdh
                    sel_ref[kt, i] = jnp.where(
                        (c >= c0) & (c < c0 + bdh), phi_rows[:, 128 * kt:128 * kt + 128], 0.0)

        def load_set(m, u):
            w = {(i, j): stage_ref[u, tile(j, pw), tile(i)] for i in range(NB) for j in range(NB)}
            f = {ij: t.astype(F32) for ij, t in w.items()}
            row = [_total([f[j, i] for i in range(NB)]).astype(BF16) for j in range(NB)]
            sym = [(f[i, j] + f[j, i]).astype(BF16) for i, j in _BLOCK_PAIRS]
            project_ahead(m, u, row + sym, _mm_nt)
            for j in range(NB):
                w[j, j] = (f[j, j] - _total([f[i, j] for i in _others(j)])).astype(BF16)
                rqkv_ref[m * n_set + u, j] = _pack(row[j].T)
                for i in range(NB):
                    wqkv_ref[m * pairs + u * NB + j, tile(i, 64)] = _pack(w[i, j].T)

        def load_out_set(u):
            w = {(i, j): stage_ref[u, tile(i, pw), tile(j)] for i in range(NB) for j in range(NB)}
            f = {ij: t.astype(F32) for ij, t in w.items()}
            for j in range(NB):
                ro_ref[j, tile(u, dh)] = _pack(_total([f[j, i] for i in range(NB)]).astype(BF16))
                w[j, j] = (f[j, j] - _total([f[i, j] for i in _others(j)])).astype(BF16)
                for i in range(NB):
                    wo_ref[tile(u * NB + i, dh), tile(j)] = _pack(w[i, j])

        zero_ref[0] = 0
        for cp in (cp_wphi, cp_mem0, cp_xe, cp_set(0, 0)):
            cp.start()
        cp_wphi.wait()
        build_selectors()
        cp_xe.wait()
        cp_set(0, 1).start()
        a, b = (_layernorm(xe_ref[:, k].astype(F32).reshape(n_seg * 8, dm)) for k in range(2))
        hb_ref[...] = _pack(b.astype(BF16))
        store_ahead_lhs(a, b)

        def load_body(r, carry):
            u = lax.rem(r, n_set)
            cp_set(0, u).wait()
            later = r + RING - 1
            for m in range(4):
                @pl.when((later >= m * n_set) & (later < (m + 1) * n_set))
                def _():
                    cp_set(m, later - m * n_set).start()

                @pl.when(r == 2 * m + 1)
                def _():
                    cp_last(m).start()

            @pl.when(r == 2)
            def _():
                cp_x.start()

            load_set(lax.div(r, n_set), u)
            return carry

        lax.fori_loop(0, 3 * n_set, load_body, 0)
        cp_set(3, n_set - 1).start()
        cp_x.wait()
        for m in range(4):
            cp_last(m).wait()
        wo_ref[tile(last, dh)] = _pack(last_ref[3])
        bounds = [seq * u // n_set // 128 * 128 for u in range(n_set + 1)]
        for u in range(n_set):
            cp_set(3, u).wait()
            early_ref[u] = _mm_nt(_unpack(hb_ref[...]), last_ref[u])
            wqkv_ref[u * pairs + last] = _pack(last_ref[u].T)
            load_out_set(u)
            x = res_ref[bounds[u]:bounds[u + 1]].astype(F32)
            xres_ref[bounds[u]:bounds[u + 1]] = x
            hn_ref[bounds[u]:bounds[u + 1]] = _pack(_layernorm(x))
        cp_mem0.wait()

    def layers(ya_ref, lhs_ref, o_ref, mem_ref, kt_ref, v_ref, p_ref,
               bqkv_ref, bwo_ref, bq_ref, bkv_ref, bo_ref, ht_ref, ot_ref, kv_ref, z_ref):
        cp_bqkv = pltpu.make_async_copy(bqkv_hbm, bqkv_ref, sem_b.at[0])
        cp_bwo = pltpu.make_async_copy(bwo_hbm, bwo_ref, sem_b.at[1])

        cut = dh % 128

        def stack(a, b):
            gap = jnp.zeros((off - rows, a.shape[1]), F32)
            tail = jnp.zeros((128 - off - rows, a.shape[1]), F32)
            return jnp.concatenate([a, gap, b, tail], axis=0).astype(BF16)

        def store_keys(j, t):
            outer = _pack(stack(t[:, 0:128], t[:, 256:384]).T)
            inner = _pack(stack(t[:, 128:256], t[:, 128:256]).T)
            low = _iota((64, 128), 1) < off
            kt_ref[j, 0:64] = jnp.where(low, outer, 0)
            kt_ref[j, 64:64 + cut // 2] = jnp.where(low[:cut // 2], inner[:cut // 2], 0)
            kt_ref[j, 64 + cut // 2:128] = jnp.where(low[cut // 2:], 0, inner[cut // 2:])
            kt_ref[j, 128:192] = jnp.where(low, 0, outer)

        def load_values(j):
            t = v_ref[j]
            low = _iota((rows, 128), 1) < cut
            none = jnp.zeros((rows, 128), F32)
            first = jnp.concatenate([t[:, 0:128], jnp.where(low, t[:, 128:256], 0.0), none], axis=1)
            second = jnp.concatenate([none, jnp.where(low, 0.0, t[:, 128:256]), t[:, 256:384]], axis=1)
            return stack(first, second)

        def a_step(s, first_layer):
            h = jnp.concatenate([mem_ref[...], pltpu.bitcast(hn_ref[rows_of(s, seg), :], F32)], axis=0)
            mine = rows_of(s, 8)
            qi = _iota((rows, 128), 0)
            ki = _iota((rows, 128), 1)
            in_a = ki < rows
            in_b = (ki >= off) & (ki < off + rows)
            see_a = in_a & ((qi < n_mem) | (qi >= ki))
            see_b = in_b & ((qi < n_mem) | (qi >= ki - off))
            fill_a = jnp.where(in_a, MASK_FILL, -jnp.inf)
            fill_b = jnp.where(in_b, MASK_FILL, -jnp.inf)
            blocks = sorted(itertools.product(range(NB), repeat=2), key=max)
            for i, j in blocks:
                lhs_ref[i, j] = _step_lhs(lambda k: h[:, tile(k)], i, j)

            def project(m, u):
                prod = {(i, j): _mm(lhs_ref[i, j], _unpack(wqkv_ref[m * pairs + u * NB + j, tile(i, 64)]))
                        for i, j in blocks}
                ahead = [ahead_ref[m * (pairs - 1) + u * NB + j, mine] for j in range(NB)]
                return zip(range(u * NB, (u + 1) * NB), _step_rows(prod, ahead))

            def project_last(m):
                w = _unpack(wqkv_ref[m * pairs + last])
                if first_layer:
                    return jnp.concatenate([_mm(h[:-8], w), early_ref[m, mine]], axis=0)
                return _mm(h, w)

            def scores(j):
                sc = _mm(o_ref[j], _unpack(kt_ref[j])) * scale
                sa = jnp.where(see_a, sc, fill_a)
                sb = jnp.where(see_b, sc, fill_b)
                ea = jnp.exp(sa - jnp.max(sa, axis=-1, keepdims=True))
                eb = jnp.exp(sb - jnp.max(sb, axis=-1, keepdims=True))
                ra = _recip(jnp.sum(ea, axis=-1, keepdims=True))
                rb = _recip(jnp.sum(eb, axis=-1, keepdims=True))
                p_ref[j] = ea * ra + eb * rb

            def attend(j):
                o = _mm(p_ref[j], load_values(j))
                o_ref[j] = o
                if j < last:
                    ahead_ref[j, mine] = o[-16:-8]
                    ahead_ref[last + j, mine] = o[-8:]

            def project_out(sets, order):
                side = lambda f: jnp.concatenate([f(u * NB) for u in sets], axis=1)
                return {(i, j): _mm(
                    _step_lhs(lambda k: side(lambda p: o_ref[p + k]), i, j),
                    _unpack(jnp.concatenate(
                        [wo_ref[tile(u * NB + i, dh), tile(j)] for u in sets], axis=0)))
                    for i, j in order}

            of_set = lambda u: range(u * NB, (u + 1) * NB)
            for u in range(n_set):
                for j, t in project(1, u):
                    store_keys(j, t)
            store_keys(last, project_last(1))
            o_ref[last] = project_last(0)
            for u in range(n_set):
                for j, t in project(0, u):
                    o_ref[j] = t
                for j in of_set(u - 1) if u else (last,):
                    scores(j)
            v_ref[last] = project_last(2)
            for u in range(n_set):
                for j, t in project(2, u):
                    v_ref[j] = t
                if u == 0:
                    for j in of_set(n_set - 1):
                        scores(j)
                for j in of_set(u - 1) if u else (last,):
                    attend(j)
            direct = _mm(o_ref[last], _unpack(wo_ref[tile(last, dh)]))
            by_column = [(i, j) for j in range(NB) for i in range(NB)]
            most = project_out(range(n_set - 1), by_column[:2 * NB])
            for j in of_set(n_set - 1):
                attend(j)
            most.update(project_out(range(n_set - 1), by_column[2 * NB:]))
            rest = project_out((n_set - 1,), by_column)
            prod = {ij: most[ij] + rest[ij] for ij in by_column}
            for j, t in enumerate(_step_rows(prod, [None] * NB)):
                t = t + direct[:, tile(j)]
                mem_ref[:, tile(j)] = t[:n_mem]
                ya_ref[s, :, :, tile(j)] = t[n_mem:].reshape(seg // 8, 8, 128)

        def a_start():
            group = lambda k: pltpu.bitcast(jnp.concatenate(
                [hn_ref[tile(s * (seg // 8) + k, 8)] for s in range(n_seg)], axis=0), F32)
            store_ahead_lhs(group(seg // 8 - 2), group(seg // 8 - 1))

            def ahead_body(r, carry):
                m, u = lax.div(r, n_set), lax.rem(r, n_set)
                block = lambda i, j: _unpack(wqkv_ref[m * pairs + u * NB + j, tile(i, 64)]).astype(F32)
                row = [_unpack(rqkv_ref[r, j]) for j in range(NB)]
                sym = [(block(i, j) + block(j, i)).astype(BF16) for i, j in _BLOCK_PAIRS]
                project_ahead(m, u, row + sym, _mm)
                return carry

            lax.fori_loop(0, 3 * n_set, ahead_body, 0)

        def a_finish():
            block = lambda i, j: _unpack(jnp.concatenate(
                [wo_ref[tile(u * NB + i, dh), tile(j)] for u in range(n_set)], axis=0)).astype(F32)
            rhs = [_unpack(ro_ref[j]) for j in range(NB)]
            rhs += [(block(i, j) + block(j, i)).astype(BF16) for i, j in _BLOCK_PAIRS]
            n = n_seg // 4
            for s0 in range(0, n_seg, n):
                side = lambda p: jnp.concatenate(
                    [ahead_ref[p + u * NB, s0 * 8:(s0 + n) * 8] for u in range(n_set)], axis=1)
                lhs = _ahead_lhs([side(k) for k in range(NB)], [side(last + k) for k in range(NB)])
                for j, y in enumerate(_ahead_sums([_mm(t, w) for t, w in zip(lhs, rhs)])):
                    y = y.reshape(n, 8, 128)
                    ya_ref[s0:s0 + n, seg // 8 - 2, :, tile(j)] += y
                    ya_ref[s0:s0 + n, seg // 8 - 1, :, tile(j)] -= LAMBDA[j] * y

        def a_layer(first_layer):
            n_loop = n_seg // UNROLL

            def a_body(i, carry):
                for k in range(UNROLL):
                    a_step(i * UNROLL + k, first_layer)
                return carry

            if first_layer:
                cp_bqkv.start()
                cp_bwo.start()
            else:
                a_start()
            mem_ref[...] = mem0_ref[...].astype(F32)
            lax.fori_loop(0, n_loop, a_body, 0)
            if first_layer:
                cp_bqkv.wait()
                cp_bwo.wait()
                b_fold_weights()
            for s in range(n_loop * UNROLL, n_seg):
                a_step(s, first_layer)
            a_finish()

        def b_fold_weights():
            def fold(m):
                out = {}
                for kt in range(dm // 128):
                    gs = groups_of(kt)
                    block = jnp.concatenate([sel_ref[kt, i] for i in range(len(gs))], axis=0)
                    part = _mm_nt(block, bqkv_ref[:, m * dm + 128 * kt:m * dm + 128 * kt + 128])
                    for i, g in enumerate(gs):
                        t = part[i * grp:(i + 1) * grp]
                        out[g] = out[g] + t if g in out else t
                return [out[g] * LOG2E for g in range(n_grp)]

            def store(ref, blocks):
                for i in range(0, len(blocks), 2):
                    two = jnp.concatenate(blocks[i:i + 2], axis=0).astype(BF16)
                    ref[i * bdh:(i + 2) * bdh, :] = _pack(two)

            wk = fold(1)
            wv = bqkv_ref[:, 2 * dm:3 * dm].T.astype(F32)
            store(bkv_ref, [w for g in range(n_grp) for w in (wk[g], wv[g * grp:(g + 1) * grp])])
            store(bq_ref, fold(0))
            bo_ref[...] = _pack(bwo_ref[...])

        def b_kv():
            n_chunk = seq // KV_CHUNK
            tokens = lambda i: slice(i * KV_CHUNK, (i + 1) * KV_CHUNK)

            def normalize(i):
                xn = xres_ref[tokens(i), :] + ya_ref[tile(i, KV_CHUNK // seg)].reshape(KV_CHUNK, dm)
                xres_ref[tokens(i), :] = xn
                ht_ref[:, tokens(i)] = _pack(_layernorm(xn).astype(BF16).T)

            work = [(i, g) for i in range(n_chunk) for g in range(n_grp)]
            ready = {}
            normalize(0)
            for n in range(len(work) + KV_LAG):
                if n < len(work):
                    i, g = work[n]
                    if g == 0 and i + 1 < n_chunk:
                        normalize(i + 1)
                    t = _mm(_unpack(bkv_ref[g * grp:(g + 1) * grp, :]), _unpack(ht_ref[:, tokens(i)]))
                    phi = _hedgehog(t[:grp])
                    ready[n] = (t[grp:], phi.astype(BF16))
                    z = phi if i == 0 else z_ref[g] + phi
                    if i == n_chunk - 1:
                        z = jnp.broadcast_to(jnp.sum(z, axis=-1, keepdims=True), z.shape)
                    z_ref[g] = z
                if n >= KV_LAG:
                    i, g = work[n - KV_LAG]
                    t = _mm_nt(*ready.pop(n - KV_LAG))
                    if i > 0:
                        t = kv_ref[g] + t
                    if i == n_chunk - 1:
                        second = (_iota(t.shape, 1) & 1) == 1
                        t = jnp.where((_iota(t.shape, 0) >= bdh) == second, t, 0.0)
                    kv_ref[g] = t

        n_chunk = seq // CHUNK
        tokens = lambda i: slice(i * CHUNK, (i + 1) * CHUNK)

        def cp_out(i):
            return pltpu.make_async_copy(res_ref.at[tokens(i)], out_hbm.at[tokens(i)], sem_out.at[i])

        def b_out(last_layer):
            zero = zero_ref[0]
            half = n_grp // 2
            n_sub = CHUNK // SUB
            work = [(i, gg) for i in range(n_chunk) for gg in range(half)]
            ready = {}

            def staged(i, r0, n):
                return pl.ds(pl.multiple_of(zero + seq + (i % 2) * (CHUNK // 2) + r0, 8), n)

            def features(g, p):
                phi = _hedgehog(p)
                t = phi * jnp.concatenate([z_ref[g]] * (CHUNK // 128), axis=1)
                den = functools.reduce(jnp.add, [t[r:r + 8] for r in range(0, 2 * grp, 8)])
                inv = _recip(_pair_reduce(den, jnp.add) + DEN_EPS)
                other = pltpu.roll(inv, 1, 0)
                r = _iota(inv.shape, 0)
                return phi.astype(BF16), jnp.concatenate(
                    [jnp.where((r + r0 >= bdh) == ((r & 1) == 1), inv, other) for r0 in range(0, grp, 8)],
                    axis=0)

            finished = []

            def normalize():
                sl = finished.pop(0)
                hn_ref[sl, :] = _pack(_layernorm(xres_ref[sl, :]))

            def finish(i, k):
                if len(finished) > LN_LAG:
                    normalize()
                sl = slice(i * CHUNK + k * SUB, i * CHUNK + (k + 1) * SUB)
                o = _unpack(hn_ref[staged(i, k * SUB // 2, SUB // 2), :])
                xn = xres_ref[sl, :] + _mm(o, _unpack(bo_ref[...]))
                if last_layer:
                    res_ref[sl, :] = xn.astype(BF16)
                    if k == n_sub - 1:
                        cp_out(i).start()
                else:
                    xres_ref[sl, :] = xn
                    finished.append(sl)

            pending = []
            for n in range(len(work) + B_LAG):
                if n < len(work):
                    i, gg = work[n]
                    t = _mm(_unpack(bq_ref[gg * grp:(gg + 1) * grp, :]), _unpack(ht_ref[:, tokens(i)]))
                    ready[n] = [features(2 * gg + k, t[k * grp:(k + 1) * grp]) for k in range(2)]
                while pending and pending[0][0] <= n:
                    finish(*pending.pop(0)[1:])
                if n >= B_LAG:
                    i, gg = work[n - B_LAG]
                    for k, (phi, inv) in enumerate(ready.pop(n - B_LAG)):
                        g = 2 * gg + k
                        ot_ref[g * grp:(g + 1) * grp, :] = _mm(kv_ref[g], phi) * inv
                    if gg == half - 1:
                        hn_ref[staged(i, 0, CHUNK // 2), :] = _pack(ot_ref[...].astype(BF16).T)
                        pending += [(n + OUT_LAG + k * half // n_sub, i, k) for k in range(n_sub)]
            for _, i, k in pending:
                finish(i, k)
            while finished:
                normalize()

        a_layer(True)
        with jax.named_scope("L_b_kv"):
            b_kv()
        with jax.named_scope("L_b_out"):
            b_out(False)
        a_layer(False)
        with jax.named_scope("L_b_kv"):
            b_kv()
        with jax.named_scope("L_b_out"):
            b_out(True)
        for i in range(n_chunk):
            cp_out(i).wait()

    pl.run_scoped(
        load,
        pltpu.VMEM((bdh, bdh, B_HEADS), BF16),
        pltpu.VMEM((n_seg, 2, 8, dm), BF16),
        pltpu.VMEM((n_seg * 4, dm), U32),
        pltpu.VMEM((RING, NB * pw, dm), BF16),
        pltpu.VMEM((4, pw, dm), BF16),
    )
    pl.run_scoped(
        layers,
        pltpu.VMEM((n_seg, seg // 8, 8, dm), F32),
        pltpu.VMEM((NB, NB, rows - 8, 128), F32),
        pltpu.VMEM((pairs, rows, pw), F32),
        pltpu.VMEM((n_mem, dm), F32),
        pltpu.VMEM((pairs, dh, 128), U32),
        pltpu.VMEM((pairs, rows, pw), F32),
        pltpu.VMEM((pairs, rows, 128), F32),
        pltpu.VMEM((dm, 3 * dm), BF16),
        pltpu.VMEM((dm, dm), BF16),
        pltpu.VMEM((dm // 2, dm), U32),
        pltpu.VMEM((dm, dm), U32),
        pltpu.VMEM((dm // 2, dm), U32),
        pltpu.VMEM((dm // 2, seq), U32),
        pltpu.VMEM((dm, CHUNK), F32),
        pltpu.VMEM((n_grp, grp, 2 * grp), F32),
        pltpu.VMEM((n_grp, 2 * grp, 128), F32),
    )


@functools.partial(jax.jit, static_argnames=("A_seg_len",))
def pallas_interleave_layers__memory_aug_recurrent_mem_tr__linear_kernel_hedgehog__prompt_kernel(
    A_x: jax.Array,
    A_mem0: jax.Array,
    A_Wq: jax.Array,
    A_Wk: jax.Array,
    A_Wv: jax.Array,
    A_Wo: jax.Array,
    A_seg_len: int,
    B_x: jax.Array,
    B_wqkv: jax.Array,
    B_w_phi: jax.Array,
    B_wo: jax.Array,
):
    del B_x
    batch, seq, dm = A_x.shape
    _, heads, dh = A_Wq.shape
    n_mem = A_mem0.shape[1]
    seg = int(A_seg_len)
    n_seg = seq // seg
    rows = n_mem + seg
    pw = 2 * dh
    pairs = heads // 2
    bdh = dm // B_HEADS
    assert batch == 1 and seq % CHUNK == 0 and KV_CHUNK % seg == 0 and seg % 8 == 0 and seg >= 16
    assert n_mem % 8 == 0 and rows <= 48
    assert heads % 2 == 0 and pw == 3 * 128 and dm == NB * 128 and pairs == RING * NB + 1 and (2 * bdh) % 8 == 0

    w_t = lambda w: jnp.transpose(w, (1, 2, 0)).reshape(heads * dh, dm)
    hbm = pl.BlockSpec(memory_space=pl.ANY)

    out = pl.pallas_call(
        functools.partial(_kernel, seg=seg, heads=heads, dh=dh),
        out_shape=jax.ShapeDtypeStruct((seq, dm), A_x.dtype),
        in_specs=[hbm] * 10,
        out_specs=hbm,
        scratch_shapes=[
            pltpu.VMEM((n_mem, dm), BF16),
            pltpu.VMEM((NB + len(_BLOCK_PAIRS), n_seg * 4, 128), U32),
            pltpu.VMEM((seq, dm), F32),
            pltpu.VMEM((seq + CHUNK, dm), U32),
            pltpu.VMEM((3 * pairs, dm // 2, pw), U32),
            pltpu.VMEM((3 * RING, NB, 64, pw), U32),
            pltpu.VMEM((pairs * dh, dm), U32),
            pltpu.VMEM((NB, RING * dh, 128), U32),
            pltpu.VMEM((3 * (pairs - 1), n_seg * 8, pw), F32),
            pltpu.VMEM((3, n_seg * 8, pw), F32),
            pltpu.VMEM((dm // 128, 127 // (2 * bdh) + 2, 2 * bdh, 128), F32),
            pltpu.VMEM((seq, dm), BF16),
            pltpu.SMEM((1,), jnp.int32),
            pltpu.SemaphoreType.DMA((4,)),
            pltpu.SemaphoreType.DMA((2,)),
            pltpu.SemaphoreType.DMA((RING,)),
            pltpu.SemaphoreType.DMA((4,)),
            pltpu.SemaphoreType.DMA((seq // CHUNK,)),
        ],
        compiler_params=pltpu.CompilerParams(vmem_limit_bytes=126 * 1024 * 1024),
    )(
        A_x.reshape(n_seg, seg // 8, 8, dm),
        A_x.reshape(seq, dm),
        A_mem0.reshape(n_mem, dm),
        w_t(A_Wq), w_t(A_Wk), w_t(A_Wv),
        A_Wo.reshape(heads * dh, dm),
        B_wqkv,
        jnp.transpose(B_w_phi, (1, 2, 0)),
        B_wo,
    )
    return out.reshape(batch, seq, dm)
```

```python
import functools
import itertools

import jax
import jax.numpy as jnp
from jax import lax
import jax.experimental.pallas as pl
import jax.experimental.pallas.tpu as pltpu

F32 = jnp.float32
BF16 = jnp.bfloat16
U32 = jnp.uint32

B_HEADS = 32
LN_EPS = 1e-05
DEN_EPS = 1e-06
MASK_FILL = -1000000000.0
LOG2E = 1.4426950408889634

LAMBDA = (-1.75, -0.5625, 0.0, 0.5625, 1.75)
NB = len(LAMBDA)
UNROLL = 3
RING = 3
CHUNK = 256
B_LAG = 3
KV_CHUNK = 128
KV_LAG = 3
SUB = 64
OUT_LAG = 4
LN_LAG = 1

_NN = (((1,), (0,)), ((), ()))
_NT = (((1,), (1,)), ((), ()))


def _mm(a, b):
    return lax.dot_general(a, b, _NN, preferred_element_type=F32)


def _mm_nt(a, b):
    return lax.dot_general(a, b, _NT, preferred_element_type=F32)


def _pack(w):
    return pltpu.bitcast(w, jnp.uint32)


def _unpack(w):
    return pltpu.bitcast(w, BF16)


def _iota(shape, dim):
    return lax.broadcasted_iota(jnp.int32, shape, dim)


def _recip(x):
    r = pl.reciprocal(x, approx=True)
    return r * (2.0 - x * r)


def _layernorm(x):
    m = jnp.mean(x, axis=-1, keepdims=True)
    xc = x - m
    v = jnp.mean(xc * xc, axis=-1, keepdims=True)
    return xc * lax.rsqrt(v + LN_EPS)


def _pair_reduce(v, op):
    v = op(v, pltpu.roll(v, 4, 0))
    return op(v, pltpu.roll(v, 2, 0))


def _hedgehog(p):
    rows = [p[i:i + 8] for i in range(0, p.shape[0], 8)]
    hi = _pair_reduce(functools.reduce(jnp.maximum, rows), jnp.maximum)
    lo = _pair_reduce(functools.reduce(jnp.minimum, rows), jnp.minimum)
    ep = [jnp.exp2(r - hi) for r in rows]
    en = [jnp.exp2(lo - r) for r in rows]
    rp = _recip(_pair_reduce(functools.reduce(jnp.add, ep), jnp.add))
    rn = _recip(_pair_reduce(functools.reduce(jnp.add, en), jnp.add))
    return jnp.concatenate([e * rp for e in ep] + [e * rn for e in en], axis=0)


def _total(terms):
    return functools.reduce(jnp.add, terms)


_BLOCK_PAIRS = tuple(itertools.combinations(range(NB), 2))


def _kappa(i, j):
    return 1.0 / (LAMBDA[j] - LAMBDA[i])


def _others(j):
    return [i for i in range(NB) if i != j]


def _ahead_lhs(a, b):
    c = [b[j] + LAMBDA[j] * a[j] for j in range(NB)]
    return list(a) + [_kappa(i, j) * (c[i] + c[j]) for i, j in _BLOCK_PAIRS]


def _ahead_sums(product):
    y = [None] * NB
    for i in range(NB):
        y[i] = product(i) if y[i] is None else y[i] + product(i)
        for j in range(i + 1, NB):
            t = product(NB + _BLOCK_PAIRS.index((i, j)))
            y[i], y[j] = y[i] + t, -t if y[j] is None else y[j] - t
    return y


def _step_lhs(x, i, j):
    t = x(j) if i == j else x(i) + x(j)
    return jnp.concatenate([t[:-16], t[-8:] + LAMBDA[j] * t[-16:-8]], axis=0)


class _StepSums:
    def __init__(self, ahead):
        self.y, self.w = list(ahead), [None] * NB

    def add(self, product, order, fill):
        plus = lambda u, t: t if u is None else u + t
        for n, (i, j) in enumerate(order):
            t = product(i, j)
            for job in fill[len(fill) * n // len(order):len(fill) * (n + 1) // len(order)]:
                job()
            self.w[j] = plus(self.w[j], t)
            if i != j:
                g = _kappa(i, j) * t[-8:]
                self.y[j] = plus(self.y[j], g)
                self.y[i] = -g if self.y[i] is None else self.y[i] - g
        return self

    def columns(self):
        return [jnp.concatenate([w[:-8], y, w[-8:] - lam * y], axis=0)
                for w, y, lam in zip(self.w, self.y, LAMBDA)]


def _kernel(
    x_hbm, x_flat_hbm, mem0_hbm, wq_hbm, wk_hbm, wv_hbm, wo_hbm, bqkv_hbm, wphi_hbm, bwo_hbm,
    out_hbm,
    mem0_ref, al_ref, xres_ref, hn_ref, wqkv_ref, rqkv_ref, wo_ref, ro_ref, ahead_ref,
    sel_ref, res_ref, zero_ref,
    sem_x, sem_b, sem_w, sem_tok, sem_last, sem_out,
    *, seg, heads, dh,
):
    seq, dm = out_hbm.shape
    n_mem = mem0_ref.shape[0]
    n_seg = seq // seg
    rows = n_mem + seg
    pairs = heads // 2
    pw = 2 * dh
    off = -(-rows // 16) * 16
    scale = dh ** (-0.5)
    bdh = dm // B_HEADS
    grp = 2 * bdh
    n_grp = B_HEADS // 2
    n_set = pairs // NB
    last = pairs - 1
    tile = lambda k, n=128: slice(k * n, (k + 1) * n)
    of_set = lambda u: range(u * NB, (u + 1) * NB)

    def rows_of(j, n):
        return pl.ds(j * n if isinstance(j, int) else pl.multiple_of(j * n, n), n)

    def groups_of(kt):
        return range(128 * kt // grp, (128 * kt + 127) // grp + 1)

    def store_ahead_lhs(s, a, b):
        split = lambda t: [t[:, tile(k)] for k in range(NB)]
        for r, t in enumerate(_ahead_lhs(split(a), split(b))):
            al_ref[r, 4 * s:4 * s + t.shape[0] // 2] = _pack(t.astype(BF16))

    def project_ahead(m, u, product):
        n = n_seg * 8 // 2
        for c in range(pw // 128):
            for r0 in range(0, n_seg * 8, n):
                apply = lambda r: product(_unpack(al_ref[r, r0 // 2:(r0 + n) // 2]), r, tile(c))
                for j, y in enumerate(_ahead_sums(apply)):
                    ahead_ref[m * (pairs - 1) + u * NB + j, r0:r0 + n, tile(c)] = y

    def load(wphi_ref, xe_ref, stage_ref, out_stage_ref, last_ref, last_out_ref):
        cp_xe = pltpu.make_async_copy(x_hbm.at[:, pl.ds(seg // 8 - 2, 2)], xe_ref, sem_x.at[0])
        cp_mem0 = pltpu.make_async_copy(mem0_hbm, mem0_ref, sem_x.at[1])
        cp_wphi = pltpu.make_async_copy(wphi_hbm, wphi_ref, sem_x.at[2])

        weights = (wq_hbm, wk_hbm, wv_hbm)
        n_round = 3 * n_set
        x_rows = seq // (n_round - 1)

        def cp_set(m, u):
            return pltpu.make_async_copy(
                weights[m].at[rows_of(u, NB * pw)], stage_ref.at[u], sem_w.at[0, u])

        def cp_out_rows(t, u):
            return pltpu.make_async_copy(
                wo_hbm.at[pl.ds(u * NB, NB), t], out_stage_ref.at[u], sem_w.at[1, u])

        def cp_x(i):
            sl = rows_of(i, x_rows)
            return pltpu.make_async_copy(x_flat_hbm.at[sl], res_ref.at[sl], sem_tok.at[i])

        def cp_last(m):
            return pltpu.make_async_copy(weights[m].at[rows_of(last, pw)], last_ref.at[m], sem_last.at[m])

        cp_last_out = pltpu.make_async_copy(wo_hbm.at[last], last_out_ref, sem_last.at[3])

        def build_selectors():
            eh_r = _iota((B_HEADS, dm), 0)
            eh_c = _iota((B_HEADS, dm), 1)
            phi_f = None
            for d in range(bdh):
                eh = jnp.where(eh_c == eh_r * bdh + d, 1.0, 0.0).astype(BF16)
                t = _mm(wphi_ref[d], eh)
                phi_f = t if phi_f is None else phi_f + t
            pick = jnp.where((_iota((grp, bdh), 0) >> 1) == _iota((grp, bdh), 1), 1.0, 0.0)
            phi_rows = _mm(pick, phi_f.astype(BF16))
            r = _iota((grp, 128), 0)
            for kt in range(dm // 128):
                c = _iota((grp, 128), 1) + 128 * kt
                for i, g in enumerate(groups_of(kt)):
                    c0 = (2 * g + (r & 1)) * bdh
                    sel_ref[kt, i] = jnp.where(
                        (c >= c0) & (c < c0 + bdh), phi_rows[:, 128 * kt:128 * kt + 128], 0.0)

        def load_set(m, u):
            w = lambda use, i, j: stage_ref[u + zero_ref[use], tile(j, pw), tile(i)]
            f = lambda *a: w(*a).astype(F32)
            row = [_total([f(0, j, i) for i in range(NB)]).astype(BF16) for j in range(NB)]
            sym = [(f(1, i, j) + f(1, j, i)).astype(BF16) for i, j in _BLOCK_PAIRS]
            project_ahead(m, u, lambda t, r, c: _mm_nt(t, (row + sym)[r][c]))
            for j in range(NB):
                rqkv_ref[m * n_set + u, j] = _pack(row[j].T)
                diag = (f(2, j, j) - _total([f(2, i, j) for i in _others(j)])).astype(BF16)
                for i in range(NB):
                    t = diag if i == j else w(2, i, j)
                    wqkv_ref[m * pairs + u * NB + j, tile(i, 64)] = _pack(t.T)

        def load_out_rows(t, u):
            for r in range(0, 128, 16):
                w = {(i, j): out_stage_ref[u, i, r:r + 16, tile(j)]
                     for i in range(NB) for j in range(NB)}
                f = {ij: v.astype(F32) for ij, v in w.items()}
                packed = lambda k: rows_of(k * (dh // 8) + t * 8 + r // 16, 8)
                for j in range(NB):
                    ro_ref[j, packed(u)] = _pack(_total([f[j, i] for i in range(NB)]).astype(BF16))
                    w[j, j] = (f[j, j] - _total([f[i, j] for i in _others(j)])).astype(BF16)
                    for i in range(NB):
                        wo_ref[packed(u * NB + i), tile(j)] = _pack(w[i, j])

        def load_tokens(i):
            for k in range(x_rows // seg):
                sl = rows_of(i * (x_rows // seg) + k, seg)
                x = res_ref[sl].astype(F32)
                xres_ref[sl] = x
                hn_ref[sl] = _pack(_layernorm(x))

        for k in range(zero_ref.shape[0]):
            zero_ref[k] = 0
        for cp in (cp_wphi, cp_mem0, cp_xe):
            cp.start()
        cp_wphi.wait()
        cp_set(0, 0).start()
        build_selectors()
        cp_xe.wait()
        for cp in (cp_out_rows(0, 0), cp_x(0), cp_set(0, 1)):
            cp.start()
        n = 8
        for s in range(0, n_seg, n):
            rows_ab = (xe_ref[s:s + n, k].astype(F32).reshape(8 * n, dm) for k in range(2))
            store_ahead_lhs(s, *map(_layernorm, rows_ab))

        def following(m, u):
            wrap = u == n_set - 1
            return jnp.where(wrap, m + 1, m), jnp.where(wrap, 0, u + 1)

        def load_body(r, carry):
            before, now = carry
            after = following(*now)
            later = following(*after)
            side = jnp.maximum(r - 1, 0)
            cp_set(0, now[1]).wait()

            @pl.when(r != 1)
            def _():
                cp_out_rows(*before).wait()
                cp_x(side).wait()

            for m in range(3):
                pl.when(later[0] == m)(cp_set(m, later[1]).start)

            @pl.when(r + 2 < n_round)
            def _():
                cp_out_rows(*after).start()
                cp_x(r + 1).start()

            @pl.when(r + 2 == n_round)
            def _():
                for cp in [cp_out_rows(*after), cp_last_out] + [cp_last(m) for m in range(3)]:
                    cp.start()

            load_set(*now)
            load_out_rows(*before)
            load_tokens(side)
            return now, after

        lax.fori_loop(0, n_round, load_body, ((0, 0), (0, 0)))
        for cp in [cp_out_rows(2, n_set - 1), cp_last_out] + [cp_last(m) for m in range(3)]:
            cp.wait()
        for m in range(3):
            wqkv_ref[m * pairs + last] = _pack(last_ref[m].T)
        load_out_rows(2, n_set - 1)
        wo_ref[tile(last, dh)] = _pack(last_out_ref[...].reshape(pw, dm))
        cp_mem0.wait()

    def layers(ya_ref, o_ref, mem_ref, kt_ref, vb_ref, p_ref,
               bqkv_ref, bwo_ref, bq_ref, bkv_ref, bo_ref, ht_ref, ot_ref, kv_ref, z_ref, set_refs):
        cp_bqkv = pltpu.make_async_copy(bqkv_hbm, bqkv_ref, sem_b.at[0])
        cp_bwo = pltpu.make_async_copy(bwo_hbm, bwo_ref, sem_b.at[1])

        cut = dh % 128

        def stack(a, b):
            gap = jnp.zeros((off - rows, a.shape[1]), F32)
            tail = jnp.zeros((128 - off - rows, a.shape[1]), F32)
            return jnp.concatenate([a, gap, b, tail], axis=0).astype(BF16)

        def store_keys(j, t):
            outer = _pack(stack(t[:, 0:128], t[:, 256:384]).T)
            inner = _pack(stack(t[:, 128:256], t[:, 128:256]).T)
            low = _iota((64, 128), 1) < off
            kt_ref[j, 0:64] = jnp.where(low, outer, 0)
            kt_ref[j, 64:64 + cut // 2] = jnp.where(low[:cut // 2], inner[:cut // 2], 0)
            kt_ref[j, 64 + cut // 2:128] = jnp.where(low[cut // 2:], 0, inner[cut // 2:])
            kt_ref[j, 128:192] = jnp.where(low, 0, outer)

        def store_values(j, t):
            t = _pack(jnp.concatenate([t, jnp.zeros((off - rows, pw), F32)], axis=0).astype(BF16))
            low = _iota((off // 2, 128), 1) < cut
            vb_ref[j, 0:off // 2, 0:128] = t[:, 0:128]
            vb_ref[j, 0:off // 2, 128:256] = jnp.where(low, t[:, 128:256], 0)
            vb_ref[j, off // 2:off, 128:256] = jnp.where(low, 0, t[:, 128:256])
            vb_ref[j, off // 2:off, 256:384] = t[:, 256:384]

        def a_step(s):
            h = jnp.concatenate([mem_ref[...], pltpu.bitcast(hn_ref[rows_of(s, seg), :], F32)], axis=0)
            mine = rows_of(s, 8)
            zero = zero_ref[0]
            qi = _iota((rows, 128), 0)
            ki = _iota((rows, 128), 1)
            in_a = ki < rows
            in_b = (ki >= off) & (ki < off + rows)
            see_a = in_a & ((qi < n_mem) | (qi >= ki))
            see_b = in_b & ((qi < n_mem) | (qi >= ki - off))
            fill_a = jnp.where(in_a, MASK_FILL, -jnp.inf)
            fill_b = jnp.where(in_b, MASK_FILL, -jnp.inf)
            by_column = [(i, j) for j in range(NB) for i in range(NB)]
            by_pair = sorted(by_column, key=lambda ij: (min(ij), max(ij)))
            lhs = {(i, j): _step_lhs(lambda k: h[:, tile(k)], i, j) for i, j in by_column}

            def project(m, u, fill, order=by_column):
                product = lambda i, j: _mm(
                    lhs[i, j], _unpack(wqkv_ref[m * pairs + u * NB + j, tile(i, 64)]))
                ahead = [ahead_ref[m * (pairs - 1) + u * NB + j, mine] for j in range(NB)]
                for j, t in zip(of_set(u), _StepSums(ahead).add(product, order, fill).columns()):
                    store[m](j, t)

            def store_queries(j, t):
                o_ref[j] = t

            store = (store_queries, store_keys, store_values)
            parts = []

            def project_last(m, c):
                parts.append(_mm(h, _unpack(wqkv_ref[m * pairs + last, :, tile(c)])))
                if len(parts) == pw // 128:
                    store[m](last, jnp.concatenate(parts, axis=1))
                    parts.clear()

            def scores(j):
                sc = _mm(o_ref[j], _unpack(kt_ref[j])) * scale
                sa = jnp.where(see_a, sc, fill_a)
                sb = jnp.where(see_b, sc, fill_b)
                ea = jnp.exp(sa - jnp.max(sa, axis=-1, keepdims=True))
                eb = jnp.exp(sb - jnp.max(sb, axis=-1, keepdims=True))
                ra = _recip(jnp.sum(ea, axis=-1, keepdims=True))
                rb = _recip(jnp.sum(eb, axis=-1, keepdims=True))
                p_ref[j] = ea * ra + eb * rb

            def attend(j):
                o = _mm(p_ref[j], _unpack(vb_ref[j]))
                if j == last:
                    o_ref[j] = o
                else:
                    set_refs[j // NB][0, j % NB] = o
                    ahead_ref[j, mine] = o[-16:-8]
                    ahead_ref[last + j, mine] = o[-8:]

            out = _StepSums([None] * NB)

            def project_out(u, fill):
                product = lambda i, j: _mm(
                    _step_lhs(lambda k: set_refs[u][zero, k], i, j),
                    _unpack(wo_ref[tile(u * NB + i, dh), tile(j)]))
                out.add(product, by_pair, fill)

            direct = {}

            def out_last(c):
                direct[c] = _mm(o_ref[last], _unpack(wo_ref[tile(last, dh), tile(c)]))

            jobs = lambda f, args: [functools.partial(f, a) for a in args]
            last_jobs = lambda m: jobs(functools.partial(project_last, m), range(pw // 128))
            project(1, 0, [], sorted(by_column, key=lambda ij: max(2, *ij)))
            project(0, 0, last_jobs(1))
            project(1, 1, last_jobs(0))
            project(2, 0, jobs(scores, of_set(0)))
            project(0, 1, last_jobs(2) + jobs(scores, (last,)))
            project(1, 2, jobs(attend, of_set(0)))
            project(2, 1, jobs(scores, of_set(1)))
            project(0, 2, jobs(attend, (last,)))
            project(2, 2, jobs(attend, of_set(1)))
            project_out(0, jobs(scores, of_set(2)))
            project_out(1, jobs(attend, of_set(2)) + jobs(out_last, range(2)))
            project_out(2, jobs(out_last, range(2, NB)))
            y = jnp.concatenate([t + direct[c] for c, t in enumerate(out.columns())], axis=1)
            mem_ref[...] = y[:n_mem]
            ya_ref[s] = y[n_mem:].reshape(seg // 8, 8, dm)

        def a_start():
            group = lambda s, k: pltpu.bitcast(jnp.concatenate(
                [hn_ref[tile((t + 1) * (seg // 8) + k, 8)] for t in range(s, s + 8)], axis=0), F32)
            for s in range(0, n_seg, 8):
                store_ahead_lhs(s, group(s, -2), group(s, -1))

            def ahead_body(r, carry):
                m, u = lax.div(r, n_set), lax.rem(r, n_set)
                block = lambda i, j: _unpack(wqkv_ref[m * pairs + u * NB + j, tile(i, 64)]).astype(F32)
                row = [_unpack(rqkv_ref[r, j]) for j in range(NB)]
                sym = [(block(i, j) + block(j, i)).astype(BF16) for i, j in _BLOCK_PAIRS]
                project_ahead(m, u, lambda t, r, c: _mm(t, (row + sym)[r][:, c]))
                return carry

            lax.fori_loop(0, 3 * n_set, ahead_body, 0)

        def a_finish():
            block = lambda i, j: _unpack(jnp.concatenate(
                [wo_ref[tile(u * NB + i, dh), tile(j)] for u in range(n_set)], axis=0)).astype(F32)
            rhs = [_unpack(ro_ref[j]) for j in range(NB)]
            rhs += [(block(i, j) + block(j, i)).astype(BF16) for i, j in _BLOCK_PAIRS]
            n = n_seg // 4
            for s0 in range(0, n_seg, n):
                side = lambda p: jnp.concatenate(
                    [ahead_ref[p + u * NB, s0 * 8:(s0 + n) * 8] for u in range(n_set)], axis=1)
                lhs = _ahead_lhs([side(k) for k in range(NB)], [side(last + k) for k in range(NB)])
                for j, y in enumerate(_ahead_sums(lambda r: _mm(lhs[r], rhs[r]))):
                    y = y.reshape(n, 8, 128)
                    ya_ref[s0:s0 + n, seg // 8 - 2, :, tile(j)] += y
                    ya_ref[s0:s0 + n, seg // 8 - 1, :, tile(j)] -= LAMBDA[j] * y

        def a_layer(first_layer):
            n_loop = n_seg // UNROLL

            def a_body(i, carry):
                for k in range(UNROLL):
                    a_step(i * UNROLL + k)
                return carry

            if first_layer:
                vb_ref[...] = jnp.zeros(vb_ref.shape, U32)
                cp_bqkv.start()
                cp_bwo.start()
            else:
                a_start()
            mem_ref[...] = mem0_ref[...].astype(F32)
            lax.fori_loop(0, n_loop, a_body, 0)
            if first_layer:
                cp_bqkv.wait()
                cp_bwo.wait()
                b_fold_weights()
            for s in range(n_loop * UNROLL, n_seg):
                a_step(s)
            a_finish()

        def b_fold_weights():
            def fold(m):
                out = {}
                for kt in range(dm // 128):
                    gs = groups_of(kt)
                    block = jnp.concatenate([sel_ref[kt, i] for i in range(len(gs))], axis=0)
                    part = _mm_nt(block, bqkv_ref[:, m * dm + 128 * kt:m * dm + 128 * kt + 128])
                    for i, g in enumerate(gs):
                        t = part[i * grp:(i + 1) * grp]
                        out[g] = out[g] + t if g in out else t
                return [out[g] * LOG2E for g in range(n_grp)]

            def store(ref, blocks):
                for i in range(0, len(blocks), 2):
                    two = jnp.concatenate(blocks[i:i + 2], axis=0).astype(BF16)
                    ref[i * bdh:(i + 2) * bdh, :] = _pack(two)

            wk = fold(1)
            wv = bqkv_ref[:, 2 * dm:3 * dm].T.astype(F32)
            store(bkv_ref, [w for g in range(n_grp) for w in (wk[g], wv[g * grp:(g + 1) * grp])])
            store(bq_ref, fold(0))
            bo_ref[...] = _pack(bwo_ref[...])

        def b_kv():
            n_chunk = seq // KV_CHUNK
            tokens = lambda i: slice(i * KV_CHUNK, (i + 1) * KV_CHUNK)

            def normalize(i):
                xn = xres_ref[tokens(i), :] + ya_ref[tile(i, KV_CHUNK // seg)].reshape(KV_CHUNK, dm)
                xres_ref[tokens(i), :] = xn
                ht_ref[:, tokens(i)] = _pack(_layernorm(xn).astype(BF16).T)

            work = [(i, g) for i in range(n_chunk) for g in range(n_grp)]
            ready = {}
            normalize(0)
            for n in range(len(work) + KV_LAG):
                if n < len(work):
                    i, g = work[n]
                    if g == 0 and i + 1 < n_chunk:
                        normalize(i + 1)
                    t = _mm(_unpack(bkv_ref[g * grp:(g + 1) * grp, :]), _unpack(ht_ref[:, tokens(i)]))
                    phi = _hedgehog(t[:grp])
                    ready[n] = (t[grp:], phi.astype(BF16))
                    z = phi if i == 0 else z_ref[g] + phi
                    if i == n_chunk - 1:
                        z = jnp.broadcast_to(jnp.sum(z, axis=-1, keepdims=True), z.shape)
                    z_ref[g] = z
                if n >= KV_LAG:
                    i, g = work[n - KV_LAG]
                    t = _mm_nt(*ready.pop(n - KV_LAG))
                    if i > 0:
                        t = kv_ref[g] + t
                    if i == n_chunk - 1:
                        second = (_iota(t.shape, 1) & 1) == 1
                        t = jnp.where((_iota(t.shape, 0) >= bdh) == second, t, 0.0)
                    kv_ref[g] = t

        n_chunk = seq // CHUNK
        tokens = lambda i: slice(i * CHUNK, (i + 1) * CHUNK)

        def cp_out(i):
            return pltpu.make_async_copy(res_ref.at[tokens(i)], out_hbm.at[tokens(i)], sem_out.at[i])

        def b_out(last_layer):
            zero = zero_ref[0]
            half = n_grp // 2
            n_sub = CHUNK // SUB
            work = [(i, gg) for i in range(n_chunk) for gg in range(half)]
            ready = {}

            def staged(i, r0, n):
                return pl.ds(pl.multiple_of(zero + seq + (i % 2) * (CHUNK // 2) + r0, 8), n)

            def features(g, p):
                phi = _hedgehog(p)
                t = phi * jnp.concatenate([z_ref[g]] * (CHUNK // 128), axis=1)
                den = functools.reduce(jnp.add, [t[r:r + 8] for r in range(0, 2 * grp, 8)])
                inv = _recip(_pair_reduce(den, jnp.add) + DEN_EPS)
                other = pltpu.roll(inv, 1, 0)
                r = _iota(inv.shape, 0)
                return phi.astype(BF16), jnp.concatenate(
                    [jnp.where((r + r0 >= bdh) == ((r & 1) == 1), inv, other) for r0 in range(0, grp, 8)],
                    axis=0)

            finished = []

            def normalize():
                sl = finished.pop(0)
                hn_ref[sl, :] = _pack(_layernorm(xres_ref[sl, :]))

            def finish(i, k):
                if len(finished) > LN_LAG:
                    normalize()
                sl = slice(i * CHUNK + k * SUB, i * CHUNK + (k + 1) * SUB)
                o = _unpack(hn_ref[staged(i, k * SUB // 2, SUB // 2), :])
                xn = xres_ref[sl, :] + _mm(o, _unpack(bo_ref[...]))
                if last_layer:
                    res_ref[sl, :] = xn.astype(BF16)
                    if k == n_sub - 1:
                        cp_out(i).start()
                else:
                    xres_ref[sl, :] = xn
                    finished.append(sl)

            pending = []
            for n in range(len(work) + B_LAG):
                if n < len(work):
                    i, gg = work[n]
                    t = _mm(_unpack(bq_ref[gg * grp:(gg + 1) * grp, :]), _unpack(ht_ref[:, tokens(i)]))
                    ready[n] = [features(2 * gg + k, t[k * grp:(k + 1) * grp]) for k in range(2)]
                while pending and pending[0][0] <= n:
                    finish(*pending.pop(0)[1:])
                if n >= B_LAG:
                    i, gg = work[n - B_LAG]
                    for k, (phi, inv) in enumerate(ready.pop(n - B_LAG)):
                        g = 2 * gg + k
                        ot_ref[g * grp:(g + 1) * grp, :] = _mm(kv_ref[g], phi) * inv
                    if gg == half - 1:
                        hn_ref[staged(i, 0, CHUNK // 2), :] = _pack(ot_ref[...].astype(BF16).T)
                        pending += [(n + OUT_LAG + k * half // n_sub, i, k) for k in range(n_sub)]
            for _, i, k in pending:
                finish(i, k)
            while finished:
                normalize()

        a_layer(True)
        with jax.named_scope("L_b_kv"):
            b_kv()
        with jax.named_scope("L_b_out"):
            b_out(False)
        a_layer(False)
        with jax.named_scope("L_b_kv"):
            b_kv()
        with jax.named_scope("L_b_out"):
            b_out(True)
        for i in range(n_chunk):
            cp_out(i).wait()

    pl.run_scoped(
        load,
        pltpu.VMEM((bdh, bdh, B_HEADS), BF16),
        pltpu.VMEM((n_seg, 2, 8, dm), BF16),
        pltpu.VMEM((RING, NB * pw, dm), BF16),
        pltpu.VMEM((RING, NB, 128, dm), BF16),
        pltpu.VMEM((3, pw, dm), BF16),
        pltpu.VMEM((pw // 128, 128, dm), BF16),
    )
    pl.run_scoped(
        layers,
        pltpu.VMEM((n_seg, seg // 8, 8, dm), F32),
        pltpu.VMEM((pairs, rows, pw), F32),
        pltpu.VMEM((n_mem, dm), F32),
        pltpu.VMEM((pairs, dh, 128), U32),
        pltpu.VMEM((pairs, 64, pw), U32),
        pltpu.VMEM((pairs, rows, 128), F32),
        pltpu.VMEM((dm, 3 * dm), BF16),
        pltpu.VMEM((dm, dm), BF16),
        pltpu.VMEM((dm // 2, dm), U32),
        pltpu.VMEM((dm, dm), U32),
        pltpu.VMEM((dm // 2, dm), U32),
        pltpu.VMEM((dm // 2, seq), U32),
        pltpu.VMEM((dm, CHUNK), F32),
        pltpu.VMEM((n_grp, grp, 2 * grp), F32),
        pltpu.VMEM((n_grp, 2 * grp, 128), F32),
        [pltpu.VMEM((1, NB, rows, pw), F32)] * n_set,
    )


@functools.partial(jax.jit, static_argnames=("A_seg_len",))
def pallas_interleave_layers__memory_aug_recurrent_mem_tr__linear_kernel_hedgehog__prompt_kernel(
    A_x: jax.Array,
    A_mem0: jax.Array,
    A_Wq: jax.Array,
    A_Wk: jax.Array,
    A_Wv: jax.Array,
    A_Wo: jax.Array,
    A_seg_len: int,
    B_x: jax.Array,
    B_wqkv: jax.Array,
    B_w_phi: jax.Array,
    B_wo: jax.Array,
):
    del B_x
    batch, seq, dm = A_x.shape
    _, heads, dh = A_Wq.shape
    n_mem = A_mem0.shape[1]
    seg = int(A_seg_len)
    n_seg = seq // seg
    rows = n_mem + seg
    pw = 2 * dh
    pairs = heads // 2
    bdh = dm // B_HEADS
    assert batch == 1 and seq % CHUNK == 0 and KV_CHUNK % seg == 0 and seg % 8 == 0 and seg >= 16
    assert n_mem % 8 == 0 and rows <= 48
    assert heads % 2 == 0 and pw == 3 * 128 and dm == NB * 128 and pairs == RING * NB + 1 and (2 * bdh) % 8 == 0

    w_t = lambda w: jnp.transpose(w, (1, 2, 0)).reshape(heads * dh, dm)
    hbm = pl.BlockSpec(memory_space=pl.ANY)

    out = pl.pallas_call(
        functools.partial(_kernel, seg=seg, heads=heads, dh=dh),
        out_shape=jax.ShapeDtypeStruct((seq, dm), A_x.dtype),
        in_specs=[hbm] * 10,
        out_specs=hbm,
        scratch_shapes=[
            pltpu.VMEM((n_mem, dm), BF16),
            pltpu.VMEM((NB + len(_BLOCK_PAIRS), n_seg * 4, 128), U32),
            pltpu.VMEM((seq, dm), F32),
            pltpu.VMEM((seq + CHUNK, dm), U32),
            pltpu.VMEM((3 * pairs, dm // 2, pw), U32),
            pltpu.VMEM((3 * RING, NB, 64, pw), U32),
            pltpu.VMEM((pairs * dh, dm), U32),
            pltpu.VMEM((NB, RING * dh, 128), U32),
            pltpu.VMEM((3 * (pairs - 1), n_seg * 8, pw), F32),
            pltpu.VMEM((dm // 128, 127 // (2 * bdh) + 2, 2 * bdh, 128), F32),
            pltpu.VMEM((seq, dm), BF16),
            pltpu.SMEM((3,), jnp.int32),
            pltpu.SemaphoreType.DMA((3,)),
            pltpu.SemaphoreType.DMA((2,)),
            pltpu.SemaphoreType.DMA((2, RING)),
            pltpu.SemaphoreType.DMA((3 * RING - 1,)),
            pltpu.SemaphoreType.DMA((4,)),
            pltpu.SemaphoreType.DMA((seq // CHUNK,)),
        ],
        compiler_params=pltpu.CompilerParams(vmem_limit_bytes=126 * 1024 * 1024),
    )(
        A_x.reshape(n_seg, seg // 8, 8, dm),
        A_x.reshape(seq, dm),
        A_mem0.reshape(n_mem, dm),
        w_t(A_Wq), w_t(A_Wk), w_t(A_Wv),
        A_Wo.reshape(pairs, pw // 128, 128, dm),
        B_wqkv,
        jnp.transpose(B_w_phi, (1, 2, 0)),
        B_wo,
    )
    return out.reshape(batch, seq, dm)
```

```python
import functools
import itertools

import jax
import jax.numpy as jnp
from jax import lax
import jax.experimental.pallas as pl
import jax.experimental.pallas.tpu as pltpu

F32 = jnp.float32
BF16 = jnp.bfloat16
U32 = jnp.uint32

B_HEADS = 32
LN_EPS = 1e-05
DEN_EPS = 1e-06
MASK_FILL = -1000000000.0
LOG2E = 1.4426950408889634

LAMBDA = (-1.75, -0.5625, 0.0, 0.5625, 1.75)
NB = len(LAMBDA)
UNROLL = 3
RING = 3
CHUNK = 256
B_LAG = 3
KV_CHUNK = 128
KV_LAG = 3
SUB = 64
OUT_LAG = 4
LN_LAG = 1

_NN = (((1,), (0,)), ((), ()))
_NT = (((1,), (1,)), ((), ()))


def _mm(a, b):
    return lax.dot_general(a, b, _NN, preferred_element_type=F32)


def _mm_nt(a, b):
    return lax.dot_general(a, b, _NT, preferred_element_type=F32)


def _pack(w):
    return pltpu.bitcast(w, jnp.uint32)


def _unpack(w):
    return pltpu.bitcast(w, BF16)


def _iota(shape, dim):
    return lax.broadcasted_iota(jnp.int32, shape, dim)


def _recip(x):
    r = pl.reciprocal(x, approx=True)
    return r * (2.0 - x * r)


def _layernorm(x):
    m = jnp.mean(x, axis=-1, keepdims=True)
    xc = x - m
    v = jnp.mean(xc * xc, axis=-1, keepdims=True)
    return xc * lax.rsqrt(v + LN_EPS)


def _pair_reduce(v, op):
    v = op(v, pltpu.roll(v, 4, 0))
    return op(v, pltpu.roll(v, 2, 0))


def _hedgehog(p):
    rows = [p[i:i + 8] for i in range(0, p.shape[0], 8)]
    hi = _pair_reduce(functools.reduce(jnp.maximum, rows), jnp.maximum)
    lo = _pair_reduce(functools.reduce(jnp.minimum, rows), jnp.minimum)
    ep = [jnp.exp2(r - hi) for r in rows]
    en = [jnp.exp2(lo - r) for r in rows]
    rp = _recip(_pair_reduce(functools.reduce(jnp.add, ep), jnp.add))
    rn = _recip(_pair_reduce(functools.reduce(jnp.add, en), jnp.add))
    return jnp.concatenate([e * rp for e in ep] + [e * rn for e in en], axis=0)


def _total(terms):
    return functools.reduce(jnp.add, terms)


_BLOCK_PAIRS = tuple(itertools.combinations(range(NB), 2))


def _kappa(i, j):
    return 1.0 / (LAMBDA[j] - LAMBDA[i])


def _others(j):
    return [i for i in range(NB) if i != j]


def _ahead_lhs(a, b):
    c = [b[j] + LAMBDA[j] * a[j] for j in range(NB)]
    return list(a) + [_kappa(i, j) * (c[i] + c[j]) for i, j in _BLOCK_PAIRS]


def _ahead_sums(product):
    y = [None] * NB
    for i in range(NB):
        y[i] = product(i) if y[i] is None else y[i] + product(i)
        for j in range(i + 1, NB):
            t = product(NB + _BLOCK_PAIRS.index((i, j)))
            y[i], y[j] = y[i] + t, -t if y[j] is None else y[j] - t
    return y


def _step_lhs(x, i, j):
    t = x(j) if i == j else x(i) + x(j)
    return jnp.concatenate([t[:-16], t[-8:] + LAMBDA[j] * t[-16:-8]], axis=0)


class _StepSums:
    def __init__(self, ahead):
        self.y, self.w = list(ahead), [None] * NB

    def add(self, product, order):
        plus = lambda u, t: t if u is None else u + t
        for i, j in order:
            t = product(i, j)
            self.w[j] = plus(self.w[j], t)
            if i != j:
                g = _kappa(i, j) * t[-8:]
                self.y[j] = plus(self.y[j], g)
                self.y[i] = -g if self.y[i] is None else self.y[i] - g
        return self

    def columns(self):
        return [jnp.concatenate([w[:-8], y, w[-8:] - lam * y], axis=0)
                for w, y, lam in zip(self.w, self.y, LAMBDA)]


def _kernel(
    x_hbm, mem0_hbm, wq_hbm, wk_hbm, wv_hbm, wo_hbm, bqkv_hbm, wphi_hbm, bwo_hbm,
    out_hbm,
    mem0_ref, al_ref, xres_ref, hn_ref, wqkv_ref, rqkv_ref, wo_ref, ro_ref, ahead_ref,
    sel_ref, zero_ref,
    sem_x, sem_b, sem_w, sem_tok, sem_last, sem_out,
    *, seg, heads, dh,
):
    seq, dm = out_hbm.shape
    n_mem = mem0_ref.shape[0]
    n_seg = seq // seg
    rows = n_mem + seg
    pairs = heads // 2
    pw = 2 * dh
    off = -(-rows // 16) * 16
    scale = dh ** (-0.5)
    bdh = dm // B_HEADS
    grp = 2 * bdh
    n_grp = B_HEADS // 2
    n_set = pairs // NB
    last = pairs - 1
    tile = lambda k, n=128: slice(k * n, (k + 1) * n)
    of_set = lambda u: range(u * NB, (u + 1) * NB)

    def rows_of(j, n):
        return pl.ds(j * n if isinstance(j, int) else pl.multiple_of(j * n, n), n)

    def groups_of(kt):
        return range(128 * kt // grp, (128 * kt + 127) // grp + 1)

    def store_ahead_lhs(s, a, b):
        split = lambda t: [t[:, tile(k)] for k in range(NB)]
        for r, t in enumerate(_ahead_lhs(split(a), split(b))):
            al_ref[r, 4 * s:4 * s + t.shape[0] // 2] = _pack(t.astype(BF16))

    def project_ahead(m, u, product):
        n = n_seg * 8 // 2
        for c in range(pw // 128):
            for r0 in range(0, n_seg * 8, n):
                apply = lambda r: product(_unpack(al_ref[r, r0 // 2:(r0 + n) // 2]), r, tile(c))
                for j, y in enumerate(_ahead_sums(apply)):
                    ahead_ref[m * (pairs - 1) + u * NB + j, r0:r0 + n, tile(c)] = y

    def load(wphi_ref, xe_ref, xp_ref, stage_ref, out_stage_ref, last_ref, last_out_ref):
        cp_xe = pltpu.make_async_copy(x_hbm.at[:, pl.ds(seg // 8 - 2, 2)], xe_ref, sem_x.at[0])
        cp_mem0 = pltpu.make_async_copy(mem0_hbm, mem0_ref, sem_x.at[1])
        cp_wphi = pltpu.make_async_copy(wphi_hbm, wphi_ref, sem_x.at[2])

        weights = (wq_hbm, wk_hbm, wv_hbm)
        n_round = 3 * n_set
        x_segs = n_seg // (n_round - 1)
        plain = seg // 8 - 2

        def cp_set(m, u):
            return pltpu.make_async_copy(
                weights[m].at[rows_of(u, NB * pw)], stage_ref.at[u], sem_w.at[0, u])

        def cp_out_rows(t, u):
            return pltpu.make_async_copy(
                wo_hbm.at[pl.ds(u * NB, NB), t], out_stage_ref.at[u], sem_w.at[1, u])

        def cp_x(i):
            sl = pl.ds(i * x_segs, x_segs)
            return pltpu.make_async_copy(x_hbm.at[sl, pl.ds(0, plain)], xp_ref.at[sl], sem_tok.at[i])

        def cp_last(m):
            return pltpu.make_async_copy(weights[m].at[rows_of(last, pw)], last_ref.at[m], sem_last.at[m])

        cp_last_out = pltpu.make_async_copy(wo_hbm.at[last], last_out_ref, sem_last.at[3])

        def build_selectors():
            eh_r = _iota((B_HEADS, dm), 0)
            eh_c = _iota((B_HEADS, dm), 1)
            phi_f = None
            for d in range(bdh):
                eh = jnp.where(eh_c == eh_r * bdh + d, 1.0, 0.0).astype(BF16)
                t = _mm(wphi_ref[d], eh)
                phi_f = t if phi_f is None else phi_f + t
            pick = jnp.where((_iota((grp, bdh), 0) >> 1) == _iota((grp, bdh), 1), 1.0, 0.0)
            phi_rows = _mm(pick, phi_f.astype(BF16))
            r = _iota((grp, 128), 0)
            for kt in range(dm // 128):
                c = _iota((grp, 128), 1) + 128 * kt
                for i, g in enumerate(groups_of(kt)):
                    c0 = (2 * g + (r & 1)) * bdh
                    sel_ref[kt, i] = jnp.where(
                        (c >= c0) & (c < c0 + bdh), phi_rows[:, 128 * kt:128 * kt + 128], 0.0)

        def load_set(m, u):
            w = lambda use, i, j: stage_ref[u + zero_ref[use], tile(j, pw), tile(i)]
            f = lambda *a: w(*a).astype(F32)
            row = [_total([f(0, j, i) for i in range(NB)]).astype(BF16) for j in range(NB)]
            sym = [(f(1, i, j) + f(1, j, i)).astype(BF16) for i, j in _BLOCK_PAIRS]
            project_ahead(m, u, lambda t, r, c: _mm_nt(t, (row + sym)[r][c]))
            for j in range(NB):
                rqkv_ref[m * n_set + u, j] = _pack(row[j].T)
                diag = (f(2, j, j) - _total([f(2, i, j) for i in _others(j)])).astype(BF16)
                for i in range(NB):
                    t = diag if i == j else w(2, i, j)
                    wqkv_ref[m * pairs + u * NB + j, tile(i, 64)] = _pack(t.T)

        def load_out_rows(t, u):
            for r in range(0, 128, 16):
                w = {(i, j): out_stage_ref[u, i, r:r + 16, tile(j)]
                     for i in range(NB) for j in range(NB)}
                f = {ij: v.astype(F32) for ij, v in w.items()}
                packed = lambda k: rows_of(k * (dh // 8) + t * 8 + r // 16, 8)
                for j in range(NB):
                    ro_ref[j, packed(u)] = _pack(_total([f[j, i] for i in range(NB)]).astype(BF16))
                    w[j, j] = (f[j, j] - _total([f[i, j] for i in _others(j)])).astype(BF16)
                    for i in range(NB):
                        wo_ref[packed(u * NB + i), tile(j)] = _pack(w[i, j])

        def start_rows(s, k, x):
            x = x.astype(F32).reshape(-1, dm)
            h = _layernorm(x)
            for t in range(x.shape[0] // 8):
                sl = rows_of((s + t) * (seg // 8) + k, 8)
                xres_ref[sl] = x[tile(t, 8)]
                hn_ref[sl] = _pack(h[tile(t, 8)])
            return h

        for k in range(zero_ref.shape[0]):
            zero_ref[k] = 0
        for cp in (cp_wphi, cp_mem0, cp_xe):
            cp.start()
        cp_wphi.wait()
        cp_set(0, 0).start()
        build_selectors()
        cp_xe.wait()
        for cp in (cp_out_rows(0, 0), cp_x(0), cp_set(0, 1)):
            cp.start()
        for s in range(0, n_seg, x_segs):
            store_ahead_lhs(s, *(start_rows(s, plain + k, xe_ref[s:s + x_segs, k]) for k in range(2)))

        def following(m, u):
            wrap = u == n_set - 1
            return jnp.where(wrap, m + 1, m), jnp.where(wrap, 0, u + 1)

        def load_body(r, carry):
            before, now = carry
            after = following(*now)
            later = following(*after)
            side = jnp.maximum(r - 1, 0)
            cp_set(0, now[1]).wait()

            @pl.when(r != 1)
            def _():
                cp_out_rows(*before).wait()
                cp_x(side).wait()

            for m in range(3):
                pl.when(later[0] == m)(cp_set(m, later[1]).start)

            @pl.when(r + 2 < n_round)
            def _():
                cp_out_rows(*after).start()
                cp_x(r + 1).start()

            @pl.when(r + 2 == n_round)
            def _():
                for cp in [cp_out_rows(*after), cp_last_out] + [cp_last(m) for m in range(3)]:
                    cp.start()

            load_set(*now)
            load_out_rows(*before)
            for k in range(plain):
                start_rows(side * x_segs, k, xp_ref[pl.ds(side * x_segs, x_segs), k])
            return now, after

        lax.fori_loop(0, n_round, load_body, ((0, 0), (0, 0)))
        for cp in [cp_out_rows(2, n_set - 1), cp_last_out] + [cp_last(m) for m in range(3)]:
            cp.wait()
        for m in range(3):
            wqkv_ref[m * pairs + last] = _pack(last_ref[m].T)
        load_out_rows(2, n_set - 1)
        wo_ref[tile(last, dh)] = _pack(last_out_ref[...].reshape(pw, dm))
        cp_mem0.wait()

    def layers(ya_ref, o_ref, mem_ref, kt_ref, vb_ref, p_ref,
               bqkv_ref, bwo_ref, bq_ref, bkv_ref, bo_ref, ht_ref, ot_ref, kv_ref, z_ref, res_ref):
        cp_bqkv = pltpu.make_async_copy(bqkv_hbm, bqkv_ref, sem_b.at[0])
        cp_bwo = pltpu.make_async_copy(bwo_hbm, bwo_ref, sem_b.at[1])

        cut = dh % 128

        def stack(a, b):
            gap = jnp.zeros((off - rows, a.shape[1]), F32)
            tail = jnp.zeros((128 - off - rows, a.shape[1]), F32)
            return jnp.concatenate([a, gap, b, tail], axis=0).astype(BF16)

        def store_keys(j, t):
            outer = _pack(stack(t[:, 0:128], t[:, 256:384]).T)
            inner = _pack(stack(t[:, 128:256], t[:, 128:256]).T)
            low = _iota((64, 128), 1) < off
            kt_ref[j, 0:64] = jnp.where(low, outer, 0)
            kt_ref[j, 64:64 + cut // 2] = jnp.where(low[:cut // 2], inner[:cut // 2], 0)
            kt_ref[j, 64 + cut // 2:128] = jnp.where(low[cut // 2:], 0, inner[cut // 2:])
            kt_ref[j, 128:192] = jnp.where(low, 0, outer)

        def store_values(j, t):
            t = _pack(jnp.concatenate([t, jnp.zeros((off - rows, pw), F32)], axis=0).astype(BF16))
            low = _iota((off // 2, 128), 1) < cut
            vb_ref[j, 0:off // 2, 0:128] = t[:, 0:128]
            vb_ref[j, 0:off // 2, 128:256] = jnp.where(low, t[:, 128:256], 0)
            vb_ref[j, off // 2:off, 128:256] = jnp.where(low, 0, t[:, 128:256])
            vb_ref[j, off // 2:off, 256:384] = t[:, 256:384]

        def a_step(s):
            h = jnp.concatenate([mem_ref[...], pltpu.bitcast(hn_ref[rows_of(s, seg), :], F32)], axis=0)
            mine = rows_of(s, 8)
            qi = _iota((rows, 128), 0)
            ki = _iota((rows, 128), 1)
            in_a = ki < rows
            in_b = (ki >= off) & (ki < off + rows)
            see_a = in_a & ((qi < n_mem) | (qi >= ki))
            see_b = in_b & ((qi < n_mem) | (qi >= ki - off))
            fill_a = jnp.where(in_a, MASK_FILL, -jnp.inf)
            fill_b = jnp.where(in_b, MASK_FILL, -jnp.inf)
            by_column = [(i, j) for j in range(NB) for i in range(NB)]
            lhs = {(i, j): _step_lhs(lambda k: h[:, tile(k)], i, j) for i, j in by_column}

            def store_queries(j, t):
                o_ref[j] = t

            store = (store_queries, store_keys, store_values)

            def project(m, u, order=by_column):
                product = lambda i, j: _mm(
                    lhs[i, j], _unpack(wqkv_ref[m * pairs + u * NB + j, tile(i, 64)]))
                ahead = [ahead_ref[m * (pairs - 1) + u * NB + j, mine] for j in range(NB)]
                for j, t in zip(of_set(u), _StepSums(ahead).add(product, order).columns()):
                    store[m](j, t)

            def scores(j):
                sc = _mm(o_ref[j], _unpack(kt_ref[j])) * scale
                sa = jnp.where(see_a, sc, fill_a)
                sb = jnp.where(see_b, sc, fill_b)
                e = jnp.exp(jnp.maximum(sa - jnp.max(sa, axis=-1, keepdims=True),
                                        sb - jnp.max(sb, axis=-1, keepdims=True)))
                sum_a = jnp.sum(jnp.where(in_a, e, 0.0), axis=-1, keepdims=True)
                sum_b = jnp.sum(jnp.where(in_a, 0.0, e), axis=-1, keepdims=True)
                p_ref[j] = e * _recip(jnp.where(in_a, sum_a, sum_b))

            def attend(j):
                o = _mm(p_ref[j], _unpack(vb_ref[j]))
                o_ref[j] = o
                if j < last:
                    ahead_ref[j, mine] = o[-16:-8]
                    ahead_ref[last + j, mine] = o[-8:]

            out = _StepSums([None] * NB)

            def project_out(u):
                product = lambda i, j: _mm(
                    _step_lhs(lambda k: o_ref[u * NB + k], i, j),
                    _unpack(wo_ref[tile(u * NB + i, dh), tile(j)]))
                out.add(product, sorted(by_column, key=sorted))

            out_last = lambda c: _mm(o_ref[last], _unpack(wo_ref[tile(last, dh), tile(c)]))

            project(1, 0, sorted(by_column, key=lambda ij: max(2, *ij)))
            for m in (1, 0, 2):
                store[m](last, _mm(h, _unpack(wqkv_ref[m * pairs + last])))
            for m, u in ((1, 1), (1, 2), (0, 0), (2, 0), (0, 1), (2, 1), (0, 2)):
                project(m, u)
            ready = [*of_set(0), *of_set(1), last]
            for j in ready:
                scores(j)
            project(2, 2)
            for j in of_set(2):
                scores(j)
            for j in ready:
                attend(j)
            project_out(0)
            for j in of_set(2):
                attend(j)
            direct = [out_last(c) for c in range(NB - 1)]
            project_out(1)
            project_out(2)
            direct.append(out_last(NB - 1))
            y = jnp.concatenate([t + d for t, d in zip(out.columns(), direct)], axis=1)
            mem_ref[...] = y[:n_mem]
            ya_ref[s] = y[n_mem:].reshape(seg // 8, 8, dm)

        def a_start():
            group = lambda s, k: pltpu.bitcast(jnp.concatenate(
                [hn_ref[tile((t + 1) * (seg // 8) + k, 8)] for t in range(s, s + 8)], axis=0), F32)
            for s in range(0, n_seg, 8):
                store_ahead_lhs(s, group(s, -2), group(s, -1))

            def ahead_body(r, carry):
                m, u = lax.div(r, n_set), lax.rem(r, n_set)
                block = lambda i, j: _unpack(wqkv_ref[m * pairs + u * NB + j, tile(i, 64)]).astype(F32)
                row = [_unpack(rqkv_ref[r, j]) for j in range(NB)]
                sym = [(block(i, j) + block(j, i)).astype(BF16) for i, j in _BLOCK_PAIRS]
                project_ahead(m, u, lambda t, r, c: _mm(t, (row + sym)[r][:, c]))
                return carry

            lax.fori_loop(0, 3 * n_set, ahead_body, 0)

        def a_finish():
            block = lambda i, j: _unpack(jnp.concatenate(
                [wo_ref[tile(u * NB + i, dh), tile(j)] for u in range(n_set)], axis=0)).astype(F32)
            rhs = [_unpack(ro_ref[j]) for j in range(NB)]
            rhs += [(block(i, j) + block(j, i)).astype(BF16) for i, j in _BLOCK_PAIRS]
            n = n_seg // 4
            for s0 in range(0, n_seg, n):
                side = lambda p: jnp.concatenate(
                    [ahead_ref[p + u * NB, s0 * 8:(s0 + n) * 8] for u in range(n_set)], axis=1)
                lhs = _ahead_lhs([side(k) for k in range(NB)], [side(last + k) for k in range(NB)])
                for j, y in enumerate(_ahead_sums(lambda r: _mm(lhs[r], rhs[r]))):
                    y = y.reshape(n, 8, 128)
                    ya_ref[s0:s0 + n, seg // 8 - 2, :, tile(j)] += y
                    ya_ref[s0:s0 + n, seg // 8 - 1, :, tile(j)] -= LAMBDA[j] * y

        def a_layer(first_layer):
            n_loop = n_seg // UNROLL

            def a_body(i, carry):
                for k in range(UNROLL):
                    a_step(i * UNROLL + k)
                return carry

            if first_layer:
                vb_ref[...] = jnp.zeros(vb_ref.shape, U32)
                cp_bqkv.start()
                cp_bwo.start()
            else:
                a_start()
            mem_ref[...] = mem0_ref[...].astype(F32)
            lax.fori_loop(0, n_loop, a_body, 0)
            if first_layer:
                cp_bqkv.wait()
                cp_bwo.wait()
                b_fold_weights()
            for s in range(n_loop * UNROLL, n_seg):
                a_step(s)
            a_finish()

        def b_fold_weights():
            def fold(m):
                out = {}
                for kt in range(dm // 128):
                    gs = groups_of(kt)
                    block = jnp.concatenate([sel_ref[kt, i] for i in range(len(gs))], axis=0)
                    part = _mm_nt(block, bqkv_ref[:, m * dm + 128 * kt:m * dm + 128 * kt + 128])
                    for i, g in enumerate(gs):
                        t = part[i * grp:(i + 1) * grp]
                        out[g] = out[g] + t if g in out else t
                return [out[g] * LOG2E for g in range(n_grp)]

            def store(ref, blocks):
                for i in range(0, len(blocks), 2):
                    two = jnp.concatenate(blocks[i:i + 2], axis=0).astype(BF16)
                    ref[i * bdh:(i + 2) * bdh, :] = _pack(two)

            wk = fold(1)
            wv = bqkv_ref[:, 2 * dm:3 * dm].T.astype(F32)
            store(bkv_ref, [w for g in range(n_grp) for w in (wk[g], wv[g * grp:(g + 1) * grp])])
            store(bq_ref, fold(0))
            bo_ref[...] = _pack(bwo_ref[...])

        def b_kv():
            n_chunk = seq // KV_CHUNK
            tokens = lambda i: slice(i * KV_CHUNK, (i + 1) * KV_CHUNK)

            def normalize(i):
                xn = xres_ref[tokens(i), :] + ya_ref[tile(i, KV_CHUNK // seg)].reshape(KV_CHUNK, dm)
                xres_ref[tokens(i), :] = xn
                ht_ref[:, tokens(i)] = _pack(_layernorm(xn).astype(BF16).T)

            work = [(i, g) for i in range(n_chunk) for g in range(n_grp)]
            ready = {}
            normalize(0)
            for n in range(len(work) + KV_LAG):
                if n < len(work):
                    i, g = work[n]
                    if g == 0 and i + 1 < n_chunk:
                        normalize(i + 1)
                    t = _mm(_unpack(bkv_ref[g * grp:(g + 1) * grp, :]), _unpack(ht_ref[:, tokens(i)]))
                    phi = _hedgehog(t[:grp])
                    ready[n] = (t[grp:], phi.astype(BF16))
                    z = phi if i == 0 else z_ref[g] + phi
                    if i == n_chunk - 1:
                        z = jnp.broadcast_to(jnp.sum(z, axis=-1, keepdims=True), z.shape)
                    z_ref[g] = z
                if n >= KV_LAG:
                    i, g = work[n - KV_LAG]
                    t = _mm_nt(*ready.pop(n - KV_LAG))
                    if i > 0:
                        t = kv_ref[g] + t
                    if i == n_chunk - 1:
                        second = (_iota(t.shape, 1) & 1) == 1
                        t = jnp.where((_iota(t.shape, 0) >= bdh) == second, t, 0.0)
                    kv_ref[g] = t

        n_chunk = seq // CHUNK
        tokens = lambda i: slice(i * CHUNK, (i + 1) * CHUNK)

        def cp_out(i):
            return pltpu.make_async_copy(res_ref.at[tokens(i)], out_hbm.at[tokens(i)], sem_out.at[i])

        def b_out(last_layer):
            zero = zero_ref[0]
            half = n_grp // 2
            n_sub = CHUNK // SUB
            work = [(i, gg) for i in range(n_chunk) for gg in range(half)]
            ready = {}

            def staged(i, r0, n):
                return pl.ds(pl.multiple_of(zero + seq + (i % 2) * (CHUNK // 2) + r0, 8), n)

            def features(g, p):
                phi = _hedgehog(p)
                t = phi * jnp.concatenate([z_ref[g]] * (CHUNK // 128), axis=1)
                den = functools.reduce(jnp.add, [t[r:r + 8] for r in range(0, 2 * grp, 8)])
                inv = _recip(_pair_reduce(den, jnp.add) + DEN_EPS)
                other = pltpu.roll(inv, 1, 0)
                r = _iota(inv.shape, 0)
                return phi.astype(BF16), jnp.concatenate(
                    [jnp.where((r + r0 >= bdh) == ((r & 1) == 1), inv, other) for r0 in range(0, grp, 8)],
                    axis=0)

            finished = []

            def normalize():
                sl = finished.pop(0)
                hn_ref[sl, :] = _pack(_layernorm(xres_ref[sl, :]))

            def finish(i, k):
                if len(finished) > LN_LAG:
                    normalize()
                sl = slice(i * CHUNK + k * SUB, i * CHUNK + (k + 1) * SUB)
                o = _unpack(hn_ref[staged(i, k * SUB // 2, SUB // 2), :])
                xn = xres_ref[sl, :] + _mm(o, _unpack(bo_ref[...]))
                if last_layer:
                    res_ref[sl, :] = xn.astype(BF16)
                    if k == n_sub - 1:
                        cp_out(i).start()
                else:
                    xres_ref[sl, :] = xn
                    finished.append(sl)

            pending = []
            for n in range(len(work) + B_LAG):
                if n < len(work):
                    i, gg = work[n]
                    t = _mm(_unpack(bq_ref[gg * grp:(gg + 1) * grp, :]), _unpack(ht_ref[:, tokens(i)]))
                    ready[n] = [features(2 * gg + k, t[k * grp:(k + 1) * grp]) for k in range(2)]
                while pending and pending[0][0] <= n:
                    finish(*pending.pop(0)[1:])
                if n >= B_LAG:
                    i, gg = work[n - B_LAG]
                    for k, (phi, inv) in enumerate(ready.pop(n - B_LAG)):
                        g = 2 * gg + k
                        ot_ref[g * grp:(g + 1) * grp, :] = _mm(kv_ref[g], phi) * inv
                    if gg == half - 1:
                        hn_ref[staged(i, 0, CHUNK // 2), :] = _pack(ot_ref[...].astype(BF16).T)
                        pending += [(n + OUT_LAG + k * half // n_sub, i, k) for k in range(n_sub)]
            for _, i, k in pending:
                finish(i, k)
            while finished:
                normalize()

        a_layer(True)
        with jax.named_scope("L_b_kv"):
            b_kv()
        with jax.named_scope("L_b_out"):
            b_out(False)
        a_layer(False)
        with jax.named_scope("L_b_kv"):
            b_kv()
        with jax.named_scope("L_b_out"):
            b_out(True)
        for i in range(n_chunk):
            cp_out(i).wait()

    pl.run_scoped(
        load,
        pltpu.VMEM((bdh, bdh, B_HEADS), BF16),
        pltpu.VMEM((n_seg, 2, 8, dm), BF16),
        pltpu.VMEM((n_seg, seg // 8 - 2, 8, dm), BF16),
        pltpu.VMEM((RING, NB * pw, dm), BF16),
        pltpu.VMEM((RING, NB, 128, dm), BF16),
        pltpu.VMEM((3, pw, dm), BF16),
        pltpu.VMEM((pw // 128, 128, dm), BF16),
    )
    pl.run_scoped(
        layers,
        pltpu.VMEM((n_seg, seg // 8, 8, dm), F32),
        pltpu.VMEM((pairs, rows, pw), F32),
        pltpu.VMEM((n_mem, dm), F32),
        pltpu.VMEM((pairs, dh, 128), U32),
        pltpu.VMEM((pairs, 64, pw), U32),
        pltpu.VMEM((pairs, rows, 128), F32),
        pltpu.VMEM((dm, 3 * dm), BF16),
        pltpu.VMEM((dm, dm), BF16),
        pltpu.VMEM((dm // 2, dm), U32),
        pltpu.VMEM((dm, dm), U32),
        pltpu.VMEM((dm // 2, dm), U32),
        pltpu.VMEM((dm // 2, seq), U32),
        pltpu.VMEM((dm, CHUNK), F32),
        pltpu.VMEM((n_grp, grp, 2 * grp), F32),
        pltpu.VMEM((n_grp, 2 * grp, 128), F32),
        pltpu.VMEM((seq, dm), BF16),
    )


@functools.partial(jax.jit, static_argnames=("A_seg_len",))
def pallas_interleave_layers__memory_aug_recurrent_mem_tr__linear_kernel_hedgehog__prompt_kernel(
    A_x: jax.Array,
    A_mem0: jax.Array,
    A_Wq: jax.Array,
    A_Wk: jax.Array,
    A_Wv: jax.Array,
    A_Wo: jax.Array,
    A_seg_len: int,
    B_x: jax.Array,
    B_wqkv: jax.Array,
    B_w_phi: jax.Array,
    B_wo: jax.Array,
):
    del B_x
    batch, seq, dm = A_x.shape
    _, heads, dh = A_Wq.shape
    n_mem = A_mem0.shape[1]
    seg = int(A_seg_len)
    n_seg = seq // seg
    rows = n_mem + seg
    pw = 2 * dh
    pairs = heads // 2
    bdh = dm // B_HEADS
    assert batch == 1 and seq % CHUNK == 0 and KV_CHUNK % seg == 0 and seg % 8 == 0 and seg > 16
    assert n_mem % 8 == 0 and rows <= 48
    assert heads % 2 == 0 and pw == 3 * 128 and dm == NB * 128 and pairs == RING * NB + 1 and (2 * bdh) % 8 == 0

    w_t = lambda w: jnp.transpose(w, (1, 2, 0)).reshape(heads * dh, dm)
    hbm = pl.BlockSpec(memory_space=pl.ANY)

    out = pl.pallas_call(
        functools.partial(_kernel, seg=seg, heads=heads, dh=dh),
        out_shape=jax.ShapeDtypeStruct((seq, dm), A_x.dtype),
        in_specs=[hbm] * 9,
        out_specs=hbm,
        scratch_shapes=[
            pltpu.VMEM((n_mem, dm), BF16),
            pltpu.VMEM((NB + len(_BLOCK_PAIRS), n_seg * 4, 128), U32),
            pltpu.VMEM((seq, dm), F32),
            pltpu.VMEM((seq + CHUNK, dm), U32),
            pltpu.VMEM((3 * pairs, dm // 2, pw), U32),
            pltpu.VMEM((3 * RING, NB, 64, pw), U32),
            pltpu.VMEM((pairs * dh, dm), U32),
            pltpu.VMEM((NB, RING * dh, 128), U32),
            pltpu.VMEM((3 * (pairs - 1), n_seg * 8, pw), F32),
            pltpu.VMEM((dm // 128, 127 // (2 * bdh) + 2, 2 * bdh, 128), F32),
            pltpu.SMEM((3,), jnp.int32),
            pltpu.SemaphoreType.DMA((3,)),
            pltpu.SemaphoreType.DMA((2,)),
            pltpu.SemaphoreType.DMA((2, RING)),
            pltpu.SemaphoreType.DMA((3 * RING - 1,)),
            pltpu.SemaphoreType.DMA((4,)),
            pltpu.SemaphoreType.DMA((seq // CHUNK,)),
        ],
        compiler_params=pltpu.CompilerParams(
            vmem_limit_bytes=126 * 1024 * 1024,
            flags={"XLA_TPU_EVENLY_DISTRIBUTE_CRITICAL_NODES": True},
        ),
    )(
        A_x.reshape(n_seg, seg // 8, 8, dm),
        A_mem0.reshape(n_mem, dm),
        w_t(A_Wq), w_t(A_Wk), w_t(A_Wv),
        A_Wo.reshape(pairs, pw // 128, 128, dm),
        B_wqkv,
        jnp.transpose(B_w_phi, (1, 2, 0)),
        B_wo,
    )
    return out.reshape(batch, seq, dm)
```

```python
import functools
import itertools

import jax
import jax.numpy as jnp
from jax import lax
import jax.experimental.pallas as pl
import jax.experimental.pallas.tpu as pltpu

F32 = jnp.float32
BF16 = jnp.bfloat16
U32 = jnp.uint32

B_HEADS = 32
LN_EPS = 1e-05
DEN_EPS = 1e-06
MASK_FILL = -1000000000.0
LOG2E = 1.4426950408889634

LAMBDA = (-1.75, -0.5625, 0.0, 0.5625, 1.75)
NB = len(LAMBDA)
UNROLL = 3
RING = 3
CHUNK = 256
B_LAG = 3
KV_CHUNK = 128
KV_LAG = 3
SUB = 64
OUT_LAG = 6
LN_LAG = 1

_NN = (((1,), (0,)), ((), ()))
_NT = (((1,), (1,)), ((), ()))


def _mm(a, b):
    return lax.dot_general(a, b, _NN, preferred_element_type=F32)


def _mm_nt(a, b):
    return lax.dot_general(a, b, _NT, preferred_element_type=F32)


def _pack(w):
    return pltpu.bitcast(w, jnp.uint32)


def _unpack(w):
    return pltpu.bitcast(w, BF16)


def _iota(shape, dim):
    return lax.broadcasted_iota(jnp.int32, shape, dim)


def _recip(x):
    r = pl.reciprocal(x, approx=True)
    return r * (2.0 - x * r)


def _layernorm(x):
    m = jnp.mean(x, axis=-1, keepdims=True)
    xc = x - m
    v = jnp.mean(xc * xc, axis=-1, keepdims=True)
    return xc * lax.rsqrt(v + LN_EPS)


def _pair_reduce(v, op):
    v = op(v, pltpu.roll(v, 4, 0))
    return op(v, pltpu.roll(v, 2, 0))


def _hedgehog(p):
    rows = [p[i:i + 8] for i in range(0, p.shape[0], 8)]
    hi = _pair_reduce(functools.reduce(jnp.maximum, rows), jnp.maximum)
    lo = _pair_reduce(functools.reduce(jnp.minimum, rows), jnp.minimum)
    ep = [jnp.exp2(r - hi) for r in rows]
    en = [jnp.exp2(lo - r) for r in rows]
    rp = _recip(_pair_reduce(functools.reduce(jnp.add, ep), jnp.add))
    rn = _recip(_pair_reduce(functools.reduce(jnp.add, en), jnp.add))
    return jnp.concatenate([e * rp for e in ep] + [e * rn for e in en], axis=0)


def _total(terms):
    return functools.reduce(jnp.add, terms)


_BLOCK_PAIRS = tuple(itertools.combinations(range(NB), 2))


def _kappa(i, j):
    return 1.0 / (LAMBDA[j] - LAMBDA[i])


def _others(j):
    return [i for i in range(NB) if i != j]


def _ahead_lhs(a, b):
    c = [b[j] + LAMBDA[j] * a[j] for j in range(NB)]
    return list(a) + [_kappa(i, j) * (c[i] + c[j]) for i, j in _BLOCK_PAIRS]


def _ahead_sums(product):
    y = [None] * NB
    for i in range(NB):
        y[i] = product(i) if y[i] is None else y[i] + product(i)
        for j in range(i + 1, NB):
            t = product(NB + _BLOCK_PAIRS.index((i, j)))
            y[i], y[j] = y[i] + t, -t if y[j] is None else y[j] - t
    return y


def _step_lhs(x, i, j):
    t = x(j) if i == j else x(i) + x(j)
    return jnp.concatenate([t[:-16], t[-8:] + LAMBDA[j] * t[-16:-8]], axis=0)


class _StepSums:
    def __init__(self, ahead):
        self.y, self.w = list(ahead), [None] * NB

    def add(self, product, order):
        plus = lambda u, t: t if u is None else u + t
        for i, j in order:
            t = product(i, j)
            self.w[j] = plus(self.w[j], t)
            if i != j:
                g = _kappa(i, j) * t[-8:]
                self.y[j] = plus(self.y[j], g)
                self.y[i] = -g if self.y[i] is None else self.y[i] - g
        return self

    def columns(self):
        return [jnp.concatenate([w[:-8], y, w[-8:] - lam * y], axis=0)
                for w, y, lam in zip(self.w, self.y, LAMBDA)]


def _kernel(
    x_hbm, mem0_hbm, wq_hbm, wk_hbm, wv_hbm, wo_hbm, bqkv_hbm, wphi_hbm, bwo_hbm,
    out_hbm,
    mem0_ref, al_ref, xres_ref, hn_ref, wqkv_ref, rqkv_ref, wo_ref, ro_ref, ahead_ref,
    sel_ref, zero_ref,
    sem_x, sem_b, sem_w, sem_tok, sem_last, sem_out,
    *, seg, heads, dh,
):
    seq, dm = out_hbm.shape
    n_mem = mem0_ref.shape[0]
    n_seg = seq // seg
    rows = n_mem + seg
    pairs = heads // 2
    pw = 2 * dh
    off = -(-rows // 16) * 16
    scale = dh ** (-0.5)
    bdh = dm // B_HEADS
    grp = 2 * bdh
    n_grp = B_HEADS // 2
    n_set = pairs // NB
    last = pairs - 1
    tile = lambda k, n=128: slice(k * n, (k + 1) * n)
    of_set = lambda u: range(u * NB, (u + 1) * NB)

    def rows_of(j, n):
        return pl.ds(j * n if isinstance(j, int) else pl.multiple_of(j * n, n), n)

    def groups_of(kt):
        return range(128 * kt // grp, (128 * kt + 127) // grp + 1)

    def store_ahead_lhs(s, a, b):
        split = lambda t: [t[:, tile(k)] for k in range(NB)]
        for r, t in enumerate(_ahead_lhs(split(a), split(b))):
            al_ref[r, 4 * s:4 * s + t.shape[0] // 2] = _pack(t.astype(BF16))

    def project_ahead(m, u, product):
        n = n_seg * 8 // 2
        for c in range(pw // 128):
            for r0 in range(0, n_seg * 8, n):
                apply = lambda r: product(_unpack(al_ref[r, r0 // 2:(r0 + n) // 2]), r, tile(c))
                for j, y in enumerate(_ahead_sums(apply)):
                    ahead_ref[m * (pairs - 1) + u * NB + j, r0:r0 + n, tile(c)] = y

    def load(wphi_ref, xe_ref, xp_ref, stage_ref, out_stage_ref, last_ref, last_out_ref):
        cp_xe = pltpu.make_async_copy(x_hbm.at[:, pl.ds(seg // 8 - 2, 2)], xe_ref, sem_x.at[0])
        cp_mem0 = pltpu.make_async_copy(mem0_hbm, mem0_ref, sem_x.at[1])
        cp_wphi = pltpu.make_async_copy(wphi_hbm, wphi_ref, sem_x.at[2])

        weights = (wq_hbm, wk_hbm, wv_hbm)
        n_round = 3 * n_set
        x_segs = n_seg // (n_round - 1)
        plain = seg // 8 - 2

        def cp_set(m, u):
            return pltpu.make_async_copy(
                weights[m].at[rows_of(u, NB * pw)], stage_ref.at[u], sem_w.at[0, u])

        def cp_out_rows(t, u):
            return pltpu.make_async_copy(
                wo_hbm.at[pl.ds(u * NB, NB), t], out_stage_ref.at[u], sem_w.at[1, u])

        def cp_x(i):
            sl = pl.ds(i * x_segs, x_segs)
            return pltpu.make_async_copy(x_hbm.at[sl, pl.ds(0, plain)], xp_ref.at[sl], sem_tok.at[i])

        def cp_last(m):
            return pltpu.make_async_copy(weights[m].at[rows_of(last, pw)], last_ref.at[m], sem_last.at[m])

        cp_last_out = pltpu.make_async_copy(wo_hbm.at[last], last_out_ref, sem_last.at[3])

        def build_selectors():
            eh_r = _iota((B_HEADS, dm), 0)
            eh_c = _iota((B_HEADS, dm), 1)
            phi_f = None
            for d in range(bdh):
                eh = jnp.where(eh_c == eh_r * bdh + d, 1.0, 0.0).astype(BF16)
                t = _mm(wphi_ref[d], eh)
                phi_f = t if phi_f is None else phi_f + t
            pick = jnp.where((_iota((grp, bdh), 0) >> 1) == _iota((grp, bdh), 1), 1.0, 0.0)
            phi_rows = _mm(pick, phi_f.astype(BF16))
            r = _iota((grp, 128), 0)
            for kt in range(dm // 128):
                c = _iota((grp, 128), 1) + 128 * kt
                for i, g in enumerate(groups_of(kt)):
                    c0 = (2 * g + (r & 1)) * bdh
                    sel_ref[kt, i] = jnp.where(
                        (c >= c0) & (c < c0 + bdh), phi_rows[:, 128 * kt:128 * kt + 128], 0.0)

        def load_set(m, u):
            w = lambda use, i, j: stage_ref[u + zero_ref[use], tile(j, pw), tile(i)]
            f = lambda *a: w(*a).astype(F32)
            row = [_total([f(0, j, i) for i in range(NB)]).astype(BF16) for j in range(NB)]
            sym = [(f(1, i, j) + f(1, j, i)).astype(BF16) for i, j in _BLOCK_PAIRS]
            project_ahead(m, u, lambda t, r, c: _mm_nt(t, (row + sym)[r][c]))
            for j in range(NB):
                rqkv_ref[m * n_set + u, j] = _pack(row[j].T)
                diag = (f(2, j, j) - _total([f(2, i, j) for i in _others(j)])).astype(BF16)
                for i in range(NB):
                    t = diag if i == j else w(2, i, j)
                    wqkv_ref[m * pairs + u * NB + j, tile(i, 64)] = _pack(t.T)

        def load_out_rows(t, u):
            for r in range(0, 128, 16):
                w = {(i, j): out_stage_ref[u, i, r:r + 16, tile(j)]
                     for i in range(NB) for j in range(NB)}
                f = {ij: v.astype(F32) for ij, v in w.items()}
                packed = lambda k: rows_of(k * (dh // 8) + t * 8 + r // 16, 8)
                for j in range(NB):
                    ro_ref[j, packed(u)] = _pack(_total([f[j, i] for i in range(NB)]).astype(BF16))
                    w[j, j] = (f[j, j] - _total([f[i, j] for i in _others(j)])).astype(BF16)
                    for i in range(NB):
                        wo_ref[packed(u * NB + i), tile(j)] = _pack(w[i, j])

        def start_rows(s, k, x):
            x = x.astype(F32).reshape(-1, dm)
            h = _layernorm(x)
            for t in range(x.shape[0] // 8):
                sl = rows_of((s + t) * (seg // 8) + k, 8)
                xres_ref[sl] = x[tile(t, 8)]
                hn_ref[sl] = _pack(h[tile(t, 8)])
            return h

        for k in range(zero_ref.shape[0]):
            zero_ref[k] = 0
        for cp in (cp_wphi, cp_mem0, cp_xe):
            cp.start()
        cp_wphi.wait()
        cp_set(0, 0).start()
        build_selectors()
        cp_xe.wait()
        for cp in (cp_out_rows(0, 0), cp_x(0), cp_set(0, 1)):
            cp.start()
        for s in range(0, n_seg, x_segs):
            store_ahead_lhs(s, *(start_rows(s, plain + k, xe_ref[s:s + x_segs, k]) for k in range(2)))

        def following(m, u):
            wrap = u == n_set - 1
            return jnp.where(wrap, m + 1, m), jnp.where(wrap, 0, u + 1)

        def load_body(r, carry):
            before, now = carry
            after = following(*now)
            later = following(*after)
            side = jnp.maximum(r - 1, 0)
            cp_set(0, now[1]).wait()

            @pl.when(r != 1)
            def _():
                cp_out_rows(*before).wait()
                cp_x(side).wait()

            for m in range(3):
                pl.when(later[0] == m)(cp_set(m, later[1]).start)

            @pl.when(r + 2 < n_round)
            def _():
                cp_out_rows(*after).start()
                cp_x(r + 1).start()

            @pl.when(r + 2 == n_round)
            def _():
                for cp in [cp_out_rows(*after), cp_last_out] + [cp_last(m) for m in range(3)]:
                    cp.start()

            load_set(*now)
            load_out_rows(*before)
            for k in range(plain):
                start_rows(side * x_segs, k, xp_ref[pl.ds(side * x_segs, x_segs), k])
            return now, after

        lax.fori_loop(0, n_round, load_body, ((0, 0), (0, 0)))
        for cp in [cp_out_rows(2, n_set - 1), cp_last_out] + [cp_last(m) for m in range(3)]:
            cp.wait()
        for m in range(3):
            wqkv_ref[m * pairs + last] = _pack(last_ref[m].T)
        load_out_rows(2, n_set - 1)
        wo_ref[tile(last, dh)] = _pack(last_out_ref[...].reshape(pw, dm))
        cp_mem0.wait()

    def layers(ya_ref, o_ref, mem_ref, kt_ref, vb_ref, p_ref,
               bqkv_ref, bwo_ref, bq_ref, bkv_ref, bo_ref, ht_ref, ot_ref, kv_ref, z_ref, res_ref):
        cp_bqkv = pltpu.make_async_copy(bqkv_hbm, bqkv_ref, sem_b.at[0])
        cp_bwo = pltpu.make_async_copy(bwo_hbm, bwo_ref, sem_b.at[1])

        cut = dh % 128

        def stack(a, b):
            gap = jnp.zeros((off - rows, a.shape[1]), F32)
            tail = jnp.zeros((128 - off - rows, a.shape[1]), F32)
            return jnp.concatenate([a, gap, b, tail], axis=0).astype(BF16)

        def store_keys(j, t):
            outer = _pack(stack(t[:, 0:128], t[:, 256:384]).T)
            inner = _pack(stack(t[:, 128:256], t[:, 128:256]).T)
            low = _iota((64, 128), 1) < off
            kt_ref[j, 0:64] = jnp.where(low, outer, 0)
            kt_ref[j, 64:64 + cut // 2] = jnp.where(low[:cut // 2], inner[:cut // 2], 0)
            kt_ref[j, 64 + cut // 2:128] = jnp.where(low[cut // 2:], 0, inner[cut // 2:])
            kt_ref[j, 128:192] = jnp.where(low, 0, outer)

        def store_values(j, t):
            t = _pack(jnp.concatenate([t, jnp.zeros((off - rows, pw), F32)], axis=0).astype(BF16))
            low = _iota((off // 2, 128), 1) < cut
            vb_ref[j, 0:off // 2, 0:128] = t[:, 0:128]
            vb_ref[j, 0:off // 2, 128:256] = jnp.where(low, t[:, 128:256], 0)
            vb_ref[j, off // 2:off, 128:256] = jnp.where(low, 0, t[:, 128:256])
            vb_ref[j, off // 2:off, 256:384] = t[:, 256:384]

        def a_step(s):
            h = jnp.concatenate([mem_ref[...], pltpu.bitcast(hn_ref[rows_of(s, seg), :], F32)], axis=0)
            mine = rows_of(s, 8)
            qi = _iota((rows, 128), 0)
            ki = _iota((rows, 128), 1)
            in_a = ki < rows
            in_b = (ki >= off) & (ki < off + rows)
            see_a = in_a & ((qi < n_mem) | (qi >= ki))
            see_b = in_b & ((qi < n_mem) | (qi >= ki - off))
            fill_a = jnp.where(in_a, MASK_FILL, -jnp.inf)
            fill_b = jnp.where(in_b, MASK_FILL, -jnp.inf)
            by_column = [(i, j) for j in range(NB) for i in range(NB)]
            lhs = {(i, j): _step_lhs(lambda k: h[:, tile(k)], i, j) for i, j in by_column}

            def store_queries(j, t):
                o_ref[j] = t

            store = (store_queries, store_keys, store_values)

            def project(m, u, order=by_column):
                product = lambda i, j: _mm(
                    lhs[i, j], _unpack(wqkv_ref[m * pairs + u * NB + j, tile(i, 64)]))
                ahead = [ahead_ref[m * (pairs - 1) + u * NB + j, mine] for j in range(NB)]
                for j, t in zip(of_set(u), _StepSums(ahead).add(product, order).columns()):
                    store[m](j, t)

            def scores(j):
                sc = _mm(o_ref[j], _unpack(kt_ref[j])) * scale
                sa = jnp.where(see_a, sc, fill_a)
                sb = jnp.where(see_b, sc, fill_b)
                e = jnp.exp(jnp.maximum(sa - jnp.max(sa, axis=-1, keepdims=True),
                                        sb - jnp.max(sb, axis=-1, keepdims=True)))
                sum_a = jnp.sum(jnp.where(in_a, e, 0.0), axis=-1, keepdims=True)
                sum_b = jnp.sum(jnp.where(in_a, 0.0, e), axis=-1, keepdims=True)
                p_ref[j] = e * _recip(jnp.where(in_a, sum_a, sum_b))

            def attend(j):
                o = _mm(p_ref[j], _unpack(vb_ref[j]))
                o_ref[j] = o
                if j < last:
                    ahead_ref[j, mine] = o[-16:-8]
                    ahead_ref[last + j, mine] = o[-8:]

            out = _StepSums([None] * NB)

            def project_out(u):
                product = lambda i, j: _mm(
                    _step_lhs(lambda k: o_ref[u * NB + k], i, j),
                    _unpack(wo_ref[tile(u * NB + i, dh), tile(j)]))
                out.add(product, sorted(by_column, key=sorted))

            out_last = lambda c: _mm(o_ref[last], _unpack(wo_ref[tile(last, dh), tile(c)]))

            project(1, 0, sorted(by_column, key=lambda ij: max(2, *ij)))
            for m in (1, 0, 2):
                store[m](last, _mm(h, _unpack(wqkv_ref[m * pairs + last])))
            for m, u in ((1, 1), (1, 2), (0, 0), (2, 0), (0, 1), (2, 1), (0, 2)):
                project(m, u)
            ready = [*of_set(0), *of_set(1), last]
            for j in ready:
                scores(j)
            project(2, 2)
            for j in of_set(2):
                scores(j)
            for j in ready:
                attend(j)
            project_out(0)
            for j in of_set(2):
                attend(j)
            direct = [out_last(c) for c in range(NB - 1)]
            project_out(1)
            project_out(2)
            direct.append(out_last(NB - 1))
            y = jnp.concatenate([t + d for t, d in zip(out.columns(), direct)], axis=1)
            mem_ref[...] = y[:n_mem]
            ya_ref[s] = y[n_mem:].reshape(seg // 8, 8, dm)

        def a_start():
            group = lambda s, k: pltpu.bitcast(jnp.concatenate(
                [hn_ref[tile((t + 1) * (seg // 8) + k, 8)] for t in range(s, s + 8)], axis=0), F32)

            @pl.when(zero_ref[0] == 0)
            def _():
                for s in range(0, n_seg, 8):
                    store_ahead_lhs(s, group(s, -2), group(s, -1))

            def ahead_body(m, carry):
                for u in range(n_set):
                    block = lambda i, j: _unpack(
                        wqkv_ref[m * pairs + u * NB + j, tile(i, 64)]).astype(F32)
                    rhs = [_unpack(rqkv_ref[m * n_set + u, j]) for j in range(NB)]
                    rhs += [(block(i, j) + block(j, i)).astype(BF16) for i, j in _BLOCK_PAIRS]
                    project_ahead(m, u, lambda t, r, c: _mm(t, rhs[r][:, c]))
                return carry

            lax.fori_loop(0, 3, ahead_body, 0)

        def a_finish():
            block = lambda i, j: _unpack(jnp.concatenate(
                [wo_ref[tile(u * NB + i, dh), tile(j)] for u in range(n_set)], axis=0)).astype(F32)
            rhs = [_unpack(ro_ref[j]) for j in range(NB)]
            rhs += [(block(i, j) + block(j, i)).astype(BF16) for i, j in _BLOCK_PAIRS]
            n = n_seg // 4
            for s0 in range(0, n_seg, n):
                side = lambda p: jnp.concatenate(
                    [ahead_ref[p + u * NB, s0 * 8:(s0 + n) * 8] for u in range(n_set)], axis=1)
                lhs = _ahead_lhs([side(k) for k in range(NB)], [side(last + k) for k in range(NB)])
                for j, y in enumerate(_ahead_sums(lambda r: _mm(lhs[r], rhs[r]))):
                    y = y.reshape(n, 8, 128)
                    ya_ref[s0:s0 + n, seg // 8 - 2, :, tile(j)] += y
                    ya_ref[s0:s0 + n, seg // 8 - 1, :, tile(j)] -= LAMBDA[j] * y

        def a_layer(first_layer):
            n_loop = n_seg // UNROLL

            def a_body(i, carry):
                for k in range(UNROLL):
                    a_step(i * UNROLL + k)
                return carry

            if first_layer:
                vb_ref[...] = jnp.zeros(vb_ref.shape, U32)
                cp_bqkv.start()
                cp_bwo.start()
            else:
                a_start()
            mem_ref[...] = mem0_ref[...].astype(F32)
            lax.fori_loop(0, n_loop, a_body, 0)
            if first_layer:
                cp_bqkv.wait()
                cp_bwo.wait()
                b_fold_weights()
            for s in range(n_loop * UNROLL, n_seg):
                a_step(s)
            a_finish()

        def b_fold_weights():
            def fold(m):
                out = {}
                for kt in range(dm // 128):
                    gs = groups_of(kt)
                    block = jnp.concatenate([sel_ref[kt, i] for i in range(len(gs))], axis=0)
                    part = _mm_nt(block, bqkv_ref[:, m * dm + 128 * kt:m * dm + 128 * kt + 128])
                    for i, g in enumerate(gs):
                        t = part[i * grp:(i + 1) * grp]
                        out[g] = out[g] + t if g in out else t
                return [out[g] * LOG2E for g in range(n_grp)]

            def store(ref, blocks):
                for i in range(0, len(blocks), 2):
                    two = jnp.concatenate(blocks[i:i + 2], axis=0).astype(BF16)
                    ref[i * bdh:(i + 2) * bdh, :] = _pack(two)

            wk = fold(1)
            wv = bqkv_ref[:, 2 * dm:3 * dm].T.astype(F32)
            store(bkv_ref, [w for g in range(n_grp) for w in (wk[g], wv[g * grp:(g + 1) * grp])])
            store(bq_ref, fold(0))
            bo_ref[...] = _pack(bwo_ref[...])

        def b_kv():
            n_chunk = seq // KV_CHUNK
            tokens = lambda i: slice(i * KV_CHUNK, (i + 1) * KV_CHUNK)

            def normalize(i):
                xn = xres_ref[tokens(i), :] + ya_ref[tile(i, KV_CHUNK // seg)].reshape(KV_CHUNK, dm)
                xres_ref[tokens(i), :] = xn
                ht_ref[:, tokens(i)] = _pack(_layernorm(xn).astype(BF16).T)

            work = [(i, g) for i in range(n_chunk) for g in range(n_grp)]
            ready = {}
            normalize(0)
            for n in range(len(work) + KV_LAG):
                if n < len(work):
                    i, g = work[n]
                    if g == 0 and i + 1 < n_chunk:
                        normalize(i + 1)
                    t = _mm(_unpack(bkv_ref[g * grp:(g + 1) * grp, :]), _unpack(ht_ref[:, tokens(i)]))
                    phi = _hedgehog(t[:grp])
                    ready[n] = (t[grp:], phi.astype(BF16))
                    z = phi if i == 0 else z_ref[g] + phi
                    if i == n_chunk - 1:
                        z = jnp.broadcast_to(jnp.sum(z, axis=-1, keepdims=True), z.shape)
                    z_ref[g] = z
                if n >= KV_LAG:
                    i, g = work[n - KV_LAG]
                    t = _mm_nt(*ready.pop(n - KV_LAG))
                    if i > 0:
                        t = kv_ref[g] + t
                    if i == n_chunk - 1:
                        second = (_iota(t.shape, 1) & 1) == 1
                        t = jnp.where((_iota(t.shape, 0) >= bdh) == second, t, 0.0)
                    kv_ref[g] = t

        n_chunk = seq // CHUNK
        tokens = lambda i: slice(i * CHUNK, (i + 1) * CHUNK)

        def cp_out(i):
            return pltpu.make_async_copy(res_ref.at[tokens(i)], out_hbm.at[tokens(i)], sem_out.at[i])

        def b_out(last_layer):
            zero = zero_ref[0]
            half = n_grp // 2
            n_sub = CHUNK // SUB
            work = [(i, gg) for i in range(n_chunk) for gg in range(half)]
            ready = {}

            def staged(i, r0, n):
                return pl.ds(pl.multiple_of(zero + seq + (i % 2) * (CHUNK // 2) + r0, 8), n)

            def features(g, p):
                phi = _hedgehog(p)
                t = phi * jnp.concatenate([z_ref[g]] * (CHUNK // 128), axis=1)
                den = functools.reduce(jnp.add, [t[r:r + 8] for r in range(0, 2 * grp, 8)])
                inv = _recip(_pair_reduce(den, jnp.add) + DEN_EPS)
                other = pltpu.roll(inv, 1, 0)
                r = _iota(inv.shape, 0)
                return phi.astype(BF16), jnp.concatenate(
                    [jnp.where((r + r0 >= bdh) == ((r & 1) == 1), inv, other) for r0 in range(0, grp, 8)],
                    axis=0)

            finished = []

            def normalize():
                sl = finished.pop(0)
                hn_ref[sl, :] = _pack(_layernorm(xres_ref[sl, :]))

            def finish(i, k):
                if len(finished) > LN_LAG:
                    normalize()
                sl = slice(i * CHUNK + k * SUB, i * CHUNK + (k + 1) * SUB)
                o = _unpack(hn_ref[staged(i, k * SUB // 2, SUB // 2), :])
                xn = xres_ref[sl, :] + _mm(o, _unpack(bo_ref[...]))
                if last_layer:
                    res_ref[sl, :] = xn.astype(BF16)
                    if k == n_sub - 1:
                        cp_out(i).start()
                else:
                    xres_ref[sl, :] = xn
                    finished.append(sl)

            pending = []
            for n in range(len(work) + B_LAG):
                if n < len(work):
                    i, gg = work[n]
                    t = _mm(_unpack(bq_ref[gg * grp:(gg + 1) * grp, :]), _unpack(ht_ref[:, tokens(i)]))
                    ready[n] = [features(2 * gg + k, t[k * grp:(k + 1) * grp]) for k in range(2)]
                while pending and pending[0][0] <= n:
                    finish(*pending.pop(0)[1:])
                if n >= B_LAG:
                    i, gg = work[n - B_LAG]
                    for k, (phi, inv) in enumerate(ready.pop(n - B_LAG)):
                        g = 2 * gg + k
                        ot_ref[g * grp:(g + 1) * grp, :] = _mm(kv_ref[g], phi) * inv
                    if gg == half - 1:
                        hn_ref[staged(i, 0, CHUNK // 2), :] = _pack(ot_ref[...].astype(BF16).T)
                        pending += [(n + OUT_LAG + k * half // n_sub, i, k) for k in range(n_sub)]
            for _, i, k in pending:
                finish(i, k)
            while finished:
                normalize()

        a_layer(True)
        with jax.named_scope("L_b_kv"):
            b_kv()
        with jax.named_scope("L_b_out"):
            b_out(False)
        a_layer(False)
        with jax.named_scope("L_b_kv"):
            b_kv()
        with jax.named_scope("L_b_out"):
            b_out(True)
        for i in range(n_chunk):
            cp_out(i).wait()

    pl.run_scoped(
        load,
        pltpu.VMEM((bdh, bdh, B_HEADS), BF16),
        pltpu.VMEM((n_seg, 2, 8, dm), BF16),
        pltpu.VMEM((n_seg, seg // 8 - 2, 8, dm), BF16),
        pltpu.VMEM((RING, NB * pw, dm), BF16),
        pltpu.VMEM((RING, NB, 128, dm), BF16),
        pltpu.VMEM((3, pw, dm), BF16),
        pltpu.VMEM((pw // 128, 128, dm), BF16),
    )
    pl.run_scoped(
        layers,
        pltpu.VMEM((n_seg, seg // 8, 8, dm), F32),
        pltpu.VMEM((pairs, rows, pw), F32),
        pltpu.VMEM((n_mem, dm), F32),
        pltpu.VMEM((pairs, dh, 128), U32),
        pltpu.VMEM((pairs, 64, pw), U32),
        pltpu.VMEM((pairs, rows, 128), F32),
        pltpu.VMEM((dm, 3 * dm), BF16),
        pltpu.VMEM((dm, dm), BF16),
        pltpu.VMEM((dm // 2, dm), U32),
        pltpu.VMEM((dm, dm), U32),
        pltpu.VMEM((dm // 2, dm), U32),
        pltpu.VMEM((dm // 2, seq), U32),
        pltpu.VMEM((dm, CHUNK), F32),
        pltpu.VMEM((n_grp, grp, 2 * grp), F32),
        pltpu.VMEM((n_grp, 2 * grp, 128), F32),
        pltpu.VMEM((seq, dm), BF16),
    )


@functools.partial(jax.jit, static_argnames=("A_seg_len",))
def pallas_interleave_layers__memory_aug_recurrent_mem_tr__linear_kernel_hedgehog__prompt_kernel(
    A_x: jax.Array,
    A_mem0: jax.Array,
    A_Wq: jax.Array,
    A_Wk: jax.Array,
    A_Wv: jax.Array,
    A_Wo: jax.Array,
    A_seg_len: int,
    B_x: jax.Array,
    B_wqkv: jax.Array,
    B_w_phi: jax.Array,
    B_wo: jax.Array,
):
    del B_x
    batch, seq, dm = A_x.shape
    _, heads, dh = A_Wq.shape
    n_mem = A_mem0.shape[1]
    seg = int(A_seg_len)
    n_seg = seq // seg
    rows = n_mem + seg
    pw = 2 * dh
    pairs = heads // 2
    bdh = dm // B_HEADS
    assert batch == 1 and seq % CHUNK == 0 and KV_CHUNK % seg == 0 and seg % 8 == 0 and seg > 16
    assert n_mem % 8 == 0 and rows <= 48
    assert heads % 2 == 0 and pw == 3 * 128 and dm == NB * 128 and pairs == RING * NB + 1 and (2 * bdh) % 8 == 0

    w_t = lambda w: jnp.transpose(w, (1, 2, 0)).reshape(heads * dh, dm)
    hbm = pl.BlockSpec(memory_space=pl.ANY)

    out = pl.pallas_call(
        functools.partial(_kernel, seg=seg, heads=heads, dh=dh),
        out_shape=jax.ShapeDtypeStruct((seq, dm), A_x.dtype),
        in_specs=[hbm] * 9,
        out_specs=hbm,
        scratch_shapes=[
            pltpu.VMEM((n_mem, dm), BF16),
            pltpu.VMEM((NB + len(_BLOCK_PAIRS), n_seg * 4, 128), U32),
            pltpu.VMEM((seq, dm), F32),
            pltpu.VMEM((seq + CHUNK, dm), U32),
            pltpu.VMEM((3 * pairs, dm // 2, pw), U32),
            pltpu.VMEM((3 * RING, NB, 64, pw), U32),
            pltpu.VMEM((pairs * dh, dm), U32),
            pltpu.VMEM((NB, RING * dh, 128), U32),
            pltpu.VMEM((3 * (pairs - 1), n_seg * 8, pw), F32),
            pltpu.VMEM((dm // 128, 127 // (2 * bdh) + 2, 2 * bdh, 128), F32),
            pltpu.SMEM((3,), jnp.int32),
            pltpu.SemaphoreType.DMA((3,)),
            pltpu.SemaphoreType.DMA((2,)),
            pltpu.SemaphoreType.DMA((2, RING)),
            pltpu.SemaphoreType.DMA((3 * RING - 1,)),
            pltpu.SemaphoreType.DMA((4,)),
            pltpu.SemaphoreType.DMA((seq // CHUNK,)),
        ],
        compiler_params=pltpu.CompilerParams(
            vmem_limit_bytes=126 * 1024 * 1024,
            flags={"XLA_TPU_EVENLY_DISTRIBUTE_CRITICAL_NODES": True},
        ),
    )(
        A_x.reshape(n_seg, seg // 8, 8, dm),
        A_mem0.reshape(n_mem, dm),
        w_t(A_Wq), w_t(A_Wk), w_t(A_Wv),
        A_Wo.reshape(pairs, pw // 128, 128, dm),
        B_wqkv,
        jnp.transpose(B_w_phi, (1, 2, 0)),
        B_wo,
    )
    return out.reshape(batch, seq, dm)
```

```python
import functools
import itertools

import jax
import jax.numpy as jnp
from jax import lax
import jax.experimental.pallas as pl
import jax.experimental.pallas.tpu as pltpu

F32 = jnp.float32
BF16 = jnp.bfloat16
U32 = jnp.uint32

B_HEADS = 32
LN_EPS = 1e-05
DEN_EPS = 1e-06
MASK_FILL = -1000000000.0
LOG2E = 1.4426950408889634

LAMBDA = (-1.75, -0.5625, 0.0, 0.5625, 1.75)
NB = len(LAMBDA)
UNROLL = 3
RING = 3
CHUNK = 256
B_LAG = 3
KV_CHUNK = 128
KV_LAG = 3
SUB = 64
OUT_LAG = 6
LN_LAG = 1

_NN = (((1,), (0,)), ((), ()))
_NT = (((1,), (1,)), ((), ()))


def _mm(a, b):
    return lax.dot_general(a, b, _NN, preferred_element_type=F32)


def _mm_nt(a, b):
    return lax.dot_general(a, b, _NT, preferred_element_type=F32)


def _pack(w):
    return pltpu.bitcast(w, U32)


def _unpack(w):
    return pltpu.bitcast(w, BF16)


def _iota(shape, dim):
    return lax.broadcasted_iota(jnp.int32, shape, dim)


def _recip(x):
    r = pltpu.reciprocal(x, approx=True)
    return r * (2.0 - x * r)


def _layernorm(x):
    m = jnp.mean(x, axis=-1, keepdims=True)
    xc = x - m
    v = jnp.mean(xc * xc, axis=-1, keepdims=True)
    return xc * lax.rsqrt(v + LN_EPS)


def _pair_reduce(v, op):
    v = op(v, pltpu.roll(v, 4, 0))
    return op(v, pltpu.roll(v, 2, 0))


def _hedgehog(p):
    rows = [p[i:i + 8] for i in range(0, p.shape[0], 8)]
    hi = _pair_reduce(functools.reduce(jnp.maximum, rows), jnp.maximum)
    lo = _pair_reduce(functools.reduce(jnp.minimum, rows), jnp.minimum)
    ep = [jnp.exp2(r - hi) for r in rows]
    en = [jnp.exp2(lo - r) for r in rows]
    rp = _recip(_pair_reduce(functools.reduce(jnp.add, ep), jnp.add))
    rn = _recip(_pair_reduce(functools.reduce(jnp.add, en), jnp.add))
    return jnp.concatenate([e * rp for e in ep] + [e * rn for e in en], axis=0)


def _total(terms):
    return functools.reduce(jnp.add, terms)


_BLOCK_PAIRS = tuple(itertools.combinations(range(NB), 2))


def _kappa(i, j):
    return 1.0 / (LAMBDA[j] - LAMBDA[i])


def _others(j):
    return [i for i in range(NB) if i != j]


def _ahead_lhs(a, b):
    c = [b[j] + LAMBDA[j] * a[j] for j in range(NB)]
    return list(a) + [_kappa(i, j) * (c[i] + c[j]) for i, j in _BLOCK_PAIRS]


def _ahead_sums(product):
    y = [None] * NB
    for i in range(NB):
        y[i] = product(i) if y[i] is None else y[i] + product(i)
        for j in range(i + 1, NB):
            t = product(NB + _BLOCK_PAIRS.index((i, j)))
            y[i], y[j] = y[i] + t, -t if y[j] is None else y[j] - t
    return y


def _step_lhs(x, i, j):
    t = x(j) if i == j else x(i) + x(j)
    return jnp.concatenate([t[:-16], t[-8:] + LAMBDA[j] * t[-16:-8]], axis=0)


class _StepSums:
    def __init__(self, ahead):
        self.y, self.w = list(ahead), [None] * NB

    def add(self, product, order):
        plus = lambda u, t: t if u is None else u + t
        for i, j in order:
            t = product(i, j)
            self.w[j] = plus(self.w[j], t)
            if i != j:
                g = _kappa(i, j) * t[-8:]
                self.y[j] = plus(self.y[j], g)
                self.y[i] = -g if self.y[i] is None else self.y[i] - g
        return self

    def columns(self):
        return [jnp.concatenate([w[:-8], y, w[-8:] - lam * y], axis=0)
                for w, y, lam in zip(self.w, self.y, LAMBDA)]


def _kernel(
    x_hbm, mem0_hbm, wq_hbm, wk_hbm, wv_hbm, wo_hbm, bqkv_hbm, wphi_hbm, bwo_hbm,
    out_hbm,
    mem0_ref, al_ref, xres_ref, hn_ref, wqkv_ref, wlast_ref, early_ref, rqkv_ref,
    wo_ref, ro_ref, ahead_ref,
    sel_ref, zero_ref,
    sem_x, sem_b, sem_w, sem_tok, sem_last, sem_out,
    *, seg, heads, dh,
):
    seq, dm = out_hbm.shape
    n_mem = mem0_ref.shape[0]
    n_seg = seq // seg
    rows = n_mem + seg
    pairs = heads // 2
    pw = 2 * dh
    off = -(-rows // 16) * 16
    scale = dh ** (-0.5)
    bdh = dm // B_HEADS
    grp = 2 * bdh
    n_grp = B_HEADS // 2
    n_set = pairs // NB
    last = pairs - 1
    tile = lambda k, n=128: slice(k * n, (k + 1) * n)
    of_set = lambda u: range(u * NB, (u + 1) * NB)

    def rows_of(j, n):
        return pl.ds(j * n if isinstance(j, int) else pl.multiple_of(j * n, n), n)

    def groups_of(kt):
        return range(128 * kt // grp, (128 * kt + 127) // grp + 1)

    def store_ahead_lhs(s, a, b):
        split = lambda t: [t[:, tile(k)] for k in range(NB)]
        for r, t in enumerate(_ahead_lhs(split(a), split(b))):
            al_ref[r, 4 * s:4 * s + t.shape[0] // 2] = _pack(t.astype(BF16))

    def project_ahead(m, u, product):
        n = n_seg * 8 // 2
        for c in range(pw // 128):
            for r0 in range(0, n_seg * 8, n):
                apply = lambda r: product(_unpack(al_ref[r, r0 // 2:(r0 + n) // 2]), r, tile(c))
                for j, y in enumerate(_ahead_sums(apply)):
                    ahead_ref[m * last + u * NB + j, r0:r0 + n, tile(c)] = y

    def load(wphi_ref, xe_ref, hb_ref, xp_ref, stage_ref, out_stage_ref, last_ref, last_out_ref):
        cp_xe = pltpu.make_async_copy(x_hbm.at[:, pl.ds(seg // 8 - 2, 2)], xe_ref, sem_x.at[0])
        cp_mem0 = pltpu.make_async_copy(mem0_hbm, mem0_ref, sem_x.at[1])
        cp_wphi = pltpu.make_async_copy(wphi_hbm, wphi_ref, sem_x.at[2])

        weights = (wq_hbm, wk_hbm, wv_hbm)
        n_round = 3 * n_set
        x_segs = n_seg // (n_round - 1)
        plain = seg // 8 - 2

        def cp_set(m, u):
            return pltpu.make_async_copy(
                weights[m].at[rows_of(u, NB * pw)], stage_ref.at[u], sem_w.at[0, u])

        def cp_out_rows(t, u):
            return pltpu.make_async_copy(
                wo_hbm.at[pl.ds(u * NB, NB), t], out_stage_ref.at[u], sem_w.at[1, u])

        def cp_x(i):
            sl = pl.ds(i * x_segs, x_segs)
            return pltpu.make_async_copy(x_hbm.at[sl, pl.ds(0, plain)], xp_ref.at[sl], sem_tok.at[i])

        def cp_last(m, c):
            return pltpu.make_async_copy(
                weights[m].at[rows_of(last * (pw // 128) + c, 128)], last_ref.at[c], sem_last.at[c])

        cp_last_out = pltpu.make_async_copy(wo_hbm.at[last], last_out_ref, sem_last.at[3])

        def build_selectors():
            eh_r = _iota((B_HEADS, dm), 0)
            eh_c = _iota((B_HEADS, dm), 1)
            phi_f = None
            for d in range(bdh):
                eh = jnp.where(eh_c == eh_r * bdh + d, 1.0, 0.0).astype(BF16)
                t = _mm(wphi_ref[d], eh)
                phi_f = t if phi_f is None else phi_f + t
            pick = jnp.where((_iota((grp, bdh), 0) >> 1) == _iota((grp, bdh), 1), 1.0, 0.0)
            phi_rows = _mm(pick, phi_f.astype(BF16))
            r = _iota((grp, 128), 0)
            for kt in range(dm // 128):
                c = _iota((grp, 128), 1) + 128 * kt
                for i, g in enumerate(groups_of(kt)):
                    c0 = (2 * g + (r & 1)) * bdh
                    sel_ref[kt, i] = jnp.where(
                        (c >= c0) & (c < c0 + bdh), phi_rows[:, 128 * kt:128 * kt + 128], 0.0)

        def load_set(m, u):
            w = lambda use, i, j: stage_ref[u + zero_ref[use], tile(j, pw), tile(i)]
            f = lambda *a: w(*a).astype(F32)
            row = [_total([f(0, j, i) for i in range(NB)]).astype(BF16) for j in range(NB)]
            sym = [(f(1, i, j) + f(1, j, i)).astype(BF16) for i, j in _BLOCK_PAIRS]
            project_ahead(m, u, lambda t, r, c: _mm_nt(t, (row + sym)[r][c]))
            for j in range(NB):
                rqkv_ref[m * n_set + u, j] = _pack(row[j].T)
                diag = (f(2, j, j) - _total([f(2, i, j) for i in _others(j)])).astype(BF16)
                for i in range(NB):
                    t = diag if i == j else w(2, i, j)
                    wqkv_ref[m * last + u * NB + j, tile(i, 64)] = _pack(t.T)

        def load_out_rows(t, u):
            for r in range(0, 128, 16):
                w = {(i, j): out_stage_ref[u, i, r:r + 16, tile(j)]
                     for i in range(NB) for j in range(NB)}
                f = {ij: v.astype(F32) for ij, v in w.items()}
                packed = lambda k: rows_of(k * (dh // 8) + t * 8 + r // 16, 8)
                for j in range(NB):
                    ro_ref[j, packed(u)] = _pack(_total([f[j, i] for i in range(NB)]).astype(BF16))
                    w[j, j] = (f[j, j] - _total([f[i, j] for i in _others(j)])).astype(BF16)
                    for i in range(NB):
                        wo_ref[packed(u * NB + i), tile(j)] = _pack(w[i, j])

        def start_rows(s, k, x):
            x = x.astype(F32).reshape(-1, dm)
            h = _layernorm(x)
            for t in range(x.shape[0] // 8):
                sl = rows_of((s + t) * (seg // 8) + k, 8)
                xres_ref[sl] = x[tile(t, 8)]
                hn_ref[sl] = _pack(h[tile(t, 8)])
            return h

        for k in range(zero_ref.shape[0]):
            zero_ref[k] = 0
        for cp in (cp_wphi, cp_mem0, cp_xe):
            cp.start()
        cp_wphi.wait()
        cp_set(0, 0).start()
        cp_last(0, 0).start()
        build_selectors()
        cp_xe.wait()
        for cp in (cp_out_rows(0, 0), cp_x(0), cp_set(0, 1), cp_last(0, 1)):
            cp.start()
        for s in range(0, n_seg, x_segs):
            a, b = (start_rows(s, plain + k, xe_ref[s:s + x_segs, k]) for k in range(2))
            store_ahead_lhs(s, a, b)
            hb_ref[4 * s:4 * (s + x_segs)] = _pack(b.astype(BF16))

        def following(m, u):
            wrap = u == n_set - 1
            return jnp.where(wrap, m + 1, m), jnp.where(wrap, 0, u + 1)

        def load_body(r, carry):
            before, now = carry
            after = following(*now)
            later = following(*after)
            side = jnp.maximum(r - 1, 0)
            cp_set(0, now[1]).wait()
            cp_last(0, now[1]).wait()

            @pl.when(r != 1)
            def _():
                cp_out_rows(*before).wait()
                cp_x(side).wait()

            for m in range(3):
                @pl.when(later[0] == m)
                def _():
                    cp_set(m, later[1]).start()
                    cp_last(m, later[1]).start()

            @pl.when(r + 2 < n_round)
            def _():
                cp_out_rows(*after).start()
                cp_x(r + 1).start()

            @pl.when(r + 2 == n_round)
            def _():
                cp_out_rows(*after).start()
                cp_last_out.start()

            w = last_ref[now[1]]
            early_ref[now[0], now[1]] = _mm_nt(_unpack(hb_ref[...]), w)
            wlast_ref[now[0], now[1]] = _pack(w.T)
            load_set(*now)
            load_out_rows(*before)
            for k in range(plain):
                start_rows(side * x_segs, k, xp_ref[pl.ds(side * x_segs, x_segs), k])
            return now, after

        lax.fori_loop(0, n_round, load_body, ((0, 0), (0, 0)))
        cp_out_rows(2, n_set - 1).wait()
        cp_last_out.wait()
        load_out_rows(2, n_set - 1)
        wo_ref[tile(last, dh)] = _pack(last_out_ref[...].reshape(pw, dm))
        cp_mem0.wait()

    def layers(ya_ref, o_ref, mem_ref, kt_ref, vb_ref, p_ref,
               bqkv_ref, bwo_ref, bq_ref, bkv_ref, bo_ref, ht_ref, ot_ref, kv_ref, z_ref, res_ref):
        cp_bqkv = pltpu.make_async_copy(bqkv_hbm, bqkv_ref, sem_b.at[0])
        cp_bwo = pltpu.make_async_copy(bwo_hbm, bwo_ref, sem_b.at[1])

        cut = dh % 128

        def stack(a, b):
            gap = jnp.zeros((off - rows, a.shape[1]), F32)
            tail = jnp.zeros((128 - off - rows, a.shape[1]), F32)
            return jnp.concatenate([a, gap, b, tail], axis=0).astype(BF16)

        def store_keys(j, t):
            outer = _pack(stack(t[:, 0:128], t[:, 256:384]).T)
            inner = _pack(stack(t[:, 128:256], t[:, 128:256]).T)
            low = _iota((64, 128), 1) < off
            kt_ref[j, 0:64] = jnp.where(low, outer, 0)
            kt_ref[j, 64:64 + cut // 2] = jnp.where(low[:cut // 2], inner[:cut // 2], 0)
            kt_ref[j, 64 + cut // 2:128] = jnp.where(low[cut // 2:], 0, inner[cut // 2:])
            kt_ref[j, 128:192] = jnp.where(low, 0, outer)

        def store_values(j, t):
            t = _pack(jnp.concatenate([t, jnp.zeros((off - rows, pw), F32)], axis=0).astype(BF16))
            low = _iota((off // 2, 128), 1) < cut
            vb_ref[j, 0:off // 2, 0:128] = t[:, 0:128]
            vb_ref[j, 0:off // 2, 128:256] = jnp.where(low, t[:, 128:256], 0)
            vb_ref[j, off // 2:off, 128:256] = jnp.where(low, 0, t[:, 128:256])
            vb_ref[j, off // 2:off, 256:384] = t[:, 256:384]

        def a_step(s, first_layer):
            h = jnp.concatenate([mem_ref[...], pltpu.bitcast(hn_ref[rows_of(s, seg), :], F32)], axis=0)
            mine = rows_of(s, 8)
            qi = _iota((rows, 128), 0)
            ki = _iota((rows, 128), 1)
            in_a = ki < rows
            in_b = (ki >= off) & (ki < off + rows)
            see_a = in_a & ((qi < n_mem) | (qi >= ki))
            see_b = in_b & ((qi < n_mem) | (qi >= ki - off))
            fill_a = jnp.where(in_a, MASK_FILL, -jnp.inf)
            fill_b = jnp.where(in_b, MASK_FILL, -jnp.inf)
            by_column = [(i, j) for j in range(NB) for i in range(NB)]
            lhs = {(i, j): _step_lhs(lambda k: h[:, tile(k)], i, j) for i, j in by_column}

            def store_queries(j, t):
                o_ref[j] = t

            store = (store_queries, store_keys, store_values)

            def project(m, u, order=by_column):
                product = lambda i, j: _mm(
                    lhs[i, j], _unpack(wqkv_ref[m * last + u * NB + j, tile(i, 64)]))
                ahead = [ahead_ref[m * last + u * NB + j, mine] for j in range(NB)]
                for j, t in zip(of_set(u), _StepSums(ahead).add(product, order).columns()):
                    store[m](j, t)

            def scores(j):
                sc = _mm(o_ref[j], _unpack(kt_ref[j])) * scale
                sa = jnp.where(see_a, sc, fill_a)
                sb = jnp.where(see_b, sc, fill_b)
                e = jnp.exp(jnp.maximum(sa - jnp.max(sa, axis=-1, keepdims=True),
                                        sb - jnp.max(sb, axis=-1, keepdims=True)))
                sum_a = jnp.sum(jnp.where(in_a, e, 0.0), axis=-1, keepdims=True)
                sum_b = jnp.sum(jnp.where(in_a, 0.0, e), axis=-1, keepdims=True)
                p_ref[j] = e * _recip(jnp.where(in_a, sum_a, sum_b))

            def attend(j):
                o = _mm(p_ref[j], _unpack(vb_ref[j]))
                o_ref[j] = o
                if j < last:
                    ahead_ref[j, mine] = o[-16:-8]
                    ahead_ref[last + j, mine] = o[-8:]

            out = _StepSums([None] * NB)

            def project_out(u):
                product = lambda i, j: _mm(
                    _step_lhs(lambda k: o_ref[u * NB + k], i, j),
                    _unpack(wo_ref[tile(u * NB + i, dh), tile(j)]))
                out.add(product, sorted(by_column, key=sorted))

            out_last = lambda c: _mm(o_ref[last], _unpack(wo_ref[tile(last, dh), tile(c)]))

            project(1, 0, sorted(by_column, key=lambda ij: max(2, *ij)))
            for m in (1, 0, 2):
                w = _unpack(jnp.concatenate([wlast_ref[m, c] for c in range(pw // 128)], axis=1))
                if first_layer:
                    done = jnp.concatenate([early_ref[m, c, mine] for c in range(pw // 128)], axis=1)
                    store[m](last, jnp.concatenate([_mm(h[:-8], w), done], axis=0))
                else:
                    store[m](last, _mm(h, w))
            for m, u in ((1, 1), (1, 2), (0, 0), (2, 0), (0, 1), (2, 1), (0, 2)):
                project(m, u)
            ready = [*of_set(0), *of_set(1), last]
            for j in ready:
                scores(j)
            project(2, 2)
            for j in of_set(2):
                scores(j)
            for j in ready:
                attend(j)
            project_out(0)
            for j in of_set(2):
                attend(j)
            direct = [out_last(c) for c in range(NB - 1)]
            project_out(1)
            project_out(2)
            direct.append(out_last(NB - 1))
            y = jnp.concatenate([t + d for t, d in zip(out.columns(), direct)], axis=1)
            mem_ref[...] = y[:n_mem]
            ya_ref[s] = y[n_mem:].reshape(seg // 8, 8, dm)

        def a_start():
            group = lambda s, k: pltpu.bitcast(jnp.concatenate(
                [hn_ref[tile((t + 1) * (seg // 8) + k, 8)] for t in range(s, s + 8)], axis=0), F32)

            @pl.when(zero_ref[0] == 0)
            def _():
                for s in range(0, n_seg, 8):
                    store_ahead_lhs(s, group(s, -2), group(s, -1))

            def ahead_body(m, carry):
                for u in range(n_set):
                    block = lambda i, j: _unpack(
                        wqkv_ref[m * last + u * NB + j, tile(i, 64)]).astype(F32)
                    rhs = [_unpack(rqkv_ref[m * n_set + u, j]) for j in range(NB)]
                    rhs += [(block(i, j) + block(j, i)).astype(BF16) for i, j in _BLOCK_PAIRS]
                    project_ahead(m, u, lambda t, r, c: _mm(t, rhs[r][:, c]))
                return carry

            lax.fori_loop(0, 3, ahead_body, 0)

        def a_finish():
            block = lambda i, j: _unpack(jnp.concatenate(
                [wo_ref[tile(u * NB + i, dh), tile(j)] for u in range(n_set)], axis=0)).astype(F32)
            rhs = [_unpack(ro_ref[j]) for j in range(NB)]
            rhs += [(block(i, j) + block(j, i)).astype(BF16) for i, j in _BLOCK_PAIRS]
            n = n_seg // 4
            for s0 in range(0, n_seg, n):
                side = lambda p: jnp.concatenate(
                    [ahead_ref[p + u * NB, s0 * 8:(s0 + n) * 8] for u in range(n_set)], axis=1)
                lhs = _ahead_lhs([side(k) for k in range(NB)], [side(last + k) for k in range(NB)])
                for j, y in enumerate(_ahead_sums(lambda r: _mm(lhs[r], rhs[r]))):
                    y = y.reshape(n, 8, 128)
                    ya_ref[s0:s0 + n, seg // 8 - 2, :, tile(j)] += y
                    ya_ref[s0:s0 + n, seg // 8 - 1, :, tile(j)] -= LAMBDA[j] * y

        def a_layer(first_layer):
            n_loop = n_seg // UNROLL

            def a_body(i, carry):
                for k in range(UNROLL):
                    a_step(i * UNROLL + k, first_layer)
                return carry

            if first_layer:
                vb_ref[...] = jnp.zeros(vb_ref.shape, U32)
                cp_bqkv.start()
                cp_bwo.start()
            else:
                a_start()
            mem_ref[...] = mem0_ref[...].astype(F32)
            lax.fori_loop(0, n_loop, a_body, 0)
            if first_layer:
                cp_bqkv.wait()
                cp_bwo.wait()
                b_fold_weights()
            for s in range(n_loop * UNROLL, n_seg):
                a_step(s, first_layer)
            a_finish()

        def b_fold_weights():
            def fold(m):
                out = {}
                for kt in range(dm // 128):
                    gs = groups_of(kt)
                    block = jnp.concatenate([sel_ref[kt, i] for i in range(len(gs))], axis=0)
                    part = _mm_nt(block, bqkv_ref[:, m * dm + 128 * kt:m * dm + 128 * kt + 128])
                    for i, g in enumerate(gs):
                        t = part[i * grp:(i + 1) * grp]
                        out[g] = out[g] + t if g in out else t
                return [out[g] * LOG2E for g in range(n_grp)]

            def store(ref, blocks):
                for i in range(0, len(blocks), 2):
                    two = jnp.concatenate(blocks[i:i + 2], axis=0).astype(BF16)
                    ref[i * bdh:(i + 2) * bdh, :] = _pack(two)

            wk = fold(1)
            wv = bqkv_ref[:, 2 * dm:3 * dm].T.astype(F32)
            store(bkv_ref, [w for g in range(n_grp) for w in (wk[g], wv[g * grp:(g + 1) * grp])])
            store(bq_ref, fold(0))
            bo_ref[...] = _pack(bwo_ref[...])

        def b_kv():
            n_chunk = seq // KV_CHUNK
            tokens = lambda i: slice(i * KV_CHUNK, (i + 1) * KV_CHUNK)

            def normalize(i):
                xn = xres_ref[tokens(i), :] + ya_ref[tile(i, KV_CHUNK // seg)].reshape(KV_CHUNK, dm)
                xres_ref[tokens(i), :] = xn
                ht_ref[:, tokens(i)] = _pack(_layernorm(xn).astype(BF16).T)

            work = [(i, g) for i in range(n_chunk) for g in range(n_grp)]
            ready = {}
            normalize(0)
            for n in range(len(work) + KV_LAG):
                if n < len(work):
                    i, g = work[n]
                    if g == 0 and i + 1 < n_chunk:
                        normalize(i + 1)
                    t = _mm(_unpack(bkv_ref[g * grp:(g + 1) * grp, :]), _unpack(ht_ref[:, tokens(i)]))
                    phi = _hedgehog(t[:grp])
                    ready[n] = (t[grp:], phi.astype(BF16))
                    z = phi if i == 0 else z_ref[g] + phi
                    if i == n_chunk - 1:
                        z = jnp.broadcast_to(jnp.sum(z, axis=-1, keepdims=True), z.shape)
                    z_ref[g] = z
                if n >= KV_LAG:
                    i, g = work[n - KV_LAG]
                    t = _mm_nt(*ready.pop(n - KV_LAG))
                    if i > 0:
                        t = kv_ref[g] + t
                    if i == n_chunk - 1:
                        second = (_iota(t.shape, 1) & 1) == 1
                        t = jnp.where((_iota(t.shape, 0) >= bdh) == second, t, 0.0)
                    kv_ref[g] = t

        n_chunk = seq // CHUNK
        tokens = lambda i: slice(i * CHUNK, (i + 1) * CHUNK)

        def cp_out(i):
            return pltpu.make_async_copy(res_ref.at[tokens(i)], out_hbm.at[tokens(i)], sem_out.at[i])

        def b_out(last_layer):
            zero = zero_ref[0]
            half = n_grp // 2
            n_sub = CHUNK // SUB
            work = [(i, gg) for i in range(n_chunk) for gg in range(half)]
            ready = {}

            def staged(i, r0, n):
                return pl.ds(pl.multiple_of(zero + seq + (i % 2) * (CHUNK // 2) + r0, 8), n)

            def features(g, p):
                phi = _hedgehog(p)
                t = phi * jnp.concatenate([z_ref[g]] * (CHUNK // 128), axis=1)
                den = functools.reduce(jnp.add, [t[r:r + 8] for r in range(0, 2 * grp, 8)])
                inv = _recip(_pair_reduce(den, jnp.add) + DEN_EPS)
                other = pltpu.roll(inv, 1, 0)
                r = _iota(inv.shape, 0)
                return phi.astype(BF16), jnp.concatenate(
                    [jnp.where((r + r0 >= bdh) == ((r & 1) == 1), inv, other) for r0 in range(0, grp, 8)],
                    axis=0)

            finished = []

            def normalize():
                sl = finished.pop(0)
                hn_ref[sl, :] = _pack(_layernorm(xres_ref[sl, :]))

            def finish(i, k):
                if len(finished) > LN_LAG:
                    normalize()
                sl = slice(i * CHUNK + k * SUB, i * CHUNK + (k + 1) * SUB)
                o = _unpack(hn_ref[staged(i, k * SUB // 2, SUB // 2), :])
                xn = xres_ref[sl, :] + _mm(o, _unpack(bo_ref[...]))
                if last_layer:
                    res_ref[sl, :] = xn.astype(BF16)
                    if k == n_sub - 1:
                        cp_out(i).start()
                else:
                    xres_ref[sl, :] = xn
                    finished.append(sl)

            pending = []
            for n in range(len(work) + B_LAG):
                if n < len(work):
                    i, gg = work[n]
                    t = _mm(_unpack(bq_ref[gg * grp:(gg + 1) * grp, :]), _unpack(ht_ref[:, tokens(i)]))
                    ready[n] = [features(2 * gg + k, t[k * grp:(k + 1) * grp]) for k in range(2)]
                while pending and pending[0][0] <= n:
                    finish(*pending.pop(0)[1:])
                if n >= B_LAG:
                    i, gg = work[n - B_LAG]
                    for k, (phi, inv) in enumerate(ready.pop(n - B_LAG)):
                        g = 2 * gg + k
                        ot_ref[g * grp:(g + 1) * grp, :] = _mm(kv_ref[g], phi) * inv
                    if gg == half - 1:
                        hn_ref[staged(i, 0, CHUNK // 2), :] = _pack(ot_ref[...].astype(BF16).T)
                        pending += [(n + OUT_LAG + k * half // n_sub, i, k) for k in range(n_sub)]
            for _, i, k in pending:
                finish(i, k)
            while finished:
                normalize()

        a_layer(True)
        b_kv()
        b_out(False)
        a_layer(False)
        b_kv()
        b_out(True)
        for i in range(n_chunk):
            cp_out(i).wait()

    pl.run_scoped(
        load,
        pltpu.VMEM((bdh, bdh, B_HEADS), BF16),
        pltpu.VMEM((n_seg, 2, 8, dm), BF16),
        pltpu.VMEM((n_seg * 4, dm), U32),
        pltpu.VMEM((n_seg, seg // 8 - 2, 8, dm), BF16),
        pltpu.VMEM((RING, NB * pw, dm), BF16),
        pltpu.VMEM((RING, NB, 128, dm), BF16),
        pltpu.VMEM((pw // 128, 128, dm), BF16),
        pltpu.VMEM((pw // 128, 128, dm), BF16),
    )
    pl.run_scoped(
        layers,
        pltpu.VMEM((n_seg, seg // 8, 8, dm), F32),
        pltpu.VMEM((pairs, rows, pw), F32),
        pltpu.VMEM((n_mem, dm), F32),
        pltpu.VMEM((pairs, dh, 128), U32),
        pltpu.VMEM((pairs, 64, pw), U32),
        pltpu.VMEM((pairs, rows, 128), F32),
        pltpu.VMEM((dm, 3 * dm), BF16),
        pltpu.VMEM((dm, dm), BF16),
        pltpu.VMEM((dm // 2, dm), U32),
        pltpu.VMEM((dm, dm), U32),
        pltpu.VMEM((dm // 2, dm), U32),
        pltpu.VMEM((dm // 2, seq), U32),
        pltpu.VMEM((dm, CHUNK), F32),
        pltpu.VMEM((n_grp, grp, 2 * grp), F32),
        pltpu.VMEM((n_grp, 2 * grp, 128), F32),
        pltpu.VMEM((seq, dm), BF16),
    )


@functools.partial(jax.jit, static_argnames=("A_seg_len",))
def pallas_interleave_layers__memory_aug_recurrent_mem_tr__linear_kernel_hedgehog__prompt_kernel(
    A_x: jax.Array,
    A_mem0: jax.Array,
    A_Wq: jax.Array,
    A_Wk: jax.Array,
    A_Wv: jax.Array,
    A_Wo: jax.Array,
    A_seg_len: int,
    B_x: jax.Array,
    B_wqkv: jax.Array,
    B_w_phi: jax.Array,
    B_wo: jax.Array,
):
    del B_x
    batch, seq, dm = A_x.shape
    _, heads, dh = A_Wq.shape
    n_mem = A_mem0.shape[1]
    seg = int(A_seg_len)
    n_seg = seq // seg
    rows = n_mem + seg
    pw = 2 * dh
    pairs = heads // 2
    bdh = dm // B_HEADS
    assert n_seg % 16 == 0
    assert batch == 1 and seq % CHUNK == 0 and KV_CHUNK % seg == 0 and seg % 8 == 0 and seg > 16
    assert n_mem % 8 == 0 and rows <= 48
    assert heads % 2 == 0 and pw == 3 * 128 and dm == NB * 128 and pairs == RING * NB + 1 and (2 * bdh) % 8 == 0

    w_t = lambda w: jnp.transpose(w, (1, 2, 0)).reshape(heads * dh, dm)
    hbm = pl.BlockSpec(memory_space=pl.ANY)

    out = pl.pallas_call(
        functools.partial(_kernel, seg=seg, heads=heads, dh=dh),
        out_shape=jax.ShapeDtypeStruct((seq, dm), A_x.dtype),
        in_specs=[hbm] * 9,
        out_specs=hbm,
        scratch_shapes=[
            pltpu.VMEM((n_mem, dm), BF16),
            pltpu.VMEM((NB + len(_BLOCK_PAIRS), n_seg * 4, 128), U32),
            pltpu.VMEM((seq, dm), F32),
            pltpu.VMEM((seq + CHUNK, dm), U32),
            pltpu.VMEM((3 * (pairs - 1), dm // 2, pw), U32),
            pltpu.VMEM((3, pw // 128, dm // 2, 128), U32),
            pltpu.VMEM((3, pw // 128, n_seg * 8, 128), F32),
            pltpu.VMEM((3 * RING, NB, 64, pw), U32),
            pltpu.VMEM((pairs * dh, dm), U32),
            pltpu.VMEM((NB, RING * dh, 128), U32),
            pltpu.VMEM((3 * (pairs - 1), n_seg * 8, pw), F32),
            pltpu.VMEM((dm // 128, 127 // (2 * bdh) + 2, 2 * bdh, 128), F32),
            pltpu.SMEM((3,), jnp.int32),
            pltpu.SemaphoreType.DMA((3,)),
            pltpu.SemaphoreType.DMA((2,)),
            pltpu.SemaphoreType.DMA((2, RING)),
            pltpu.SemaphoreType.DMA((3 * RING - 1,)),
            pltpu.SemaphoreType.DMA((4,)),
            pltpu.SemaphoreType.DMA((seq // CHUNK,)),
        ],
        compiler_params=pltpu.CompilerParams(
            vmem_limit_bytes=126 * 1024 * 1024,
            flags={"XLA_TPU_EVENLY_DISTRIBUTE_CRITICAL_NODES": True},
        ),
    )(
        A_x.reshape(n_seg, seg // 8, 8, dm),
        A_mem0.reshape(n_mem, dm),
        w_t(A_Wq), w_t(A_Wk), w_t(A_Wv),
        A_Wo.reshape(pairs, pw // 128, 128, dm),
        B_wqkv,
        jnp.transpose(B_w_phi, (1, 2, 0)),
        B_wo,
    )
    return out.reshape(batch, seq, dm)
```

```python
import functools
import itertools

import jax
import jax.numpy as jnp
from jax import lax
import jax.experimental.pallas as pl
import jax.experimental.pallas.tpu as pltpu

F32 = jnp.float32
BF16 = jnp.bfloat16
U32 = jnp.uint32

B_HEADS = 32
LN_EPS = 1e-05
DEN_EPS = 1e-06
MASK_FILL = -1000000000.0
LOG2E = 1.4426950408889634

LAMBDA = (-1.75, -0.5625, 0.0, 0.5625, 1.75)
NB = len(LAMBDA)
UNROLL = 3
RING = 3
CHUNK = 256
B_LAG = 3
KV_CHUNK = 128
KV_LAG = 3
SUB = 64
OUT_LAG = 6
LN_LAG = 1

_NN = (((1,), (0,)), ((), ()))
_NT = (((1,), (1,)), ((), ()))


def _mm(a, b):
    return lax.dot_general(a, b, _NN, preferred_element_type=F32)


def _mm_nt(a, b):
    return lax.dot_general(a, b, _NT, preferred_element_type=F32)


def _pack(w):
    return pltpu.bitcast(w, U32)


def _unpack(w):
    return pltpu.bitcast(w, BF16)


def _iota(shape, dim):
    return lax.broadcasted_iota(jnp.int32, shape, dim)


def _recip(x):
    r = pltpu.reciprocal(x, approx=True)
    return r * (2.0 - x * r)


def _layernorm(x):
    m = jnp.mean(x, axis=-1, keepdims=True)
    xc = x - m
    v = jnp.mean(xc * xc, axis=-1, keepdims=True)
    return xc * lax.rsqrt(v + LN_EPS)


def _pair_reduce(v, op):
    v = op(v, pltpu.roll(v, 4, 0))
    return op(v, pltpu.roll(v, 2, 0))


def _hedgehog(p):
    rows = [p[i:i + 8] for i in range(0, p.shape[0], 8)]
    hi = _pair_reduce(functools.reduce(jnp.maximum, rows), jnp.maximum)
    lo = _pair_reduce(functools.reduce(jnp.minimum, rows), jnp.minimum)
    ep = [jnp.exp2(r - hi) for r in rows]
    en = [jnp.exp2(lo - r) for r in rows]
    rp = _recip(_pair_reduce(functools.reduce(jnp.add, ep), jnp.add))
    rn = _recip(_pair_reduce(functools.reduce(jnp.add, en), jnp.add))
    return jnp.concatenate([e * rp for e in ep] + [e * rn for e in en], axis=0)


def _total(terms):
    return functools.reduce(jnp.add, terms)


_BLOCK_PAIRS = tuple(itertools.combinations(range(NB), 2))


def _kappa(i, j):
    return 1.0 / (LAMBDA[j] - LAMBDA[i])


def _others(j):
    return [i for i in range(NB) if i != j]


def _ahead_lhs(a, b):
    c = [b[j] + LAMBDA[j] * a[j] for j in range(NB)]
    return list(a) + [_kappa(i, j) * (c[i] + c[j]) for i, j in _BLOCK_PAIRS]


def _ahead_sums(product):
    y = [None] * NB
    for i in range(NB):
        y[i] = product(i) if y[i] is None else y[i] + product(i)
        for j in range(i + 1, NB):
            t = product(NB + _BLOCK_PAIRS.index((i, j)))
            y[i], y[j] = y[i] + t, -t if y[j] is None else y[j] - t
    return y


def _step_lhs(x, i, j):
    t = x(j) if i == j else x(i) + x(j)
    return jnp.concatenate([t[:-16], t[-8:] + LAMBDA[j] * t[-16:-8]], axis=0)


class _StepSums:
    def __init__(self, ahead):
        self.y, self.w = list(ahead), [None] * NB

    def add(self, product, order):
        plus = lambda u, t: t if u is None else u + t
        for i, j in order:
            t = product(i, j)
            self.w[j] = plus(self.w[j], t)
            if i != j:
                g = _kappa(i, j) * t[-8:]
                self.y[j] = plus(self.y[j], g)
                self.y[i] = -g if self.y[i] is None else self.y[i] - g
        return self

    def columns(self):
        return [jnp.concatenate([w[:-8], y, w[-8:] - lam * y], axis=0)
                for w, y, lam in zip(self.w, self.y, LAMBDA)]


def _kernel(
    x_hbm, mem0_hbm, wq_hbm, wk_hbm, wv_hbm, wo_hbm, bqkv_hbm, wphi_hbm, bwo_hbm,
    out_hbm,
    mem0_ref, al_ref, xres_ref, hn_ref, wqkv_ref, wlast_ref, early_ref, rqkv_ref,
    wo_ref, ro_ref, ahead_ref,
    sel_ref, zero_ref,
    sem_x, sem_b, sem_w, sem_tok, sem_last, sem_out,
    *, seg, heads, dh,
):
    seq, dm = out_hbm.shape
    n_mem = mem0_ref.shape[0]
    n_seg = seq // seg
    rows = n_mem + seg
    pairs = heads // 2
    pw = 2 * dh
    off = -(-rows // 16) * 16
    scale = dh ** (-0.5)
    bdh = dm // B_HEADS
    grp = 2 * bdh
    n_grp = B_HEADS // 2
    n_set = pairs // NB
    last = pairs - 1
    tile = lambda k, n=128: slice(k * n, (k + 1) * n)
    of_set = lambda u: range(u * NB, (u + 1) * NB)

    def rows_of(j, n):
        return pl.ds(j * n if isinstance(j, int) else pl.multiple_of(j * n, n), n)

    def groups_of(kt):
        return range(128 * kt // grp, (128 * kt + 127) // grp + 1)

    def store_ahead_lhs(s, a, b):
        split = lambda t: [t[:, tile(k)] for k in range(NB)]
        for r, t in enumerate(_ahead_lhs(split(a), split(b))):
            al_ref[r, 4 * s:4 * s + t.shape[0] // 2] = _pack(t.astype(BF16))

    def project_ahead(m, u, product):
        n = n_seg * 8 // 2
        for c in range(pw // 128):
            for r0 in range(0, n_seg * 8, n):
                apply = lambda r: product(_unpack(al_ref[r, r0 // 2:(r0 + n) // 2]), r, tile(c))
                for j, y in enumerate(_ahead_sums(apply)):
                    ahead_ref[m * last + u * NB + j, r0:r0 + n, tile(c)] = y

    def load(wphi_ref, xe_ref, hb_ref, xp_ref, stage_ref, out_stage_ref, last_ref, last_out_ref):
        cp_xe = pltpu.make_async_copy(x_hbm.at[:, pl.ds(seg // 8 - 2, 2)], xe_ref, sem_x.at[0])
        cp_mem0 = pltpu.make_async_copy(mem0_hbm, mem0_ref, sem_x.at[1])
        cp_wphi = pltpu.make_async_copy(wphi_hbm, wphi_ref, sem_x.at[2])

        weights = (wq_hbm, wk_hbm, wv_hbm)
        n_round = 3 * n_set
        x_segs = n_seg // (n_round - 1)
        plain = seg // 8 - 2

        def cp_set(m, u):
            return pltpu.make_async_copy(
                weights[m].at[rows_of(u, NB * pw)], stage_ref.at[u], sem_w.at[0, u])

        def cp_out_rows(t, u):
            return pltpu.make_async_copy(
                wo_hbm.at[pl.ds(u * NB, NB), t], out_stage_ref.at[u], sem_w.at[1, u])

        def cp_x(i):
            sl = pl.ds(i * x_segs, x_segs)
            return pltpu.make_async_copy(x_hbm.at[sl, pl.ds(0, plain)], xp_ref.at[sl], sem_tok.at[i])

        def cp_last(m, c):
            return pltpu.make_async_copy(
                weights[m].at[rows_of(last * (pw // 128) + c, 128)], last_ref.at[c], sem_last.at[c])

        cp_last_out = pltpu.make_async_copy(wo_hbm.at[last], last_out_ref, sem_last.at[3])

        def build_selectors():
            eh_r = _iota((B_HEADS, dm), 0)
            eh_c = _iota((B_HEADS, dm), 1)
            phi_f = None
            for d in range(bdh):
                eh = jnp.where(eh_c == eh_r * bdh + d, 1.0, 0.0).astype(BF16)
                t = _mm(wphi_ref[d], eh)
                phi_f = t if phi_f is None else phi_f + t
            pick = jnp.where((_iota((grp, bdh), 0) >> 1) == _iota((grp, bdh), 1), 1.0, 0.0)
            phi_rows = _mm(pick, phi_f.astype(BF16))
            r = _iota((grp, 128), 0)
            for kt in range(dm // 128):
                c = _iota((grp, 128), 1) + 128 * kt
                for i, g in enumerate(groups_of(kt)):
                    c0 = (2 * g + (r & 1)) * bdh
                    sel_ref[kt, i] = jnp.where(
                        (c >= c0) & (c < c0 + bdh), phi_rows[:, 128 * kt:128 * kt + 128], 0.0)

        def load_set(m, u):
            w = lambda use, i, j: stage_ref[u + zero_ref[use], tile(j, pw), tile(i)]
            f = lambda *a: w(*a).astype(F32)
            row = [_total([f(0, j, i) for i in range(NB)]).astype(BF16) for j in range(NB)]
            sym = [(f(1, i, j) + f(1, j, i)).astype(BF16) for i, j in _BLOCK_PAIRS]
            project_ahead(m, u, lambda t, r, c: _mm_nt(t, (row + sym)[r][c]))
            for j in range(NB):
                rqkv_ref[m * n_set + u, j] = _pack(row[j].T)
                diag = (f(2, j, j) - _total([f(2, i, j) for i in _others(j)])).astype(BF16)
                for i in range(NB):
                    t = diag if i == j else w(2, i, j)
                    wqkv_ref[m * last + u * NB + j, tile(i, 64)] = _pack(t.T)

        def load_out_rows(t, u):
            for r in range(0, 128, 16):
                w = {(i, j): out_stage_ref[u, i, r:r + 16, tile(j)]
                     for i in range(NB) for j in range(NB)}
                f = {ij: v.astype(F32) for ij, v in w.items()}
                packed = lambda k: rows_of(k * (dh // 8) + t * 8 + r // 16, 8)
                for j in range(NB):
                    ro_ref[j, packed(u)] = _pack(_total([f[j, i] for i in range(NB)]).astype(BF16))
                    w[j, j] = (f[j, j] - _total([f[i, j] for i in _others(j)])).astype(BF16)
                    for i in range(NB):
                        wo_ref[packed(u * NB + i), tile(j)] = _pack(w[i, j])

        def start_rows(s, k, x):
            x = x.astype(F32).reshape(-1, dm)
            h = _layernorm(x)
            for t in range(x.shape[0] // 8):
                sl = rows_of((s + t) * (seg // 8) + k, 8)
                xres_ref[sl] = x[tile(t, 8)]
                hn_ref[sl] = _pack(h[tile(t, 8)])
            return h

        for k in range(zero_ref.shape[0]):
            zero_ref[k] = 0
        for cp in (cp_wphi, cp_mem0, cp_xe):
            cp.start()
        cp_wphi.wait()
        cp_set(0, 0).start()
        cp_last(0, 0).start()
        build_selectors()
        cp_xe.wait()
        for cp in (cp_out_rows(0, 0), cp_x(0), cp_set(0, 1), cp_last(0, 1)):
            cp.start()
        for s in range(0, n_seg, x_segs):
            a, b = (start_rows(s, plain + k, xe_ref[s:s + x_segs, k]) for k in range(2))
            store_ahead_lhs(s, a, b)
            hb_ref[4 * s:4 * (s + x_segs)] = _pack(b.astype(BF16))

        def following(m, u):
            wrap = u == n_set - 1
            return jnp.where(wrap, m + 1, m), jnp.where(wrap, 0, u + 1)

        def load_body(r, carry):
            before, now = carry
            after = following(*now)
            later = following(*after)
            side = jnp.maximum(r - 1, 0)
            cp_set(0, now[1]).wait()
            cp_last(0, now[1]).wait()

            @pl.when(r != 1)
            def _():
                cp_out_rows(*before).wait()
                cp_x(side).wait()

            for m in range(3):
                @pl.when(later[0] == m)
                def _():
                    cp_set(m, later[1]).start()
                    cp_last(m, later[1]).start()

            @pl.when(r + 2 < n_round)
            def _():
                cp_out_rows(*after).start()
                cp_x(r + 1).start()

            @pl.when(r + 2 == n_round)
            def _():
                cp_out_rows(*after).start()
                cp_last_out.start()

            w = last_ref[now[1]]
            early_ref[now[0], now[1]] = _mm_nt(_unpack(hb_ref[...]), w)
            wlast_ref[now[0], now[1]] = _pack(w.T)
            load_set(*now)
            load_out_rows(*before)
            for k in range(plain):
                start_rows(side * x_segs, k, xp_ref[pl.ds(side * x_segs, x_segs), k])
            return now, after

        lax.fori_loop(0, n_round, load_body, ((0, 0), (0, 0)))
        cp_out_rows(2, n_set - 1).wait()
        cp_last_out.wait()
        load_out_rows(2, n_set - 1)
        wo_ref[tile(last, dh)] = _pack(last_out_ref[...].reshape(pw, dm))
        cp_mem0.wait()

    def layers(ya_ref, o_ref, mem_ref, kt_ref, vb_ref, p_ref,
               bqkv_ref, bwo_ref, bq_ref, bkv_ref, bo_ref, ht_ref, ot_ref, kv_ref, z_ref, res_ref):
        cp_bqkv = pltpu.make_async_copy(bqkv_hbm, bqkv_ref, sem_b.at[0])
        cp_bwo = pltpu.make_async_copy(bwo_hbm, bwo_ref, sem_b.at[1])

        cut = dh % 128

        def stack(a, b):
            gap = jnp.zeros((off - rows, a.shape[1]), F32)
            tail = jnp.zeros((128 - off - rows, a.shape[1]), F32)
            return jnp.concatenate([a, gap, b, tail], axis=0).astype(BF16)

        def store_keys(j, t):
            outer = _pack(stack(t[:, 0:128], t[:, 256:384]).T)
            inner = _pack(stack(t[:, 128:256], t[:, 128:256]).T)
            low = _iota((64, 128), 1) < off
            kt_ref[j, 0:64] = jnp.where(low, outer, 0)
            kt_ref[j, 64:64 + cut // 2] = jnp.where(low[:cut // 2], inner[:cut // 2], 0)
            kt_ref[j, 64 + cut // 2:128] = jnp.where(low[cut // 2:], 0, inner[cut // 2:])
            kt_ref[j, 128:192] = jnp.where(low, 0, outer)

        def store_values(j, t):
            t = _pack(jnp.concatenate([t, jnp.zeros((off - rows, pw), F32)], axis=0).astype(BF16))
            low = _iota((off // 2, 128), 1) < cut
            vb_ref[j, 0:off // 2, 0:128] = t[:, 0:128]
            vb_ref[j, 0:off // 2, 128:256] = jnp.where(low, t[:, 128:256], 0)
            vb_ref[j, off // 2:off, 128:256] = jnp.where(low, 0, t[:, 128:256])
            vb_ref[j, off // 2:off, 256:384] = t[:, 256:384]

        def a_step(s, first_layer):
            h = jnp.concatenate([mem_ref[...], pltpu.bitcast(hn_ref[rows_of(s, seg), :], F32)], axis=0)
            mine = rows_of(s, 8)
            qi = _iota((rows, 128), 0)
            ki = _iota((rows, 128), 1)
            in_a = ki < rows
            in_b = (ki >= off) & (ki < off + rows)
            see_a = in_a & ((qi < n_mem) | (qi >= ki))
            see_b = in_b & ((qi < n_mem) | (qi >= ki - off))
            fill_a = jnp.where(in_a, MASK_FILL, -jnp.inf)
            fill_b = jnp.where(in_b, MASK_FILL, -jnp.inf)
            by_column = [(i, j) for j in range(NB) for i in range(NB)]
            lhs = {(i, j): _step_lhs(lambda k: h[:, tile(k)], i, j) for i, j in by_column}

            def store_queries(j, t):
                o_ref[j] = t

            store = (store_queries, store_keys, store_values)

            def project(m, u, order=by_column):
                product = lambda i, j: _mm(
                    lhs[i, j], _unpack(wqkv_ref[m * last + u * NB + j, tile(i, 64)]))
                ahead = [ahead_ref[m * last + u * NB + j, mine] for j in range(NB)]
                for j, t in zip(of_set(u), _StepSums(ahead).add(product, order).columns()):
                    store[m](j, t)

            def scores(j):
                sc = _mm(o_ref[j], _unpack(kt_ref[j])) * scale
                sa = jnp.where(see_a, sc, fill_a)
                sb = jnp.where(see_b, sc, fill_b)
                e = jnp.exp(jnp.maximum(sa - jnp.max(sa, axis=-1, keepdims=True),
                                        sb - jnp.max(sb, axis=-1, keepdims=True)))
                sum_a = jnp.sum(jnp.where(in_a, e, 0.0), axis=-1, keepdims=True)
                sum_b = jnp.sum(jnp.where(in_a, 0.0, e), axis=-1, keepdims=True)
                p_ref[j] = e * _recip(jnp.where(in_a, sum_a, sum_b))

            def attend(j):
                o = _mm(p_ref[j], _unpack(vb_ref[j]))
                o_ref[j] = o
                if j < last:
                    ahead_ref[j, mine] = o[-16:-8]
                    ahead_ref[last + j, mine] = o[-8:]

            out = _StepSums([None] * NB)

            def project_out(u):
                product = lambda i, j: _mm(
                    _step_lhs(lambda k: o_ref[u * NB + k], i, j),
                    _unpack(wo_ref[tile(u * NB + i, dh), tile(j)]))
                out.add(product, sorted(by_column, key=sorted))

            out_last = lambda c: _mm(o_ref[last], _unpack(wo_ref[tile(last, dh), tile(c)]))

            project(1, 0, sorted(by_column, key=lambda ij: max(2, *ij)))
            for m in (1, 0, 2):
                w = _unpack(jnp.concatenate([wlast_ref[m, c] for c in range(pw // 128)], axis=1))
                if first_layer:
                    done = jnp.concatenate([early_ref[m, c, mine] for c in range(pw // 128)], axis=1)
                    store[m](last, jnp.concatenate([_mm(h[:-8], w), done], axis=0))
                else:
                    store[m](last, _mm(h, w))
            for m, u in ((1, 1), (1, 2), (0, 0), (2, 0), (0, 1), (2, 1), (0, 2)):
                project(m, u)
            ready = [*of_set(0), *of_set(1), last]
            for j in ready:
                scores(j)
            project(2, 2)
            for j in of_set(2):
                scores(j)
            for j in ready:
                attend(j)
            project_out(0)
            for j in of_set(2):
                attend(j)
            direct = [out_last(c) for c in range(NB - 1)]
            project_out(1)
            project_out(2)
            direct.append(out_last(NB - 1))
            y = jnp.concatenate([t + d for t, d in zip(out.columns(), direct)], axis=1)
            mem_ref[...] = y[:n_mem]
            ya_ref[s] = y[n_mem:].reshape(seg // 8, 8, dm)

        def a_start():
            group = lambda s, k: pltpu.bitcast(jnp.concatenate(
                [hn_ref[tile((t + 1) * (seg // 8) + k, 8)] for t in range(s, s + 8)], axis=0), F32)

            @pl.when(zero_ref[0] == 0)
            def _():
                for s in range(0, n_seg, 8):
                    store_ahead_lhs(s, group(s, -2), group(s, -1))

            def ahead_body(m, carry):
                for u in range(n_set):
                    block = lambda i, j: _unpack(
                        wqkv_ref[m * last + u * NB + j, tile(i, 64)]).astype(F32)
                    rhs = [_unpack(rqkv_ref[m * n_set + u, j]) for j in range(NB)]
                    rhs += [(block(i, j) + block(j, i)).astype(BF16) for i, j in _BLOCK_PAIRS]
                    project_ahead(m, u, lambda t, r, c: _mm(t, rhs[r][:, c]))
                return carry

            lax.fori_loop(0, 3, ahead_body, 0)

        def a_finish():
            block = lambda i, j: _unpack(jnp.concatenate(
                [wo_ref[tile(u * NB + i, dh), tile(j)] for u in range(n_set)], axis=0)).astype(F32)
            rhs = [_unpack(ro_ref[j]) for j in range(NB)]
            rhs += [(block(i, j) + block(j, i)).astype(BF16) for i, j in _BLOCK_PAIRS]
            n = n_seg // 4
            for s0 in range(0, n_seg, n):
                side = lambda p: jnp.concatenate(
                    [ahead_ref[p + u * NB, s0 * 8:(s0 + n) * 8] for u in range(n_set)], axis=1)
                lhs = _ahead_lhs([side(k) for k in range(NB)], [side(last + k) for k in range(NB)])
                for j, y in enumerate(_ahead_sums(lambda r: _mm(lhs[r], rhs[r]))):
                    y = y.reshape(n, 8, 128)
                    ya_ref[s0:s0 + n, seg // 8 - 2, :, tile(j)] += y
                    ya_ref[s0:s0 + n, seg // 8 - 1, :, tile(j)] -= LAMBDA[j] * y

        def a_layer(first_layer):
            n_loop = n_seg // UNROLL

            def a_body(i, carry):
                for k in range(UNROLL):
                    a_step(i * UNROLL + k, first_layer)
                return carry

            if first_layer:
                vb_ref[...] = jnp.zeros(vb_ref.shape, U32)
                cp_bqkv.start()
                cp_bwo.start()
            else:
                a_start()
            mem_ref[...] = mem0_ref[...].astype(F32)
            lax.fori_loop(0, n_loop, a_body, 0)
            if first_layer:
                cp_bqkv.wait()
                cp_bwo.wait()
                b_fold_weights()
            for s in range(n_loop * UNROLL, n_seg):
                a_step(s, first_layer)
            a_finish()

        def b_fold_weights():
            def fold(m):
                out = {}
                for kt in range(dm // 128):
                    gs = groups_of(kt)
                    block = jnp.concatenate([sel_ref[kt, i] for i in range(len(gs))], axis=0)
                    part = _mm_nt(block, bqkv_ref[:, m * dm + 128 * kt:m * dm + 128 * kt + 128])
                    for i, g in enumerate(gs):
                        t = part[i * grp:(i + 1) * grp]
                        out[g] = out[g] + t if g in out else t
                return [out[g] * LOG2E for g in range(n_grp)]

            def store(ref, blocks):
                for i in range(0, len(blocks), 2):
                    two = jnp.concatenate(blocks[i:i + 2], axis=0).astype(BF16)
                    ref[i * bdh:(i + 2) * bdh, :] = _pack(two)

            wk = fold(1)
            wv = bqkv_ref[:, 2 * dm:3 * dm].T.astype(F32)
            store(bkv_ref, [w for g in range(n_grp) for w in (wk[g], wv[g * grp:(g + 1) * grp])])
            store(bq_ref, fold(0))
            bo_ref[...] = _pack(bwo_ref[...])

        def b_kv():
            n_chunk = seq // KV_CHUNK
            tokens = lambda i: slice(i * KV_CHUNK, (i + 1) * KV_CHUNK)

            def normalize(i):
                xn = xres_ref[tokens(i), :] + ya_ref[tile(i, KV_CHUNK // seg)].reshape(KV_CHUNK, dm)
                xres_ref[tokens(i), :] = xn
                ht_ref[:, tokens(i)] = _pack(_layernorm(xn).astype(BF16).T)

            work = [(i, g) for i in range(n_chunk) for g in range(n_grp)]
            ready = {}
            normalize(0)
            for n in range(len(work) + KV_LAG):
                if n < len(work):
                    i, g = work[n]
                    if g == 0 and i + 1 < n_chunk:
                        normalize(i + 1)
                    t = _mm(_unpack(bkv_ref[g * grp:(g + 1) * grp, :]), _unpack(ht_ref[:, tokens(i)]))
                    phi = _hedgehog(t[:grp])
                    ready[n] = (t[grp:], phi.astype(BF16))
                    z = phi if i == 0 else z_ref[g] + phi
                    if i == n_chunk - 1:
                        z = jnp.broadcast_to(jnp.sum(z, axis=-1, keepdims=True), z.shape)
                    z_ref[g] = z
                if n >= KV_LAG:
                    i, g = work[n - KV_LAG]
                    t = _mm_nt(*ready.pop(n - KV_LAG))
                    if i > 0:
                        t = kv_ref[g] + t
                    if i == n_chunk - 1:
                        second = (_iota(t.shape, 1) & 1) == 1
                        t = jnp.where((_iota(t.shape, 0) >= bdh) == second, t, 0.0)
                    kv_ref[g] = t

        n_chunk = seq // CHUNK
        tokens = lambda i: slice(i * CHUNK, (i + 1) * CHUNK)

        def cp_out(i):
            return pltpu.make_async_copy(res_ref.at[tile(i, SUB)], out_hbm.at[tile(i, SUB)], sem_out.at[i])

        def b_out(last_layer):
            zero = zero_ref[0]
            half = n_grp // 2
            n_sub = CHUNK // SUB
            work = [(i, gg) for i in range(n_chunk) for gg in range(half)]
            ready = {}

            def staged(i, r0, n):
                return pl.ds(pl.multiple_of(zero + seq + (i % 2) * (CHUNK // 2) + r0, 8), n)

            def features(g, p):
                phi = _hedgehog(p)
                t = phi * jnp.concatenate([z_ref[g]] * (CHUNK // 128), axis=1)
                den = functools.reduce(jnp.add, [t[r:r + 8] for r in range(0, 2 * grp, 8)])
                inv = _recip(_pair_reduce(den, jnp.add) + DEN_EPS)
                other = pltpu.roll(inv, 1, 0)
                r = _iota(inv.shape, 0)
                return phi.astype(BF16), jnp.concatenate(
                    [jnp.where((r + r0 >= bdh) == ((r & 1) == 1), inv, other) for r0 in range(0, grp, 8)],
                    axis=0)

            finished = []

            def normalize():
                sl = finished.pop(0)
                hn_ref[sl, :] = _pack(_layernorm(xres_ref[sl, :]))

            def finish(i, k):
                if len(finished) > LN_LAG:
                    normalize()
                sl = slice(i * CHUNK + k * SUB, i * CHUNK + (k + 1) * SUB)
                o = _unpack(hn_ref[staged(i, k * SUB // 2, SUB // 2), :])
                xn = xres_ref[sl, :] + _mm(o, _unpack(bo_ref[...]))
                if last_layer:
                    res_ref[sl, :] = xn.astype(BF16)
                    cp_out(i * n_sub + k).start()
                else:
                    xres_ref[sl, :] = xn
                    finished.append(sl)

            pending = []
            for n in range(len(work) + B_LAG):
                if n < len(work):
                    i, gg = work[n]
                    t = _mm(_unpack(bq_ref[gg * grp:(gg + 1) * grp, :]), _unpack(ht_ref[:, tokens(i)]))
                    ready[n] = [features(2 * gg + k, t[k * grp:(k + 1) * grp]) for k in range(2)]
                while pending and pending[0][0] <= n:
                    finish(*pending.pop(0)[1:])
                if n >= B_LAG:
                    i, gg = work[n - B_LAG]
                    for k, (phi, inv) in enumerate(ready.pop(n - B_LAG)):
                        g = 2 * gg + k
                        ot_ref[g * grp:(g + 1) * grp, :] = _mm(kv_ref[g], phi) * inv
                    if gg == half - 1:
                        hn_ref[staged(i, 0, CHUNK // 2), :] = _pack(ot_ref[...].astype(BF16).T)
                        start = n + (OUT_LAG if i < n_chunk - 2 else half)
                        pending += [(start + k * half // n_sub, i, k) for k in range(n_sub)]
            for _, i, k in pending:
                finish(i, k)
            while finished:
                normalize()

        a_layer(True)
        b_kv()
        b_out(False)
        a_layer(False)
        b_kv()
        b_out(True)
        for i in range(seq // SUB):
            cp_out(i).wait()

    pl.run_scoped(
        load,
        pltpu.VMEM((bdh, bdh, B_HEADS), BF16),
        pltpu.VMEM((n_seg, 2, 8, dm), BF16),
        pltpu.VMEM((n_seg * 4, dm), U32),
        pltpu.VMEM((n_seg, seg // 8 - 2, 8, dm), BF16),
        pltpu.VMEM((RING, NB * pw, dm), BF16),
        pltpu.VMEM((RING, NB, 128, dm), BF16),
        pltpu.VMEM((pw // 128, 128, dm), BF16),
        pltpu.VMEM((pw // 128, 128, dm), BF16),
    )
    pl.run_scoped(
        layers,
        pltpu.VMEM((n_seg, seg // 8, 8, dm), F32),
        pltpu.VMEM((pairs, rows, pw), F32),
        pltpu.VMEM((n_mem, dm), F32),
        pltpu.VMEM((pairs, dh, 128), U32),
        pltpu.VMEM((pairs, 64, pw), U32),
        pltpu.VMEM((pairs, rows, 128), F32),
        pltpu.VMEM((dm, 3 * dm), BF16),
        pltpu.VMEM((dm, dm), BF16),
        pltpu.VMEM((dm // 2, dm), U32),
        pltpu.VMEM((dm, dm), U32),
        pltpu.VMEM((dm // 2, dm), U32),
        pltpu.VMEM((dm // 2, seq), U32),
        pltpu.VMEM((dm, CHUNK), F32),
        pltpu.VMEM((n_grp, grp, 2 * grp), F32),
        pltpu.VMEM((n_grp, 2 * grp, 128), F32),
        pltpu.VMEM((seq, dm), BF16),
    )


@functools.partial(jax.jit, static_argnames=("A_seg_len",))
def pallas_interleave_layers__memory_aug_recurrent_mem_tr__linear_kernel_hedgehog__prompt_kernel(
    A_x: jax.Array,
    A_mem0: jax.Array,
    A_Wq: jax.Array,
    A_Wk: jax.Array,
    A_Wv: jax.Array,
    A_Wo: jax.Array,
    A_seg_len: int,
    B_x: jax.Array,
    B_wqkv: jax.Array,
    B_w_phi: jax.Array,
    B_wo: jax.Array,
):
    del B_x
    batch, seq, dm = A_x.shape
    _, heads, dh = A_Wq.shape
    n_mem = A_mem0.shape[1]
    seg = int(A_seg_len)
    n_seg = seq // seg
    rows = n_mem + seg
    pw = 2 * dh
    pairs = heads // 2
    bdh = dm // B_HEADS
    assert n_seg % 16 == 0
    assert batch == 1 and seq % CHUNK == 0 and KV_CHUNK % seg == 0 and seg % 8 == 0 and seg > 16
    assert n_mem % 8 == 0 and rows <= 48
    assert heads % 2 == 0 and pw == 3 * 128 and dm == NB * 128 and pairs == RING * NB + 1 and (2 * bdh) % 8 == 0

    w_t = lambda w: jnp.transpose(w, (1, 2, 0)).reshape(heads * dh, dm)
    hbm = pl.BlockSpec(memory_space=pl.ANY)

    out = pl.pallas_call(
        functools.partial(_kernel, seg=seg, heads=heads, dh=dh),
        out_shape=jax.ShapeDtypeStruct((seq, dm), A_x.dtype),
        in_specs=[hbm] * 9,
        out_specs=hbm,
        scratch_shapes=[
            pltpu.VMEM((n_mem, dm), BF16),
            pltpu.VMEM((NB + len(_BLOCK_PAIRS), n_seg * 4, 128), U32),
            pltpu.VMEM((seq, dm), F32),
            pltpu.VMEM((seq + CHUNK, dm), U32),
            pltpu.VMEM((3 * (pairs - 1), dm // 2, pw), U32),
            pltpu.VMEM((3, pw // 128, dm // 2, 128), U32),
            pltpu.VMEM((3, pw // 128, n_seg * 8, 128), F32),
            pltpu.VMEM((3 * RING, NB, 64, pw), U32),
            pltpu.VMEM((pairs * dh, dm), U32),
            pltpu.VMEM((NB, RING * dh, 128), U32),
            pltpu.VMEM((3 * (pairs - 1), n_seg * 8, pw), F32),
            pltpu.VMEM((dm // 128, 127 // (2 * bdh) + 2, 2 * bdh, 128), F32),
            pltpu.SMEM((3,), jnp.int32),
            pltpu.SemaphoreType.DMA((3,)),
            pltpu.SemaphoreType.DMA((2,)),
            pltpu.SemaphoreType.DMA((2, RING)),
            pltpu.SemaphoreType.DMA((3 * RING - 1,)),
            pltpu.SemaphoreType.DMA((4,)),
            pltpu.SemaphoreType.DMA((seq // SUB,)),
        ],
        compiler_params=pltpu.CompilerParams(
            vmem_limit_bytes=126 * 1024 * 1024,
            flags={"XLA_TPU_EVENLY_DISTRIBUTE_CRITICAL_NODES": True},
        ),
    )(
        A_x.reshape(n_seg, seg // 8, 8, dm),
        A_mem0.reshape(n_mem, dm),
        w_t(A_Wq), w_t(A_Wk), w_t(A_Wv),
        A_Wo.reshape(pairs, pw // 128, 128, dm),
        B_wqkv,
        jnp.transpose(B_w_phi, (1, 2, 0)),
        B_wo,
    )
    return out.reshape(batch, seq, dm)
```
